```python
import jax
import jax.numpy as jnp

def _softmax(x, axis=-1):
    return jax.nn.softmax(x, axis=axis)

def _gelu(x):
    return jax.nn.gelu(x, approximate=True)

def _silu(x):
    return jax.nn.silu(x)

def _sigmoid(x):
    return jax.nn.sigmoid(x)

def _layernorm(x, axis=-1, eps=1e-05):
    m = jnp.mean(x, axis=axis, keepdims=True)
    v = jnp.var(x, axis=axis, keepdims=True)
    return (x - m) / jnp.sqrt(v + eps)

def _scatter_add(tgt, idx, src, axis=0):
    return tgt.at[idx].add(src)

def _segment_sum(src, seg, n):
    return jax.ops.segment_sum(src, seg, n)

class _Rng:

    def __init__(self, key):
        self._k = key

    def _next(self):
        self._k, sub = jax.random.split(self._k)
        return sub

    def normal(self, shape):
        return jax.random.normal(self._next(), shape, dtype=jnp.bfloat16)

    def randint(self, lo, hi, shape):
        return jax.random.randint(self._next(), shape, lo, hi, dtype=jnp.int32)

    def uniform(self, shape, lo=0.0, hi=1.0):
        return jax.random.uniform(self._next(), shape, jnp.bfloat16, lo, hi)

    def permutation(self, n):
        return jax.random.permutation(self._next(), n)
kernel_name = 'gated_mix__memory_aug_recurrent_mem_tr__mixer_s_mlp__prompt'

def setup_inputs():
    _rng = _Rng(jax.random.key(int.from_bytes(__import__("os").urandom(4), "little")))
    _w = lambda a: (lambda t: t.astype(jnp.bfloat16) if jnp.issubdtype(t.dtype, jnp.floating) else t)(jnp.asarray(a))

    def _A_setup():
        B, S, Dm = (1, 2048, 1024)
        H, Dh = (32, 128)
        M, seg = (8, 32)
        seg = min(seg, S)
        S = S // seg * seg
        return {'x': _w((lambda *s: _rng.normal(s) * 0.05)(B, S, Dm)), 'mem0': _w((lambda *s: _rng.normal(s) * 0.05)(B, M, Dm)), 'Wq': _w((lambda *s: _rng.normal(s) * 0.05)(Dm, H, Dh) * Dm ** (-0.5)), 'Wk': _w((lambda *s: _rng.normal(s) * 0.05)(Dm, H, Dh) * Dm ** (-0.5)), 'Wv': _w((lambda *s: _rng.normal(s) * 0.05)(Dm, H, Dh) * Dm ** (-0.5)), 'Wo': _w((lambda *s: _rng.normal(s) * 0.05)(H, Dh, Dm) * (H * Dh) ** (-0.5)), 'seg_len': seg}
    _A_in = _A_setup()

    def _B_setup():
        B, S, D, F = (1, 2048, 1024, 3584)
        return {'x': _w((lambda *s: _rng.normal(s) * 0.05)(B, S, D)), 'w1': _w((lambda *s: _rng.normal(s) * 0.05)(D, D) * D ** (-0.5)), 'w2': _w((lambda *s: _rng.normal(s) * 0.05)(D, D) * D ** (-0.5)), 'w3': _w((lambda *s: _rng.normal(s) * 0.05)(D, F) * D ** (-0.5)), 'w4': _w((lambda *s: _rng.normal(s) * 0.05)(F, D) * F ** (-0.5))}
    _B_in = _B_setup()
    return {'A_x': _A_in['x'], 'A_mem0': _A_in['mem0'], 'A_Wq': _A_in['Wq'], 'A_Wk': _A_in['Wk'], 'A_Wv': _A_in['Wv'], 'A_Wo': _A_in['Wo'], 'A_seg_len': _A_in['seg_len'], 'B_x': _B_in['x'], 'B_w1': _B_in['w1'], 'B_w2': _B_in['w2'], 'B_w3': _B_in['w3'], 'B_w4': _B_in['w4'], 'gate_w': _w((lambda *s: _rng.normal(s) * 0.05)(1024))}

def reference(A_x, A_mem0, A_Wq, A_Wk, A_Wv, A_Wo, A_seg_len, B_x, B_w1, B_w2, B_w3, B_w4, gate_w):

    def _A_ref(x, mem0, Wq, Wk, Wv, Wo, seg_len):
        B, S, Dm = x.shape
        H, Dh = (Wq.shape[1], Wq.shape[2])
        M = mem0.shape[1]
        scale = Dh ** (-0.5)
        n_seg = S // seg_len
        L = M + seg_len
        idx = jnp.arange(L)
        mask = (idx[:, None] < M) | (idx[:, None] >= idx[None, :])
        mem = mem0
        outs = []
        for s in range(n_seg):
            xs = x[:, s * seg_len:(s + 1) * seg_len, :].copy()
            h = jnp.concatenate([mem, xs], axis=1)
            q = jnp.einsum('btd,dhe->bhte', h, Wq)
            k = jnp.einsum('btd,dhe->bhte', h, Wk)
            v = jnp.einsum('btd,dhe->bhte', h, Wv)
            scores = jnp.einsum('bhqe,bhke->bhqk', q, k) * scale
            scores = jnp.where(mask[None, None], scores, -1000000000.0)
            p = _softmax(scores, axis=-1)
            o = jnp.einsum('bhqk,bhke->bhqe', p, v)
            o = jnp.einsum('bhte,hed->btd', o, Wo)
            mem = o[:, :M, :].copy()
            outs.append(o[:, M:, :])
        return jnp.concatenate(outs, axis=1)

    def _B_ref(x, w1, w2, w3, w4):
        B, S, D = x.shape
        h = _gelu(_layernorm(x, axis=-1) @ w1)
        c = D // 4
        g0 = jnp.pad(h[:, :, 0 * c:1 * c], ((0, 0), (1, 0), (0, 0)))[:, :S, :]
        g1 = jnp.pad(h[:, :, 1 * c:2 * c], ((0, 0), (0, 1), (0, 0)))[:, 1:, :]
        g2 = jnp.pad(h[:, :, 2 * c:3 * c], ((0, 0), (2, 0), (0, 0)))[:, :S, :]
        g3 = jnp.pad(h[:, :, 3 * c:], ((0, 0), (0, 2), (0, 0)))[:, 2:, :]
        hs = jnp.concatenate([g0, g1, g2, g3], axis=-1) @ w2
        x1 = x + hs
        h2 = _gelu(_layernorm(x1, axis=-1) @ w3) @ w4
        return x1 + h2
    x = A_x
    g = _sigmoid((x * gate_w).sum(-1, keepdims=True))
    a = _A_ref(x, A_mem0, A_Wq, A_Wk, A_Wv, A_Wo, A_seg_len)
    b = _B_ref(x, B_w1, B_w2, B_w3, B_w4)
    return g * a + (1 - g) * b
```

```python
import functools
import math

import jax
import jax.numpy as jnp
import jax.experimental.pallas as pl
import jax.experimental.pallas.tpu as pltpu

F32 = jnp.float32
BF16 = jnp.bfloat16
U32 = jnp.uint32

S = 2048
D = 1024
H = 32
DH = 128
M = 8
SEG = 32
L = M + SEG
FF = 3584
PAIR = 2 * SEG
NPAIR = S // PAIR
TM = 256
NCH = S // TM
PITCH = 520
EPS = 1e-5
NEG = -1e9


def _gelu(x):
    c = math.sqrt(2.0 / math.pi)
    return 0.5 * x * (1.0 + jnp.tanh(c * (x + 0.044715 * (x * x * x))))


def _layernorm(x):
    m = jnp.mean(x, axis=-1, keepdims=True)
    xc = x - m
    v = jnp.mean(xc * xc, axis=-1, keepdims=True)
    return xc * jax.lax.rsqrt(v + EPS)


def _slab_of(which, h):
    return which * H + (h % 2) * (H // 2) + h // 2


def _kernel(x_hbm, mem0_ref, wq_hbm, wk_hbm, wv_hbm, wo_hbm,
            w1_hbm, w2_hbm, w3_hbm, w4_hbm, gw_ref,
            out_hbm,
            x_v, stage_v, wqkv_v, wo_v, w1_v, w2_v, w3_v, w4_v,
            h1_v, bb_v, g_v, mem_v, obuf_v, sems, osems):
    cp_x = pltpu.make_async_copy(x_hbm, x_v, sems.at[0])
    cp_w1 = pltpu.make_async_copy(w1_hbm, w1_v, sems.at[1])
    cp_w2 = pltpu.make_async_copy(w2_hbm, w2_v, sems.at[2])
    cp_w3 = pltpu.make_async_copy(w3_hbm, w3_v, sems.at[3])
    cp_w4 = pltpu.make_async_copy(w4_hbm, w4_v, sems.at[4])
    cp_qkv = [pltpu.make_async_copy(w, stage_v.at[i], sems.at[5 + i])
              for i, w in enumerate((wq_hbm, wk_hbm, wv_hbm))]
    cp_wo = [pltpu.make_async_copy(wo_hbm.at[:, pl.ds(128 * j, 128)], wo_v.at[j], sems.at[8 + j])
             for j in range(D // 128)]
    cp_x.start()
    cp_w1.start()
    cp_x.wait()
    cp_w1.wait()
    cp_w2.start()
    cp_w3.start()
    cp_w4.start()
    for c in cp_qkv:
        c.start()
    for c in cp_wo:
        c.start()

    h1_v[pl.ds(0, 8), :] = jnp.zeros((8, D), F32)
    h1_v[pl.ds(S + 8, 8), :] = jnp.zeros((8, D), F32)

    def b1_body(i, carry):
        r0 = pl.multiple_of(i * TM, TM)
        xf = x_v[pl.ds(r0, TM), :].astype(F32)
        ln = _layernorm(xf).astype(BF16)
        h = jnp.dot(ln, w1_v[...], preferred_element_type=F32)
        h1_v[pl.ds(r0 + 8, TM), :] = _gelu(h)
        return carry

    jax.lax.fori_loop(0, NCH, b1_body, 0)

    cp_w2.wait()
    cp_w3.wait()
    cp_w4.wait()

    c4 = D // 4
    for i in range(NCH):
        r0 = i * TM
        parts = [
            h1_v[pl.ds(r0 + 8 - 1, TM), pl.ds(0 * c4, c4)],
            h1_v[pl.ds(r0 + 8 + 1, TM), pl.ds(1 * c4, c4)],
            h1_v[pl.ds(r0 + 8 - 2, TM), pl.ds(2 * c4, c4)],
            h1_v[pl.ds(r0 + 8 + 2, TM), pl.ds(3 * c4, c4)],
        ]
        bb_v[pl.ds(r0, TM), :] = jnp.concatenate(parts, axis=1)

    def b2_body(i, carry):
        r0 = pl.multiple_of(i * TM, TM)
        hs_in = bb_v[pl.ds(r0, TM), :].astype(BF16)
        xf = x_v[pl.ds(r0, TM), :].astype(F32)
        x1 = xf + jnp.dot(hs_in, w2_v[...], preferred_element_type=F32)
        ln = _layernorm(x1).astype(BF16)
        h = _gelu(jnp.dot(ln, w3_v[...], preferred_element_type=F32)).astype(BF16)
        b = x1 + jnp.dot(h, w4_v[...], preferred_element_type=F32)
        z = jnp.sum(xf * gw_ref[...].astype(F32), axis=-1, keepdims=True)
        g = 1.0 / (1.0 + jnp.exp(-z))
        bb_v[pl.ds(r0, TM), :] = (1.0 - g) * b
        g_v[pl.ds(r0, TM), :] = jnp.broadcast_to(g, (TM, 128))
        return carry

    jax.lax.fori_loop(0, NCH, b2_body, 0)

    for c in cp_qkv:
        c.wait()
    for c in cp_wo:
        c.wait()

    for which in range(3):
        def relayout_body(i, carry, which=which):
            base = pl.multiple_of(i * 64, 64)
            blk = pltpu.bitcast(stage_v[which, pl.ds(base, 64), :], U32)
            a = blk[0:16]
            b = blk[16:32]
            lo = (a & jnp.uint32(0xFFFF)) | (b << 16)
            hi = (a >> 16) | (b & jnp.uint32(0xFFFF0000))
            s0 = which * H * PITCH
            wqkv_v[pl.ds(s0 + i, 16, stride=PITCH), :] = lo
            wqkv_v[pl.ds(s0 + 16 * PITCH + i, 16, stride=PITCH), :] = hi
            return carry

        jax.lax.fori_loop(0, D // 2, relayout_body, 0, unroll=8)

    mem_v[...] = mem0_ref[...].astype(F32)
    wo_u = wo_v.bitcast(U32)
    c_exp = (DH ** -0.5) * math.log2(math.e)
    neg_raw = NEG / (DH ** -0.5)

    row = jax.lax.broadcasted_iota(jnp.int32, (L, 128), 0)
    col = jax.lax.broadcasted_iota(jnp.int32, (L, 128), 1)
    allowed = (row < M) | (row >= col)
    real = col < L

    def wslab(which, h):
        s = _slab_of(which, h) * PITCH
        return pltpu.bitcast(wqkv_v[pl.ds(s, 512), :], BF16)

    zpad = jnp.zeros((128 - L, DH), F32)
    z8 = jnp.zeros((8, DH), F32)

    def attend(q, k, v):
        qb = jnp.concatenate([q, z8], axis=0).astype(BF16)
        kb = jnp.concatenate([k, zpad], axis=0).astype(BF16)
        vb = jnp.concatenate([v, zpad], axis=0).astype(BF16)
        s = jax.lax.dot_general(qb, kb, (((1,), (1,)), ((), ())),
                                preferred_element_type=F32)[0:L]
        s = jnp.where(allowed, s, neg_raw)
        s = jnp.where(real, s, -jnp.inf)
        m = jnp.max(s, axis=-1, keepdims=True)
        p = jnp.exp2((s - m) * c_exp)
        l = jnp.sum(p, axis=-1, keepdims=True)
        pb = jnp.concatenate([p, z8], axis=0).astype(BF16)
        o = jnp.dot(pb, vb, preferred_element_type=F32)[0:L]
        return o / l

    def out_proj(o_bf):
        return jnp.concatenate(
            [jnp.dot(o_bf, pltpu.bitcast(wo_u[j], BF16), preferred_element_type=F32)
             for j in range(D // 128)], axis=1)

    def out_copy(t, slot):
        return pltpu.make_async_copy(obuf_v.at[slot], out_hbm.at[pl.ds(t * PAIR, PAIR), :],
                                     osems.at[slot])

    def a_body(t, carry):
        r0 = pl.multiple_of(t * PAIR, PAIR)
        slot = t % 2
        xf = x_v[pl.ds(r0, PAIR), :].astype(F32)

        lhs = jnp.concatenate([mem_v[...], xf[0:40]], axis=0).astype(BF16)
        o_a = []
        extra = []
        for h in range(H):
            q = jnp.dot(lhs, wslab(0, h), preferred_element_type=F32)
            k = jnp.dot(lhs, wslab(1, h), preferred_element_type=F32)
            v = jnp.dot(lhs, wslab(2, h), preferred_element_type=F32)
            extra.append((q[40:48], k[40:48], v[40:48]))
            o_a.append(attend(q[0:40], k[0:40], v[0:40]))
        o_a = jnp.concatenate(o_a, axis=1)
        y_a = out_proj(o_a[0:32].astype(BF16))
        mem_b = y_a[0:8].astype(BF16).astype(F32)

        lhs = jnp.concatenate([mem_b, xf[40:64]], axis=0).astype(BF16)
        o_b = []
        for h in range(H):
            q = jnp.dot(lhs, wslab(0, h), preferred_element_type=F32)
            k = jnp.dot(lhs, wslab(1, h), preferred_element_type=F32)
            v = jnp.dot(lhs, wslab(2, h), preferred_element_type=F32)
            eq, ek, ev = extra[h]
            q = jnp.concatenate([q[0:8], eq, q[8:32]], axis=0)
            k = jnp.concatenate([k[0:8], ek, k[8:32]], axis=0)
            v = jnp.concatenate([v[0:8], ev, v[8:32]], axis=0)
            o_b.append(attend(q, k, v))
        o_b = jnp.concatenate(o_b, axis=1)
        y_b = out_proj(jnp.concatenate([o_b, o_a[32:40]], axis=0).astype(BF16))
        mem_v[...] = y_b[0:8].astype(BF16).astype(F32)

        a = jnp.concatenate([y_a[8:32], y_b[40:48], y_b[8:40]], axis=0)
        g = g_v[pl.ds(r0, PAIR), :]
        g = jnp.concatenate([g] * (D // 128), axis=1)
        res = g * a + bb_v[pl.ds(r0, PAIR), :]

        @pl.when(t >= 2)
        def _():
            out_copy(t - 2, slot).wait()

        obuf_v[slot] = res.astype(BF16)
        out_copy(t, slot).start()
        return carry

    jax.lax.fori_loop(0, NPAIR, a_body, 0)
    out_copy(NPAIR - 2, 0).wait()
    out_copy(NPAIR - 1, 1).wait()


@functools.partial(jax.jit, static_argnames=("A_seg_len",))
def pallas_gated_mix__memory_aug_recurrent_mem_tr__mixer_s_mlp__prompt_kernel(
    A_x, A_mem0, A_Wq, A_Wk, A_Wv, A_Wo, A_seg_len, B_x, B_w1, B_w2, B_w3, B_w4, gate_w,
):
    assert A_seg_len == SEG
    assert A_x.shape == (1, S, D) and A_Wq.shape == (D, H, DH) and A_mem0.shape == (1, M, D)
    x = A_x.reshape(S, D)
    mem0 = A_mem0.reshape(M, D)
    wq = A_Wq.reshape(D * H, DH)
    wk = A_Wk.reshape(D * H, DH)
    wv = A_Wv.reshape(D * H, DH)
    wo = A_Wo.reshape(H * DH, D)
    gw = gate_w.reshape(1, D)

    any_spec = pl.BlockSpec(memory_space=pl.ANY)
    vmem_spec = pl.BlockSpec(memory_space=pltpu.VMEM)
    out = pl.pallas_call(
        _kernel,
        out_shape=jax.ShapeDtypeStruct((S, D), BF16),
        in_specs=[any_spec, vmem_spec, any_spec, any_spec, any_spec, any_spec,
                  any_spec, any_spec, any_spec, any_spec, vmem_spec],
        out_specs=any_spec,
        scratch_shapes=[
            pltpu.VMEM((S, D), BF16),
            pltpu.VMEM((3, D * H, DH), BF16),
            pltpu.VMEM((3 * H * PITCH, 128), U32),
            pltpu.VMEM((D // 128, H * DH, 128), BF16),
            pltpu.VMEM((D, D), BF16),
            pltpu.VMEM((D, D), BF16),
            pltpu.VMEM((D, FF), BF16),
            pltpu.VMEM((FF, D), BF16),
            pltpu.VMEM((S + 16, D), F32),
            pltpu.VMEM((S, D), F32),
            pltpu.VMEM((S, 128), F32),
            pltpu.VMEM((M, D), F32),
            pltpu.VMEM((2, PAIR, D), BF16),
            pltpu.SemaphoreType.DMA((16,)),
            pltpu.SemaphoreType.DMA((2,)),
        ],
        compiler_params=pltpu.CompilerParams(vmem_limit_bytes=120 * 1024 * 1024),
    )(x, mem0, wq, wk, wv, wo, B_w1, B_w2, B_w3, B_w4, gw)
    return out.reshape(1, S, D)
```

```python
import functools
import math

import jax
import jax.numpy as jnp
import jax.experimental.pallas as pl
import jax.experimental.pallas.tpu as pltpu

F32 = jnp.float32
BF16 = jnp.bfloat16
U32 = jnp.uint32

S = 2048
D = 1024
H = 32
DH = 128
M = 8
SEG = 32
L = M + SEG
FF = 3584
PAIR = 2 * SEG
NPAIR = S // PAIR
TM = 256
NCH = S // TM
PITCH = 520
EPS = 1e-5
NEG = -1e9


def _gelu(x):
    c = math.sqrt(2.0 / math.pi)
    return 0.5 * x * (1.0 + jnp.tanh(c * (x + 0.044715 * (x * x * x))))


def _layernorm(x):
    m = jnp.mean(x, axis=-1, keepdims=True)
    xc = x - m
    v = jnp.mean(xc * xc, axis=-1, keepdims=True)
    return xc * jax.lax.rsqrt(v + EPS)


def _slab_of(which, h):
    return which * H + (h % 2) * (H // 2) + h // 2


def _kernel(x_hbm, mem0_ref, wq_hbm, wk_hbm, wv_hbm, wo_hbm,
            w1_hbm, w2_hbm, w3_hbm, w4_hbm, gw_ref,
            out_hbm,
            x_v, stage_v, wqkv_v, wo_v, w1_v, w2_v, w3_v, w4_v,
            h1_v, bb_v, g_v, mem_v, obuf_v, sems, osems):
    cp_x = pltpu.make_async_copy(x_hbm, x_v, sems.at[0])
    cp_w1 = pltpu.make_async_copy(w1_hbm, w1_v, sems.at[1])
    cp_w2 = pltpu.make_async_copy(w2_hbm, w2_v, sems.at[2])
    cp_w3 = pltpu.make_async_copy(w3_hbm, w3_v, sems.at[3])
    cp_w4 = pltpu.make_async_copy(w4_hbm, w4_v, sems.at[4])
    cp_qkv = [pltpu.make_async_copy(w, stage_v.at[i], sems.at[5 + i])
              for i, w in enumerate((wq_hbm, wk_hbm, wv_hbm))]
    cp_wo = [pltpu.make_async_copy(wo_hbm.at[:, pl.ds(128 * j, 128)], wo_v.at[j], sems.at[8 + j])
             for j in range(D // 128)]
    cp_x.start()
    cp_w1.start()
    cp_x.wait()
    cp_w1.wait()
    cp_w2.start()
    cp_w3.start()
    cp_w4.start()
    for c in cp_qkv:
        c.start()
    for c in cp_wo:
        c.start()

    h1_v[pl.ds(0, 8), :] = jnp.zeros((8, D), F32)
    h1_v[pl.ds(S + 8, 8), :] = jnp.zeros((8, D), F32)

    def b1_body(i, carry):
        r0 = pl.multiple_of(i * TM, TM)
        xf = x_v[pl.ds(r0, TM), :].astype(F32)
        ln = _layernorm(xf).astype(BF16)
        h = jnp.dot(ln, w1_v[...], preferred_element_type=F32)
        h1_v[pl.ds(r0 + 8, TM), :] = _gelu(h)
        return carry

    jax.lax.fori_loop(0, NCH, b1_body, 0)

    cp_w2.wait()
    cp_w3.wait()
    cp_w4.wait()

    c4 = D // 4
    for i in range(NCH):
        r0 = i * TM
        parts = [
            h1_v[pl.ds(r0 + 8 - 1, TM), pl.ds(0 * c4, c4)],
            h1_v[pl.ds(r0 + 8 + 1, TM), pl.ds(1 * c4, c4)],
            h1_v[pl.ds(r0 + 8 - 2, TM), pl.ds(2 * c4, c4)],
            h1_v[pl.ds(r0 + 8 + 2, TM), pl.ds(3 * c4, c4)],
        ]
        bb_v[pl.ds(r0, TM), :] = jnp.concatenate(parts, axis=1)

    def b2_body(i, carry):
        r0 = pl.multiple_of(i * TM, TM)
        hs_in = bb_v[pl.ds(r0, TM), :].astype(BF16)
        xf = x_v[pl.ds(r0, TM), :].astype(F32)
        x1 = xf + jnp.dot(hs_in, w2_v[...], preferred_element_type=F32)
        ln = _layernorm(x1).astype(BF16)
        h = _gelu(jnp.dot(ln, w3_v[...], preferred_element_type=F32)).astype(BF16)
        b = x1 + jnp.dot(h, w4_v[...], preferred_element_type=F32)
        z = jnp.sum(xf * gw_ref[...].astype(F32), axis=-1, keepdims=True)
        g = 1.0 / (1.0 + jnp.exp(-z))
        bb_v[pl.ds(r0, TM), :] = (1.0 - g) * b
        g_v[pl.ds(r0, TM), :] = jnp.broadcast_to(g, (TM, 128))
        return carry

    jax.lax.fori_loop(0, NCH, b2_body, 0)

    for c in cp_qkv:
        c.wait()
    for c in cp_wo:
        c.wait()

    for which in range(3):
        def relayout_body(i, carry, which=which):
            base = pl.multiple_of(i * 64, 64)
            blk = pltpu.bitcast(stage_v[which, pl.ds(base, 64), :], U32)
            a = blk[0:16]
            b = blk[16:32]
            lo = (a & jnp.uint32(0xFFFF)) | (b << 16)
            hi = (a >> 16) | (b & jnp.uint32(0xFFFF0000))
            s0 = which * H * PITCH
            wqkv_v[pl.ds(s0 + i, 16, stride=PITCH), :] = lo
            wqkv_v[pl.ds(s0 + 16 * PITCH + i, 16, stride=PITCH), :] = hi
            return carry

        jax.lax.fori_loop(0, D // 2, relayout_body, 0, unroll=8)

    mem_v[...] = mem0_ref[...].astype(F32)
    wo_u = wo_v.bitcast(U32)
    c_exp = (DH ** -0.5) * math.log2(math.e)
    neg_raw = NEG / (DH ** -0.5)

    row = jax.lax.broadcasted_iota(jnp.int32, (L, 128), 0)
    col = jax.lax.broadcasted_iota(jnp.int32, (L, 128), 1)
    allowed = (row < M) | (row >= col)
    real = col < L

    def wslab(which, h):
        s = _slab_of(which, h) * PITCH
        return pltpu.bitcast(wqkv_v[pl.ds(s, 512), :], BF16)

    zpad = jnp.zeros((128 - L, DH), F32)
    z8 = jnp.zeros((8, DH), F32)

    def to_bf(q, k, v):
        qb = jnp.concatenate([q, z8], axis=0).astype(BF16)
        kb = jnp.concatenate([k, zpad], axis=0).astype(BF16)
        vb = jnp.concatenate([v, zpad], axis=0).astype(BF16)
        return qb, kb, vb

    def scores(qb, kb):
        s = jax.lax.dot_general(qb, kb, (((1,), (1,)), ((), ())),
                                preferred_element_type=F32)[0:L]
        s = jnp.where(allowed, s, neg_raw)
        s = jnp.where(real, s, -jnp.inf)
        m = jnp.max(s, axis=-1, keepdims=True)
        p = jnp.exp2((s - m) * c_exp)
        l = jnp.sum(p, axis=-1, keepdims=True)
        pb = jnp.concatenate([p, z8], axis=0).astype(BF16)
        return pb, l

    def pv(pb, l, vb):
        o = jnp.dot(pb, vb, preferred_element_type=F32)[0:L]
        return o * pl.reciprocal(l, approx=False)

    def wo_part(o_bf, h0, h1, j):
        w = pltpu.bitcast(wo_u[j, pl.ds(h0 * 64, (h1 - h0) * 64), :], BF16)
        return jnp.dot(o_bf, w, preferred_element_type=F32)

    def segment(lhs, assemble, wo_rows):
        qkv = [None] * H
        pl_ = [None] * H
        ob = [None] * H

        def do_qkv(h):
            q = jnp.dot(lhs, wslab(0, h), preferred_element_type=F32)
            k = jnp.dot(lhs, wslab(1, h), preferred_element_type=F32)
            v = jnp.dot(lhs, wslab(2, h), preferred_element_type=F32)
            qkv[h] = to_bf(*assemble(h, q, k, v))

        def do_s(h):
            pl_[h] = scores(qkv[h][0], qkv[h][1])

        def do_pv(h):
            ob[h] = wo_rows(h, pv(pl_[h][0], pl_[h][1], qkv[h][2])).astype(BF16)

        G = 2
        NG = H // G
        for g in range(NG):
            for h in range(g * G, (g + 1) * G):
                do_qkv(h)
            if g >= 1:
                for h in range((g - 1) * G, g * G):
                    do_s(h)
            if g >= 2:
                for h in range((g - 2) * G, (g - 1) * G):
                    do_pv(h)
        HA = H - 3 * G
        oa = jnp.concatenate(ob[0:HA], axis=1)
        ya = []
        nj = D // 128
        for j in range(nj):
            ya.append(wo_part(oa, 0, HA, j))
            if j == 1:
                for h in range(H - G, H):
                    do_s(h)
                for h in range(H - 2 * G, H - G):
                    do_pv(h)
            if j == 4:
                for h in range(H - G, H):
                    do_pv(h)
        ot = jnp.concatenate(ob[HA:H], axis=1)
        y = [ya[j] + wo_part(ot, HA, H, j) for j in range(nj)]
        return jnp.concatenate(y, axis=1)

    def out_copy(t, slot):
        return pltpu.make_async_copy(obuf_v.at[slot], out_hbm.at[pl.ds(t * PAIR, PAIR), :],
                                     osems.at[slot])

    def a_body(t, carry):
        r0 = pl.multiple_of(t * PAIR, PAIR)
        slot = t % 2
        xf = x_v[pl.ds(r0, PAIR), :].astype(F32)

        lhs = jnp.concatenate([mem_v[...], xf[0:40]], axis=0).astype(BF16)
        extra = [None] * H
        o_left = [None] * H

        def asm_a(h, q, k, v):
            extra[h] = (q[40:48], k[40:48], v[40:48])
            return q[0:40], k[0:40], v[0:40]

        def rows_a(h, o):
            o_left[h] = o[32:40]
            return o[0:32]

        y_a = segment(lhs, asm_a, rows_a)
        mem_b = y_a[0:8].astype(BF16).astype(F32)

        lhs = jnp.concatenate([mem_b, xf[40:64]], axis=0).astype(BF16)

        def asm_b(h, q, k, v):
            eq, ek, ev = extra[h]
            return (jnp.concatenate([q[0:8], eq, q[8:32]], axis=0),
                    jnp.concatenate([k[0:8], ek, k[8:32]], axis=0),
                    jnp.concatenate([v[0:8], ev, v[8:32]], axis=0))

        def rows_b(h, o):
            return jnp.concatenate([o, o_left[h]], axis=0)

        y_b = segment(lhs, asm_b, rows_b)
        mem_v[...] = y_b[0:8].astype(BF16).astype(F32)

        a = jnp.concatenate([y_a[8:32], y_b[40:48], y_b[8:40]], axis=0)
        g = g_v[pl.ds(r0, PAIR), :]
        g = jnp.concatenate([g] * (D // 128), axis=1)
        res = g * a + bb_v[pl.ds(r0, PAIR), :]

        @pl.when(t >= 2)
        def _():
            out_copy(t - 2, slot).wait()

        obuf_v[slot] = res.astype(BF16)
        out_copy(t, slot).start()
        return carry

    jax.lax.fori_loop(0, NPAIR, a_body, 0)
    out_copy(NPAIR - 2, 0).wait()
    out_copy(NPAIR - 1, 1).wait()


@functools.partial(jax.jit, static_argnames=("A_seg_len",))
def pallas_gated_mix__memory_aug_recurrent_mem_tr__mixer_s_mlp__prompt_kernel(
    A_x, A_mem0, A_Wq, A_Wk, A_Wv, A_Wo, A_seg_len, B_x, B_w1, B_w2, B_w3, B_w4, gate_w,
):
    assert A_seg_len == SEG
    assert A_x.shape == (1, S, D) and A_Wq.shape == (D, H, DH) and A_mem0.shape == (1, M, D)
    x = A_x.reshape(S, D)
    mem0 = A_mem0.reshape(M, D)
    wq = A_Wq.reshape(D * H, DH)
    wk = A_Wk.reshape(D * H, DH)
    wv = A_Wv.reshape(D * H, DH)
    wo = A_Wo.reshape(H * DH, D)
    gw = gate_w.reshape(1, D)

    any_spec = pl.BlockSpec(memory_space=pl.ANY)
    vmem_spec = pl.BlockSpec(memory_space=pltpu.VMEM)
    out = pl.pallas_call(
        _kernel,
        out_shape=jax.ShapeDtypeStruct((S, D), BF16),
        in_specs=[any_spec, vmem_spec, any_spec, any_spec, any_spec, any_spec,
                  any_spec, any_spec, any_spec, any_spec, vmem_spec],
        out_specs=any_spec,
        scratch_shapes=[
            pltpu.VMEM((S, D), BF16),
            pltpu.VMEM((3, D * H, DH), BF16),
            pltpu.VMEM((3 * H * PITCH, 128), U32),
            pltpu.VMEM((D // 128, H * DH, 128), BF16),
            pltpu.VMEM((D, D), BF16),
            pltpu.VMEM((D, D), BF16),
            pltpu.VMEM((D, FF), BF16),
            pltpu.VMEM((FF, D), BF16),
            pltpu.VMEM((S + 16, D), F32),
            pltpu.VMEM((S, D), F32),
            pltpu.VMEM((S, 128), F32),
            pltpu.VMEM((M, D), F32),
            pltpu.VMEM((2, PAIR, D), BF16),
            pltpu.SemaphoreType.DMA((16,)),
            pltpu.SemaphoreType.DMA((2,)),
        ],
        compiler_params=pltpu.CompilerParams(vmem_limit_bytes=120 * 1024 * 1024),
    )(x, mem0, wq, wk, wv, wo, B_w1, B_w2, B_w3, B_w4, gw)
    return out.reshape(1, S, D)
```

```python
import functools
import math

import jax
import jax.numpy as jnp
import jax.experimental.pallas as pl
import jax.experimental.pallas.tpu as pltpu

F32 = jnp.float32
BF16 = jnp.bfloat16
U32 = jnp.uint32

S = 2048
D = 1024
H = 32
DH = 128
M = 8
SEG = 32
L = M + SEG
FF = 3584
PAIR = 2 * SEG
NPAIR = S // PAIR
TM = 256
NCH = S // TM
PITCH = 520
EPS = 1e-5
S_LAG = 1
PV_LAG = 3
TAIL_AT = (1, 3, 5)
NEG = -1e9


def _gelu(x):
    c = math.sqrt(2.0 / math.pi)
    return 0.5 * x * (1.0 + jnp.tanh(c * (x + 0.044715 * (x * x * x))))


def _layernorm(x):
    m = jnp.mean(x, axis=-1, keepdims=True)
    xc = x - m
    v = jnp.mean(xc * xc, axis=-1, keepdims=True)
    return xc * jax.lax.rsqrt(v + EPS)


def _slab_of(which, h):
    return which * H + (h % 2) * (H // 2) + h // 2


def _kernel(x_hbm, mem0_ref, wq_hbm, wk_hbm, wv_hbm, wo_hbm,
            w1_hbm, w2_hbm, w3_hbm, w4_hbm, gw_ref,
            out_hbm,
            x_v, stage_v, wqkv_v, wo_v, w1_v, w2_v, w3_v, w4_v,
            h1_v, bb_v, g_v, mem_v, obuf_v, sems, osems):
    cp_x = pltpu.make_async_copy(x_hbm, x_v, sems.at[0])
    cp_w1 = pltpu.make_async_copy(w1_hbm, w1_v, sems.at[1])
    cp_w2 = pltpu.make_async_copy(w2_hbm, w2_v, sems.at[2])
    cp_w3 = pltpu.make_async_copy(w3_hbm, w3_v, sems.at[3])
    cp_w4 = pltpu.make_async_copy(w4_hbm, w4_v, sems.at[4])
    cp_qkv = [pltpu.make_async_copy(w, stage_v.at[i], sems.at[5 + i])
              for i, w in enumerate((wq_hbm, wk_hbm, wv_hbm))]
    cp_wo = [pltpu.make_async_copy(wo_hbm.at[:, pl.ds(128 * j, 128)], wo_v.at[j], sems.at[8 + j])
             for j in range(D // 128)]
    cp_x.start()
    cp_w1.start()
    cp_x.wait()
    cp_w1.wait()
    cp_w2.start()
    cp_w3.start()
    cp_w4.start()
    for c in cp_qkv:
        c.start()
    for c in cp_wo:
        c.start()

    h1_v[pl.ds(0, 8), :] = jnp.zeros((8, D), F32)
    h1_v[pl.ds(S + 8, 8), :] = jnp.zeros((8, D), F32)

    def b1_body(i, carry):
        r0 = pl.multiple_of(i * TM, TM)
        xf = x_v[pl.ds(r0, TM), :].astype(F32)
        ln = _layernorm(xf).astype(BF16)
        h = jnp.dot(ln, w1_v[...], preferred_element_type=F32)
        h1_v[pl.ds(r0 + 8, TM), :] = _gelu(h)
        return carry

    jax.lax.fori_loop(0, NCH, b1_body, 0)

    cp_w2.wait()
    cp_w3.wait()
    cp_w4.wait()

    c4 = D // 4
    for i in range(NCH):
        r0 = i * TM
        parts = [
            h1_v[pl.ds(r0 + 8 - 1, TM), pl.ds(0 * c4, c4)],
            h1_v[pl.ds(r0 + 8 + 1, TM), pl.ds(1 * c4, c4)],
            h1_v[pl.ds(r0 + 8 - 2, TM), pl.ds(2 * c4, c4)],
            h1_v[pl.ds(r0 + 8 + 2, TM), pl.ds(3 * c4, c4)],
        ]
        bb_v[pl.ds(r0, TM), :] = jnp.concatenate(parts, axis=1)

    def b2_body(i, carry):
        r0 = pl.multiple_of(i * TM, TM)
        hs_in = bb_v[pl.ds(r0, TM), :].astype(BF16)
        xf = x_v[pl.ds(r0, TM), :].astype(F32)
        x1 = xf + jnp.dot(hs_in, w2_v[...], preferred_element_type=F32)
        ln = _layernorm(x1).astype(BF16)
        h = _gelu(jnp.dot(ln, w3_v[...], preferred_element_type=F32)).astype(BF16)
        b = x1 + jnp.dot(h, w4_v[...], preferred_element_type=F32)
        z = jnp.sum(xf * gw_ref[...].astype(F32), axis=-1, keepdims=True)
        g = 1.0 / (1.0 + jnp.exp(-z))
        bb_v[pl.ds(r0, TM), :] = (1.0 - g) * b
        g_v[pl.ds(r0, TM), :] = jnp.broadcast_to(g, (TM, 128))
        return carry

    jax.lax.fori_loop(0, NCH, b2_body, 0)

    for c in cp_qkv:
        c.wait()
    for c in cp_wo:
        c.wait()

    for which in range(3):
        def relayout_body(i, carry, which=which):
            base = pl.multiple_of(i * 64, 64)
            blk = pltpu.bitcast(stage_v[which, pl.ds(base, 64), :], U32)
            a = blk[0:16]
            b = blk[16:32]
            lo = (a & jnp.uint32(0xFFFF)) | (b << 16)
            hi = (a >> 16) | (b & jnp.uint32(0xFFFF0000))
            s0 = which * H * PITCH
            wqkv_v[pl.ds(s0 + i, 16, stride=PITCH), :] = lo
            wqkv_v[pl.ds(s0 + 16 * PITCH + i, 16, stride=PITCH), :] = hi
            return carry

        jax.lax.fori_loop(0, D // 2, relayout_body, 0, unroll=8)

    mem_v[...] = mem0_ref[...].astype(F32)
    wo_u = wo_v.bitcast(U32)
    c_exp = (DH ** -0.5) * math.log2(math.e)
    neg_raw = NEG / (DH ** -0.5)

    L2 = 2 * L
    row = jax.lax.broadcasted_iota(jnp.int32, (L2, 128), 0)
    col = jax.lax.broadcasted_iota(jnp.int32, (L2, 128), 1)
    second = row >= L
    rowl = jnp.where(second, row - L, row)
    coll = jnp.where(second, col - L, col)
    real = (coll >= 0) & (coll < L)
    allowed = real & ((rowl < M) | (rowl >= coll))
    fill = jnp.where(real, neg_raw, -jnp.inf).astype(F32)

    def wslab(which, h):
        s = _slab_of(which, h) * PITCH
        return pltpu.bitcast(wqkv_v[pl.ds(s, 512), :], BF16)

    zpad = jnp.zeros((128 - L2, DH), F32)

    def scores(qb, kb):
        s = jax.lax.dot_general(qb, kb, (((1,), (1,)), ((), ())),
                                preferred_element_type=F32)
        s = jnp.where(allowed, s, fill)
        m = jnp.max(s, axis=-1, keepdims=True)
        p = jnp.exp2((s - m) * c_exp)
        l = jnp.sum(p, axis=-1, keepdims=True)
        r = pl.reciprocal(l, approx=True)
        r = r * (2.0 - l * r)
        return (p * r).astype(BF16)

    def wo_part(o_bf, h0, h1, j):
        w = pltpu.bitcast(wo_u[j, pl.ds(h0 * 64, (h1 - h0) * 64), :], BF16)
        return jnp.dot(o_bf, w, preferred_element_type=F32)

    def segment(lhs, assemble, wo_rows):
        NP = H // 2
        qkv = [None] * NP
        pb = [None] * NP
        ob = [None] * H

        def do_qkv(p):
            t = []
            for h in (2 * p, 2 * p + 1):
                q = jnp.dot(lhs, wslab(0, h), preferred_element_type=F32)
                k = jnp.dot(lhs, wslab(1, h), preferred_element_type=F32)
                v = jnp.dot(lhs, wslab(2, h), preferred_element_type=F32)
                t.append(assemble(h, q, k, v))
            qb = jnp.concatenate([t[0][0], t[1][0]], axis=0).astype(BF16)
            kb = jnp.concatenate([t[0][1], t[1][1], zpad], axis=0).astype(BF16)
            vb = jnp.concatenate([t[0][2], t[1][2], zpad], axis=0).astype(BF16)
            qkv[p] = (qb, kb, vb)

        def do_s(p):
            pb[p] = scores(qkv[p][0], qkv[p][1])

        def do_pv(p):
            o = jnp.dot(pb[p], qkv[p][2], preferred_element_type=F32)
            ob[2 * p] = wo_rows(2 * p, o[0:L]).astype(BF16)
            ob[2 * p + 1] = wo_rows(2 * p + 1, o[L:L2]).astype(BF16)

        for p in range(NP):
            do_qkv(p)
            if p >= S_LAG:
                do_s(p - S_LAG)
            if p >= PV_LAG:
                do_pv(p - PV_LAG)
        HA = 2 * (NP - PV_LAG - 1)
        oa = jnp.concatenate(ob[0:HA], axis=1)
        ya = []
        nj = D // 128
        nxt = NP
        for j in range(nj):
            ya.append(wo_part(oa, 0, HA, j))
            if j in TAIL_AT:
                if nxt - S_LAG < NP:
                    do_s(nxt - S_LAG)
                if nxt - PV_LAG < NP:
                    do_pv(nxt - PV_LAG)
                nxt += 1
        assert nxt - PV_LAG >= NP
        ot = jnp.concatenate(ob[HA:H], axis=1)
        y = [wo_part(ot, HA, H, j) + ya[j] for j in range(nj)]
        return jnp.concatenate(y, axis=1)

    def out_copy(t, slot):
        return pltpu.make_async_copy(obuf_v.at[slot], out_hbm.at[pl.ds(t * PAIR, PAIR), :],
                                     osems.at[slot])

    def a_body(t, carry):
        r0 = pl.multiple_of(t * PAIR, PAIR)
        slot = t % 2
        xf = x_v[pl.ds(r0, PAIR), :].astype(F32)

        lhs = jnp.concatenate([mem_v[...], xf[0:40]], axis=0).astype(BF16)
        extra = [None] * H
        o_left = [None] * H

        def asm_a(h, q, k, v):
            extra[h] = (q[40:48], k[40:48], v[40:48])
            return q[0:40], k[0:40], v[0:40]

        def rows_a(h, o):
            o_left[h] = o[32:40]
            return o[0:32]

        y_a = segment(lhs, asm_a, rows_a)
        mem_b = y_a[0:8].astype(BF16).astype(F32)

        lhs = jnp.concatenate([mem_b, xf[40:64]], axis=0).astype(BF16)

        def asm_b(h, q, k, v):
            eq, ek, ev = extra[h]
            return (jnp.concatenate([q[0:8], eq, q[8:32]], axis=0),
                    jnp.concatenate([k[0:8], ek, k[8:32]], axis=0),
                    jnp.concatenate([v[0:8], ev, v[8:32]], axis=0))

        def rows_b(h, o):
            return jnp.concatenate([o, o_left[h]], axis=0)

        y_b = segment(lhs, asm_b, rows_b)
        mem_v[...] = y_b[0:8].astype(BF16).astype(F32)

        a = jnp.concatenate([y_a[8:32], y_b[40:48], y_b[8:40]], axis=0)
        g = g_v[pl.ds(r0, PAIR), :]
        g = jnp.concatenate([g] * (D // 128), axis=1)
        res = g * a + bb_v[pl.ds(r0, PAIR), :]

        @pl.when(t >= 2)
        def _():
            out_copy(t - 2, slot).wait()

        obuf_v[slot] = res.astype(BF16)
        out_copy(t, slot).start()
        return carry

    jax.lax.fori_loop(0, NPAIR, a_body, 0)
    out_copy(NPAIR - 2, 0).wait()
    out_copy(NPAIR - 1, 1).wait()


@functools.partial(jax.jit, static_argnames=("A_seg_len",))
def pallas_gated_mix__memory_aug_recurrent_mem_tr__mixer_s_mlp__prompt_kernel(
    A_x, A_mem0, A_Wq, A_Wk, A_Wv, A_Wo, A_seg_len, B_x, B_w1, B_w2, B_w3, B_w4, gate_w,
):
    assert A_seg_len == SEG
    assert A_x.shape == (1, S, D) and A_Wq.shape == (D, H, DH) and A_mem0.shape == (1, M, D)
    x = A_x.reshape(S, D)
    mem0 = A_mem0.reshape(M, D)
    wq = A_Wq.reshape(D * H, DH)
    wk = A_Wk.reshape(D * H, DH)
    wv = A_Wv.reshape(D * H, DH)
    wo = A_Wo.reshape(H * DH, D)
    gw = gate_w.reshape(1, D)

    any_spec = pl.BlockSpec(memory_space=pl.ANY)
    vmem_spec = pl.BlockSpec(memory_space=pltpu.VMEM)
    out = pl.pallas_call(
        _kernel,
        out_shape=jax.ShapeDtypeStruct((S, D), BF16),
        in_specs=[any_spec, vmem_spec, any_spec, any_spec, any_spec, any_spec,
                  any_spec, any_spec, any_spec, any_spec, vmem_spec],
        out_specs=any_spec,
        scratch_shapes=[
            pltpu.VMEM((S, D), BF16),
            pltpu.VMEM((3, D * H, DH), BF16),
            pltpu.VMEM((3 * H * PITCH, 128), U32),
            pltpu.VMEM((D // 128, H * DH, 128), BF16),
            pltpu.VMEM((D, D), BF16),
            pltpu.VMEM((D, D), BF16),
            pltpu.VMEM((D, FF), BF16),
            pltpu.VMEM((FF, D), BF16),
            pltpu.VMEM((S + 16, D), F32),
            pltpu.VMEM((S, D), F32),
            pltpu.VMEM((S, 128), F32),
            pltpu.VMEM((M, D), F32),
            pltpu.VMEM((2, PAIR, D), BF16),
            pltpu.SemaphoreType.DMA((16,)),
            pltpu.SemaphoreType.DMA((2,)),
        ],
        compiler_params=pltpu.CompilerParams(vmem_limit_bytes=120 * 1024 * 1024),
    )(x, mem0, wq, wk, wv, wo, B_w1, B_w2, B_w3, B_w4, gw)
    return out.reshape(1, S, D)
```

```python
import functools
import math

import jax
import jax.numpy as jnp
import jax.experimental.pallas as pl
import jax.experimental.pallas.tpu as pltpu

F32 = jnp.float32
BF16 = jnp.bfloat16
U32 = jnp.uint32

S = 2048
D = 1024
H = 32
DH = 128
M = 8
SEG = 32
L = M + SEG
FF = 3584
PAIR = 2 * SEG
NPAIR = S // PAIR
T1 = 256
N1 = S // T1
T3 = 256
N3 = S // T3
DP = D // N3
OP = H * DH // N3
UNROLL_A = 1
PITCH = 520
EPS = 1e-5
NCHAIN1 = 2
S_LAG = 1
PV_LAG = 3
TAIL_AT = (1, 3, 5)
NEG = -1e9


def _gelu(x):
    c = math.sqrt(2.0 / math.pi)
    return 0.5 * x * (1.0 + jnp.tanh(c * (x + 0.044715 * (x * x * x))))


def _layernorm(x):
    m = jnp.mean(x, axis=-1, keepdims=True)
    xc = x - m
    v = jnp.mean(xc * xc, axis=-1, keepdims=True)
    return xc * jax.lax.rsqrt(v + EPS)


def _slab_of(which, h):
    return which * H + (h % 2) * (H // 2) + h // 2


def _kernel(x_hbm, mem0_ref, wq_hbm, wk_hbm, wv_hbm, wo_hbm,
            w1_hbm, w2_hbm, w3_hbm, w4_hbm, gw_ref,
            out_hbm,
            x_v, stq_v, sto_v, wqkv_v, wo_v, w1_v, w2_v, w3_v, w4_v,
            h1_v, x1_v, g_v, ln1_v, ln3_v, mem_v, out_v, zero_v, sems, xsems, psems, osem):
    def cp_x(i):
        r0 = i * T1 if isinstance(i, int) else pl.multiple_of(i * T1, T1)
        return pltpu.make_async_copy(x_hbm.at[pl.ds(r0, T1)], x_v.at[pl.ds(r0, T1)], xsems.at[i])

    cp_w1 = pltpu.make_async_copy(w1_hbm, w1_v, sems.at[1])
    cp_w2 = pltpu.make_async_copy(w2_hbm, w2_v, sems.at[2])
    cp_w3 = pltpu.make_async_copy(w3_hbm, w3_v, sems.at[3])
    cp_w4 = pltpu.make_async_copy(w4_hbm, w4_v, sems.at[4])

    def piece_copies(i, slot):
        cps = [pltpu.make_async_copy(w.at[pl.ds(i * (DP * H), DP * H)], stq_v.at[slot, k],
                                     psems.at[slot, k])
               for k, w in enumerate((wq_hbm, wk_hbm, wv_hbm))]
        cps.append(pltpu.make_async_copy(wo_hbm.at[pl.ds(i * OP, OP)], sto_v.at[slot],
                                         psems.at[slot, 3]))
        return cps

    cp_x(0).start()
    cp_w1.start()
    cp_x(1).start()
    h1_v[pl.ds(8, 8), :] = jnp.zeros((8, D), F32)
    h1_v[pl.ds(S, 8), :] = jnp.zeros((8, D), F32)
    zero_v[...] = jnp.zeros((16, 128), U32)
    gw = gw_ref[...].astype(F32)

    def tie(x, tok):
        head = pltpu.bitcast(pltpu.bitcast(x[:, 0:128], U32) | tok, F32)
        return jnp.concatenate([head, x[:, 128:]], axis=1)

    def ln_rows(x, tok, zero):
        if tok is not None:
            x = tie(x, tok)
        part = x[:, 0:128]
        for j in range(1, D // 128):
            part = part + x[:, j * 128:(j + 1) * 128]
        m = jnp.sum(part, axis=-1, keepdims=True) * (1.0 / D)
        xc = x - m
        v = jnp.mean(xc * xc, axis=-1, keepdims=True)
        y = xc * jax.lax.rsqrt(v + EPS)
        tok = None if zero is None else pltpu.bitcast(y[:, 0:128], U32) & zero
        return x, y, tok

    def prep1(blk, slot, chain):
        r0 = pl.multiple_of(blk * T1, T1)
        zero = zero_v[...] if chain else None
        toks = [None] * NCHAIN1
        for k in range(T1 // 16):
            xf = x_v[pl.ds(r0 + k * 16, 16), :].astype(F32)
            xf, y, toks[k % NCHAIN1] = ln_rows(xf, toks[k % NCHAIN1], zero)
            ln1_v[slot, pl.ds(k * 16, 16), :] = y.astype(BF16)
            z = jnp.sum(xf * gw, axis=-1, keepdims=True)
            g_v[pl.ds(r0 + k * 16, 16), :] = jnp.broadcast_to(1.0 / (1.0 + jnp.exp(-z)), (16, 128))

    cp_x(0).wait()
    prep1(0, 0, False)
    cp_w1.wait()
    for i in range(2, N1):
        cp_x(i).start()

    c4 = D // 4

    def p1_body(i, carry):
        r0 = pl.multiple_of(i * T1, T1)
        slot = i % 2

        @pl.when(i == 2)
        def _():
            cp_w2.start()
            cp_w3.start()
            cp_w4.start()
            for c in piece_copies(0, 0):
                c.start()

        @pl.when(i + 1 < N1)
        def _():
            cp_x(i + 1).wait()

        lhs = ln1_v[slot]
        prep1(jnp.minimum(i + 1, N1 - 1), 1 - slot, True)
        h = _gelu(jnp.dot(lhs, w1_v[...], preferred_element_type=F32))
        win = h1_v.at[pl.ds(r0, T1 + 16)]
        for k, sh in enumerate((1, -1, 2, -2)):
            win[pl.ds(8 + sh, T1), pl.ds(k * c4, c4)] = h[:, k * c4:(k + 1) * c4]
        return carry

    with jax.named_scope('p1_body'):
        jax.lax.fori_loop(0, N1, p1_body, 0)
    cp_w2.wait()

    def p2_body(i, carry):
        r0 = pl.multiple_of(i * T1, T1)
        hs = h1_v[pl.ds(r0 + 8, T1), :].astype(BF16)
        x1_v[pl.ds(r0, T1), :] = (jnp.dot(hs, w2_v[...], preferred_element_type=F32)
                                  + x_v[pl.ds(r0, T1), :].astype(F32))
        return carry

    with jax.named_scope('p2_body'):
        jax.lax.fori_loop(0, N1, p2_body, 0)

    def prep3(blk, slot, chain):
        r0 = pl.multiple_of(blk * T3, T3)
        zero = zero_v[...] if chain else None
        tok = None
        for k in range(T3 // 16):
            _, y, tok = ln_rows(x1_v[pl.ds(r0 + k * 16, 16), :], tok, zero)
            ln3_v[slot, pl.ds(k * 16, 16), :] = y.astype(BF16)
        return tok

    prep3(0, 0, False)
    cp_w3.wait()
    cp_w4.wait()

    def p3_body(i, carry):
        r0 = pl.multiple_of(i * T3, T3)
        slot = i % 2

        @pl.when(i + 1 < N3)
        def _():
            for c in piece_copies(i + 1, 1 - slot):
                c.start()

        for c in piece_copies(i, slot):
            c.wait()

        lhs = ln3_v[slot]
        tok = prep3(jnp.minimum(i + 1, N3 - 1), 1 - slot, True)
        zero = zero_v[...]
        for which in range(3):
            for j in range(DP // 2):
                blk = pltpu.bitcast(stq_v[slot, which, pl.ds(j * 64, 64), :], U32)
                a = blk[0:16] | tok
                c = blk[16:32]
                lo = (a & jnp.uint32(0xFFFF)) | (c << 16)
                a = a | (lo & zero)
                hi = (a >> 16) | (c & jnp.uint32(0xFFFF0000))
                tok = hi & zero
                s0 = which * H * PITCH + i * (DP // 2) + j
                wqkv_v[pl.ds(s0, 16, stride=PITCH), :] = lo
                wqkv_v[pl.ds(s0 + 16 * PITCH, 16, stride=PITCH), :] = hi
        o0 = pl.multiple_of(i * (OP // 2), OP // 2)
        for j in range(D // 128):
            for k in range(OP // 32):
                w = pltpu.bitcast(sto_v[slot, pl.ds(k * 32, 32), pl.ds(j * 128, 128)], U32) | tok
                tok = w & zero
                wo_v[j, pl.ds(o0 + k * 16, 16), :] = w
        h = _gelu(jnp.dot(lhs, w3_v[...], preferred_element_type=F32)).astype(BF16)
        b = jnp.dot(h, w4_v[...], preferred_element_type=F32) + x1_v[pl.ds(r0, T3), :]
        g = g_v[pl.ds(r0, T3), :]
        omg = jnp.concatenate([1.0 - g] * (D // 128), axis=1)
        h1_v[pl.ds(r0, T3), :] = omg * b
        return carry

    with jax.named_scope('p3_body'):
        jax.lax.fori_loop(0, N3, p3_body, 0)

    mem_v[...] = mem0_ref[...].astype(F32)
    c_exp = (DH ** -0.5) * math.log2(math.e)
    neg_raw = NEG / (DH ** -0.5)

    L2 = 2 * L
    row = jax.lax.broadcasted_iota(jnp.int32, (L2, 128), 0)
    col = jax.lax.broadcasted_iota(jnp.int32, (L2, 128), 1)
    second = row >= L
    rowl = jnp.where(second, row - L, row)
    coll = jnp.where(second, col - L, col)
    real = (coll >= 0) & (coll < L)
    allowed = real & ((rowl < M) | (rowl >= coll))
    fill = jnp.where(real, neg_raw, -jnp.inf).astype(F32)

    def wslab(which, h):
        s = _slab_of(which, h) * PITCH
        return pltpu.bitcast(wqkv_v[pl.ds(s, 512), :], BF16)

    zpad = jnp.zeros((128 - L2, DH), F32)

    def scores(qb, kb):
        s = jax.lax.dot_general(qb, kb, (((1,), (1,)), ((), ())),
                                preferred_element_type=F32)
        s = jnp.where(allowed, s, fill)
        m = jnp.max(s, axis=-1, keepdims=True)
        p = jnp.exp2((s - m) * c_exp)
        l = jnp.sum(p, axis=-1, keepdims=True)
        r = pl.reciprocal(l, approx=True)
        r = r * (2.0 - l * r)
        return (p * r).astype(BF16)

    def wo_part(o_bf, h0, h1, j):
        w = pltpu.bitcast(wo_v[j, pl.ds(h0 * 64, (h1 - h0) * 64), :], BF16)
        return jnp.dot(o_bf, w, preferred_element_type=F32)

    def segment(lhs, assemble, wo_rows):
        NP = H // 2
        qkv = [None] * NP
        pb = [None] * NP
        ob = [None] * H

        def do_qkv(p):
            t = []
            for h in (2 * p, 2 * p + 1):
                q = jnp.dot(lhs, wslab(0, h), preferred_element_type=F32)
                k = jnp.dot(lhs, wslab(1, h), preferred_element_type=F32)
                v = jnp.dot(lhs, wslab(2, h), preferred_element_type=F32)
                t.append(assemble(h, q, k, v))
            qb = jnp.concatenate([t[0][0], t[1][0]], axis=0).astype(BF16)
            kb = jnp.concatenate([t[0][1], t[1][1], zpad], axis=0).astype(BF16)
            vb = jnp.concatenate([t[0][2], t[1][2], zpad], axis=0).astype(BF16)
            qkv[p] = (qb, kb, vb)

        def do_s(p):
            pb[p] = scores(qkv[p][0], qkv[p][1])

        def do_pv(p):
            o = jnp.dot(pb[p], qkv[p][2], preferred_element_type=F32)
            ob[2 * p] = wo_rows(2 * p, o[0:L]).astype(BF16)
            ob[2 * p + 1] = wo_rows(2 * p + 1, o[L:L2]).astype(BF16)

        for p in range(NP):
            do_qkv(p)
            if p >= S_LAG:
                do_s(p - S_LAG)
            if p >= PV_LAG:
                do_pv(p - PV_LAG)
        HA = 2 * (NP - PV_LAG - 1)
        oa = jnp.concatenate(ob[0:HA], axis=1)
        ya = []
        nj = D // 128
        nxt = NP
        for j in range(nj):
            ya.append(wo_part(oa, 0, HA, j))
            if j in TAIL_AT:
                if nxt - S_LAG < NP:
                    do_s(nxt - S_LAG)
                if nxt - PV_LAG < NP:
                    do_pv(nxt - PV_LAG)
                nxt += 1
        assert nxt - PV_LAG >= NP
        ot = jnp.concatenate(ob[HA:H], axis=1)
        y = [wo_part(ot, HA, H, j) + ya[j] for j in range(nj)]
        return jnp.concatenate(y, axis=1)

    def pair(r0, mem):
        xf = x_v[pl.ds(r0, PAIR), :].astype(F32)

        lhs = jnp.concatenate([mem, xf[0:40]], axis=0).astype(BF16)
        extra = [None] * H
        o_left = [None] * H

        def asm_a(h, q, k, v):
            extra[h] = (q[40:48], k[40:48], v[40:48])
            return q[0:40], k[0:40], v[0:40]

        def rows_a(h, o):
            o_left[h] = o[32:40]
            return o[0:32]

        y_a = segment(lhs, asm_a, rows_a)

        lhs = jnp.concatenate([y_a[0:8], xf[40:64]], axis=0).astype(BF16)

        def asm_b(h, q, k, v):
            eq, ek, ev = extra[h]
            return (jnp.concatenate([q[0:8], eq, q[8:32]], axis=0),
                    jnp.concatenate([k[0:8], ek, k[8:32]], axis=0),
                    jnp.concatenate([v[0:8], ev, v[8:32]], axis=0))

        def rows_b(h, o):
            return jnp.concatenate([o, o_left[h]], axis=0)

        y_b = segment(lhs, asm_b, rows_b)

        a = jnp.concatenate([y_a[8:32], y_b[40:48], y_b[8:40]], axis=0)
        g = g_v[pl.ds(r0, PAIR), :]
        g = jnp.concatenate([g] * (D // 128), axis=1)
        out_v[pl.ds(r0, PAIR), :] = (g * a + h1_v[pl.ds(r0, PAIR), :]).astype(BF16)
        return y_b[0:8]

    rows_it = UNROLL_A * PAIR

    def a_body(t, carry):
        base = pl.multiple_of(t * rows_it, rows_it)
        mem = mem_v[...]
        for u in range(UNROLL_A):
            mem = pair(pl.multiple_of(base + u * PAIR, PAIR), mem)
        mem_v[...] = mem
        pltpu.make_async_copy(out_v.at[pl.ds(base, rows_it)], out_hbm.at[pl.ds(base, rows_it)],
                              osem).start()
        return carry

    with jax.named_scope('a_body'):
        jax.lax.fori_loop(0, S // rows_it, a_body, 0)
    pltpu.make_async_copy(out_v, out_hbm, osem).wait()


@functools.partial(jax.jit, static_argnames=("A_seg_len",))
def pallas_gated_mix__memory_aug_recurrent_mem_tr__mixer_s_mlp__prompt_kernel(
    A_x, A_mem0, A_Wq, A_Wk, A_Wv, A_Wo, A_seg_len, B_x, B_w1, B_w2, B_w3, B_w4, gate_w,
):
    assert A_seg_len == SEG
    assert A_x.shape == (1, S, D) and A_Wq.shape == (D, H, DH) and A_mem0.shape == (1, M, D)
    x = A_x.reshape(S, D)
    mem0 = A_mem0.reshape(M, D)
    wq = A_Wq.reshape(D * H, DH)
    wk = A_Wk.reshape(D * H, DH)
    wv = A_Wv.reshape(D * H, DH)
    wo = A_Wo.reshape(H * DH, D)
    gw = gate_w.reshape(1, D)

    any_spec = pl.BlockSpec(memory_space=pl.ANY)
    vmem_spec = pl.BlockSpec(memory_space=pltpu.VMEM)
    out = pl.pallas_call(
        _kernel,
        out_shape=jax.ShapeDtypeStruct((S, D), BF16),
        in_specs=[any_spec, vmem_spec, any_spec, any_spec, any_spec, any_spec,
                  any_spec, any_spec, any_spec, any_spec, vmem_spec],
        out_specs=any_spec,
        scratch_shapes=[
            pltpu.VMEM((S, D), BF16),
            pltpu.VMEM((2, 3, DP * H, DH), BF16),
            pltpu.VMEM((2, OP, D), BF16),
            pltpu.VMEM((3 * H * PITCH, 128), U32),
            pltpu.VMEM((D // 128, H * DH // 2, 128), U32),
            pltpu.VMEM((D, D), BF16),
            pltpu.VMEM((D, D), BF16),
            pltpu.VMEM((D, FF), BF16),
            pltpu.VMEM((FF, D), BF16),
            pltpu.VMEM((S + 16, D), F32),
            pltpu.VMEM((S, D), F32),
            pltpu.VMEM((S, 128), F32),
            pltpu.VMEM((2, T1, D), BF16),
            pltpu.VMEM((2, T3, D), BF16),
            pltpu.VMEM((M, D), F32),
            pltpu.VMEM((S, D), BF16),
            pltpu.VMEM((16, 128), U32),
            pltpu.SemaphoreType.DMA((5,)),
            pltpu.SemaphoreType.DMA((N1,)),
            pltpu.SemaphoreType.DMA((2, 4)),
            pltpu.SemaphoreType.DMA(()),
        ],
        compiler_params=pltpu.CompilerParams(vmem_limit_bytes=120 * 1024 * 1024),
    )(x, mem0, wq, wk, wv, wo, B_w1, B_w2, B_w3, B_w4, gw)
    return out.reshape(1, S, D)
```

```python
import functools
import math

import jax
import jax.numpy as jnp
import jax.experimental.pallas as pl
import jax.experimental.pallas.tpu as pltpu

F32 = jnp.float32
BF16 = jnp.bfloat16
U32 = jnp.uint32

S = 2048
D = 1024
H = 32
DH = 128
M = 8
SEG = 32
L = M + SEG
FF = 3584
PAIR = 2 * SEG
NPAIR = S // PAIR
T1 = 256
N1 = S // T1
T3 = 256
N3 = S // T3
DP = D // N3
OP = H * DH // N3
UNROLL_A = 1
PITCH = 520
SEM_X = 6
SEM_P = SEM_X + N1
NSEM = SEM_P + 8
EPS = 1e-5
NCHAIN1 = 2
S_LAG = 1
PV_LAG = 3
TAIL_AT = (1, 3, 5)
NEG = -1e9


def _gelu(x):
    c = math.sqrt(2.0 / math.pi)
    return 0.5 * x * (1.0 + jnp.tanh(c * (x + 0.044715 * (x * x * x))))


def _layernorm(x):
    m = jnp.mean(x, axis=-1, keepdims=True)
    xc = x - m
    v = jnp.mean(xc * xc, axis=-1, keepdims=True)
    return xc * jax.lax.rsqrt(v + EPS)


def _slab_of(which, h):
    return which * H + (h % 2) * (H // 2) + h // 2


def _kernel(x_hbm, mem0_hbm, wq_hbm, wk_hbm, wv_hbm, wo_hbm,
            w1_hbm, w2_hbm, w3_hbm, w4_hbm, gw_hbm,
            out_hbm,
            x_v, stq_v, sto_v, wqkv_v, wo_v, w1_v, w2_v, w3_v, w4_v,
            h1_v, x1_v, g_v, ln1_v, ln3_v, mem0_v, gw_v, mem_v, out_v, zero_v, sems, osem):
    def cp_x(i):
        r0 = i * T1 if isinstance(i, int) else pl.multiple_of(i * T1, T1)
        return pltpu.make_async_copy(x_hbm.at[pl.ds(r0, T1)], x_v.at[pl.ds(r0, T1)],
                                     sems.at[SEM_X + i])

    cp_gw = pltpu.make_async_copy(gw_hbm, gw_v, sems.at[0])
    cp_w1 = pltpu.make_async_copy(w1_hbm, w1_v, sems.at[1])
    cp_w2 = pltpu.make_async_copy(w2_hbm, w2_v, sems.at[2])
    cp_w3 = pltpu.make_async_copy(w3_hbm, w3_v, sems.at[3])
    cp_w4 = pltpu.make_async_copy(w4_hbm, w4_v, sems.at[4])
    cp_m0 = pltpu.make_async_copy(mem0_hbm, mem0_v, sems.at[5])

    def piece_copies(i, slot):
        cps = [pltpu.make_async_copy(w.at[pl.ds(i * (DP * H), DP * H)], stq_v.at[slot, k],
                                     sems.at[SEM_P + 4 * slot + k])
               for k, w in enumerate((wq_hbm, wk_hbm, wv_hbm))]
        cps.append(pltpu.make_async_copy(wo_hbm.at[pl.ds(i * OP, OP)], sto_v.at[slot],
                                         sems.at[SEM_P + 4 * slot + 3]))
        return cps

    cp_gw.start()
    cp_x(0).start()
    cp_w1.start()
    for i in range(1, N1):
        cp_x(i).start()
    cp_w2.start()
    cp_m0.start()
    cp_w3.start()
    cp_w4.start()
    for c in piece_copies(0, 0):
        c.start()
    h1_v[pl.ds(8, 8), :] = jnp.zeros((8, D), F32)
    h1_v[pl.ds(S, 8), :] = jnp.zeros((8, D), F32)
    zero_v[...] = jnp.zeros((16, 128), U32)
    cp_gw.wait()
    gw = gw_v[...].astype(F32).reshape(1, D)

    def tie(x, tok):
        head = pltpu.bitcast(pltpu.bitcast(x[:, 0:128], U32) | tok, F32)
        return jnp.concatenate([head, x[:, 128:]], axis=1)

    def ln_rows(x, tok, zero):
        if tok is not None:
            x = tie(x, tok)
        part = x[:, 0:128]
        for j in range(1, D // 128):
            part = part + x[:, j * 128:(j + 1) * 128]
        m = jnp.sum(part, axis=-1, keepdims=True) * (1.0 / D)
        xc = x - m
        v = jnp.mean(xc * xc, axis=-1, keepdims=True)
        y = xc * jax.lax.rsqrt(v + EPS)
        tok = None if zero is None else pltpu.bitcast(y[:, 0:128], U32) & zero
        return x, y, tok

    def prep1(blk, slot, chain):
        r0 = pl.multiple_of(blk * T1, T1)
        zero = zero_v[...] if chain else None
        toks = [None] * NCHAIN1
        for k in range(T1 // 16):
            xf = x_v[pl.ds(r0 + k * 16, 16), :].astype(F32)
            xf, y, toks[k % NCHAIN1] = ln_rows(xf, toks[k % NCHAIN1], zero)
            ln1_v[slot, pl.ds(k * 16, 16), :] = y.astype(BF16)
            z = jnp.sum(xf * gw, axis=-1, keepdims=True)
            g_v[pl.ds(r0 + k * 16, 16), :] = jnp.broadcast_to(1.0 / (1.0 + jnp.exp(-z)), (16, 128))

    cp_x(0).wait()
    prep1(0, 0, False)
    cp_w1.wait()

    c4 = D // 4

    def p1_body(i, carry):
        r0 = pl.multiple_of(i * T1, T1)
        slot = i % 2

        @pl.when(i + 1 < N1)
        def _():
            cp_x(i + 1).wait()

        lhs = ln1_v[slot]
        prep1(jnp.minimum(i + 1, N1 - 1), 1 - slot, True)
        h = _gelu(jnp.dot(lhs, w1_v[...], preferred_element_type=F32))
        win = h1_v.at[pl.ds(r0, T1 + 16)]
        for k, sh in enumerate((1, -1, 2, -2)):
            win[pl.ds(8 + sh, T1), pl.ds(k * c4, c4)] = h[:, k * c4:(k + 1) * c4]
        return carry

    with jax.named_scope('p1_body'):
        jax.lax.fori_loop(0, N1, p1_body, 0)
    cp_w2.wait()

    def p2_body(i, carry):
        r0 = pl.multiple_of(i * T1, T1)
        hs = h1_v[pl.ds(r0 + 8, T1), :].astype(BF16)
        x1_v[pl.ds(r0, T1), :] = (jnp.dot(hs, w2_v[...], preferred_element_type=F32)
                                  + x_v[pl.ds(r0, T1), :].astype(F32))
        return carry

    with jax.named_scope('p2_body'):
        jax.lax.fori_loop(0, N1, p2_body, 0)

    def prep3(blk, slot, chain):
        r0 = pl.multiple_of(blk * T3, T3)
        zero = zero_v[...] if chain else None
        tok = None
        for k in range(T3 // 16):
            _, y, tok = ln_rows(x1_v[pl.ds(r0 + k * 16, 16), :], tok, zero)
            ln3_v[slot, pl.ds(k * 16, 16), :] = y.astype(BF16)
        return tok

    prep3(0, 0, False)
    cp_m0.wait()
    cp_w3.wait()
    cp_w4.wait()

    def p3_body(i, carry):
        r0 = pl.multiple_of(i * T3, T3)
        slot = i % 2

        @pl.when(i + 1 < N3)
        def _():
            for c in piece_copies(i + 1, 1 - slot):
                c.start()

        for c in piece_copies(i, slot):
            c.wait()

        lhs = ln3_v[slot]
        tok = prep3(jnp.minimum(i + 1, N3 - 1), 1 - slot, True)
        zero = zero_v[...]
        for which in range(3):
            for j in range(DP // 2):
                blk = pltpu.bitcast(stq_v[slot, which, pl.ds(j * 64, 64), :], U32)
                a = blk[0:16] | tok
                c = blk[16:32]
                lo = (a & jnp.uint32(0xFFFF)) | (c << 16)
                a = a | (lo & zero)
                hi = (a >> 16) | (c & jnp.uint32(0xFFFF0000))
                tok = hi & zero
                s0 = which * H * PITCH + i * (DP // 2) + j
                wqkv_v[pl.ds(s0, 16, stride=PITCH), :] = lo
                wqkv_v[pl.ds(s0 + 16 * PITCH, 16, stride=PITCH), :] = hi
        o0 = pl.multiple_of(i * (OP // 2), OP // 2)
        for j in range(D // 128):
            for k in range(OP // 32):
                w = pltpu.bitcast(sto_v[slot, pl.ds(k * 32, 32), pl.ds(j * 128, 128)], U32) | tok
                tok = w & zero
                wo_v[j, pl.ds(o0 + k * 16, 16), :] = w
        h = _gelu(jnp.dot(lhs, w3_v[...], preferred_element_type=F32)).astype(BF16)
        b = jnp.dot(h, w4_v[...], preferred_element_type=F32) + x1_v[pl.ds(r0, T3), :]
        g = g_v[pl.ds(r0, T3), :]
        omg = jnp.concatenate([1.0 - g] * (D // 128), axis=1)
        h1_v[pl.ds(r0, T3), :] = omg * b
        return carry

    with jax.named_scope('p3_body'):
        jax.lax.fori_loop(0, N3, p3_body, 0)

    mem_v[...] = mem0_v[...].astype(F32)
    c_exp = (DH ** -0.5) * math.log2(math.e)
    neg_raw = NEG / (DH ** -0.5)

    L2 = 2 * L
    row = jax.lax.broadcasted_iota(jnp.int32, (L2, 128), 0)
    col = jax.lax.broadcasted_iota(jnp.int32, (L2, 128), 1)
    second = row >= L
    rowl = jnp.where(second, row - L, row)
    coll = jnp.where(second, col - L, col)
    real = (coll >= 0) & (coll < L)
    allowed = real & ((rowl < M) | (rowl >= coll))
    fill = jnp.where(real, neg_raw, -jnp.inf).astype(F32)

    def wslab(which, h, r0, n):
        s = _slab_of(which, h) * PITCH
        return pltpu.bitcast(wqkv_v[pl.ds(s + r0, n), :], BF16)

    zpad = jnp.zeros((128 - L2, DH), F32)

    def scores(qb, kb):
        s = jax.lax.dot_general(qb, kb, (((1,), (1,)), ((), ())),
                                preferred_element_type=F32)
        s = jnp.where(allowed, s, fill)
        m = jnp.max(s, axis=-1, keepdims=True)
        p = jnp.exp2((s - m) * c_exp)
        l = jnp.sum(p, axis=-1, keepdims=True)
        r = pl.reciprocal(l, approx=True)
        r = r * (2.0 - l * r)
        return (p * r).astype(BF16)

    def wo_part(o_bf, h0, h1, j):
        w = pltpu.bitcast(wo_v[j, pl.ds(h0 * 64, (h1 - h0) * 64), :], BF16)
        return jnp.dot(o_bf, w, preferred_element_type=F32)

    def segment(lhs, assemble, wo_rows, split_first, early_wo):
        NP = H // 2
        nj = D // 128
        qkv = [None] * NP
        pb = [None] * NP
        ob = [None] * H

        def do_qkv(p):
            slabs = [(which, h) for h in (2 * p, 2 * p + 1) for which in range(3)]
            if p == 0 and split_first:
                r = [jnp.dot(lhs[:, 0:D // 2], wslab(w, h, 0, 256), preferred_element_type=F32)
                     for w, h in slabs]
                r = [jnp.dot(lhs[:, D // 2:D], wslab(w, h, 256, 256),
                             preferred_element_type=F32) + acc
                     for (w, h), acc in zip(slabs, r)]
            else:
                r = [jnp.dot(lhs, wslab(w, h, 0, 512), preferred_element_type=F32)
                     for w, h in slabs]
            t = [assemble(2 * p, *r[0:3]), assemble(2 * p + 1, *r[3:6])]
            qb = jnp.concatenate([t[0][0], t[1][0]], axis=0).astype(BF16)
            kb = jnp.concatenate([t[0][1], t[1][1], zpad], axis=0).astype(BF16)
            vb = jnp.concatenate([t[0][2], t[1][2], zpad], axis=0).astype(BF16)
            qkv[p] = (qb, kb, vb)

        def do_s(p):
            pb[p] = scores(qkv[p][0], qkv[p][1])

        def do_pv(p):
            o = jnp.dot(pb[p], qkv[p][2], preferred_element_type=F32)
            ob[2 * p] = wo_rows(2 * p, o[0:L]).astype(BF16)
            ob[2 * p + 1] = wo_rows(2 * p + 1, o[L:L2]).astype(BF16)

        y = [None] * nj

        def do_wo(h0, h1, j):
            r = wo_part(jnp.concatenate(ob[h0:h1], axis=1), h0, h1, j)
            y[j] = r if y[j] is None else r + y[j]

        H0 = early_wo
        for p in range(NP):
            do_qkv(p)
            if H0 and p >= NP - nj:
                do_wo(0, H0, p - (NP - nj))
            if p >= S_LAG:
                do_s(p - S_LAG)
            if p >= PV_LAG:
                do_pv(p - PV_LAG)
        HA = 2 * (NP - PV_LAG - 1)
        nxt = NP
        for j in range(nj):
            do_wo(H0, HA, j)
            if j in TAIL_AT:
                if nxt - S_LAG < NP:
                    do_s(nxt - S_LAG)
                if nxt - PV_LAG < NP:
                    do_pv(nxt - PV_LAG)
                nxt += 1
        assert nxt - PV_LAG >= NP
        for j in range(nj):
            do_wo(HA, H, j)
        return jnp.concatenate(y, axis=1)

    def pair(r0, mem):
        xf = x_v[pl.ds(r0, PAIR), :].astype(F32)

        lhs = jnp.concatenate([mem, xf[0:40]], axis=0).astype(BF16)
        extra = [None] * H
        o_left = [None] * H

        def asm_a(h, q, k, v):
            extra[h] = (q[40:48], k[40:48], v[40:48])
            return q[0:40], k[0:40], v[0:40]

        def rows_a(h, o):
            o_left[h] = o[32:40]
            return o[0:32]

        y_a = segment(lhs, asm_a, rows_a, False, 0)

        lhs = jnp.concatenate([y_a[0:8], xf[40:64]], axis=0).astype(BF16)

        def asm_b(h, q, k, v):
            eq, ek, ev = extra[h]
            return (jnp.concatenate([q[0:8], eq, q[8:32]], axis=0),
                    jnp.concatenate([k[0:8], ek, k[8:32]], axis=0),
                    jnp.concatenate([v[0:8], ev, v[8:32]], axis=0))

        def rows_b(h, o):
            return jnp.concatenate([o, o_left[h]], axis=0)

        y_b = segment(lhs, asm_b, rows_b, True, 8)

        a = jnp.concatenate([y_a[8:32], y_b[40:48], y_b[8:40]], axis=0)
        g = g_v[pl.ds(r0, PAIR), :]
        g = jnp.concatenate([g] * (D // 128), axis=1)
        out_v[pl.ds(r0, PAIR), :] = (g * a + h1_v[pl.ds(r0, PAIR), :]).astype(BF16)
        return y_b[0:8]

    rows_it = UNROLL_A * PAIR

    def a_body(t, carry):
        base = pl.multiple_of(t * rows_it, rows_it)
        mem = mem_v[...]
        for u in range(UNROLL_A):
            mem = pair(pl.multiple_of(base + u * PAIR, PAIR), mem)
        mem_v[...] = mem
        pltpu.make_async_copy(out_v.at[pl.ds(base, rows_it)], out_hbm.at[pl.ds(base, rows_it)],
                              osem).start()
        return carry

    with jax.named_scope('a_body'):
        jax.lax.fori_loop(0, S // rows_it, a_body, 0)
    pltpu.make_async_copy(out_v, out_hbm, osem).wait()


@functools.partial(jax.jit, static_argnames=("A_seg_len",))
def pallas_gated_mix__memory_aug_recurrent_mem_tr__mixer_s_mlp__prompt_kernel(
    A_x, A_mem0, A_Wq, A_Wk, A_Wv, A_Wo, A_seg_len, B_x, B_w1, B_w2, B_w3, B_w4, gate_w,
):
    assert A_seg_len == SEG
    assert A_x.shape == (1, S, D) and A_Wq.shape == (D, H, DH) and A_mem0.shape == (1, M, D)
    x = A_x.reshape(S, D)
    mem0 = A_mem0.reshape(M, D)
    wq = A_Wq.reshape(D * H, DH)
    wk = A_Wk.reshape(D * H, DH)
    wv = A_Wv.reshape(D * H, DH)
    wo = A_Wo.reshape(H * DH, D)

    any_spec = pl.BlockSpec(memory_space=pl.ANY)
    out = pl.pallas_call(
        _kernel,
        out_shape=jax.ShapeDtypeStruct((S, D), BF16),
        in_specs=[any_spec] * 11,
        out_specs=any_spec,
        scratch_shapes=[
            pltpu.VMEM((S, D), BF16),
            pltpu.VMEM((2, 3, DP * H, DH), BF16),
            pltpu.VMEM((2, OP, D), BF16),
            pltpu.VMEM((3 * H * PITCH, 128), U32),
            pltpu.VMEM((D // 128, H * DH // 2, 128), U32),
            pltpu.VMEM((D, D), BF16),
            pltpu.VMEM((D, D), BF16),
            pltpu.VMEM((D, FF), BF16),
            pltpu.VMEM((FF, D), BF16),
            pltpu.VMEM((S + 16, D), F32),
            pltpu.VMEM((S, D), F32),
            pltpu.VMEM((S, 128), F32),
            pltpu.VMEM((2, T1, D), BF16),
            pltpu.VMEM((2, T3, D), BF16),
            pltpu.VMEM((M, D), BF16),
            pltpu.VMEM((D,), BF16),
            pltpu.VMEM((M, D), F32),
            pltpu.VMEM((S, D), BF16),
            pltpu.VMEM((16, 128), U32),
            pltpu.SemaphoreType.DMA((NSEM,)),
            pltpu.SemaphoreType.DMA(()),
        ],
        compiler_params=pltpu.CompilerParams(vmem_limit_bytes=120 * 1024 * 1024,
                                             disable_bounds_checks=True),
    )(x, mem0, wq, wk, wv, wo, B_w1, B_w2, B_w3, B_w4, gate_w)
    return out.reshape(1, S, D)
```

```python
import functools
import math

import jax
import jax.numpy as jnp
import jax.experimental.pallas as pl
import jax.experimental.pallas.tpu as pltpu

F32 = jnp.float32
BF16 = jnp.bfloat16
U32 = jnp.uint32

S = 2048
D = 1024
H = 32
DH = 128
M = 8
SEG = 32
L = M + SEG
FF = 3584
PAIR = 2 * SEG
NPAIR = S // PAIR
T1 = 256
N1 = S // T1
T2 = 512
N2 = S // T2
T3 = 256
N3 = S // T3
DP = D // N3
OP = H * DH // N3
UNROLL_A = 1
PITCH = 520
SEM_X = 12
SEM_P = SEM_X + N1
NSEM = SEM_P + 8
EPS = 1e-5
NCHAIN0 = 5
NCHAIN1 = 2
HOP = 4
S_LAG = 1
PV_LAG = 3
TAIL_AT = (1, 3, 5)
NEG = -1e9


def _gelu(x):
    c = math.sqrt(2.0 / math.pi)
    return 0.5 * x * (1.0 + jnp.tanh(c * (x + 0.044715 * (x * x * x))))


def _layernorm(x):
    m = jnp.mean(x, axis=-1, keepdims=True)
    xc = x - m
    v = jnp.mean(xc * xc, axis=-1, keepdims=True)
    return xc * jax.lax.rsqrt(v + EPS)


def _slab_of(which, h):
    return which * H + (h % 2) * (H // 2) + h // 2


def _kernel(x_hbm, mem0_hbm, wq_hbm, wk_hbm, wv_hbm, wo_hbm,
            w1_hbm, w2_hbm, w3_hbm, w4_hbm, gw_hbm,
            out_hbm,
            x_v, stq_v, sto_v, wqkv_v, wo_v, w1_v, w2_v, w3_v, w4_v,
            h1_v, x1_v, g_v, ln1_v, ln3_v, mem0_v, gw_v, mem_v, out_v, zero_v, sems, osem):
    def cp_x(i):
        r0 = i * T1 if isinstance(i, int) else pl.multiple_of(i * T1, T1)
        return pltpu.make_async_copy(x_hbm.at[pl.ds(r0, T1)], x_v.at[pl.ds(r0, T1)],
                                     sems.at[SEM_X + i])

    c4 = D // 4
    cp_gw = pltpu.make_async_copy(gw_hbm, gw_v, sems.at[0])
    cp_m0 = pltpu.make_async_copy(mem0_hbm, mem0_v, sems.at[1])
    cp_w3 = pltpu.make_async_copy(w3_hbm, w3_v, sems.at[2])
    cp_w4 = pltpu.make_async_copy(w4_hbm, w4_v, sems.at[3])
    cp_w1 = [pltpu.make_async_copy(w1_hbm.at[:, pl.ds(q * c4, c4)], w1_v.at[q], sems.at[4 + q])
             for q in range(4)]
    cp_w2 = [pltpu.make_async_copy(w2_hbm.at[:, pl.ds(q * c4, c4)], w2_v.at[q], sems.at[8 + q])
             for q in range(4)]

    def piece_copies(i, slot):
        cps = [pltpu.make_async_copy(w.at[pl.ds(i * (DP * H), DP * H)], stq_v.at[slot, k],
                                     sems.at[SEM_P + 4 * slot + k])
               for k, w in enumerate((wq_hbm, wk_hbm, wv_hbm))]
        cps.append(pltpu.make_async_copy(wo_hbm.at[pl.ds(i * OP, OP)], sto_v.at[slot],
                                         sems.at[SEM_P + 4 * slot + 3]))
        return cps

    cp_x(0).start()
    for c in cp_w1:
        c.start()
    for i in range(1, N1):
        cp_x(i).start()
    for c in cp_w2:
        c.start()
    cp_gw.start()
    cp_m0.start()
    cp_w3.start()
    cp_w4.start()
    for c in piece_copies(0, 0):
        c.start()
    h1_v[pl.ds(8, 8), :] = jnp.zeros((8, D), F32)
    h1_v[pl.ds(S, 8), :] = jnp.zeros((8, D), F32)
    zero_v[...] = jnp.zeros((16, 128), U32)

    def ln_rows(x, tok, zero):
        if tok is not None:
            head = pltpu.bitcast(pltpu.bitcast(x[:, 0:128], U32) | tok, F32)
            x = jnp.concatenate([head, x[:, 128:]], axis=1)
        y = _layernorm(x)
        tok = None if zero is None else pltpu.bitcast(y[:, 0:128], U32) & zero
        return y, tok

    def ln_block(load, store, rows, nchain):
        zero = zero_v[...] if nchain else None
        toks = [None] * max(nchain, 1)
        for k in range(rows // 16):
            y, toks[k % len(toks)] = ln_rows(load(k), toks[k % len(toks)], zero)
            store(k, y.astype(BF16))
        return toks[(rows // 16 - 1) % len(toks)]

    def prep1(blk, slot, nchain):
        r0 = blk * T1 if isinstance(blk, int) else pl.multiple_of(blk * T1, T1)

        def store(k, y):
            ln1_v[slot, pl.ds(k * 16, 16), :] = y

        ln_block(lambda k: x_v[pl.ds(r0 + k * 16, 16), :].astype(F32), store, T1, nchain)

    def p1_quarter(lhs, r0, q):
        h = _gelu(jnp.dot(lhs, w1_v[q], preferred_element_type=F32))
        win = h1_v.at[pl.ds(r0, T1 + 16)]
        win[pl.ds(8 + (1, -1, 2, -2)[q], T1), pl.ds(q * c4, c4)] = h

    cp_x(0).wait()
    prep1(0, 0, 0)
    for q in range(4):
        cp_w1[q].wait()
        if q == 3:
            cp_x(1).wait()
        lhs = ln1_v[0]
        if q == 3:
            prep1(1, 1, NCHAIN0)
        p1_quarter(lhs, 0, q)

    def p1_body(i, carry):
        r0 = pl.multiple_of(i * T1, T1)
        slot = i % 2

        @pl.when(i + 1 < N1)
        def _():
            cp_x(i + 1).wait()

        lhs = ln1_v[slot]
        prep1(jnp.minimum(i + 1, N1 - 1), 1 - slot, NCHAIN1)
        for q in range(4):
            p1_quarter(lhs, r0, q)
        return carry

    with jax.named_scope('p1_body'):
        jax.lax.fori_loop(1, N1, p1_body, 0)
    for c in cp_w2:
        c.wait()

    def p2_body(i, carry):
        r0 = pl.multiple_of(i * T2, T2)
        hs = h1_v[pl.ds(r0 + 8, T2), :].astype(BF16)
        for q in range(4):
            x1_v[pl.ds(r0, T2), pl.ds(q * c4, c4)] = (
                jnp.dot(hs, w2_v[q], preferred_element_type=F32)
                + x_v[pl.ds(r0, T2), pl.ds(q * c4, c4)].astype(F32))
        return carry

    with jax.named_scope('p2_body'):
        jax.lax.fori_loop(0, N2, p2_body, 0)

    def prep3(blk, slot, nchain):
        r0 = blk * T3 if isinstance(blk, int) else pl.multiple_of(blk * T3, T3)

        def store(k, y):
            ln3_v[slot, pl.ds(k * 16, 16), :] = y

        return ln_block(lambda k: x1_v[pl.ds(r0 + k * 16, 16), :], store, T3, nchain)

    prep3(0, 0, 0)
    cp_gw.wait()
    cp_m0.wait()
    cp_w3.wait()
    cp_w4.wait()

    def p3_body(i, carry):
        r0 = pl.multiple_of(i * T3, T3)
        slot = i % 2

        @pl.when(i + 1 < N3)
        def _():
            for c in piece_copies(i + 1, 1 - slot):
                c.start()

        for c in piece_copies(i, slot):
            c.wait()

        lhs = ln3_v[slot]
        tok = prep3(jnp.minimum(i + 1, N3 - 1), 1 - slot, 1)
        zero = zero_v[...]
        for which in range(3):
            for j in range(DP // 2):
                blk = pltpu.bitcast(stq_v[slot, which, pl.ds(j * 64, 64), :], U32)
                a = blk[0:16] | tok
                c = blk[16:32]
                lo = (a & jnp.uint32(0xFFFF)) | (c << 16)
                a = a | (lo & zero)
                hi = (a >> 16) | (c & jnp.uint32(0xFFFF0000))
                tok = hi & zero
                if j % HOP == HOP - 1:
                    tok = pltpu.roll(tok, 1, 1)
                s0 = which * H * PITCH + i * (DP // 2) + j
                wqkv_v[pl.ds(s0, 16, stride=PITCH), :] = lo
                wqkv_v[pl.ds(s0 + 16 * PITCH, 16, stride=PITCH), :] = hi
        o0 = pl.multiple_of(i * (OP // 2), OP // 2)
        for j in range(D // 128):
            for k in range(OP // 32):
                w = pltpu.bitcast(sto_v[slot, pl.ds(k * 32, 32), pl.ds(j * 128, 128)], U32) | tok
                tok = w & zero
                if k % (2 * HOP) == 2 * HOP - 1:
                    tok = pltpu.roll(tok, 1, 1)
                wo_v[j, pl.ds(o0 + k * 16, 16), :] = w

        h = _gelu(jnp.dot(lhs, w3_v[...], preferred_element_type=F32)).astype(BF16)
        b = jnp.dot(h, w4_v[...], preferred_element_type=F32) + x1_v[pl.ds(r0, T3), :]
        gw = gw_v[...].astype(F32).reshape(1, D)
        z = jnp.sum(x_v[pl.ds(r0, T3), :].astype(F32) * gw, axis=-1, keepdims=True)
        g = 1.0 / (1.0 + jnp.exp(-z))
        g_v[pl.ds(r0, T3), :] = jnp.broadcast_to(g, (T3, 128))
        h1_v[pl.ds(r0, T3), :] = (1.0 - g) * b
        return carry

    with jax.named_scope('p3_body'):
        jax.lax.fori_loop(0, N3, p3_body, 0)

    mem_v[...] = mem0_v[...].astype(F32)
    c_exp = (DH ** -0.5) * math.log2(math.e)
    neg_raw = NEG / (DH ** -0.5)

    L2 = 2 * L
    row = jax.lax.broadcasted_iota(jnp.int32, (L2, 128), 0)
    col = jax.lax.broadcasted_iota(jnp.int32, (L2, 128), 1)
    second = row >= L
    rowl = jnp.where(second, row - L, row)
    coll = jnp.where(second, col - L, col)
    real = (coll >= 0) & (coll < L)
    allowed = real & ((rowl < M) | (rowl >= coll))
    fill = jnp.where(real, neg_raw, -jnp.inf).astype(F32)

    def wslab(which, h, r0, n):
        s = _slab_of(which, h) * PITCH
        return pltpu.bitcast(wqkv_v[pl.ds(s + r0, n), :], BF16)

    zpad = jnp.zeros((128 - L2, DH), F32)

    def scores(qb, kb):
        s = jax.lax.dot_general(qb, kb, (((1,), (1,)), ((), ())),
                                preferred_element_type=F32)
        s = jnp.where(allowed, s, fill)
        m = jnp.max(s, axis=-1, keepdims=True)
        p = jnp.exp2((s - m) * c_exp)
        l = jnp.sum(p, axis=-1, keepdims=True)
        r = pl.reciprocal(l, approx=True)
        r = r * (2.0 - l * r)
        return (p * r).astype(BF16)

    def wo_part(o_bf, h0, h1, j):
        w = pltpu.bitcast(wo_v[j, pl.ds(h0 * 64, (h1 - h0) * 64), :], BF16)
        return jnp.dot(o_bf, w, preferred_element_type=F32)

    def segment(lhs, assemble, wo_rows, split_first, early_wo):
        NP = H // 2
        nj = D // 128
        qkv = [None] * NP
        pb = [None] * NP
        ob = [None] * H

        def do_qkv(p):
            slabs = [(which, h) for h in (2 * p, 2 * p + 1) for which in range(3)]
            if p == 0 and split_first:
                r = [jnp.dot(lhs[:, 0:D // 2], wslab(w, h, 0, 256), preferred_element_type=F32)
                     for w, h in slabs]
                r = [jnp.dot(lhs[:, D // 2:D], wslab(w, h, 256, 256),
                             preferred_element_type=F32) + acc
                     for (w, h), acc in zip(slabs, r)]
            else:
                r = [jnp.dot(lhs, wslab(w, h, 0, 512), preferred_element_type=F32)
                     for w, h in slabs]
            t = [assemble(2 * p, *r[0:3]), assemble(2 * p + 1, *r[3:6])]
            qb = jnp.concatenate([t[0][0], t[1][0]], axis=0).astype(BF16)
            kb = jnp.concatenate([t[0][1], t[1][1], zpad], axis=0).astype(BF16)
            vb = jnp.concatenate([t[0][2], t[1][2], zpad], axis=0).astype(BF16)
            qkv[p] = (qb, kb, vb)

        def do_s(p):
            pb[p] = scores(qkv[p][0], qkv[p][1])

        def do_pv(p):
            o = jnp.dot(pb[p], qkv[p][2], preferred_element_type=F32)
            ob[2 * p] = wo_rows(2 * p, o[0:L]).astype(BF16)
            ob[2 * p + 1] = wo_rows(2 * p + 1, o[L:L2]).astype(BF16)

        y = [None] * nj

        def do_wo(h0, h1, j):
            r = wo_part(jnp.concatenate(ob[h0:h1], axis=1), h0, h1, j)
            y[j] = r if y[j] is None else r + y[j]

        H0 = early_wo
        for p in range(NP):
            do_qkv(p)
            if H0 and p >= NP - nj:
                do_wo(0, H0, p - (NP - nj))
            if p >= S_LAG:
                do_s(p - S_LAG)
            if p >= PV_LAG:
                do_pv(p - PV_LAG)
        HA = 2 * (NP - PV_LAG - 1)
        nxt = NP
        for j in range(nj):
            do_wo(H0, HA, j)
            if j in TAIL_AT:
                if nxt - S_LAG < NP:
                    do_s(nxt - S_LAG)
                if nxt - PV_LAG < NP:
                    do_pv(nxt - PV_LAG)
                nxt += 1
        assert nxt - PV_LAG >= NP
        for j in range(nj):
            do_wo(HA, H, j)
        return jnp.concatenate(y, axis=1)

    def pair(r0, mem):
        xf = x_v[pl.ds(r0, PAIR), :].astype(F32)

        lhs = jnp.concatenate([mem, xf[0:40]], axis=0).astype(BF16)
        extra = [None] * H
        o_left = [None] * H

        def asm_a(h, q, k, v):
            extra[h] = (q[40:48], k[40:48], v[40:48])
            return q[0:40], k[0:40], v[0:40]

        def rows_a(h, o):
            o_left[h] = o[32:40]
            return o[0:32]

        y_a = segment(lhs, asm_a, rows_a, False, 0)

        lhs = jnp.concatenate([y_a[0:8], xf[40:64]], axis=0).astype(BF16)

        def asm_b(h, q, k, v):
            eq, ek, ev = extra[h]
            return (jnp.concatenate([q[0:8], eq, q[8:32]], axis=0),
                    jnp.concatenate([k[0:8], ek, k[8:32]], axis=0),
                    jnp.concatenate([v[0:8], ev, v[8:32]], axis=0))

        def rows_b(h, o):
            return jnp.concatenate([o, o_left[h]], axis=0)

        y_b = segment(lhs, asm_b, rows_b, True, 8)

        a = jnp.concatenate([y_a[8:32], y_b[40:48], y_b[8:40]], axis=0)
        g = g_v[pl.ds(r0, PAIR), :]
        g = jnp.concatenate([g] * (D // 128), axis=1)
        out_v[pl.ds(r0, PAIR), :] = (g * a + h1_v[pl.ds(r0, PAIR), :]).astype(BF16)
        return y_b[0:8]

    rows_it = UNROLL_A * PAIR

    def a_body(t, carry):
        base = pl.multiple_of(t * rows_it, rows_it)
        mem = mem_v[...]
        for u in range(UNROLL_A):
            mem = pair(pl.multiple_of(base + u * PAIR, PAIR), mem)
        mem_v[...] = mem
        pltpu.make_async_copy(out_v.at[pl.ds(base, rows_it)], out_hbm.at[pl.ds(base, rows_it)],
                              osem).start()
        return carry

    with jax.named_scope('a_body'):
        jax.lax.fori_loop(0, S // rows_it, a_body, 0)
    pltpu.make_async_copy(out_v, out_hbm, osem).wait()


@functools.partial(jax.jit, static_argnames=("A_seg_len",))
def pallas_gated_mix__memory_aug_recurrent_mem_tr__mixer_s_mlp__prompt_kernel(
    A_x, A_mem0, A_Wq, A_Wk, A_Wv, A_Wo, A_seg_len, B_x, B_w1, B_w2, B_w3, B_w4, gate_w,
):
    assert A_seg_len == SEG
    assert A_x.shape == (1, S, D) and A_Wq.shape == (D, H, DH) and A_mem0.shape == (1, M, D)
    x = A_x.reshape(S, D)
    mem0 = A_mem0.reshape(M, D)
    wq = A_Wq.reshape(D * H, DH)
    wk = A_Wk.reshape(D * H, DH)
    wv = A_Wv.reshape(D * H, DH)
    wo = A_Wo.reshape(H * DH, D)

    any_spec = pl.BlockSpec(memory_space=pl.ANY)
    out = pl.pallas_call(
        _kernel,
        out_shape=jax.ShapeDtypeStruct((S, D), BF16),
        in_specs=[any_spec] * 11,
        out_specs=any_spec,
        scratch_shapes=[
            pltpu.VMEM((S, D), BF16),
            pltpu.VMEM((2, 3, DP * H, DH), BF16),
            pltpu.VMEM((2, OP, D), BF16),
            pltpu.VMEM((3 * H * PITCH, 128), U32),
            pltpu.VMEM((D // 128, H * DH // 2, 128), U32),
            pltpu.VMEM((4, D, D // 4), BF16),
            pltpu.VMEM((4, D, D // 4), BF16),
            pltpu.VMEM((D, FF), BF16),
            pltpu.VMEM((FF, D), BF16),
            pltpu.VMEM((S + 16, D), F32),
            pltpu.VMEM((S, D), F32),
            pltpu.VMEM((S, 128), F32),
            pltpu.VMEM((2, T1, D), BF16),
            pltpu.VMEM((2, T3, D), BF16),
            pltpu.VMEM((M, D), BF16),
            pltpu.VMEM((D,), BF16),
            pltpu.VMEM((M, D), F32),
            pltpu.VMEM((S, D), BF16),
            pltpu.VMEM((16, 128), U32),
            pltpu.SemaphoreType.DMA((NSEM,)),
            pltpu.SemaphoreType.DMA(()),
        ],
        compiler_params=pltpu.CompilerParams(vmem_limit_bytes=120 * 1024 * 1024,
                                             disable_bounds_checks=True),
    )(x, mem0, wq, wk, wv, wo, B_w1, B_w2, B_w3, B_w4, gate_w)
    return out.reshape(1, S, D)
```

```python
import math

import jax
import jax.numpy as jnp
import jax.experimental.pallas as pl
import jax.experimental.pallas.tpu as pltpu

F32 = jnp.float32
BF16 = jnp.bfloat16
U32 = jnp.uint32

S = 2048
D = 1024
H = 32
DH = 128
M = 8
SEG = 32
L = M + SEG
FF = 3584
PAIR = 2 * SEG
NPAIR = S // PAIR
T1 = 256
N1 = S // T1
T2 = 512
N2 = S // T2
T3 = 256
N3 = S // T3
DP = D // N3
OP = H * DH // N3
UNROLL_A = 1
PITCH = 520
SEM_X = 12
SEM_P = SEM_X + N1
NSEM = SEM_P + 8
EPS = 1e-5
NCHAIN0 = 5
NCHAIN1 = 2
HOP = 4
NGV_A = 2
NGV_B = 1
EARLY_A = 0
EARLY_B = 8
V_LAG = 2
S_LAG = 1
PV_LAG = 3
TAIL_AT = (1, 3, 5)
NEG = -1e9


def _gelu(x):
    c = math.sqrt(2.0 / math.pi)
    return 0.5 * x * (1.0 + jnp.tanh(c * (x + 0.044715 * (x * x * x))))


def _layernorm(x):
    m = jnp.mean(x, axis=-1, keepdims=True)
    xc = x - m
    v = jnp.mean(xc * xc, axis=-1, keepdims=True)
    return xc * jax.lax.rsqrt(v + EPS)


def _slab_of(which, h):
    return which * H + (h % 2) * (H // 2) + h // 2


def _kernel(x_hbm, mem0_hbm, wq_hbm, wk_hbm, wv_hbm, wo_hbm,
            w1_hbm, w2_hbm, w3_hbm, w4_hbm, gw_hbm,
            out_hbm,
            x_v, stq_v, sto_v, wqkv_v, wo_v, w1_v, w2_v, w3_v, w4_v,
            h1_v, x1_v, g_v, ln1_v, ln3_v, mem0_v, gw_v, mem_v, out_v, zero_v, sems, osem):
    def cp_x(i):
        r0 = i * T1 if isinstance(i, int) else pl.multiple_of(i * T1, T1)
        return pltpu.make_async_copy(x_hbm.at[pl.ds(r0, T1)], x_v.at[pl.ds(r0, T1)],
                                     sems.at[SEM_X + i])

    c4 = D // 4
    cp_gw = pltpu.make_async_copy(gw_hbm, gw_v, sems.at[0])
    cp_m0 = pltpu.make_async_copy(mem0_hbm, mem0_v, sems.at[1])
    cp_w3 = pltpu.make_async_copy(w3_hbm, w3_v, sems.at[2])
    cp_w4 = pltpu.make_async_copy(w4_hbm, w4_v, sems.at[3])
    cp_w1 = [pltpu.make_async_copy(w1_hbm.at[:, pl.ds(q * c4, c4)], w1_v.at[q], sems.at[4 + q])
             for q in range(4)]
    cp_w2 = [pltpu.make_async_copy(w2_hbm.at[:, pl.ds(q * c4, c4)], w2_v.at[q], sems.at[8 + q])
             for q in range(4)]

    def piece_copies(i, slot):
        cps = [pltpu.make_async_copy(w.at[pl.ds(i * (DP * H), DP * H)], stq_v.at[slot, k],
                                     sems.at[SEM_P + 4 * slot + k])
               for k, w in enumerate((wq_hbm, wk_hbm, wv_hbm))]
        cps.append(pltpu.make_async_copy(wo_hbm.at[pl.ds(i * OP, OP)], sto_v.at[slot],
                                         sems.at[SEM_P + 4 * slot + 3]))
        return cps

    cp_x(0).start()
    for c in cp_w1:
        c.start()
    for i in range(1, N1):
        cp_x(i).start()
    for c in cp_w2:
        c.start()
    cp_gw.start()
    cp_m0.start()
    cp_w3.start()
    cp_w4.start()
    for c in piece_copies(0, 0):
        c.start()
    h1_v[pl.ds(8, 8), :] = jnp.zeros((8, D), F32)
    h1_v[pl.ds(S, 8), :] = jnp.zeros((8, D), F32)
    zero_v[...] = jnp.zeros((16, 128), U32)

    def ln_rows(x, tok, zero):
        if tok is not None:
            head = pltpu.bitcast(pltpu.bitcast(x[:, 0:128], U32) | tok, F32)
            x = jnp.concatenate([head, x[:, 128:]], axis=1)
        y = _layernorm(x)
        tok = None if zero is None else pltpu.bitcast(y[:, 0:128], U32) & zero
        return y, tok

    def ln_block(load, store, rows, nchain):
        zero = zero_v[...] if nchain else None
        toks = [None] * max(nchain, 1)
        for k in range(rows // 16):
            y, toks[k % len(toks)] = ln_rows(load(k), toks[k % len(toks)], zero)
            store(k, y.astype(BF16))
        return toks[(rows // 16 - 1) % len(toks)]

    def prep1(blk, slot, nchain):
        r0 = blk * T1 if isinstance(blk, int) else pl.multiple_of(blk * T1, T1)

        def store(k, y):
            ln1_v[slot, pl.ds(k * 16, 16), :] = y

        ln_block(lambda k: x_v[pl.ds(r0 + k * 16, 16), :].astype(F32), store, T1, nchain)

    def p1_quarter(lhs, r0, q):
        h = _gelu(jnp.dot(lhs, w1_v[q], preferred_element_type=F32))
        win = h1_v.at[pl.ds(r0, T1 + 16)]
        win[pl.ds(8 + (1, -1, 2, -2)[q], T1), pl.ds(q * c4, c4)] = h

    cp_x(0).wait()
    prep1(0, 0, 0)
    for q in range(4):
        cp_w1[q].wait()
        if q == 3:
            cp_x(1).wait()
        lhs = ln1_v[0]
        if q == 3:
            prep1(1, 1, NCHAIN0)
        p1_quarter(lhs, 0, q)

    def p1_body(i, carry):
        r0 = pl.multiple_of(i * T1, T1)
        slot = i % 2

        @pl.when(i + 1 < N1)
        def _():
            cp_x(i + 1).wait()

        lhs = ln1_v[slot]
        prep1(jnp.minimum(i + 1, N1 - 1), 1 - slot, NCHAIN1)
        for q in range(4):
            p1_quarter(lhs, r0, q)
        return carry

    with jax.named_scope('p1_body'):
        jax.lax.fori_loop(1, N1, p1_body, 0)
    for c in cp_w2:
        c.wait()

    def p2_body(i, carry):
        r0 = pl.multiple_of(i * T2, T2)
        hs = h1_v[pl.ds(r0 + 8, T2), :].astype(BF16)
        for q in range(4):
            x1_v[pl.ds(r0, T2), pl.ds(q * c4, c4)] = (
                jnp.dot(hs, w2_v[q], preferred_element_type=F32)
                + x_v[pl.ds(r0, T2), pl.ds(q * c4, c4)].astype(F32))
        return carry

    with jax.named_scope('p2_body'):
        jax.lax.fori_loop(0, N2, p2_body, 0)

    def prep3(blk, slot, nchain):
        r0 = blk * T3 if isinstance(blk, int) else pl.multiple_of(blk * T3, T3)

        def store(k, y):
            ln3_v[slot, pl.ds(k * 16, 16), :] = y

        return ln_block(lambda k: x1_v[pl.ds(r0 + k * 16, 16), :], store, T3, nchain)

    prep3(0, 0, 0)
    cp_gw.wait()
    cp_m0.wait()
    cp_w3.wait()
    cp_w4.wait()

    def p3_body(i, carry):
        r0 = pl.multiple_of(i * T3, T3)
        slot = i % 2

        @pl.when(i + 1 < N3)
        def _():
            for c in piece_copies(i + 1, 1 - slot):
                c.start()

        for c in piece_copies(i, slot):
            c.wait()

        lhs = ln3_v[slot]
        tok = prep3(jnp.minimum(i + 1, N3 - 1), 1 - slot, 1)
        zero = zero_v[...]
        for which in range(3):
            for j in range(DP // 2):
                blk = pltpu.bitcast(stq_v[slot, which, pl.ds(j * 64, 64), :], U32)
                a = blk[0:16] | tok
                c = blk[16:32]
                lo = (a & jnp.uint32(0xFFFF)) | (c << 16)
                a = a | (lo & zero)
                hi = (a >> 16) | (c & jnp.uint32(0xFFFF0000))
                tok = hi & zero
                if j % HOP == HOP - 1:
                    tok = pltpu.roll(tok, 1, 1)
                s0 = which * H * PITCH + i * (DP // 2) + j
                wqkv_v[pl.ds(s0, 16, stride=PITCH), :] = lo
                wqkv_v[pl.ds(s0 + 16 * PITCH, 16, stride=PITCH), :] = hi
        o0 = pl.multiple_of(i * (OP // 2), OP // 2)
        for j in range(D // 128):
            for k in range(OP // 32):
                w = pltpu.bitcast(sto_v[slot, pl.ds(k * 32, 32), pl.ds(j * 128, 128)], U32) | tok
                tok = w & zero
                if k % (2 * HOP) == 2 * HOP - 1:
                    tok = pltpu.roll(tok, 1, 1)
                wo_v[j, pl.ds(o0 + k * 16, 16), :] = w

        h = _gelu(jnp.dot(lhs, w3_v[...], preferred_element_type=F32)).astype(BF16)
        b = jnp.dot(h, w4_v[...], preferred_element_type=F32) + x1_v[pl.ds(r0, T3), :]
        gw = gw_v[...].astype(F32).reshape(1, D)
        z = jnp.sum(x_v[pl.ds(r0, T3), :].astype(F32) * gw, axis=-1, keepdims=True)
        g = 1.0 / (1.0 + jnp.exp(-z))
        g_v[pl.ds(r0, T3), :] = jnp.broadcast_to(g, (T3, 128))
        h1_v[pl.ds(r0, T3), :] = (1.0 - g) * b
        return carry

    with jax.named_scope('p3_body'):
        jax.lax.fori_loop(0, N3, p3_body, 0)

    mem_v[...] = mem0_v[...].astype(F32)
    c_exp = (DH ** -0.5) * math.log2(math.e)
    neg_raw = NEG / (DH ** -0.5)

    L2 = 2 * L

    def make_mask(ngv):
        rm = L - 8 * ngv
        row = jax.lax.broadcasted_iota(jnp.int32, (2 * rm, 128), 0)
        col = jax.lax.broadcasted_iota(jnp.int32, (2 * rm, 128), 1)
        second = row >= rm
        rowl = jnp.where(second, row - rm, row)
        coll = jnp.where(second, col - L, col)
        real = (coll >= 0) & (coll < L)
        allowed = real & ((rowl < M) | (rowl + 8 * ngv >= coll))
        return allowed, jnp.where(real, neg_raw, -jnp.inf).astype(F32)

    masks = {n: make_mask(n) for n in {NGV_A, NGV_B}}
    sub = jax.lax.broadcasted_iota(jnp.int32, (8, 1), 0)
    neg_c = NEG * math.log2(math.e)

    def wslab(which, h, r0, n, tok=None):
        s = _slab_of(which, h) * PITCH
        w = wqkv_v[pl.ds(s + r0, n), :]
        if tok is not None:
            w = jnp.concatenate([w[0:56], w[56:64] | tok, w[64:]], axis=0)
        return pltpu.bitcast(w, BF16)

    zpad = jnp.zeros((128 - L2, DH), F32)

    def recip(l):
        r = pl.reciprocal(l, approx=True)
        return r * (2.0 - l * r)

    def scores(qb, kb, ngv):
        allowed, fill = masks[ngv]
        s = jax.lax.dot_general(qb, kb, (((1,), (1,)), ((), ())),
                                preferred_element_type=F32)
        s = jnp.where(allowed, s, fill)
        m = jnp.max(s, axis=-1, keepdims=True)
        p = jnp.exp2((s - m) * c_exp)
        l = jnp.sum(p, axis=-1, keepdims=True)
        return (p * recip(l)).astype(BF16)

    def tree(op, xs):
        xs = list(xs)
        while len(xs) > 1:
            xs = [op(xs[i], xs[i + 1]) if i + 1 < len(xs) else xs[i]
                  for i in range(0, len(xs), 2)]
        return xs[0]

    def vpu_group(q, k, v, g):
        nk = 8 * (g + 1)
        qs = q * c_exp
        s = []
        for j in range(nk):
            sj = jnp.sum(qs * k[j:j + 1], axis=-1, keepdims=True)
            if j > 8 * g:
                sj = jnp.where(sub >= j - 8 * g, sj, neg_c)
            s.append(sj)
        m = jnp.maximum(tree(jnp.maximum, s), neg_c)
        p = [jnp.exp2(sj - m) for sj in s]
        pm = jnp.exp2(neg_c - m)
        l = tree(jnp.add, p) + pm * float(L - nk)
        acc = [pm * jnp.sum(v[nk:L], axis=0, keepdims=True), None]
        for j in range(nk):
            t = p[j] * v[j:j + 1]
            acc[j % 2] = t if acc[j % 2] is None else acc[j % 2] + t
        return (acc[0] + acc[1]) * recip(l)

    def wo_part(o_bf, h0, h1, j):
        w = pltpu.bitcast(wo_v[j, pl.ds(h0 * 64, (h1 - h0) * 64), :], BF16)
        return jnp.dot(o_bf, w, preferred_element_type=F32)

    def segment(lhs_q, lhs_kv, ngv, unpack, wo_rows, split_first, early_wo, zero):
        NP = H // 2
        nj = D // 128
        mxu_groups = [0] + list(range(ngv + 1, 5))
        rm = 8 * len(mxu_groups)
        qkv = [None] * NP
        pb = [None] * NP
        ob = [None] * H
        og = [dict() for _ in range(H)]

        def do_qkv(p):
            slabs = [(which, h) for h in (2 * p, 2 * p + 1) for which in range(3)]
            lhs = [lhs_q if w == 0 else lhs_kv for w, _ in slabs]
            toks = [None] * 6
            if p >= V_LAG:
                units = [o for h in (2 * (p - V_LAG), 2 * (p - V_LAG) + 1)
                         for o in og[h].values()]
                for n, o in enumerate(units):
                    toks[n * 6 // len(units)] = pltpu.bitcast(o, U32) & zero
            if p == 0 and split_first:
                r = [jnp.dot(x[:, 0:D // 2], wslab(w, h, 0, 256), preferred_element_type=F32)
                     for (w, h), x in zip(slabs, lhs)]
                r = [jnp.dot(x[:, D // 2:D], wslab(w, h, 256, 256),
                             preferred_element_type=F32) + acc
                     for (w, h), x, acc in zip(slabs, lhs, r)]
            else:
                r = [jnp.dot(x, wslab(w, h, 0, 512, tok), preferred_element_type=F32)
                     for (w, h), x, tok in zip(slabs, lhs, toks)]
            t = [unpack(2 * p, *r[0:3]), unpack(2 * p + 1, *r[3:6])]
            for i in range(2):
                q, k, v, jobs = t[i]
                for name, job in jobs.items():
                    og[2 * p + i][name] = vpu_group(*job)
                for g in range(1, ngv + 1):
                    if g in q:
                        og[2 * p + i][g] = vpu_group(q[g], k, v, g)
            qb = jnp.concatenate([t[i][0][g] for i in range(2) for g in mxu_groups],
                                 axis=0).astype(BF16)
            kb = jnp.concatenate([t[0][1], t[1][1], zpad], axis=0).astype(BF16)
            vb = jnp.concatenate([t[0][2], t[1][2], zpad], axis=0).astype(BF16)
            qkv[p] = (qb, kb, vb)

        def do_s(p):
            pb[p] = scores(qkv[p][0], qkv[p][1], ngv)

        def do_pv(p):
            o = jnp.dot(pb[p], qkv[p][2], preferred_element_type=F32)
            for i in range(2):
                rows = dict(og[2 * p + i])
                for n, g in enumerate(mxu_groups):
                    rows[g] = o[i * rm + 8 * n:i * rm + 8 * n + 8]
                ob[2 * p + i] = wo_rows(rows).astype(BF16)

        y = [None] * nj

        def do_wo(h0, h1, j):
            r = wo_part(jnp.concatenate(ob[h0:h1], axis=1), h0, h1, j)
            y[j] = r if y[j] is None else r + y[j]

        H0 = early_wo
        for p in range(NP):
            do_qkv(p)
            if H0 and p >= NP - nj:
                do_wo(0, H0, p - (NP - nj))
            if p >= S_LAG:
                do_s(p - S_LAG)
            if p >= PV_LAG:
                do_pv(p - PV_LAG)
        HA = 2 * (NP - PV_LAG - 1)
        nxt = NP
        for j in range(nj):
            do_wo(H0, HA, j)
            if j in TAIL_AT:
                if nxt - S_LAG < NP:
                    do_s(nxt - S_LAG)
                if nxt - PV_LAG < NP:
                    do_pv(nxt - PV_LAG)
                nxt += 1
        assert nxt - PV_LAG >= NP
        for j in range(nj):
            do_wo(HA, H, j)
        return jnp.concatenate(y, axis=1)

    def pair(r0, mem):
        xf = x_v[pl.ds(r0, PAIR), :].astype(F32)
        zero = zero_v[pl.ds(0, 8), :]
        x1s = jnp.concatenate([xf[0:8], xf[32:40]], axis=0).astype(BF16)
        keep = [None] * H

        def cat(*xs):
            return jnp.concatenate(xs, axis=0)

        lhs = cat(mem, xf[8:32]).astype(BF16)

        def unpack_a(h, q, k, v):
            ka = cat(k[0:8], k[32:40], k[8:32])
            va = cat(v[0:8], v[32:40], v[8:32])
            keep[h] = (ka, va, k[40:48], v[40:48])
            return {0: q[0:8], 2: q[8:16], 3: q[16:24], 4: q[24:32]}, ka, va, {}

        y_a = segment(lhs, cat(lhs, x1s), NGV_A, unpack_a,
                      lambda o: cat(o[0], o[2], o[3], o[4]), False, EARLY_A, zero)

        lhs = cat(y_a[0:8], xf[40:64]).astype(BF16)

        def unpack_b(h, q, k, v):
            ka, va, k1, v1 = keep[h]
            return ({0: q[0:8], 1: q[40:48], 2: q[8:16], 3: q[16:24], 4: q[24:32]},
                    cat(k[0:8], k1, k[8:32]), cat(v[0:8], v1, v[8:32]),
                    {'a1': (q[32:40], ka, va, 1)})

        y_b = segment(cat(lhs, x1s), lhs, NGV_B, unpack_b,
                      lambda o: cat(o[0], o[1], o[2], o[3], o[4], o['a1']), True, EARLY_B,
                      zero)

        a = cat(y_b[40:48], y_a[8:32], y_b[8:40])
        g = g_v[pl.ds(r0, PAIR), :]
        g = jnp.concatenate([g] * (D // 128), axis=1)
        out_v[pl.ds(r0, PAIR), :] = (g * a + h1_v[pl.ds(r0, PAIR), :]).astype(BF16)
        return y_b[0:8]

    rows_it = UNROLL_A * PAIR

    def a_body(t, carry):
        base = pl.multiple_of(t * rows_it, rows_it)
        mem = mem_v[...]
        for u in range(UNROLL_A):
            mem = pair(pl.multiple_of(base + u * PAIR, PAIR), mem)
        mem_v[...] = mem
        pltpu.make_async_copy(out_v.at[pl.ds(base, rows_it)], out_hbm.at[pl.ds(base, rows_it)],
                              osem).start()
        return carry

    with jax.named_scope('a_body'):
        jax.lax.fori_loop(0, S // rows_it, a_body, 0)
    pltpu.make_async_copy(out_v, out_hbm, osem).wait()


@jax.jit
def pallas_gated_mix__memory_aug_recurrent_mem_tr__mixer_s_mlp__prompt_kernel(
    A_x, A_mem0, A_Wq, A_Wk, A_Wv, A_Wo, A_seg_len, B_x, B_w1, B_w2, B_w3, B_w4, gate_w,
):
    assert A_x.shape == (1, S, D) and A_Wq.shape == (D, H, DH) and A_mem0.shape == (1, M, D)
    x = A_x.reshape(S, D)
    mem0 = A_mem0.reshape(M, D)
    wq = A_Wq.reshape(D * H, DH)
    wk = A_Wk.reshape(D * H, DH)
    wv = A_Wv.reshape(D * H, DH)
    wo = A_Wo.reshape(H * DH, D)

    any_spec = pl.BlockSpec(memory_space=pl.ANY)
    out = pl.pallas_call(
        _kernel,
        out_shape=jax.ShapeDtypeStruct((S, D), BF16),
        in_specs=[any_spec] * 11,
        out_specs=any_spec,
        scratch_shapes=[
            pltpu.VMEM((S, D), BF16),
            pltpu.VMEM((2, 3, DP * H, DH), BF16),
            pltpu.VMEM((2, OP, D), BF16),
            pltpu.VMEM((3 * H * PITCH, 128), U32),
            pltpu.VMEM((D // 128, H * DH // 2, 128), U32),
            pltpu.VMEM((4, D, D // 4), BF16),
            pltpu.VMEM((4, D, D // 4), BF16),
            pltpu.VMEM((D, FF), BF16),
            pltpu.VMEM((FF, D), BF16),
            pltpu.VMEM((S + 16, D), F32),
            pltpu.VMEM((S, D), F32),
            pltpu.VMEM((S, 128), F32),
            pltpu.VMEM((2, T1, D), BF16),
            pltpu.VMEM((2, T3, D), BF16),
            pltpu.VMEM((M, D), BF16),
            pltpu.VMEM((D,), BF16),
            pltpu.VMEM((M, D), F32),
            pltpu.VMEM((S, D), BF16),
            pltpu.VMEM((16, 128), U32),
            pltpu.SemaphoreType.DMA((NSEM,)),
            pltpu.SemaphoreType.DMA(()),
        ],
        compiler_params=pltpu.CompilerParams(vmem_limit_bytes=120 * 1024 * 1024,
                                             disable_bounds_checks=True),
    )(x, mem0, wq, wk, wv, wo, B_w1, B_w2, B_w3, B_w4, gate_w)
    return out.reshape(1, S, D)
```

```python
import math

import jax
import jax.numpy as jnp
import jax.experimental.pallas as pl
import jax.experimental.pallas.tpu as pltpu

F32 = jnp.float32
BF16 = jnp.bfloat16
U32 = jnp.uint32

S = 2048
D = 1024
H = 32
DH = 128
M = 8
SEG = 32
L = M + SEG
FF = 3584
PAIR = 2 * SEG
NPAIR = S // PAIR
T1 = 256
N1 = S // T1
T2 = 512
N2 = S // T2
T3 = 256
N3 = S // T3
DP = D // N3
OP = H * DH // N3
UNROLL_A = 1
PITCH = 520
SEM_X = 12
SEM_P = SEM_X + N1
NSEM = SEM_P + 8
EPS = 1e-5
NCHAIN0 = 5
NCHAIN1 = 2
HOP = 4
NGV_A = 2
NGV_B = 1
NJOB = NGV_A + NGV_B
EARLY_A = 2
EARLY_B = 3
TAIL_A = 1.5
TAIL_B = 1.1
WO_SLOTS = 10
CHUNK = 8
T_V = 6
T_S = 6
T_PV = 18
TAIL_H = 8
NEG = -1e9


def _gelu(x):
    c = math.sqrt(2.0 / math.pi)
    return 0.5 * x * (1.0 + jnp.tanh(c * (x + 0.044715 * (x * x * x))))


def _layernorm(x):
    m = jnp.mean(x, axis=-1, keepdims=True)
    xc = x - m
    v = jnp.mean(xc * xc, axis=-1, keepdims=True)
    return xc * jax.lax.rsqrt(v + EPS)


def _slab_of(which, h):
    return which * H + (h % 2) * (H // 2) + h // 2


def _kernel(x_hbm, mem0_hbm, wq_hbm, wk_hbm, wv_hbm, wo_hbm,
            w1_hbm, w2_hbm, w3_hbm, w4_hbm, gw_hbm,
            out_hbm,
            x_v, stq_v, sto_v, wqkv_v, wo_v, w1_v, w2_v, w3_v, w4_v,
            h1_v, x1_v, g_v, ln1_v, ln3_v, mem0_v, gw_v, mem_v, out_v, kv_v, zero_v, sems, osem):
    def cp_x(i):
        r0 = i * T1 if isinstance(i, int) else pl.multiple_of(i * T1, T1)
        return pltpu.make_async_copy(x_hbm.at[pl.ds(r0, T1)], x_v.at[pl.ds(r0, T1)],
                                     sems.at[SEM_X + i])

    c4 = D // 4
    cp_gw = pltpu.make_async_copy(gw_hbm, gw_v, sems.at[0])
    cp_m0 = pltpu.make_async_copy(mem0_hbm, mem0_v, sems.at[1])
    cp_w3 = pltpu.make_async_copy(w3_hbm, w3_v, sems.at[2])
    cp_w4 = pltpu.make_async_copy(w4_hbm, w4_v, sems.at[3])
    cp_w1 = [pltpu.make_async_copy(w1_hbm.at[:, pl.ds(q * c4, c4)], w1_v.at[q], sems.at[4 + q])
             for q in range(4)]
    cp_w2 = [pltpu.make_async_copy(w2_hbm.at[:, pl.ds(q * c4, c4)], w2_v.at[q], sems.at[8 + q])
             for q in range(4)]

    def piece_copies(i, slot):
        cps = [pltpu.make_async_copy(w.at[pl.ds(i * (DP * H), DP * H)], stq_v.at[slot, k],
                                     sems.at[SEM_P + 4 * slot + k])
               for k, w in enumerate((wq_hbm, wk_hbm, wv_hbm))]
        cps.append(pltpu.make_async_copy(wo_hbm.at[pl.ds(i * OP, OP)], sto_v.at[slot],
                                         sems.at[SEM_P + 4 * slot + 3]))
        return cps

    cp_x(0).start()
    for c in cp_w1:
        c.start()
    for i in range(1, N1):
        cp_x(i).start()
    for c in cp_w2:
        c.start()
    cp_gw.start()
    cp_m0.start()
    cp_w3.start()
    cp_w4.start()
    for c in piece_copies(0, 0):
        c.start()
    h1_v[pl.ds(8, 8), :] = jnp.zeros((8, D), F32)
    h1_v[pl.ds(S, 8), :] = jnp.zeros((8, D), F32)
    zero_v[...] = jnp.zeros((16, 128), U32)

    def ln_rows(x, tok, zero):
        if tok is not None:
            head = pltpu.bitcast(pltpu.bitcast(x[:, 0:128], U32) | tok, F32)
            x = jnp.concatenate([head, x[:, 128:]], axis=1)
        y = _layernorm(x)
        tok = None if zero is None else pltpu.bitcast(y[:, 0:128], U32) & zero
        return y, tok

    def ln_block(load, store, rows, nchain):
        zero = zero_v[...] if nchain else None
        toks = [None] * max(nchain, 1)
        for k in range(rows // 16):
            y, toks[k % len(toks)] = ln_rows(load(k), toks[k % len(toks)], zero)
            store(k, y.astype(BF16))
        return toks[(rows // 16 - 1) % len(toks)]

    def prep1(blk, slot, nchain):
        r0 = blk * T1 if isinstance(blk, int) else pl.multiple_of(blk * T1, T1)

        def store(k, y):
            ln1_v[slot, pl.ds(k * 16, 16), :] = y

        ln_block(lambda k: x_v[pl.ds(r0 + k * 16, 16), :].astype(F32), store, T1, nchain)

    def p1_quarter(lhs, r0, q):
        h = _gelu(jnp.dot(lhs, w1_v[q], preferred_element_type=F32))
        win = h1_v.at[pl.ds(r0, T1 + 16)]
        win[pl.ds(8 + (1, -1, 2, -2)[q], T1), pl.ds(q * c4, c4)] = h

    cp_x(0).wait()
    prep1(0, 0, 0)
    for q in range(4):
        cp_w1[q].wait()
        if q == 3:
            cp_x(1).wait()
        lhs = ln1_v[0]
        if q == 3:
            prep1(1, 1, NCHAIN0)
        p1_quarter(lhs, 0, q)

    def p1_body(i, carry):
        r0 = pl.multiple_of(i * T1, T1)
        slot = i % 2

        @pl.when(i + 1 < N1)
        def _():
            cp_x(i + 1).wait()

        lhs = ln1_v[slot]
        prep1(jnp.minimum(i + 1, N1 - 1), 1 - slot, NCHAIN1)
        for q in range(4):
            p1_quarter(lhs, r0, q)
        return carry

    with jax.named_scope('p1_body'):
        jax.lax.fori_loop(1, N1, p1_body, 0)
    for c in cp_w2:
        c.wait()

    def p2_body(i, carry):
        r0 = pl.multiple_of(i * T2, T2)
        hs = h1_v[pl.ds(r0 + 8, T2), :].astype(BF16)
        for q in range(4):
            x1_v[pl.ds(r0, T2), pl.ds(q * c4, c4)] = (
                jnp.dot(hs, w2_v[q], preferred_element_type=F32)
                + x_v[pl.ds(r0, T2), pl.ds(q * c4, c4)].astype(F32))
        return carry

    with jax.named_scope('p2_body'):
        jax.lax.fori_loop(0, N2, p2_body, 0)

    def prep3(blk, slot, nchain):
        r0 = blk * T3 if isinstance(blk, int) else pl.multiple_of(blk * T3, T3)

        def store(k, y):
            ln3_v[slot, pl.ds(k * 16, 16), :] = y

        return ln_block(lambda k: x1_v[pl.ds(r0 + k * 16, 16), :], store, T3, nchain)

    prep3(0, 0, 0)
    cp_gw.wait()
    cp_m0.wait()
    cp_w3.wait()
    cp_w4.wait()

    def p3_body(i, carry):
        r0 = pl.multiple_of(i * T3, T3)
        slot = i % 2

        @pl.when(i + 1 < N3)
        def _():
            for c in piece_copies(i + 1, 1 - slot):
                c.start()

        for c in piece_copies(i, slot):
            c.wait()

        lhs = ln3_v[slot]
        tok = prep3(jnp.minimum(i + 1, N3 - 1), 1 - slot, 1)
        zero = zero_v[...]
        for which in range(3):
            for j in range(DP // 2):
                blk = pltpu.bitcast(stq_v[slot, which, pl.ds(j * 64, 64), :], U32)
                a = blk[0:16] | tok
                c = blk[16:32]
                lo = (a & jnp.uint32(0xFFFF)) | (c << 16)
                a = a | (lo & zero)
                hi = (a >> 16) | (c & jnp.uint32(0xFFFF0000))
                tok = hi & zero
                if j % HOP == HOP - 1:
                    tok = pltpu.roll(tok, 1, 1)
                s0 = which * H * PITCH + i * (DP // 2) + j
                wqkv_v[pl.ds(s0, 16, stride=PITCH), :] = lo
                wqkv_v[pl.ds(s0 + 16 * PITCH, 16, stride=PITCH), :] = hi
        o0 = pl.multiple_of(i * (OP // 2), OP // 2)
        for j in range(D // 128):
            for k in range(OP // 32):
                w = pltpu.bitcast(sto_v[slot, pl.ds(k * 32, 32), pl.ds(j * 128, 128)], U32) | tok
                tok = w & zero
                if k % (2 * HOP) == 2 * HOP - 1:
                    tok = pltpu.roll(tok, 1, 1)
                wo_v[j, pl.ds(o0 + k * 16, 16), :] = w

        h = _gelu(jnp.dot(lhs, w3_v[...], preferred_element_type=F32)).astype(BF16)
        b = jnp.dot(h, w4_v[...], preferred_element_type=F32) + x1_v[pl.ds(r0, T3), :]
        gw = gw_v[...].astype(F32).reshape(1, D)
        z = jnp.sum(x_v[pl.ds(r0, T3), :].astype(F32) * gw, axis=-1, keepdims=True)
        g = 1.0 / (1.0 + jnp.exp(-z))
        g_v[pl.ds(r0, T3), :] = jnp.broadcast_to(g, (T3, 128))
        h1_v[pl.ds(r0, T3), :] = (1.0 - g) * b
        return carry

    with jax.named_scope('p3_body'):
        jax.lax.fori_loop(0, N3, p3_body, 0)

    mem_v[...] = mem0_v[...].astype(F32)
    c_exp = (DH ** -0.5) * math.log2(math.e)
    neg_raw = NEG / (DH ** -0.5)

    L2 = 2 * L

    def make_mask(ngv):
        rm = L - 8 * ngv
        row = jax.lax.broadcasted_iota(jnp.int32, (2 * rm, 128), 0)
        col = jax.lax.broadcasted_iota(jnp.int32, (2 * rm, 128), 1)
        second = row >= rm
        rowl = jnp.where(second, row - rm, row)
        coll = jnp.where(second, col - L, col)
        real = (coll >= 0) & (coll < L)
        allowed = real & ((rowl < M) | (rowl + 8 * ngv >= coll))
        return allowed, jnp.where(real, neg_raw, -jnp.inf).astype(F32)

    masks = {n: make_mask(n) for n in {NGV_A, NGV_B}}
    sub = jax.lax.broadcasted_iota(jnp.int32, (8, 1), 0)
    neg_c = NEG * math.log2(math.e)

    def tied(w, toks):
        for tok in toks:
            w = jnp.concatenate([w[0:56], w[56:64] | tok, w[64:]], axis=0)
        return pltpu.bitcast(w, BF16)

    zpad = jnp.zeros((128 - L2, DH), F32)

    def recip(l):
        r = pl.reciprocal(l, approx=True)
        return r * (2.0 - l * r)

    def tree(op, xs):
        xs = list(xs)
        while len(xs) > 1:
            xs = [op(xs[i], xs[i + 1]) if i + 1 < len(xs) else xs[i]
                  for i in range(0, len(xs), 2)]
        return xs[0]

    def stash(slot, k, v, g):
        n = 8 * (g + 2)
        kb = slot * 2 * L
        kv_v[pl.ds(kb, n), :] = jnp.concatenate([k[8 * g:8 * g + 8], k[0:n - 8]], axis=0)
        kv_v[pl.ds(kb + L, n), :] = jnp.concatenate([v[8 * g:8 * g + 8], v[0:n - 8]], axis=0)
        return kb + n - 8, kb + L + n - 8, jnp.sum(v[n - 8:L], axis=0, keepdims=True)

    def vpu_group(q, parked, g):
        k0, v0, vskip = parked
        nk = 8 * (g + 1)
        qs = q * c_exp
        m = jnp.full((8, 1), neg_c, F32)
        l = jnp.full((8, 1), float(L - nk), F32)
        acc = vskip
        for c0 in range(0, nk, CHUNK):
            sc = []
            for r in range(c0, min(c0 + CHUNK, nk)):
                sr = jnp.sum(qs * kv_v[pl.ds(k0 - r, 8), :], axis=-1, keepdims=True)
                if r > 8 * g:
                    sr = jnp.where(sub >= r - 8 * g, sr, neg_c)
                sc.append(sr)
            m_new = jnp.maximum(tree(jnp.maximum, sc), m)
            alpha = jnp.exp2(m - m_new)
            m = m_new
            l = l * alpha
            acc = acc * alpha
            for n, sr in enumerate(sc):
                pr = jnp.exp2(sr - m)
                l = l + pr
                acc = acc + pr * kv_v[pl.ds(v0 - c0 - n, 8), :]
        return acc * recip(l)

    def segment(lhs_q, lhs_kv, ngv, unpack, wo_rows, split_first, early, tail_scale, zero):
        NP = H // 2
        nj = D // 128
        NT = 6 * NP
        allowed, fill = masks[ngv]
        mxu_groups = [0] + list(range(ngv + 1, 5))
        rm = 8 * len(mxu_groups)
        proj = {}
        qkv = [None] * NP
        pb = [None] * NP
        og = [dict() for _ in range(H)]
        ocat = {}
        y = [None] * nj
        events = {}
        anchors = {}
        now = [0]

        def when(t):
            return t if t < NT else NT + int((t - NT + 1) * tail_scale) - 1

        def tick(fn, *args):
            fn(anchors.pop(now[0], []), *args)
            for f, a in events.pop(now[0], []):
                f(*a)
            now[0] += 1

        def slab(toks, which, h, r0, n):
            x = lhs_q if which == 0 else lhs_kv
            w = tied(wqkv_v[pl.ds(_slab_of(which, h) * PITCH + r0, n), :], toks)
            r = jnp.dot(x[:, 2 * r0:2 * (r0 + n)], w, preferred_element_type=F32)
            proj[(which, h)] = r + proj[(which, h)] if (which, h) in proj else r

        def finish_pair(p):
            t = [unpack(h, *[proj[(w, h)] for w in range(3)]) for h in (2 * p, 2 * p + 1)]
            jobs = [(2 * p + i, name, job) for i in range(2) for name, job in t[i][3].items()]
            for n, (h, name, job) in enumerate(jobs):
                og[h][name] = vpu_group(*job)
                anchors.setdefault(when(now[0] + T_V + n * 6 // len(jobs)), []).append(
                    pltpu.bitcast(og[h][name], U32) & zero)
            qb = jnp.concatenate([t[i][0][g] for i in range(2) for g in mxu_groups],
                                 axis=0).astype(BF16)
            kb = jnp.concatenate([t[0][1], t[1][1], zpad], axis=0).astype(BF16)
            vb = jnp.concatenate([t[0][2], t[1][2], zpad], axis=0).astype(BF16)
            qkv[p] = (qb, kb, vb)

        def do_s(p):
            sc = jax.lax.dot_general(qkv[p][0], qkv[p][1], (((1,), (1,)), ((), ())),
                                     preferred_element_type=F32)
            sc = jnp.where(allowed, sc, fill)
            e = jnp.exp2((sc - jnp.max(sc, axis=-1, keepdims=True)) * c_exp)
            l = jnp.sum(e, axis=-1, keepdims=True)
            pb[p] = (e * recip(l)).astype(BF16)

        def do_pv(p):
            o = jnp.dot(pb[p], qkv[p][2], preferred_element_type=F32)
            for i in range(2):
                for n, g in enumerate(mxu_groups):
                    og[2 * p + i][g] = o[i * rm + 8 * n:i * rm + 8 * n + 8]

        def do_wo(toks, h0, h1, j):
            if (h0, h1) not in ocat:
                ocat[(h0, h1)] = jnp.concatenate(
                    [wo_rows(og[h]) for h in range(h0, h1)], axis=1).astype(BF16)
            w = tied(wo_v[j, pl.ds(h0 * 64, (h1 - h0) * 64), :], toks)
            r = jnp.dot(ocat[(h0, h1)], w, preferred_element_type=F32)
            y[j] = r if y[j] is None else r + y[j]

        wo_early = [(4 * c, 4 * c + 4, j) for c in range(early) for j in range(nj)]
        first = NP - WO_SLOTS
        for p in range(NP):
            slabs = [(which, h) for h in (2 * p, 2 * p + 1) for which in range(3)]
            mine = []
            if p >= first:
                lo = (p - first) * len(wo_early) // WO_SLOTS
                mine = wo_early[lo:(p - first + 1) * len(wo_early) // WO_SLOTS]
            if p == 0 and split_first:
                for w, h in slabs:
                    slab([], w, h, 0, 256)
                for w, h in slabs:
                    tick(slab, w, h, 256, 256)
            else:
                for n, (w, h) in enumerate(slabs):
                    for item in mine[n * len(mine) // 6:(n + 1) * len(mine) // 6]:
                        do_wo([], *item)
                    tick(slab, w, h, 0, 512)
            finish_pair(p)
            events.setdefault(when(now[0] - 1 + T_S), []).append((do_s, (p,)))
            events.setdefault(when(now[0] - 1 + T_PV), []).append((do_pv, (p,)))
        HA = H - TAIL_H
        for j in range(nj):
            for h0 in range(4 * early, HA, 4):
                tick(do_wo, h0, h0 + 4, j)
        assert not events and not anchors
        for j in range(nj):
            do_wo([], HA, H, j)
        return jnp.concatenate(y, axis=1)

    def pair(r0, mem):
        xf = x_v[pl.ds(r0, PAIR), :].astype(F32)
        zero = zero_v[pl.ds(0, 8), :]
        x1s = jnp.concatenate([xf[0:8], xf[32:40]], axis=0).astype(BF16)
        keep = [None] * H

        def cat(*xs):
            return jnp.concatenate(xs, axis=0)

        lhs = cat(mem, xf[8:32]).astype(BF16)

        def unpack_a(h, q, k, v):
            ka = cat(k[0:8], k[32:40], k[8:32])
            va = cat(v[0:8], v[32:40], v[8:32])
            keep[h] = (stash(NJOB * h, ka, va, 1), k[40:48], v[40:48])
            qg = {0: q[0:8], 2: q[8:16], 3: q[16:24], 4: q[24:32]}
            return qg, ka, va, {g: (qg[g], stash(NJOB * h + g - 1, ka, va, g), g)
                                for g in range(2, NGV_A + 1)}

        y_a = segment(lhs, cat(lhs, x1s), NGV_A, unpack_a,
                      lambda o: cat(o[0], o[2], o[3], o[4]), False, EARLY_A, TAIL_A, zero)

        lhs = cat(y_a[0:8], xf[40:64]).astype(BF16)

        def unpack_b(h, q, k, v):
            parked_a1, k1, v1 = keep[h]
            kb = cat(k[0:8], k1, k[8:32])
            vb = cat(v[0:8], v1, v[8:32])
            qg = {0: q[0:8], 1: q[40:48], 2: q[8:16], 3: q[16:24], 4: q[24:32]}
            jobs = {'a1': (q[32:40], parked_a1, 1)}
            jobs.update({g: (qg[g], stash(NJOB * h + NGV_A + g - 1, kb, vb, g), g)
                         for g in range(1, NGV_B + 1)})
            return qg, kb, vb, jobs

        y_b = segment(cat(lhs, x1s), lhs, NGV_B, unpack_b,
                      lambda o: cat(o[0], o[1], o[2], o[3], o[4], o['a1']), True, EARLY_B,
                      TAIL_B, zero)

        a = cat(y_b[40:48], y_a[8:32], y_b[8:40])
        g = g_v[pl.ds(r0, PAIR), :]
        g = jnp.concatenate([g] * (D // 128), axis=1)
        out_v[pl.ds(r0, PAIR), :] = (g * a + h1_v[pl.ds(r0, PAIR), :]).astype(BF16)
        return y_b[0:8]

    rows_it = UNROLL_A * PAIR

    def a_body(t, carry):
        base = pl.multiple_of(t * rows_it, rows_it)
        mem = mem_v[...]
        for u in range(UNROLL_A):
            mem = pair(pl.multiple_of(base + u * PAIR, PAIR), mem)
        mem_v[...] = mem
        pltpu.make_async_copy(out_v.at[pl.ds(base, rows_it)], out_hbm.at[pl.ds(base, rows_it)],
                              osem).start()
        return carry

    with jax.named_scope('a_body'):
        jax.lax.fori_loop(0, S // rows_it, a_body, 0)
    pltpu.make_async_copy(out_v, out_hbm, osem).wait()


@jax.jit
def pallas_gated_mix__memory_aug_recurrent_mem_tr__mixer_s_mlp__prompt_kernel(
    A_x, A_mem0, A_Wq, A_Wk, A_Wv, A_Wo, A_seg_len, B_x, B_w1, B_w2, B_w3, B_w4, gate_w,
):
    assert A_x.shape == (1, S, D) and A_Wq.shape == (D, H, DH) and A_mem0.shape == (1, M, D)
    x = A_x.reshape(S, D)
    mem0 = A_mem0.reshape(M, D)
    wq = A_Wq.reshape(D * H, DH)
    wk = A_Wk.reshape(D * H, DH)
    wv = A_Wv.reshape(D * H, DH)
    wo = A_Wo.reshape(H * DH, D)

    any_spec = pl.BlockSpec(memory_space=pl.ANY)
    out = pl.pallas_call(
        _kernel,
        out_shape=jax.ShapeDtypeStruct((S, D), BF16),
        in_specs=[any_spec] * 11,
        out_specs=any_spec,
        scratch_shapes=[
            pltpu.VMEM((S, D), BF16),
            pltpu.VMEM((2, 3, DP * H, DH), BF16),
            pltpu.VMEM((2, OP, D), BF16),
            pltpu.VMEM((3 * H * PITCH, 128), U32),
            pltpu.VMEM((D // 128, H * DH // 2, 128), U32),
            pltpu.VMEM((4, D, D // 4), BF16),
            pltpu.VMEM((4, D, D // 4), BF16),
            pltpu.VMEM((D, FF), BF16),
            pltpu.VMEM((FF, D), BF16),
            pltpu.VMEM((S + 16, D), F32),
            pltpu.VMEM((S, D), F32),
            pltpu.VMEM((S, 128), F32),
            pltpu.VMEM((2, T1, D), BF16),
            pltpu.VMEM((2, T3, D), BF16),
            pltpu.VMEM((M, D), BF16),
            pltpu.VMEM((D,), BF16),
            pltpu.VMEM((M, D), F32),
            pltpu.VMEM((S, D), BF16),
            pltpu.VMEM((NJOB * H * 2 * L, 128), F32),
            pltpu.VMEM((16, 128), U32),
            pltpu.SemaphoreType.DMA((NSEM,)),
            pltpu.SemaphoreType.DMA(()),
        ],
        compiler_params=pltpu.CompilerParams(vmem_limit_bytes=120 * 1024 * 1024,
                                             disable_bounds_checks=True),
    )(x, mem0, wq, wk, wv, wo, B_w1, B_w2, B_w3, B_w4, gate_w)
    return out.reshape(1, S, D)
```

```python
import math

import jax
import jax.numpy as jnp
import jax.experimental.pallas as pl
import jax.experimental.pallas.tpu as pltpu

F32 = jnp.float32
BF16 = jnp.bfloat16
U32 = jnp.uint32

S = 2048
D = 1024
H = 32
DH = 128
M = 8
SEG = 32
L = M + SEG
FF = 3584
PAIR = 2 * SEG
NPAIR = S // PAIR
T1 = 256
N1 = S // T1
T2 = 512
N2 = S // T2
T3 = 256
N3 = S // T3
DP = D // N3
OP = H * DH // N3
UNROLL_A = 1
PITCH = 520
SEM_X = 12
SEM_P = SEM_X + N1
NSEM = SEM_P + 8
EPS = 1e-5
NCHAIN0 = 5
NCHAIN1 = 2
HOP = 4
NGV_A = 2
NGV_B = 1
NJOB = NGV_A + NGV_B
EARLY_A = 2
EARLY_B = 3
WO_SLOTS = 10
CHUNK = 8
D_G = 0
D_J0 = 450
D_JK = 6
D_S = 500
D_PV = 1400
D_SM = 600
D_O = 170
TAIL_H = 8
NEG = -1e9


def _gelu(x):
    c = math.sqrt(2.0 / math.pi)
    return 0.5 * x * (1.0 + jnp.tanh(c * (x + 0.044715 * (x * x * x))))


def _layernorm(x):
    m = jnp.mean(x, axis=-1, keepdims=True)
    xc = x - m
    v = jnp.mean(xc * xc, axis=-1, keepdims=True)
    return xc * jax.lax.rsqrt(v + EPS)


def _slab_of(which, h):
    return which * H + (h % 2) * (H // 2) + h // 2


def _kernel(x_hbm, mem0_hbm, wq_hbm, wk_hbm, wv_hbm, wo_hbm,
            w1_hbm, w2_hbm, w3_hbm, w4_hbm, gw_hbm,
            out_hbm,
            x_v, stq_v, sto_v, wqkv_v, wo_v, w1_v, w2_v, w3_v, w4_v,
            h1_v, x1_v, g_v, ln1_v, ln3_v, mem0_v, gw_v, mem_v, out_v, kv_v, zero_v, sems, osem):
    def cp_x(i):
        r0 = i * T1 if isinstance(i, int) else pl.multiple_of(i * T1, T1)
        return pltpu.make_async_copy(x_hbm.at[pl.ds(r0, T1)], x_v.at[pl.ds(r0, T1)],
                                     sems.at[SEM_X + i])

    c4 = D // 4
    cp_gw = pltpu.make_async_copy(gw_hbm, gw_v, sems.at[0])
    cp_m0 = pltpu.make_async_copy(mem0_hbm, mem0_v, sems.at[1])
    cp_w3 = pltpu.make_async_copy(w3_hbm, w3_v, sems.at[2])
    cp_w4 = pltpu.make_async_copy(w4_hbm, w4_v, sems.at[3])
    cp_w1 = [pltpu.make_async_copy(w1_hbm.at[:, pl.ds(q * c4, c4)], w1_v.at[q], sems.at[4 + q])
             for q in range(4)]
    cp_w2 = [pltpu.make_async_copy(w2_hbm.at[:, pl.ds(q * c4, c4)], w2_v.at[q], sems.at[8 + q])
             for q in range(4)]

    def piece_copies(i, slot):
        cps = [pltpu.make_async_copy(w.at[pl.ds(i * (DP * H), DP * H)], stq_v.at[slot, k],
                                     sems.at[SEM_P + 4 * slot + k])
               for k, w in enumerate((wq_hbm, wk_hbm, wv_hbm))]
        cps.append(pltpu.make_async_copy(wo_hbm.at[pl.ds(i * OP, OP)], sto_v.at[slot],
                                         sems.at[SEM_P + 4 * slot + 3]))
        return cps

    cp_x(0).start()
    for c in cp_w1:
        c.start()
    for i in range(1, N1):
        cp_x(i).start()
    for c in cp_w2:
        c.start()
    cp_gw.start()
    cp_m0.start()
    cp_w3.start()
    cp_w4.start()
    for c in piece_copies(0, 0):
        c.start()
    h1_v[pl.ds(8, 8), :] = jnp.zeros((8, D), F32)
    h1_v[pl.ds(S, 8), :] = jnp.zeros((8, D), F32)
    zero_v[...] = jnp.zeros((16, 128), U32)

    def ln_rows(x, tok, zero):
        if tok is not None:
            head = pltpu.bitcast(pltpu.bitcast(x[:, 0:128], U32) | tok, F32)
            x = jnp.concatenate([head, x[:, 128:]], axis=1)
        y = _layernorm(x)
        tok = None if zero is None else pltpu.bitcast(y[:, 0:128], U32) & zero
        return y, tok

    def ln_block(load, store, rows, nchain):
        zero = zero_v[...] if nchain else None
        toks = [None] * max(nchain, 1)
        for k in range(rows // 16):
            y, toks[k % len(toks)] = ln_rows(load(k), toks[k % len(toks)], zero)
            store(k, y.astype(BF16))
        return toks[(rows // 16 - 1) % len(toks)]

    def prep1(blk, slot, nchain):
        r0 = blk * T1 if isinstance(blk, int) else pl.multiple_of(blk * T1, T1)

        def store(k, y):
            ln1_v[slot, pl.ds(k * 16, 16), :] = y

        ln_block(lambda k: x_v[pl.ds(r0 + k * 16, 16), :].astype(F32), store, T1, nchain)

    def p1_quarter(lhs, r0, q):
        h = _gelu(jnp.dot(lhs, w1_v[q], preferred_element_type=F32))
        win = h1_v.at[pl.ds(r0, T1 + 16)]
        win[pl.ds(8 + (1, -1, 2, -2)[q], T1), pl.ds(q * c4, c4)] = h

    cp_x(0).wait()
    prep1(0, 0, 0)
    for q in range(4):
        cp_w1[q].wait()
        if q == 3:
            cp_x(1).wait()
        lhs = ln1_v[0]
        if q == 3:
            prep1(1, 1, NCHAIN0)
        p1_quarter(lhs, 0, q)

    def p1_body(i, carry):
        r0 = pl.multiple_of(i * T1, T1)
        slot = i % 2

        @pl.when(i + 1 < N1)
        def _():
            cp_x(i + 1).wait()

        lhs = ln1_v[slot]
        prep1(jnp.minimum(i + 1, N1 - 1), 1 - slot, NCHAIN1)
        for q in range(4):
            p1_quarter(lhs, r0, q)
        return carry

    with jax.named_scope('p1_body'):
        jax.lax.fori_loop(1, N1, p1_body, 0)
    for c in cp_w2:
        c.wait()

    def p2_body(i, carry):
        r0 = pl.multiple_of(i * T2, T2)
        hs = h1_v[pl.ds(r0 + 8, T2), :].astype(BF16)
        for q in range(4):
            x1_v[pl.ds(r0, T2), pl.ds(q * c4, c4)] = (
                jnp.dot(hs, w2_v[q], preferred_element_type=F32)
                + x_v[pl.ds(r0, T2), pl.ds(q * c4, c4)].astype(F32))
        return carry

    with jax.named_scope('p2_body'):
        jax.lax.fori_loop(0, N2, p2_body, 0)

    def prep3(blk, slot, nchain):
        r0 = blk * T3 if isinstance(blk, int) else pl.multiple_of(blk * T3, T3)

        def store(k, y):
            ln3_v[slot, pl.ds(k * 16, 16), :] = y

        return ln_block(lambda k: x1_v[pl.ds(r0 + k * 16, 16), :], store, T3, nchain)

    prep3(0, 0, 0)
    cp_gw.wait()
    cp_m0.wait()
    cp_w3.wait()
    cp_w4.wait()

    def p3_body(i, carry):
        r0 = pl.multiple_of(i * T3, T3)
        slot = i % 2

        @pl.when(i + 1 < N3)
        def _():
            for c in piece_copies(i + 1, 1 - slot):
                c.start()

        for c in piece_copies(i, slot):
            c.wait()

        lhs = ln3_v[slot]
        tok = prep3(jnp.minimum(i + 1, N3 - 1), 1 - slot, 1)
        zero = zero_v[...]
        for which in range(3):
            for j in range(DP // 2):
                blk = pltpu.bitcast(stq_v[slot, which, pl.ds(j * 64, 64), :], U32)
                a = blk[0:16] | tok
                c = blk[16:32]
                lo = (a & jnp.uint32(0xFFFF)) | (c << 16)
                a = a | (lo & zero)
                hi = (a >> 16) | (c & jnp.uint32(0xFFFF0000))
                tok = hi & zero
                if j % HOP == HOP - 1:
                    tok = pltpu.roll(tok, 1, 1)
                s0 = which * H * PITCH + i * (DP // 2) + j
                wqkv_v[pl.ds(s0, 16, stride=PITCH), :] = lo
                wqkv_v[pl.ds(s0 + 16 * PITCH, 16, stride=PITCH), :] = hi
        o0 = pl.multiple_of(i * (OP // 2), OP // 2)
        for j in range(D // 128):
            for k in range(OP // 32):
                w = pltpu.bitcast(sto_v[slot, pl.ds(k * 32, 32), pl.ds(j * 128, 128)], U32) | tok
                tok = w & zero
                if k % (2 * HOP) == 2 * HOP - 1:
                    tok = pltpu.roll(tok, 1, 1)
                wo_v[j, pl.ds(o0 + k * 16, 16), :] = w

        h = _gelu(jnp.dot(lhs, w3_v[...], preferred_element_type=F32)).astype(BF16)
        b = jnp.dot(h, w4_v[...], preferred_element_type=F32) + x1_v[pl.ds(r0, T3), :]
        gw = gw_v[...].astype(F32).reshape(1, D)
        z = jnp.sum(x_v[pl.ds(r0, T3), :].astype(F32) * gw, axis=-1, keepdims=True)
        g = 1.0 / (1.0 + jnp.exp(-z))
        g_v[pl.ds(r0, T3), :] = jnp.broadcast_to(g, (T3, 128))
        h1_v[pl.ds(r0, T3), :] = (1.0 - g) * b
        return carry

    with jax.named_scope('p3_body'):
        jax.lax.fori_loop(0, N3, p3_body, 0)

    mem_v[...] = mem0_v[...].astype(F32)
    c_exp = (DH ** -0.5) * math.log2(math.e)
    neg_raw = NEG / (DH ** -0.5)

    L2 = 2 * L

    def make_mask(ngv):
        rm = L - 8 * ngv
        row = jax.lax.broadcasted_iota(jnp.int32, (2 * rm, 128), 0)
        col = jax.lax.broadcasted_iota(jnp.int32, (2 * rm, 128), 1)
        second = row >= rm
        rowl = jnp.where(second, row - rm, row)
        coll = jnp.where(second, col - L, col)
        real = (coll >= 0) & (coll < L)
        allowed = real & ((rowl < M) | (rowl + 8 * ngv >= coll))
        return allowed, jnp.where(real, neg_raw, -jnp.inf).astype(F32)

    masks = {n: make_mask(n) for n in {NGV_A, NGV_B}}
    sub = jax.lax.broadcasted_iota(jnp.int32, (8, 1), 0)
    neg_c = NEG * math.log2(math.e)

    def tied(w, toks):
        for tok in toks:
            w = jnp.concatenate([w[0:56], w[56:64] | tok, w[64:]], axis=0)
        return pltpu.bitcast(w, BF16)

    zpad = jnp.zeros((128 - L2, DH), F32)

    def recip(l):
        r = pl.reciprocal(l, approx=True)
        return r * (2.0 - l * r)

    def tree(op, xs):
        xs = list(xs)
        while len(xs) > 1:
            xs = [op(xs[i], xs[i + 1]) if i + 1 < len(xs) else xs[i]
                  for i in range(0, len(xs), 2)]
        return xs[0]

    def stash(slot, k, v, g):
        n = 8 * (g + 2)
        kb = slot * 2 * L
        kv_v[pl.ds(kb, n), :] = jnp.concatenate([k[8 * g:8 * g + 8], k[0:n - 8]], axis=0)
        kv_v[pl.ds(kb + L, n), :] = jnp.concatenate([v[8 * g:8 * g + 8], v[0:n - 8]], axis=0)
        return kb + n - 8, kb + L + n - 8, jnp.sum(v[n - 8:L], axis=0, keepdims=True)

    def vpu_group(q, parked, g):
        k0, v0, vskip = parked
        nk = 8 * (g + 1)
        qs = q * c_exp
        m = jnp.full((8, 1), neg_c, F32)
        l = jnp.full((8, 1), float(L - nk), F32)
        acc = vskip
        for c0 in range(0, nk, CHUNK):
            sc = []
            for r in range(c0, min(c0 + CHUNK, nk)):
                sr = jnp.sum(qs * kv_v[pl.ds(k0 - r, 8), :], axis=-1, keepdims=True)
                if r > 8 * g:
                    sr = jnp.where(sub >= r - 8 * g, sr, neg_c)
                sc.append(sr)
            m_new = jnp.maximum(tree(jnp.maximum, sc), m)
            alpha = jnp.exp2(m - m_new)
            m = m_new
            l = l * alpha
            acc = acc * alpha
            for n, sr in enumerate(sc):
                pr = jnp.exp2(sr - m)
                l = l + pr
                acc = acc + pr * kv_v[pl.ds(v0 - c0 - n, 8), :]
        return acc * recip(l)

    def segment(lhs_q, lhs_kv, wo_m, ngv, unpack, wo_rows, split_first, early, zero):
        NP = H // 2
        nj = D // 128
        HA = H - TAIL_H
        allowed, fill = masks[ngv]
        mxu_groups = [0] + list(range(ngv + 1, 5))
        rm = 8 * len(mxu_groups)
        proj = {}
        qkv = [None] * NP
        pb = [None] * NP
        og = [dict() for _ in range(H)]
        ocat = {}
        y = [None] * nj

        def slab(toks, which, h, r0, n):
            x = lhs_q if which == 0 else lhs_kv
            w = tied(wqkv_v[pl.ds(_slab_of(which, h) * PITCH + r0, n), :], toks)
            r = jnp.dot(x[:, 2 * r0:2 * (r0 + n)], w, preferred_element_type=F32)
            proj[(which, h)] = r + proj[(which, h)] if (which, h) in proj else r
            return proj[(which, h)]

        def do_wo(toks, h0, h1, j):
            if (h0, h1) not in ocat:
                ocat[(h0, h1)] = jnp.concatenate(
                    [wo_rows(og[h]) for h in range(h0, h1)], axis=1).astype(BF16)
            w = tied(wo_v[j, pl.ds(h0 * 64, (h1 - h0) * 64), :], toks)
            r = jnp.dot(ocat[(h0, h1)], w, preferred_element_type=F32)
            y[j] = r if y[j] is None else r + y[j]
            return y[j]

        ticks = []
        pair_end = {}
        wo_early = [(4 * c, 4 * c + 4, j) for c in range(early) for j in range(nj)]
        first = NP - WO_SLOTS
        for p in range(NP):
            slabs = [(which, h) for h in (2 * p, 2 * p + 1) for which in range(3)]
            rows = [(lhs_q if w == 0 else lhs_kv).shape[0] for w, _ in slabs]
            if p == 0 and split_first:
                for r0 in (0, 256):
                    ticks += [(slab, (w, h, r0, 256), m) for (w, h), m in zip(slabs, rows)]
            else:
                mine = []
                if p >= first:
                    lo = (p - first) * len(wo_early) // WO_SLOTS
                    mine = wo_early[lo:(p - first + 1) * len(wo_early) // WO_SLOTS]
                for n, ((w, h), m) in enumerate(zip(slabs, rows)):
                    ticks += [(do_wo, item, wo_m)
                              for item in mine[n * len(mine) // 6:(n + 1) * len(mine) // 6]]
                    ticks.append((slab, (w, h, 0, 512), 2 * m + rm // 6))
            pair_end[len(ticks) - 1] = p
        ticks += [(do_wo, (h0, h0 + 4, j), wo_m)
                  for j in range(nj) for h0 in range(4 * early, HA, 4)]
        ends = []
        for _, _, dur in ticks:
            ends.append(dur + (ends[-1] if ends else 0))

        def index(t):
            return next(i for i, e in enumerate(ends) if e >= t)

        events = {}
        anchors = {}

        def run_job(res, h, name, job, i_done):
            gate = pltpu.bitcast(res[0:8], U32) & zero
            q = pltpu.bitcast(pltpu.bitcast(job[0], U32) | gate, F32)
            og[h][name] = vpu_group(q, *job[1:])
            anchors.setdefault(i_done, []).append(pltpu.bitcast(og[h][name], U32) & zero)

        def do_s(res, p):
            sc = jax.lax.dot_general(qkv[p][0], qkv[p][1], (((1,), (1,)), ((), ())),
                                     preferred_element_type=F32)
            sc = jnp.where(allowed, sc, fill)
            e = jnp.exp2((sc - jnp.max(sc, axis=-1, keepdims=True)) * c_exp)
            l = jnp.sum(e, axis=-1, keepdims=True)
            pb[p] = (e * recip(l)).astype(BF16)

        def do_pv(res, p):
            o = jnp.dot(pb[p], qkv[p][2], preferred_element_type=F32)
            for i in range(2):
                for n, g in enumerate(mxu_groups):
                    og[2 * p + i][g] = o[i * rm + 8 * n:i * rm + 8 * n + 8]

        def finish_pair(p, i):
            u = [unpack(h, *[proj[(w, h)] for w in range(3)]) for h in (2 * p, 2 * p + 1)]
            jobs = [(2 * p + k, name, job) for k in range(2) for name, job in u[k][3].items()]
            span = ends[i] - ends[i - 6] if p == NP - 1 else (
                ends[[k for k, v in pair_end.items() if v == p + 1][0]] - ends[i])
            span = min(span, ends[-2] - ends[i] - D_J0 - D_JK * 8 * (ngv + 1) - D_G)
            total = sum(job[2] + 1 for _, _, job in jobs)
            done = 0
            for h, name, job in jobs:
                g = max(index(ends[i] + D_G + span * done // total), i + 1)
                done += job[2] + 1
                events.setdefault(g, []).append(
                    (run_job, (h, name, job,
                               index(ends[g] + D_J0 + D_JK * 8 * (job[2] + 1)) + 1)))
            qb = jnp.concatenate([u[k][0][g] for k in range(2) for g in mxu_groups],
                                 axis=0).astype(BF16)
            kb = jnp.concatenate([u[0][1], u[1][1], zpad], axis=0).astype(BF16)
            vb = jnp.concatenate([u[0][2], u[1][2], zpad], axis=0).astype(BF16)
            qkv[p] = (qb, kb, vb)
            t_pv = min(ends[i] + D_PV, ends[-1] - D_O)
            events.setdefault(index(min(ends[i] + D_S, t_pv - D_SM)), []).append((do_s, (p,)))
            events.setdefault(index(t_pv), []).append((do_pv, (p,)))

        for i, (fn, args, _) in enumerate(ticks):
            res = fn(anchors.pop(i, []), *args)
            if i in pair_end:
                finish_pair(pair_end[i], i)
            for f, a in events.pop(i, []):
                f(res, *a)
        assert not events
        for j in range(nj):
            do_wo([], HA, H, j)
        return jnp.concatenate(y, axis=1)

    def pair(r0, mem):
        xf = x_v[pl.ds(r0, PAIR), :].astype(F32)
        zero = zero_v[pl.ds(0, 8), :]
        x1s = jnp.concatenate([xf[0:8], xf[32:40]], axis=0).astype(BF16)
        keep = [None] * H

        def cat(*xs):
            return jnp.concatenate(xs, axis=0)

        lhs = cat(mem, xf[8:32]).astype(BF16)

        def unpack_a(h, q, k, v):
            ka = cat(k[0:8], k[32:40], k[8:32])
            va = cat(v[0:8], v[32:40], v[8:32])
            keep[h] = (stash(NJOB * h, ka, va, 1), k[40:48], v[40:48])
            qg = {0: q[0:8], 2: q[8:16], 3: q[16:24], 4: q[24:32]}
            return qg, ka, va, {g: (qg[g], stash(NJOB * h + g - 1, ka, va, g), g)
                                for g in range(2, NGV_A + 1)}

        y_a = segment(lhs, cat(lhs, x1s), 32, NGV_A, unpack_a,
                      lambda o: cat(o[0], o[2], o[3], o[4]), False, EARLY_A, zero)

        lhs = cat(y_a[0:8], xf[40:64]).astype(BF16)

        def unpack_b(h, q, k, v):
            parked_a1, k1, v1 = keep[h]
            kb = cat(k[0:8], k1, k[8:32])
            vb = cat(v[0:8], v1, v[8:32])
            qg = {0: q[0:8], 1: q[40:48], 2: q[8:16], 3: q[16:24], 4: q[24:32]}
            jobs = {'a1': (q[32:40], parked_a1, 1)}
            jobs.update({g: (qg[g], stash(NJOB * h + NGV_A + g - 1, kb, vb, g), g)
                         for g in range(1, NGV_B + 1)})
            return qg, kb, vb, jobs

        y_b = segment(cat(lhs, x1s), lhs, 48, NGV_B, unpack_b,
                      lambda o: cat(o[0], o[1], o[2], o[3], o[4], o['a1']), True, EARLY_B,
                      zero)

        a = cat(y_b[40:48], y_a[8:32], y_b[8:40])
        g = g_v[pl.ds(r0, PAIR), :]
        g = jnp.concatenate([g] * (D // 128), axis=1)
        out_v[pl.ds(r0, PAIR), :] = (g * a + h1_v[pl.ds(r0, PAIR), :]).astype(BF16)
        return y_b[0:8]

    rows_it = UNROLL_A * PAIR

    def a_body(t, carry):
        base = pl.multiple_of(t * rows_it, rows_it)
        mem = mem_v[...]
        for u in range(UNROLL_A):
            mem = pair(pl.multiple_of(base + u * PAIR, PAIR), mem)
        mem_v[...] = mem
        pltpu.make_async_copy(out_v.at[pl.ds(base, rows_it)], out_hbm.at[pl.ds(base, rows_it)],
                              osem).start()
        return carry

    with jax.named_scope('a_body'):
        jax.lax.fori_loop(0, S // rows_it, a_body, 0)
    pltpu.make_async_copy(out_v, out_hbm, osem).wait()


@jax.jit
def pallas_gated_mix__memory_aug_recurrent_mem_tr__mixer_s_mlp__prompt_kernel(
    A_x, A_mem0, A_Wq, A_Wk, A_Wv, A_Wo, A_seg_len, B_x, B_w1, B_w2, B_w3, B_w4, gate_w,
):
    assert A_x.shape == (1, S, D) and A_Wq.shape == (D, H, DH) and A_mem0.shape == (1, M, D)
    x = A_x.reshape(S, D)
    mem0 = A_mem0.reshape(M, D)
    wq = A_Wq.reshape(D * H, DH)
    wk = A_Wk.reshape(D * H, DH)
    wv = A_Wv.reshape(D * H, DH)
    wo = A_Wo.reshape(H * DH, D)

    any_spec = pl.BlockSpec(memory_space=pl.ANY)
    out = pl.pallas_call(
        _kernel,
        out_shape=jax.ShapeDtypeStruct((S, D), BF16),
        in_specs=[any_spec] * 11,
        out_specs=any_spec,
        scratch_shapes=[
            pltpu.VMEM((S, D), BF16),
            pltpu.VMEM((2, 3, DP * H, DH), BF16),
            pltpu.VMEM((2, OP, D), BF16),
            pltpu.VMEM((3 * H * PITCH, 128), U32),
            pltpu.VMEM((D // 128, H * DH // 2, 128), U32),
            pltpu.VMEM((4, D, D // 4), BF16),
            pltpu.VMEM((4, D, D // 4), BF16),
            pltpu.VMEM((D, FF), BF16),
            pltpu.VMEM((FF, D), BF16),
            pltpu.VMEM((S + 16, D), F32),
            pltpu.VMEM((S, D), F32),
            pltpu.VMEM((S, 128), F32),
            pltpu.VMEM((2, T1, D), BF16),
            pltpu.VMEM((2, T3, D), BF16),
            pltpu.VMEM((M, D), BF16),
            pltpu.VMEM((D,), BF16),
            pltpu.VMEM((M, D), F32),
            pltpu.VMEM((S, D), BF16),
            pltpu.VMEM((NJOB * H * 2 * L, 128), F32),
            pltpu.VMEM((16, 128), U32),
            pltpu.SemaphoreType.DMA((NSEM,)),
            pltpu.SemaphoreType.DMA(()),
        ],
        compiler_params=pltpu.CompilerParams(vmem_limit_bytes=120 * 1024 * 1024,
                                             disable_bounds_checks=True),
    )(x, mem0, wq, wk, wv, wo, B_w1, B_w2, B_w3, B_w4, gate_w)
    return out.reshape(1, S, D)
```

```python
import math

import jax
import jax.numpy as jnp
import jax.experimental.pallas as pl
import jax.experimental.pallas.tpu as pltpu

F32 = jnp.float32
BF16 = jnp.bfloat16
U32 = jnp.uint32

S = 2048
D = 1024
H = 32
DH = 128
M = 8
SEG = 32
L = M + SEG
FF = 3584
PAIR = 2 * SEG
NPAIR = S // PAIR
T1 = 256
N1 = S // T1
T2 = 512
N2 = S // T2
T3 = 256
N3 = S // T3
DP = D // N3
OP = H * DH // N3
UNROLL_A = 1
PITCH = 520
SEM_X = 12
SEM_P = SEM_X + N1
NSEM = SEM_P + 8
EPS = 1e-5
NCHAIN0 = 5
NCHAIN1 = 2
HOP = 4
NGV_A = 3
NGV_B = 2
NJOB = NGV_A + NGV_B
EARLY_A = 2
EARLY_B = 3
WO_SLOTS = 10
CHUNK = 8
D_G = 0
D_JA = 530
D_JB = 600
D_F = 100
D_S = 500
D_PV = 1400
D_SM = 600
D_O = 170
TAIL_H = 8
NEG = -1e9


def _gelu(x):
    c = math.sqrt(2.0 / math.pi)
    return 0.5 * x * (1.0 + jnp.tanh(c * (x + 0.044715 * (x * x * x))))


def _layernorm(x):
    m = jnp.mean(x, axis=-1, keepdims=True)
    xc = x - m
    v = jnp.mean(xc * xc, axis=-1, keepdims=True)
    return xc * jax.lax.rsqrt(v + EPS)


def _slab_of(which, h):
    return which * H + (h % 2) * (H // 2) + h // 2


def _kernel(x_hbm, mem0_hbm, wq_hbm, wk_hbm, wv_hbm, wo_hbm,
            w1_hbm, w2_hbm, w3_hbm, w4_hbm, gw_hbm,
            out_hbm,
            x_v, stq_v, sto_v, wqkv_v, wo_v, w1_v, w2_v, w3_v, w4_v,
            h1_v, x1_v, g_v, ln1_v, ln3_v, mem0_v, gw_v, mem_v, out_v, kv_v, zero_v, sems, osem):
    def cp_x(i):
        r0 = i * T1 if isinstance(i, int) else pl.multiple_of(i * T1, T1)
        return pltpu.make_async_copy(x_hbm.at[pl.ds(r0, T1)], x_v.at[pl.ds(r0, T1)],
                                     sems.at[SEM_X + i])

    c4 = D // 4
    cp_gw = pltpu.make_async_copy(gw_hbm, gw_v, sems.at[0])
    cp_m0 = pltpu.make_async_copy(mem0_hbm, mem0_v, sems.at[1])
    cp_w3 = pltpu.make_async_copy(w3_hbm, w3_v, sems.at[2])
    cp_w4 = pltpu.make_async_copy(w4_hbm, w4_v, sems.at[3])
    cp_w1 = [pltpu.make_async_copy(w1_hbm.at[:, pl.ds(q * c4, c4)], w1_v.at[q], sems.at[4 + q])
             for q in range(4)]
    cp_w2 = [pltpu.make_async_copy(w2_hbm.at[:, pl.ds(q * c4, c4)], w2_v.at[q], sems.at[8 + q])
             for q in range(4)]

    def piece_copies(i, slot):
        cps = [pltpu.make_async_copy(w.at[pl.ds(i * (DP * H), DP * H)], stq_v.at[slot, k],
                                     sems.at[SEM_P + 4 * slot + k])
               for k, w in enumerate((wq_hbm, wk_hbm, wv_hbm))]
        cps.append(pltpu.make_async_copy(wo_hbm.at[pl.ds(i * OP, OP)], sto_v.at[slot],
                                         sems.at[SEM_P + 4 * slot + 3]))
        return cps

    cp_x(0).start()
    for c in cp_w1:
        c.start()
    for i in range(1, N1):
        cp_x(i).start()
    for c in cp_w2:
        c.start()
    cp_gw.start()
    cp_m0.start()
    cp_w3.start()
    cp_w4.start()
    for c in piece_copies(0, 0):
        c.start()
    h1_v[pl.ds(8, 8), :] = jnp.zeros((8, D), F32)
    h1_v[pl.ds(S, 8), :] = jnp.zeros((8, D), F32)
    zero_v[...] = jnp.zeros((16, 128), U32)

    def ln_rows(x, tok, zero):
        if tok is not None:
            head = pltpu.bitcast(pltpu.bitcast(x[:, 0:128], U32) | tok, F32)
            x = jnp.concatenate([head, x[:, 128:]], axis=1)
        y = _layernorm(x)
        tok = None if zero is None else pltpu.bitcast(y[:, 0:128], U32) & zero
        return y, tok

    def ln_block(load, store, rows, nchain):
        zero = zero_v[...] if nchain else None
        toks = [None] * max(nchain, 1)
        for k in range(rows // 16):
            y, toks[k % len(toks)] = ln_rows(load(k), toks[k % len(toks)], zero)
            store(k, y.astype(BF16))
        return toks[(rows // 16 - 1) % len(toks)]

    def prep1(blk, slot, nchain):
        r0 = blk * T1 if isinstance(blk, int) else pl.multiple_of(blk * T1, T1)

        def store(k, y):
            ln1_v[slot, pl.ds(k * 16, 16), :] = y

        ln_block(lambda k: x_v[pl.ds(r0 + k * 16, 16), :].astype(F32), store, T1, nchain)

    def p1_quarter(lhs, r0, q):
        h = _gelu(jnp.dot(lhs, w1_v[q], preferred_element_type=F32))
        win = h1_v.at[pl.ds(r0, T1 + 16)]
        win[pl.ds(8 + (1, -1, 2, -2)[q], T1), pl.ds(q * c4, c4)] = h

    cp_x(0).wait()
    prep1(0, 0, 0)
    for q in range(4):
        cp_w1[q].wait()
        if q == 3:
            cp_x(1).wait()
        lhs = ln1_v[0]
        if q == 3:
            prep1(1, 1, NCHAIN0)
        p1_quarter(lhs, 0, q)

    def p1_body(i, carry):
        r0 = pl.multiple_of(i * T1, T1)
        slot = i % 2

        @pl.when(i + 1 < N1)
        def _():
            cp_x(i + 1).wait()

        lhs = ln1_v[slot]
        prep1(jnp.minimum(i + 1, N1 - 1), 1 - slot, NCHAIN1)
        for q in range(4):
            p1_quarter(lhs, r0, q)
        return carry

    with jax.named_scope('p1_body'):
        jax.lax.fori_loop(1, N1, p1_body, 0)
    for c in cp_w2:
        c.wait()

    def p2_body(i, carry):
        r0 = pl.multiple_of(i * T2, T2)
        hs = h1_v[pl.ds(r0 + 8, T2), :].astype(BF16)
        for q in range(4):
            x1_v[pl.ds(r0, T2), pl.ds(q * c4, c4)] = (
                jnp.dot(hs, w2_v[q], preferred_element_type=F32)
                + x_v[pl.ds(r0, T2), pl.ds(q * c4, c4)].astype(F32))
        return carry

    with jax.named_scope('p2_body'):
        jax.lax.fori_loop(0, N2, p2_body, 0)

    def prep3(blk, slot, nchain):
        r0 = blk * T3 if isinstance(blk, int) else pl.multiple_of(blk * T3, T3)

        def store(k, y):
            ln3_v[slot, pl.ds(k * 16, 16), :] = y

        return ln_block(lambda k: x1_v[pl.ds(r0 + k * 16, 16), :], store, T3, nchain)

    prep3(0, 0, 0)
    cp_gw.wait()
    cp_m0.wait()
    cp_w3.wait()
    cp_w4.wait()

    def p3_body(i, carry):
        r0 = pl.multiple_of(i * T3, T3)
        slot = i % 2

        @pl.when(i + 1 < N3)
        def _():
            for c in piece_copies(i + 1, 1 - slot):
                c.start()

        for c in piece_copies(i, slot):
            c.wait()

        lhs = ln3_v[slot]
        tok = prep3(jnp.minimum(i + 1, N3 - 1), 1 - slot, 1)
        zero = zero_v[...]
        for which in range(3):
            for j in range(DP // 2):
                blk = pltpu.bitcast(stq_v[slot, which, pl.ds(j * 64, 64), :], U32)
                a = blk[0:16] | tok
                c = blk[16:32]
                lo = (a & jnp.uint32(0xFFFF)) | (c << 16)
                a = a | (lo & zero)
                hi = (a >> 16) | (c & jnp.uint32(0xFFFF0000))
                tok = hi & zero
                if j % HOP == HOP - 1:
                    tok = pltpu.roll(tok, 1, 1)
                s0 = which * H * PITCH + i * (DP // 2) + j
                wqkv_v[pl.ds(s0, 16, stride=PITCH), :] = lo
                wqkv_v[pl.ds(s0 + 16 * PITCH, 16, stride=PITCH), :] = hi
        o0 = pl.multiple_of(i * (OP // 2), OP // 2)
        for j in range(D // 128):
            for k in range(OP // 32):
                w = pltpu.bitcast(sto_v[slot, pl.ds(k * 32, 32), pl.ds(j * 128, 128)], U32) | tok
                tok = w & zero
                if k % (2 * HOP) == 2 * HOP - 1:
                    tok = pltpu.roll(tok, 1, 1)
                wo_v[j, pl.ds(o0 + k * 16, 16), :] = w

        h = _gelu(jnp.dot(lhs, w3_v[...], preferred_element_type=F32)).astype(BF16)
        b = jnp.dot(h, w4_v[...], preferred_element_type=F32) + x1_v[pl.ds(r0, T3), :]
        gw = gw_v[...].astype(F32).reshape(1, D)
        z = jnp.sum(x_v[pl.ds(r0, T3), :].astype(F32) * gw, axis=-1, keepdims=True)
        g = 1.0 / (1.0 + jnp.exp(-z))
        g_v[pl.ds(r0, T3), :] = jnp.broadcast_to(g, (T3, 128))
        h1_v[pl.ds(r0, T3), :] = (1.0 - g) * b
        return carry

    with jax.named_scope('p3_body'):
        jax.lax.fori_loop(0, N3, p3_body, 0)

    mem_v[...] = mem0_v[...].astype(F32)
    c_exp = (DH ** -0.5) * math.log2(math.e)
    neg_raw = NEG / (DH ** -0.5)

    L2 = 2 * L

    def make_mask(ngv):
        rm = L - 8 * ngv
        row = jax.lax.broadcasted_iota(jnp.int32, (2 * rm, 128), 0)
        col = jax.lax.broadcasted_iota(jnp.int32, (2 * rm, 128), 1)
        second = row >= rm
        rowl = jnp.where(second, row - rm, row)
        coll = jnp.where(second, col - L, col)
        real = (coll >= 0) & (coll < L)
        allowed = real & ((rowl < M) | (rowl + 8 * ngv >= coll))
        return allowed, jnp.where(real, neg_raw, -jnp.inf).astype(F32)

    masks = {n: make_mask(n) for n in {NGV_A, NGV_B}}
    sub = jax.lax.broadcasted_iota(jnp.int32, (8, 1), 0)
    neg_c = NEG * math.log2(math.e)

    def tied(w, toks):
        for tok in toks:
            w = jnp.concatenate([w[0:56], w[56:64] | tok, w[64:]], axis=0)
        return pltpu.bitcast(w, BF16)

    zpad = jnp.zeros((128 - L2, DH), F32)

    def recip(l):
        r = pl.reciprocal(l, approx=True)
        return r * (2.0 - l * r)

    def tree(op, xs):
        xs = list(xs)
        while len(xs) > 1:
            xs = [op(xs[i], xs[i + 1]) if i + 1 < len(xs) else xs[i]
                  for i in range(0, len(xs), 2)]
        return xs[0]

    low = jax.lax.broadcasted_iota(jnp.int32, (8, 128), 1) < 64

    def cross(x0, x1):
        lo = jnp.concatenate([low] * (x0.shape[0] // 8), axis=0)
        return jnp.where(lo, x0, x1), pltpu.roll(jnp.where(lo, x1, x0), 64, 1)

    def stash(slot, ks, ws, g):
        n = 8 * (g + 2)
        starts = []
        for i, x in enumerate(ks + ws):
            base = (4 * slot + i) * (L + 8)
            kv_v[pl.ds(base, n), :] = jnp.concatenate([x[8 * g:8 * g + 8], x[0:n - 8]], axis=0)
            starts.append(base + n - 8)
        return starts, [jnp.sum(w[n - 8:L], axis=0, keepdims=True) if n - 8 < L
                        else jnp.zeros((1, DH), F32) for w in ws]

    def vpu_start(q0, q1, parked, g):
        starts, (acc_a, acc_b) = parked
        return dict(q=(q0 * c_exp, q1 * c_exp), starts=starts, g=g,
                    m=jnp.full((8, 128), neg_c, F32),
                    l=jnp.full((8, 128), float(L - 8 * (g + 1)), F32), a=acc_a, b=acc_b)

    def vpu_chunk(st, c0, gate):
        k0, k1, wa, wb = st['starts']
        g = st['g']
        q0, q1 = [pltpu.bitcast(pltpu.bitcast(q, U32) | gate, F32) for q in st['q']]
        sc = []
        for r in range(c0, min(c0 + CHUNK, 8 * (g + 1))):
            sr = jnp.where(
                low, jnp.sum(q0 * kv_v[pl.ds(k0 - r, 8), :], axis=-1, keepdims=True),
                jnp.sum(q1 * kv_v[pl.ds(k1 - r, 8), :], axis=-1, keepdims=True))
            if r > 8 * g:
                sr = jnp.where(sub >= r - 8 * g, sr, neg_c)
            sc.append(sr)
        m = jnp.maximum(tree(jnp.maximum, sc), st['m'])
        alpha = jnp.exp2(st['m'] - m)
        l, acc_a, acc_b = st['l'] * alpha, st['a'] * alpha, st['b'] * alpha
        for n, sr in enumerate(sc):
            pr = jnp.exp2(sr - m)
            l = l + pr
            acc_a = acc_a + pr * kv_v[pl.ds(wa - c0 - n, 8), :]
            acc_b = acc_b + pr * kv_v[pl.ds(wb - c0 - n, 8), :]
        st.update(m=m, l=l, a=acc_a, b=acc_b)
        return pltpu.bitcast(l, U32) | pltpu.bitcast(acc_a, U32) | pltpu.bitcast(acc_b, U32)

    def vpu_finish(st):
        r = recip(st['l'])
        oa = st['a'] * r
        ob = pltpu.roll(st['b'] * r, 64, 1)
        return jnp.where(low, oa, ob), jnp.where(low, ob, oa)

    def segment(lhs_q, lhs_kv, wo_m, ngv, unpack, wo_rows, split_first, early, d_j, zero):
        NP = H // 2
        nj = D // 128
        HA = H - TAIL_H
        allowed, fill = masks[ngv]
        mxu_groups = [0] + list(range(ngv + 1, 5))
        rm = 8 * len(mxu_groups)
        proj = {}
        qkv = [None] * NP
        pb = [None] * NP
        og = [dict() for _ in range(H)]
        ocat = {}
        y = [None] * nj

        def slab(toks, which, h, r0, n):
            x = lhs_q if which == 0 else lhs_kv
            w = tied(wqkv_v[pl.ds(_slab_of(which, h) * PITCH + r0, n), :], toks)
            r = jnp.dot(x[:, 2 * r0:2 * (r0 + n)], w, preferred_element_type=F32)
            proj[(which, h)] = r + proj[(which, h)] if (which, h) in proj else r
            return proj[(which, h)]

        def do_wo(toks, h0, h1, j):
            if (h0, h1) not in ocat:
                ocat[(h0, h1)] = jnp.concatenate(
                    [wo_rows(og[h]) for h in range(h0, h1)], axis=1).astype(BF16)
            w = tied(wo_v[j, pl.ds(h0 * 64, (h1 - h0) * 64), :], toks)
            r = jnp.dot(ocat[(h0, h1)], w, preferred_element_type=F32)
            y[j] = r if y[j] is None else r + y[j]
            return y[j]

        ticks = []
        pair_end = {}
        wo_early = [(4 * c, 4 * c + 4, j) for c in range(early) for j in range(nj)]
        first = NP - WO_SLOTS
        for p in range(NP):
            slabs = [(which, h) for h in (2 * p, 2 * p + 1) for which in range(3)]
            rows = [(lhs_q if w == 0 else lhs_kv).shape[0] for w, _ in slabs]
            if p == 0 and split_first:
                for r0 in (0, 256):
                    ticks += [(slab, (w, h, r0, 256), m) for (w, h), m in zip(slabs, rows)]
            else:
                mine = []
                if p >= first:
                    lo = (p - first) * len(wo_early) // WO_SLOTS
                    mine = wo_early[lo:(p - first + 1) * len(wo_early) // WO_SLOTS]
                for n, ((w, h), m) in enumerate(zip(slabs, rows)):
                    ticks += [(do_wo, item, wo_m)
                              for item in mine[n * len(mine) // 6:(n + 1) * len(mine) // 6]]
                    ticks.append((slab, (w, h, 0, 512), 2 * m + rm // 6))
            pair_end[len(ticks) - 1] = p
        ticks += [(do_wo, (h0, h0 + 4, j), wo_m)
                  for j in range(nj) for h0 in range(4 * early, HA, 4)]
        ends = []
        for _, _, dur in ticks:
            ends.append(dur + (ends[-1] if ends else 0))

        def index(t):
            return next(i for i, e in enumerate(ends) if e >= t)

        events = {}
        anchors = {}
        cursor = [0]

        def run_chunk(res, p, name, st, c0, i_done):
            done = vpu_chunk(st, c0, pltpu.bitcast(res[0:8], U32) & zero)
            anchors.setdefault(i_done, []).append(done & zero)
            if c0 + CHUNK >= 8 * (st['g'] + 1):
                og[2 * p][name], og[2 * p + 1][name] = vpu_finish(st)

        def do_s(res, p):
            sc = jax.lax.dot_general(qkv[p][0], qkv[p][1], (((1,), (1,)), ((), ())),
                                     preferred_element_type=F32)
            sc = jnp.where(allowed, sc, fill)
            e = jnp.exp2((sc - jnp.max(sc, axis=-1, keepdims=True)) * c_exp)
            l = jnp.sum(e, axis=-1, keepdims=True)
            pb[p] = (e * recip(l)).astype(BF16)

        def do_pv(res, p):
            o = jnp.dot(pb[p], qkv[p][2], preferred_element_type=F32)
            for i in range(2):
                for n, g in enumerate(mxu_groups):
                    og[2 * p + i][g] = o[i * rm + 8 * n:i * rm + 8 * n + 8]

        def finish_pair(p, i):
            u, jobs = unpack(p, [[proj[(w, h)] for w in range(3)] for h in (2 * p, 2 * p + 1)])
            chunks = [(name, st, c0) for name, st in
                      [(name, vpu_start(*job)) for name, job in jobs.items()]
                      for c0 in range(0, 8 * (st['g'] + 1), CHUNK)]
            t_first = ends[min(pair_end)] + D_G
            t_last = ends[-2] - d_j - D_F
            gap = (t_last - t_first) / (NP * len(chunks) - 1)
            if p == NP - 1:
                gap = min(gap, (t_last - max(ends[i] + D_G, cursor[0])) / (len(chunks) - 1))
            for chunk in chunks:
                t = max(ends[i] + D_G, cursor[0])
                cursor[0] = t + gap
                g = max(index(t), i + 1)
                events.setdefault(g, []).append(
                    (run_chunk, (p,) + chunk + (index(ends[g] + d_j) + 1,)))
            qb = jnp.concatenate([u[k][0][g] for k in range(2) for g in mxu_groups],
                                 axis=0).astype(BF16)
            kb = jnp.concatenate([u[0][1], u[1][1], zpad], axis=0).astype(BF16)
            vb = jnp.concatenate([u[0][2], u[1][2], zpad], axis=0).astype(BF16)
            qkv[p] = (qb, kb, vb)
            t_pv = min(ends[i] + D_PV, ends[-1] - D_O)
            events.setdefault(index(min(ends[i] + D_S, t_pv - D_SM)), []).append((do_s, (p,)))
            events.setdefault(index(t_pv), []).append((do_pv, (p,)))

        for i, (fn, args, _) in enumerate(ticks):
            res = fn(anchors.pop(i, []), *args)
            if i in pair_end:
                finish_pair(pair_end[i], i)
            for f, a in events.pop(i, []):
                f(res, *a)
        assert not events
        for j in range(nj):
            do_wo([], HA, H, j)
        return jnp.concatenate(y, axis=1)

    def pair(r0, mem):
        xf = x_v[pl.ds(r0, PAIR), :].astype(F32)
        zero = zero_v[pl.ds(0, 8), :]
        x1s = jnp.concatenate([xf[0:8], xf[32:40]], axis=0).astype(BF16)
        keep = [None] * H

        def cat(*xs):
            return jnp.concatenate(xs, axis=0)

        lhs = cat(mem, xf[8:32]).astype(BF16)

        def finish(qg, ks, vs, slot, groups):
            ws = list(cross(vs[0], vs[1]))
            return ([(qg[i], ks[i], vs[i]) for i in range(2)],
                    {g: stash(slot + n, ks, ws, g) for n, g in enumerate(groups)})

        def unpack_a(p, qkv):
            qg = [{0: q[0:8], 2: q[8:16], 3: q[16:24], 4: q[24:32]} for q, _, _ in qkv]
            ks = [cat(k[0:8], k[32:40], k[8:32]) for _, k, _ in qkv]
            vs = [cat(v[0:8], v[32:40], v[8:32]) for _, _, v in qkv]
            u, parked = finish(qg, ks, vs, NJOB * p, range(1, NGV_A + 1))
            keep[p] = (parked[1], [(k[40:48], v[40:48]) for _, k, v in qkv])
            return u, {g: (qg[0][g], qg[1][g], parked[g], g) for g in range(2, NGV_A + 1)}

        y_a = segment(lhs, cat(lhs, x1s), 32, NGV_A, unpack_a,
                      lambda o: cat(o[0], o[2], o[3], o[4]), False, EARLY_A, D_JA, zero)

        lhs = cat(y_a[0:8], xf[40:64]).astype(BF16)

        def unpack_b(p, qkv):
            parked_a1, kv1 = keep[p]
            qg = [{0: q[0:8], 1: q[40:48], 2: q[8:16], 3: q[16:24], 4: q[24:32]}
                  for q, _, _ in qkv]
            ks = [cat(k[0:8], e[0], k[8:32]) for (_, k, _), e in zip(qkv, kv1)]
            vs = [cat(v[0:8], e[1], v[8:32]) for (_, _, v), e in zip(qkv, kv1)]
            u, parked = finish(qg, ks, vs, NJOB * p + NGV_A, range(1, NGV_B + 1))
            jobs = {'a1': (qkv[0][0][32:40], qkv[1][0][32:40], parked_a1, 1)}
            jobs.update({g: (qg[0][g], qg[1][g], parked[g], g) for g in range(1, NGV_B + 1)})
            return u, jobs

        y_b = segment(cat(lhs, x1s), lhs, 48, NGV_B, unpack_b,
                      lambda o: cat(o[0], o[1], o[2], o[3], o[4], o['a1']), True, EARLY_B,
                      D_JB, zero)

        a = cat(y_b[40:48], y_a[8:32], y_b[8:40])
        g = g_v[pl.ds(r0, PAIR), :]
        g = jnp.concatenate([g] * (D // 128), axis=1)
        out_v[pl.ds(r0, PAIR), :] = (g * a + h1_v[pl.ds(r0, PAIR), :]).astype(BF16)
        return y_b[0:8]

    rows_it = UNROLL_A * PAIR

    def a_body(t, carry):
        base = pl.multiple_of(t * rows_it, rows_it)
        mem = mem_v[...]
        for u in range(UNROLL_A):
            mem = pair(pl.multiple_of(base + u * PAIR, PAIR), mem)
        mem_v[...] = mem
        pltpu.make_async_copy(out_v.at[pl.ds(base, rows_it)], out_hbm.at[pl.ds(base, rows_it)],
                              osem).start()
        return carry

    with jax.named_scope('a_body'):
        jax.lax.fori_loop(0, S // rows_it, a_body, 0)
    pltpu.make_async_copy(out_v, out_hbm, osem).wait()


@jax.jit
def pallas_gated_mix__memory_aug_recurrent_mem_tr__mixer_s_mlp__prompt_kernel(
    A_x, A_mem0, A_Wq, A_Wk, A_Wv, A_Wo, A_seg_len, B_x, B_w1, B_w2, B_w3, B_w4, gate_w,
):
    assert A_x.shape == (1, S, D) and A_Wq.shape == (D, H, DH) and A_mem0.shape == (1, M, D)
    x = A_x.reshape(S, D)
    mem0 = A_mem0.reshape(M, D)
    wq = A_Wq.reshape(D * H, DH)
    wk = A_Wk.reshape(D * H, DH)
    wv = A_Wv.reshape(D * H, DH)
    wo = A_Wo.reshape(H * DH, D)

    any_spec = pl.BlockSpec(memory_space=pl.ANY)
    out = pl.pallas_call(
        _kernel,
        out_shape=jax.ShapeDtypeStruct((S, D), BF16),
        in_specs=[any_spec] * 11,
        out_specs=any_spec,
        scratch_shapes=[
            pltpu.VMEM((S, D), BF16),
            pltpu.VMEM((2, 3, DP * H, DH), BF16),
            pltpu.VMEM((2, OP, D), BF16),
            pltpu.VMEM((3 * H * PITCH, 128), U32),
            pltpu.VMEM((D // 128, H * DH // 2, 128), U32),
            pltpu.VMEM((4, D, D // 4), BF16),
            pltpu.VMEM((4, D, D // 4), BF16),
            pltpu.VMEM((D, FF), BF16),
            pltpu.VMEM((FF, D), BF16),
            pltpu.VMEM((S + 16, D), F32),
            pltpu.VMEM((S, D), F32),
            pltpu.VMEM((S, 128), F32),
            pltpu.VMEM((2, T1, D), BF16),
            pltpu.VMEM((2, T3, D), BF16),
            pltpu.VMEM((M, D), BF16),
            pltpu.VMEM((D,), BF16),
            pltpu.VMEM((M, D), F32),
            pltpu.VMEM((S, D), BF16),
            pltpu.VMEM((NJOB * H * 2 * (L + 8), 128), F32),
            pltpu.VMEM((16, 128), U32),
            pltpu.SemaphoreType.DMA((NSEM,)),
            pltpu.SemaphoreType.DMA(()),
        ],
        compiler_params=pltpu.CompilerParams(vmem_limit_bytes=120 * 1024 * 1024,
                                             disable_bounds_checks=True),
    )(x, mem0, wq, wk, wv, wo, B_w1, B_w2, B_w3, B_w4, gate_w)
    return out.reshape(1, S, D)
```

```python
import math

import jax
import jax.numpy as jnp
import jax.experimental.pallas as pl
import jax.experimental.pallas.tpu as pltpu

F32 = jnp.float32
BF16 = jnp.bfloat16
U32 = jnp.uint32

S = 2048
D = 1024
H = 32
DH = 128
M = 8
SEG = 32
L = M + SEG
FF = 3584
PAIR = 2 * SEG
NPAIR = S // PAIR
T1 = 256
N1 = S // T1
T2 = 512
N2 = S // T2
T3 = 256
N3 = S // T3
DP = D // N3
OP = H * DH // N3
UNROLL_A = 1
PITCH = 520
SEM_X = 12
SEM_P = SEM_X + N1
NSEM = SEM_P + 8
EPS = 1e-5
NCHAIN0 = 5
NCHAIN1 = 2
HOP = 4
KEYS_A = 3.0
KEYS_B = 2.0
NGV_A = [int((p + 1) * KEYS_A + 1e-6) - int(p * KEYS_A + 1e-6) for p in range(H // 2)]
NGV_B = [int((p + 1) * KEYS_B + 1e-6) - int(p * KEYS_B + 1e-6) for p in range(H // 2)]
NJOB = max(NGV_A) + max(NGV_B)
EARLY_A = 2
EARLY_B = 3
WO_SLOTS = 10
CHUNK = 8
D_G = 0
D_JA = 530
D_JB = 600
D_F = 100
D_R = 0
D_S = 500
D_PV = 1400
D_SM = 600
D_O = 170
TAIL_H = 8
NEG = -1e9


def _gelu(x):
    c = math.sqrt(2.0 / math.pi)
    return 0.5 * x * (1.0 + jnp.tanh(c * (x + 0.044715 * (x * x * x))))


def _layernorm(x):
    m = jnp.mean(x, axis=-1, keepdims=True)
    xc = x - m
    v = jnp.mean(xc * xc, axis=-1, keepdims=True)
    return xc * jax.lax.rsqrt(v + EPS)


def _slab_of(which, h):
    return which * H + (h % 2) * (H // 2) + h // 2


def _kernel(x_hbm, mem0_hbm, wq_hbm, wk_hbm, wv_hbm, wo_hbm,
            w1_hbm, w2_hbm, w3_hbm, w4_hbm, gw_hbm,
            out_hbm,
            x_v, stq_v, sto_v, wqkv_v, wo_v, w1_v, w2_v, w3_v, w4_v,
            h1_v, x1_v, g_v, ln1_v, ln3_v, mem0_v, gw_v, mem_v, out_v, kv_v, zero_v, sems, osem):
    def cp_x(i):
        r0 = i * T1 if isinstance(i, int) else pl.multiple_of(i * T1, T1)
        return pltpu.make_async_copy(x_hbm.at[pl.ds(r0, T1)], x_v.at[pl.ds(r0, T1)],
                                     sems.at[SEM_X + i])

    c4 = D // 4
    cp_gw = pltpu.make_async_copy(gw_hbm, gw_v, sems.at[0])
    cp_m0 = pltpu.make_async_copy(mem0_hbm, mem0_v, sems.at[1])
    cp_w3 = pltpu.make_async_copy(w3_hbm, w3_v, sems.at[2])
    cp_w4 = pltpu.make_async_copy(w4_hbm, w4_v, sems.at[3])
    cp_w1 = [pltpu.make_async_copy(w1_hbm.at[:, pl.ds(q * c4, c4)], w1_v.at[q], sems.at[4 + q])
             for q in range(4)]
    cp_w2 = [pltpu.make_async_copy(w2_hbm.at[:, pl.ds(q * c4, c4)], w2_v.at[q], sems.at[8 + q])
             for q in range(4)]

    def piece_copies(i, slot):
        cps = [pltpu.make_async_copy(w.at[pl.ds(i * (DP * H), DP * H)], stq_v.at[slot, k],
                                     sems.at[SEM_P + 4 * slot + k])
               for k, w in enumerate((wq_hbm, wk_hbm, wv_hbm))]
        cps.append(pltpu.make_async_copy(wo_hbm.at[pl.ds(i * OP, OP)], sto_v.at[slot],
                                         sems.at[SEM_P + 4 * slot + 3]))
        return cps

    cp_x(0).start()
    for c in cp_w1:
        c.start()
    for i in range(1, N1):
        cp_x(i).start()
    for c in cp_w2:
        c.start()
    cp_gw.start()
    cp_m0.start()
    cp_w3.start()
    cp_w4.start()
    for c in piece_copies(0, 0):
        c.start()
    h1_v[pl.ds(8, 8), :] = jnp.zeros((8, D), F32)
    h1_v[pl.ds(S, 8), :] = jnp.zeros((8, D), F32)
    zero_v[...] = jnp.zeros((16, 128), U32)

    def ln_rows(x, tok, zero):
        if tok is not None:
            head = pltpu.bitcast(pltpu.bitcast(x[:, 0:128], U32) | tok, F32)
            x = jnp.concatenate([head, x[:, 128:]], axis=1)
        y = _layernorm(x)
        tok = None if zero is None else pltpu.bitcast(y[:, 0:128], U32) & zero
        return y, tok

    def ln_block(load, store, rows, nchain):
        zero = zero_v[...] if nchain else None
        toks = [None] * max(nchain, 1)
        for k in range(rows // 16):
            y, toks[k % len(toks)] = ln_rows(load(k), toks[k % len(toks)], zero)
            store(k, y.astype(BF16))
        return toks[(rows // 16 - 1) % len(toks)]

    def prep1(blk, slot, nchain):
        r0 = blk * T1 if isinstance(blk, int) else pl.multiple_of(blk * T1, T1)

        def store(k, y):
            ln1_v[slot, pl.ds(k * 16, 16), :] = y

        ln_block(lambda k: x_v[pl.ds(r0 + k * 16, 16), :].astype(F32), store, T1, nchain)

    def p1_quarter(lhs, r0, q):
        h = _gelu(jnp.dot(lhs, w1_v[q], preferred_element_type=F32))
        win = h1_v.at[pl.ds(r0, T1 + 16)]
        win[pl.ds(8 + (1, -1, 2, -2)[q], T1), pl.ds(q * c4, c4)] = h

    cp_x(0).wait()
    prep1(0, 0, 0)
    for q in range(4):
        cp_w1[q].wait()
        if q == 3:
            cp_x(1).wait()
        lhs = ln1_v[0]
        if q == 3:
            prep1(1, 1, NCHAIN0)
        p1_quarter(lhs, 0, q)

    def p1_body(i, carry):
        r0 = pl.multiple_of(i * T1, T1)
        slot = i % 2

        @pl.when(i + 1 < N1)
        def _():
            cp_x(i + 1).wait()

        lhs = ln1_v[slot]
        prep1(jnp.minimum(i + 1, N1 - 1), 1 - slot, NCHAIN1)
        for q in range(4):
            p1_quarter(lhs, r0, q)
        return carry

    with jax.named_scope('p1_body'):
        jax.lax.fori_loop(1, N1, p1_body, 0)
    for c in cp_w2:
        c.wait()

    def p2_body(i, carry):
        r0 = pl.multiple_of(i * T2, T2)
        hs = h1_v[pl.ds(r0 + 8, T2), :].astype(BF16)
        for q in range(4):
            x1_v[pl.ds(r0, T2), pl.ds(q * c4, c4)] = (
                jnp.dot(hs, w2_v[q], preferred_element_type=F32)
                + x_v[pl.ds(r0, T2), pl.ds(q * c4, c4)].astype(F32))
        return carry

    with jax.named_scope('p2_body'):
        jax.lax.fori_loop(0, N2, p2_body, 0)

    def prep3(blk, slot, nchain):
        r0 = blk * T3 if isinstance(blk, int) else pl.multiple_of(blk * T3, T3)

        def store(k, y):
            ln3_v[slot, pl.ds(k * 16, 16), :] = y

        return ln_block(lambda k: x1_v[pl.ds(r0 + k * 16, 16), :], store, T3, nchain)

    prep3(0, 0, 0)
    cp_gw.wait()
    cp_m0.wait()
    cp_w3.wait()
    cp_w4.wait()

    def p3_body(i, carry):
        r0 = pl.multiple_of(i * T3, T3)
        slot = i % 2

        @pl.when(i + 1 < N3)
        def _():
            for c in piece_copies(i + 1, 1 - slot):
                c.start()

        for c in piece_copies(i, slot):
            c.wait()

        lhs = ln3_v[slot]
        tok = prep3(jnp.minimum(i + 1, N3 - 1), 1 - slot, 1)
        zero = zero_v[...]
        for which in range(3):
            for j in range(DP // 2):
                blk = pltpu.bitcast(stq_v[slot, which, pl.ds(j * 64, 64), :], U32)
                a = blk[0:16] | tok
                c = blk[16:32]
                lo = (a & jnp.uint32(0xFFFF)) | (c << 16)
                a = a | (lo & zero)
                hi = (a >> 16) | (c & jnp.uint32(0xFFFF0000))
                tok = hi & zero
                if j % HOP == HOP - 1:
                    tok = pltpu.roll(tok, 1, 1)
                s0 = which * H * PITCH + i * (DP // 2) + j
                wqkv_v[pl.ds(s0, 16, stride=PITCH), :] = lo
                wqkv_v[pl.ds(s0 + 16 * PITCH, 16, stride=PITCH), :] = hi
        o0 = pl.multiple_of(i * (OP // 2), OP // 2)
        for j in range(D // 128):
            for k in range(OP // 32):
                w = pltpu.bitcast(sto_v[slot, pl.ds(k * 32, 32), pl.ds(j * 128, 128)], U32) | tok
                tok = w & zero
                if k % (2 * HOP) == 2 * HOP - 1:
                    tok = pltpu.roll(tok, 1, 1)
                wo_v[j, pl.ds(o0 + k * 16, 16), :] = w

        h = _gelu(jnp.dot(lhs, w3_v[...], preferred_element_type=F32)).astype(BF16)
        b = jnp.dot(h, w4_v[...], preferred_element_type=F32) + x1_v[pl.ds(r0, T3), :]
        gw = gw_v[...].astype(F32).reshape(1, D)
        z = jnp.sum(x_v[pl.ds(r0, T3), :].astype(F32) * gw, axis=-1, keepdims=True)
        g = 1.0 / (1.0 + jnp.exp(-z))
        g_v[pl.ds(r0, T3), :] = jnp.broadcast_to(g, (T3, 128))
        h1_v[pl.ds(r0, T3), :] = (1.0 - g) * b
        return carry

    with jax.named_scope('p3_body'):
        jax.lax.fori_loop(0, N3, p3_body, 0)

    mem_v[...] = mem0_v[...].astype(F32)
    c_exp = (DH ** -0.5) * math.log2(math.e)
    neg_raw = NEG / (DH ** -0.5)

    L2 = 2 * L

    def make_mask(ngv):
        rm = L - 8 * ngv
        row = jax.lax.broadcasted_iota(jnp.int32, (2 * rm, 128), 0)
        col = jax.lax.broadcasted_iota(jnp.int32, (2 * rm, 128), 1)
        second = row >= rm
        rowl = jnp.where(second, row - rm, row)
        coll = jnp.where(second, col - L, col)
        real = (coll >= 0) & (coll < L)
        allowed = real & ((rowl < M) | (rowl + 8 * ngv >= coll))
        return allowed, jnp.where(real, neg_raw, -jnp.inf).astype(F32)

    masks = {n: make_mask(n) for n in set(NGV_A + NGV_B)}
    sub = jax.lax.broadcasted_iota(jnp.int32, (8, 1), 0)
    neg_c = NEG * math.log2(math.e)

    def tied(w, toks):
        for tok in toks:
            w = jnp.concatenate([w[0:56], w[56:64] | tok, w[64:]], axis=0)
        return pltpu.bitcast(w, BF16)

    zpad = jnp.zeros((128 - L2, DH), F32)

    def recip(l):
        r = pl.reciprocal(l, approx=True)
        return r * (2.0 - l * r)

    def tree(op, xs):
        xs = list(xs)
        while len(xs) > 1:
            xs = [op(xs[i], xs[i + 1]) if i + 1 < len(xs) else xs[i]
                  for i in range(0, len(xs), 2)]
        return xs[0]

    low = jax.lax.broadcasted_iota(jnp.int32, (8, 128), 1) < 64

    def cross(x0, x1):
        lo = jnp.concatenate([low] * (x0.shape[0] // 8), axis=0)
        return jnp.where(lo, x0, x1), pltpu.roll(jnp.where(lo, x1, x0), 64, 1)

    def stash(slot, ks, ws, g):
        n = 8 * (g + 2)
        starts = []
        for i, x in enumerate(ks + ws):
            base = (4 * slot + i) * (L + 8)
            kv_v[pl.ds(base, n), :] = jnp.concatenate([x[8 * g:8 * g + 8], x[0:n - 8]], axis=0)
            starts.append(base + n - 8)
        return starts, [jnp.sum(w[n - 8:L], axis=0, keepdims=True) if n - 8 < L
                        else jnp.zeros((1, DH), F32) for w in ws]

    def vpu_start(q0, q1, parked, g):
        starts, (acc_a, acc_b) = parked
        return dict(q=(q0 * c_exp, q1 * c_exp), starts=starts, g=g,
                    m=jnp.full((8, 128), neg_c, F32),
                    l=jnp.full((8, 128), float(L - 8 * (g + 1)), F32), a=acc_a, b=acc_b)

    def vpu_chunk(st, c0, gate):
        k0, k1, wa, wb = st['starts']
        g = st['g']
        q0, q1 = [pltpu.bitcast(pltpu.bitcast(q, U32) | gate, F32) for q in st['q']]
        sc = []
        for r in range(c0, min(c0 + CHUNK, 8 * (g + 1))):
            sr = jnp.where(
                low, jnp.sum(q0 * kv_v[pl.ds(k0 - r, 8), :], axis=-1, keepdims=True),
                jnp.sum(q1 * kv_v[pl.ds(k1 - r, 8), :], axis=-1, keepdims=True))
            if r > 8 * g:
                sr = jnp.where(sub >= r - 8 * g, sr, neg_c)
            sc.append(sr)
        m = jnp.maximum(tree(jnp.maximum, sc), st['m'])
        alpha = jnp.exp2(st['m'] - m)
        l, acc_a, acc_b = st['l'] * alpha, st['a'] * alpha, st['b'] * alpha
        for n, sr in enumerate(sc):
            pr = jnp.exp2(sr - m)
            l = l + pr
            acc_a = acc_a + pr * kv_v[pl.ds(wa - c0 - n, 8), :]
            acc_b = acc_b + pr * kv_v[pl.ds(wb - c0 - n, 8), :]
        st.update(m=m, l=l, a=acc_a, b=acc_b)
        return pltpu.bitcast(l, U32) | pltpu.bitcast(acc_a, U32) | pltpu.bitcast(acc_b, U32)

    def vpu_finish(st):
        r = recip(st['l'])
        oa = st['a'] * r
        ob = pltpu.roll(st['b'] * r, 64, 1)
        return jnp.where(low, oa, ob), jnp.where(low, ob, oa)

    def segment(lhs_q, lhs_kv, wo_m, ngv, n_chunks, unpack, wo_rows, split_first, early, d_j, zero):
        NP = H // 2
        nj = D // 128
        HA = H - TAIL_H
        mxu_groups = [[0] + list(range(n + 1, 5)) for n in ngv]
        proj = {}
        qkv = [None] * NP
        pb = [None] * NP
        og = [dict() for _ in range(H)]
        ocat = {}
        y = [None] * nj

        def slab(toks, which, h, r0, n):
            x = lhs_q if which == 0 else lhs_kv
            w = tied(wqkv_v[pl.ds(_slab_of(which, h) * PITCH + r0, n), :], toks)
            r = jnp.dot(x[:, 2 * r0:2 * (r0 + n)], w, preferred_element_type=F32)
            proj[(which, h)] = r + proj[(which, h)] if (which, h) in proj else r
            return proj[(which, h)]

        def do_wo(toks, h0, h1, j):
            if (h0, h1) not in ocat:
                ocat[(h0, h1)] = jnp.concatenate(
                    [wo_rows(og[h]) for h in range(h0, h1)], axis=1).astype(BF16)
            w = tied(wo_v[j, pl.ds(h0 * 64, (h1 - h0) * 64), :], toks)
            r = jnp.dot(ocat[(h0, h1)], w, preferred_element_type=F32)
            y[j] = r if y[j] is None else r + y[j]
            return y[j]

        ticks = []
        pair_end = {}
        wo_early = [(4 * c, 4 * c + 4, j) for c in range(early) for j in range(nj)]
        first = NP - WO_SLOTS
        for p in range(NP):
            slabs = [(which, h) for h in (2 * p, 2 * p + 1) for which in range(3)]
            rows = [(lhs_q if w == 0 else lhs_kv).shape[0] for w, _ in slabs]
            if p == 0 and split_first:
                for r0 in (0, 256):
                    ticks += [(slab, (w, h, r0, 256), m) for (w, h), m in zip(slabs, rows)]
            else:
                mine = []
                if p >= first:
                    lo = (p - first) * len(wo_early) // WO_SLOTS
                    mine = wo_early[lo:(p - first + 1) * len(wo_early) // WO_SLOTS]
                for n, ((w, h), m) in enumerate(zip(slabs, rows)):
                    ticks += [(do_wo, item, wo_m)
                              for item in mine[n * len(mine) // 6:(n + 1) * len(mine) // 6]]
                    ticks.append((slab, (w, h, 0, 512), 2 * m + 8 * len(mxu_groups[p]) // 6))
            pair_end[len(ticks) - 1] = p
        ticks += [(do_wo, (h0, h0 + 4, j), wo_m)
                  for j in range(nj) for h0 in range(4 * early, HA, 4)]
        ends = []
        for _, _, dur in ticks:
            ends.append(dur + (ends[-1] if ends else 0))

        def index(t):
            return next(i for i, e in enumerate(ends) if e >= t)

        events = {}
        anchors = {}
        cursor = [0]

        def run_chunk(res, p, name, st, c0, i_done):
            done = vpu_chunk(st, c0, pltpu.bitcast(res[0:8], U32) & zero)
            anchors.setdefault(i_done, []).append(done & zero)
            if c0 + CHUNK >= 8 * (st['g'] + 1):
                og[2 * p][name], og[2 * p + 1][name] = vpu_finish(st)
                if D_R and ends[i_done - 1] + D_R < ends[-2]:
                    anchors.setdefault(index(ends[i_done - 1] + D_R) + 1, []).append(
                        pltpu.bitcast(og[2 * p][name], U32) & zero)

        def do_s(res, p):
            sc = jax.lax.dot_general(qkv[p][0], qkv[p][1], (((1,), (1,)), ((), ())),
                                     preferred_element_type=F32)
            allowed, fill = masks[ngv[p]]
            sc = jnp.where(allowed, sc, fill)
            e = jnp.exp2((sc - jnp.max(sc, axis=-1, keepdims=True)) * c_exp)
            l = jnp.sum(e, axis=-1, keepdims=True)
            pb[p] = (e * recip(l)).astype(BF16)

        def do_pv(res, p):
            o = jnp.dot(pb[p], qkv[p][2], preferred_element_type=F32)
            rm = 8 * len(mxu_groups[p])
            for i in range(2):
                for n, g in enumerate(mxu_groups[p]):
                    og[2 * p + i][g] = o[i * rm + 8 * n:i * rm + 8 * n + 8]

        def finish_pair(p, i):
            u, jobs = unpack(p, [[proj[(w, h)] for w in range(3)] for h in (2 * p, 2 * p + 1)])
            chunks = [(name, st, c0) for name, st in
                      [(name, vpu_start(*job)) for name, job in jobs.items()]
                      for c0 in range(0, 8 * (st['g'] + 1), CHUNK)]
            t_first = ends[min(pair_end)] + D_G
            t_last = ends[-2] - d_j - D_F
            gap = (t_last - t_first) / (n_chunks - 1)
            if p == NP - 1:
                gap = min(gap, (t_last - max(ends[i] + D_G, cursor[0])) / (len(chunks) - 1))
            for chunk in chunks:
                t = max(ends[i] + D_G, cursor[0])
                cursor[0] = t + gap
                g = max(index(t), i + 1)
                events.setdefault(g, []).append(
                    (run_chunk, (p,) + chunk + (index(ends[g] + d_j) + 1,)))
            qb = jnp.concatenate([u[k][0][g] for k in range(2) for g in mxu_groups[p]],
                                 axis=0).astype(BF16)
            kb = jnp.concatenate([u[0][1], u[1][1], zpad], axis=0).astype(BF16)
            vb = jnp.concatenate([u[0][2], u[1][2], zpad], axis=0).astype(BF16)
            qkv[p] = (qb, kb, vb)
            t_pv = min(ends[i] + D_PV, ends[-1] - D_O)
            events.setdefault(index(min(ends[i] + D_S, t_pv - D_SM)), []).append((do_s, (p,)))
            events.setdefault(index(t_pv), []).append((do_pv, (p,)))

        for i, (fn, args, _) in enumerate(ticks):
            res = fn(anchors.pop(i, []), *args)
            if i in pair_end:
                finish_pair(pair_end[i], i)
            for f, a in events.pop(i, []):
                f(res, *a)
        assert not events
        for j in range(nj):
            do_wo([], HA, H, j)
        return jnp.concatenate(y, axis=1)

    def pair(r0, mem):
        xf = x_v[pl.ds(r0, PAIR), :].astype(F32)
        zero = zero_v[pl.ds(0, 8), :]
        x1s = jnp.concatenate([xf[0:8], xf[32:40]], axis=0).astype(BF16)
        keep = [None] * H

        def cat(*xs):
            return jnp.concatenate(xs, axis=0)

        lhs = cat(mem, xf[8:32]).astype(BF16)

        def finish(qg, ks, vs, slot, groups):
            ws = list(cross(vs[0], vs[1]))
            return ([(qg[i], ks[i], vs[i]) for i in range(2)],
                    {g: stash(slot + n, ks, ws, g) for n, g in enumerate(groups)})

        def unpack_a(p, qkv):
            qg = [{0: q[0:8], 2: q[8:16], 3: q[16:24], 4: q[24:32]} for q, _, _ in qkv]
            ks = [cat(k[0:8], k[32:40], k[8:32]) for _, k, _ in qkv]
            vs = [cat(v[0:8], v[32:40], v[8:32]) for _, _, v in qkv]
            u, parked = finish(qg, ks, vs, NJOB * p, range(1, NGV_A[p] + 1))
            keep[p] = (parked[1], [(k[40:48], v[40:48]) for _, k, v in qkv])
            return u, {g: (qg[0][g], qg[1][g], parked[g], g) for g in range(2, NGV_A[p] + 1)}

        y_a = segment(lhs, cat(lhs, x1s), 32, NGV_A,
                      sum(g + 1 for n in NGV_A for g in range(2, n + 1)) * 8 // CHUNK, unpack_a,
                      lambda o: cat(o[0], o[2], o[3], o[4]), False, EARLY_A, D_JA, zero)

        lhs = cat(y_a[0:8], xf[40:64]).astype(BF16)

        def unpack_b(p, qkv):
            parked_a1, kv1 = keep[p]
            qg = [{0: q[0:8], 1: q[40:48], 2: q[8:16], 3: q[16:24], 4: q[24:32]}
                  for q, _, _ in qkv]
            ks = [cat(k[0:8], e[0], k[8:32]) for (_, k, _), e in zip(qkv, kv1)]
            vs = [cat(v[0:8], e[1], v[8:32]) for (_, _, v), e in zip(qkv, kv1)]
            u, parked = finish(qg, ks, vs, NJOB * p + max(NGV_A), range(1, NGV_B[p] + 1))
            jobs = {'a1': (qkv[0][0][32:40], qkv[1][0][32:40], parked_a1, 1)}
            jobs.update({g: (qg[0][g], qg[1][g], parked[g], g) for g in range(1, NGV_B[p] + 1)})
            return u, jobs

        y_b = segment(cat(lhs, x1s), lhs, 48, NGV_B,
                      sum(2 + sum(range(2, n + 2)) for n in NGV_B) * 8 // CHUNK, unpack_b,
                      lambda o: cat(o[0], o[1], o[2], o[3], o[4], o['a1']), True, EARLY_B,
                      D_JB, zero)

        a = cat(y_b[40:48], y_a[8:32], y_b[8:40])
        g = g_v[pl.ds(r0, PAIR), :]
        g = jnp.concatenate([g] * (D // 128), axis=1)
        out_v[pl.ds(r0, PAIR), :] = (g * a + h1_v[pl.ds(r0, PAIR), :]).astype(BF16)
        return y_b[0:8]

    rows_it = UNROLL_A * PAIR

    def a_body(t, carry):
        base = pl.multiple_of(t * rows_it, rows_it)
        mem = mem_v[...]
        for u in range(UNROLL_A):
            mem = pair(pl.multiple_of(base + u * PAIR, PAIR), mem)
        mem_v[...] = mem
        pltpu.make_async_copy(out_v.at[pl.ds(base, rows_it)], out_hbm.at[pl.ds(base, rows_it)],
                              osem).start()
        return carry

    with jax.named_scope('a_body'):
        jax.lax.fori_loop(0, S // rows_it, a_body, 0)
    pltpu.make_async_copy(out_v, out_hbm, osem).wait()


@jax.jit
def pallas_gated_mix__memory_aug_recurrent_mem_tr__mixer_s_mlp__prompt_kernel(
    A_x, A_mem0, A_Wq, A_Wk, A_Wv, A_Wo, A_seg_len, B_x, B_w1, B_w2, B_w3, B_w4, gate_w,
):
    assert A_x.shape == (1, S, D) and A_Wq.shape == (D, H, DH) and A_mem0.shape == (1, M, D)
    x = A_x.reshape(S, D)
    mem0 = A_mem0.reshape(M, D)
    wq = A_Wq.reshape(D * H, DH)
    wk = A_Wk.reshape(D * H, DH)
    wv = A_Wv.reshape(D * H, DH)
    wo = A_Wo.reshape(H * DH, D)

    any_spec = pl.BlockSpec(memory_space=pl.ANY)
    out = pl.pallas_call(
        _kernel,
        out_shape=jax.ShapeDtypeStruct((S, D), BF16),
        in_specs=[any_spec] * 11,
        out_specs=any_spec,
        scratch_shapes=[
            pltpu.VMEM((S, D), BF16),
            pltpu.VMEM((2, 3, DP * H, DH), BF16),
            pltpu.VMEM((2, OP, D), BF16),
            pltpu.VMEM((3 * H * PITCH, 128), U32),
            pltpu.VMEM((D // 128, H * DH // 2, 128), U32),
            pltpu.VMEM((4, D, D // 4), BF16),
            pltpu.VMEM((4, D, D // 4), BF16),
            pltpu.VMEM((D, FF), BF16),
            pltpu.VMEM((FF, D), BF16),
            pltpu.VMEM((S + 16, D), F32),
            pltpu.VMEM((S, D), F32),
            pltpu.VMEM((S, 128), F32),
            pltpu.VMEM((2, T1, D), BF16),
            pltpu.VMEM((2, T3, D), BF16),
            pltpu.VMEM((M, D), BF16),
            pltpu.VMEM((D,), BF16),
            pltpu.VMEM((M, D), F32),
            pltpu.VMEM((S, D), BF16),
            pltpu.VMEM((NJOB * H * 2 * (L + 8), 128), F32),
            pltpu.VMEM((16, 128), U32),
            pltpu.SemaphoreType.DMA((NSEM,)),
            pltpu.SemaphoreType.DMA(()),
        ],
        compiler_params=pltpu.CompilerParams(vmem_limit_bytes=120 * 1024 * 1024,
                                             disable_bounds_checks=True),
    )(x, mem0, wq, wk, wv, wo, B_w1, B_w2, B_w3, B_w4, gate_w)
    return out.reshape(1, S, D)
```

```python
import math

import jax
import jax.numpy as jnp
import jax.experimental.pallas as pl
import jax.experimental.pallas.tpu as pltpu

F32 = jnp.float32
BF16 = jnp.bfloat16
U32 = jnp.uint32

S = 2048
D = 1024
H = 32
DH = 128
M = 8
SEG = 32
L = M + SEG
FF = 3584
PAIR = 2 * SEG
NPAIR = S // PAIR
T1 = 256
N1 = S // T1
T2 = 512
N2 = S // T2
T3 = 256
N3 = S // T3
DP = D // N3
OP = H * DH // N3
UNROLL_A = 1
PITCH = 520
NRING = 3
NSEM = 11 + NRING
EPS = 1e-5
NCHAIN0 = 10
NCHAIN1 = 5
LN1_ROWS = 8
HOP = 4
KEYS_A = 3.0
KEYS_B = 2.0
NGV_A = [int((p + 1) * KEYS_A + 1e-6) - int(p * KEYS_A + 1e-6) for p in range(H // 2)]
NGV_B = [int((p + 1) * KEYS_B + 1e-6) - int(p * KEYS_B + 1e-6) for p in range(H // 2)]
NJOB = max(NGV_A) + max(NGV_B)
EARLY_A = 2
EARLY_B = 3
WO_SLOTS = 10
CHUNK = 8
D_G = 0
D_JA = 530
D_JB = 600
D_F = 100
D_R = 0
D_S = 500
D_PV = 1400
D_SM = 600
D_O = 170
TAIL_H = 8
NEG = -1e9


def _gelu(x):
    c = math.sqrt(2.0 / math.pi)
    return 0.5 * x * (1.0 + jnp.tanh(c * (x + 0.044715 * (x * x * x))))


def _layernorm(x):
    m = jnp.mean(x, axis=-1, keepdims=True)
    xc = x - m
    v = jnp.mean(xc * xc, axis=-1, keepdims=True)
    return xc * jax.lax.rsqrt(v + EPS)


def _slab_of(which, h):
    return which * H + (h % 2) * (H // 2) + h // 2


def _kernel(x_hbm, mem0_hbm, wq_hbm, wk_hbm, wv_hbm, wo_hbm,
            w1_hbm, w2_hbm, w3_hbm, w4_hbm, gw_hbm,
            out_hbm,
            x_v, stq_v, sto_v, wqkv_v, wo_v, w1_v, w2_v, w3_v, w4_v,
            h1_v, x1_v, g_v, ln1_v, ln3_v, mem0_v, gw_v, mem_v, out_v, kv_v, zero_v, sems, osem):
    c4 = D // 4
    xcuts = (0, 1, 2, 3, 5, N1)
    cp_x = [pltpu.make_async_copy(x_hbm.at[pl.ds(lo * T1, (hi - lo) * T1)],
                                  x_v.at[pl.ds(lo * T1, (hi - lo) * T1)], sems.at[n])
            for n, (lo, hi) in enumerate(zip(xcuts[:-1], xcuts[1:]))]
    cp_w1 = [pltpu.make_async_copy(w1_hbm.at[:, pl.ds(q * c4, c4)], w1_v.at[q], sems.at[5 + q])
             for q in range(4)]
    cp_w2 = [pltpu.make_async_copy(w2_hbm.at[:, pl.ds(q * c4, c4)], w2_v.at[q], sems.at[9])
             for q in range(4)]
    cp_ffn = [pltpu.make_async_copy(src, dst, sems.at[10])
              for src, dst in ((gw_hbm, gw_v), (mem0_hbm, mem0_v), (w3_hbm, w3_v), (w4_hbm, w4_v))]

    def piece_copies(i, slot):
        cps = [pltpu.make_async_copy(w.at[pl.ds(i * (DP * H), DP * H)], stq_v.at[slot, k],
                                     sems.at[11 + slot])
               for k, w in enumerate((wq_hbm, wk_hbm, wv_hbm))]
        cps.append(pltpu.make_async_copy(wo_hbm.at[pl.ds(i * OP, OP)], sto_v.at[slot],
                                         sems.at[11 + slot]))
        return cps

    for c in (cp_x[0:1] + cp_w1 + cp_x[1:] + cp_w2 + cp_ffn
              + piece_copies(0, 0) + piece_copies(1, 1)):
        c.start()
    x1_v[pl.ds(0, T3), :] = jnp.zeros((T3, D), F32)
    h1_v[:, pl.ds(8, 8), :] = jnp.zeros((D // 128, 8, 128), F32)
    h1_v[:, pl.ds(S, 8), :] = jnp.zeros((D // 128, 8, 128), F32)
    zero_v[...] = jnp.zeros((16, 128), U32)

    def ln_rows(x, tok, zero):
        if tok is not None:
            head = pltpu.bitcast(pltpu.bitcast(x[:, 0:128], U32) | tok, F32)
            x = jnp.concatenate([head, x[:, 128:]], axis=1)
        y = _layernorm(x)
        tok = None if zero is None else pltpu.bitcast(y[:, 0:128], U32) & zero
        return y, tok

    def ln_block(load, store, rows, nchain, gr):
        zero = zero_v[pl.ds(0, gr), :] if nchain else None
        toks = [None] * max(nchain, 1)
        for k in range(rows // gr):
            y, toks[k % len(toks)] = ln_rows(load(k * gr, gr), toks[k % len(toks)], zero)
            store(k * gr, y.astype(BF16))
        return toks[(rows // gr - 1) % len(toks)]

    def prep1(blk, slot, nchain):
        r0 = blk * T1 if isinstance(blk, int) else pl.multiple_of(blk * T1, T1)

        def store(k, y):
            ln1_v[slot, pl.ds(k, y.shape[0]), :] = y

        ln_block(lambda k, n: x_v[pl.ds(r0 + k, n), :].astype(F32), store, T1, nchain, LN1_ROWS)

    def p1_quarter(lhs, r0, q):
        h = _gelu(jnp.dot(lhs, w1_v[q], preferred_element_type=F32))
        for j in range(2):
            win = h1_v.at[2 * q + j, pl.ds(r0, T1 + 16)]
            win[pl.ds(8 + (1, -1, 2, -2)[q], T1), :] = h[:, j * 128:(j + 1) * 128]

    cp_x[0].wait()
    prep1(0, 0, 0)
    for q in range(4):
        cp_w1[q].wait()
        if q == 3:
            cp_x[1].wait()
        lhs = ln1_v[0]
        if q == 3:
            prep1(1, 1, NCHAIN0)
        p1_quarter(lhs, 0, q)

    def p1_body(i, carry):
        r0 = pl.multiple_of(i * T1, T1)
        slot = i % 2

        for n in range(2, len(cp_x)):
            pl.when(i + 1 == xcuts[n])(cp_x[n].wait)

        lhs = ln1_v[slot]
        prep1(jnp.minimum(i + 1, N1 - 1), 1 - slot, NCHAIN1)
        for q in range(4):
            p1_quarter(lhs, r0, q)
        return carry

    with jax.named_scope('p1_body'):
        jax.lax.fori_loop(1, N1, p1_body, 0)
    for c in cp_w2:
        c.wait()

    def h1_rows(r0, n):
        return jnp.concatenate([h1_v[j, pl.ds(r0, n), :] for j in range(D // 128)], axis=1)

    def prep3(src, slot):
        def store(k, y):
            ln3_v[slot, pl.ds(k, y.shape[0]), :] = y

        return ln_block(lambda k, n: src[pl.ds(k, n), :], store, T3, 1, 16)

    def p2_body(i, carry):
        r0 = pl.multiple_of(i * T2, T2)
        win = x1_v.at[pl.ds(r0, 2 * T2)]
        prep3(win, 0)
        hs = h1_rows(r0 + 8, T2).astype(BF16)
        for q in range(4):
            win[pl.ds(T2, T2), pl.ds(q * c4, c4)] = (
                jnp.dot(hs, w2_v[q], preferred_element_type=F32)
                + x_v[pl.ds(r0, T2), pl.ds(q * c4, c4)].astype(F32))
        return carry

    with jax.named_scope('p2_body'):
        jax.lax.fori_loop(0, N2, p2_body, 0)

    for c in cp_ffn:
        c.wait()
    blk0 = (N2 - 2) * T2 // T3

    def p3_body(i, carry):
        r0 = pl.multiple_of((i + blk0) % N3 * T3, T3)
        r_next = pl.multiple_of((i + 1 + blk0) % N3 * T3, T3)
        slot = i % 2
        ring = i % NRING
        for c in piece_copies(i, ring):
            c.wait()

        @pl.when(i + 2 < N3)
        def _():
            for c in piece_copies(i + 2, (i + 2) % NRING):
                c.start()

        lhs = ln3_v[slot]
        tok = prep3(x1_v.at[pl.ds(T2 + r_next, T3)], 1 - slot)
        zero = zero_v[...]
        for which in range(3):
            for j in range(DP // 2):
                blk = pltpu.bitcast(stq_v[ring, which, pl.ds(j * 64, 64), :], U32)
                a = blk[0:16] | tok
                c = blk[16:32]
                lo = (a & jnp.uint32(0xFFFF)) | (c << 16)
                a = a | (lo & zero)
                hi = (a >> 16) | (c & jnp.uint32(0xFFFF0000))
                tok = hi & zero
                if j % HOP == HOP - 1:
                    tok = pltpu.roll(tok, 1, 1)
                s0 = which * H * PITCH + i * (DP // 2) + j
                wqkv_v[pl.ds(s0, 16, stride=PITCH), :] = lo
                wqkv_v[pl.ds(s0 + 16 * PITCH, 16, stride=PITCH), :] = hi
        o0 = pl.multiple_of(i * (OP // 2), OP // 2)
        for j in range(D // 128):
            for k in range(OP // 32):
                w = pltpu.bitcast(sto_v[ring, pl.ds(k * 32, 32), pl.ds(j * 128, 128)], U32) | tok
                tok = w & zero
                if k % (2 * HOP) == 2 * HOP - 1:
                    tok = pltpu.roll(tok, 1, 1)
                wo_v[j, pl.ds(o0 + k * 16, 16), :] = w

        h = _gelu(jnp.dot(lhs, w3_v[...], preferred_element_type=F32)).astype(BF16)
        b = jnp.dot(h, w4_v[...], preferred_element_type=F32) + x1_v[pl.ds(T2 + r0, T3), :]
        gw = gw_v[...].astype(F32).reshape(1, D)
        z = jnp.sum(x_v[pl.ds(r0, T3), :].astype(F32) * gw, axis=-1, keepdims=True)
        g = 1.0 / (1.0 + jnp.exp(-z))
        g_v[pl.ds(r0, T3), :] = jnp.broadcast_to(g, (T3, 128))
        b = (1.0 - g) * b
        for j in range(D // 128):
            h1_v[j, pl.ds(r0, T3), :] = b[:, j * 128:(j + 1) * 128]
        return carry

    with jax.named_scope('p3_body'):
        jax.lax.fori_loop(0, N3, p3_body, 0)

    mem_v[...] = mem0_v[...].astype(F32)
    c_exp = (DH ** -0.5) * math.log2(math.e)
    neg_raw = NEG / (DH ** -0.5)

    L2 = 2 * L

    def make_mask(ngv):
        rm = L - 8 * ngv
        row = jax.lax.broadcasted_iota(jnp.int32, (2 * rm, 128), 0)
        col = jax.lax.broadcasted_iota(jnp.int32, (2 * rm, 128), 1)
        second = row >= rm
        rowl = jnp.where(second, row - rm, row)
        coll = jnp.where(second, col - L, col)
        real = (coll >= 0) & (coll < L)
        allowed = real & ((rowl < M) | (rowl + 8 * ngv >= coll))
        return allowed, jnp.where(real, neg_raw, -jnp.inf).astype(F32)

    masks = {n: make_mask(n) for n in set(NGV_A + NGV_B)}
    sub = jax.lax.broadcasted_iota(jnp.int32, (8, 1), 0)
    neg_c = NEG * math.log2(math.e)

    def tied(w, toks):
        for tok in toks:
            w = jnp.concatenate([w[0:56], w[56:64] | tok, w[64:]], axis=0)
        return pltpu.bitcast(w, BF16)

    zpad = jnp.zeros((128 - L2, DH), F32)

    def recip(l):
        r = pl.reciprocal(l, approx=True)
        return r * (2.0 - l * r)

    def tree(op, xs):
        xs = list(xs)
        while len(xs) > 1:
            xs = [op(xs[i], xs[i + 1]) if i + 1 < len(xs) else xs[i]
                  for i in range(0, len(xs), 2)]
        return xs[0]

    low = jax.lax.broadcasted_iota(jnp.int32, (8, 128), 1) < 64

    def cross(x0, x1):
        lo = jnp.concatenate([low] * (x0.shape[0] // 8), axis=0)
        return jnp.where(lo, x0, x1), pltpu.roll(jnp.where(lo, x1, x0), 64, 1)

    def stash(slot, ks, ws, g):
        n = 8 * (g + 2)
        starts = []
        for i, x in enumerate(ks + ws):
            base = (4 * slot + i) * (L + 8)
            kv_v[pl.ds(base, n), :] = jnp.concatenate([x[8 * g:8 * g + 8], x[0:n - 8]], axis=0)
            starts.append(base + n - 8)
        return starts, [jnp.sum(w[n - 8:L], axis=0, keepdims=True) if n - 8 < L
                        else jnp.zeros((1, DH), F32) for w in ws]

    def vpu_start(q0, q1, parked, g):
        starts, (acc_a, acc_b) = parked
        return dict(q=(q0 * c_exp, q1 * c_exp), starts=starts, g=g,
                    m=jnp.full((8, 128), neg_c, F32),
                    l=jnp.full((8, 128), float(L - 8 * (g + 1)), F32), a=acc_a, b=acc_b)

    def vpu_chunk(st, c0, gate):
        k0, k1, wa, wb = st['starts']
        g = st['g']
        q0, q1 = [pltpu.bitcast(pltpu.bitcast(q, U32) | gate, F32) for q in st['q']]
        sc = []
        for r in range(c0, min(c0 + CHUNK, 8 * (g + 1))):
            sr = jnp.where(
                low, jnp.sum(q0 * kv_v[pl.ds(k0 - r, 8), :], axis=-1, keepdims=True),
                jnp.sum(q1 * kv_v[pl.ds(k1 - r, 8), :], axis=-1, keepdims=True))
            if r > 8 * g:
                sr = jnp.where(sub >= r - 8 * g, sr, neg_c)
            sc.append(sr)
        m = jnp.maximum(tree(jnp.maximum, sc), st['m'])
        alpha = jnp.exp2(st['m'] - m)
        l, acc_a, acc_b = st['l'] * alpha, st['a'] * alpha, st['b'] * alpha
        for n, sr in enumerate(sc):
            pr = jnp.exp2(sr - m)
            l = l + pr
            acc_a = acc_a + pr * kv_v[pl.ds(wa - c0 - n, 8), :]
            acc_b = acc_b + pr * kv_v[pl.ds(wb - c0 - n, 8), :]
        st.update(m=m, l=l, a=acc_a, b=acc_b)
        return pltpu.bitcast(l, U32) | pltpu.bitcast(acc_a, U32) | pltpu.bitcast(acc_b, U32)

    def vpu_finish(st):
        r = recip(st['l'])
        oa = st['a'] * r
        ob = pltpu.roll(st['b'] * r, 64, 1)
        return jnp.where(low, oa, ob), jnp.where(low, ob, oa)

    def segment(lhs_q, lhs_kv, wo_m, ngv, n_chunks, unpack, wo_rows, split_first, early, d_j, zero):
        NP = H // 2
        nj = D // 128
        HA = H - TAIL_H
        mxu_groups = [[0] + list(range(n + 1, 5)) for n in ngv]
        proj = {}
        qkv = [None] * NP
        pb = [None] * NP
        og = [dict() for _ in range(H)]
        ocat = {}
        y = [None] * nj

        def slab(toks, which, h, r0, n):
            x = lhs_q if which == 0 else lhs_kv
            w = tied(wqkv_v[pl.ds(_slab_of(which, h) * PITCH + r0, n), :], toks)
            r = jnp.dot(x[:, 2 * r0:2 * (r0 + n)], w, preferred_element_type=F32)
            proj[(which, h)] = r + proj[(which, h)] if (which, h) in proj else r
            return proj[(which, h)]

        def do_wo(toks, h0, h1, j):
            if (h0, h1) not in ocat:
                ocat[(h0, h1)] = jnp.concatenate(
                    [wo_rows(og[h]) for h in range(h0, h1)], axis=1).astype(BF16)
            w = tied(wo_v[j, pl.ds(h0 * 64, (h1 - h0) * 64), :], toks)
            r = jnp.dot(ocat[(h0, h1)], w, preferred_element_type=F32)
            y[j] = r if y[j] is None else r + y[j]
            return y[j]

        ticks = []
        pair_end = {}
        wo_early = [(4 * c, 4 * c + 4, j) for c in range(early) for j in range(nj)]
        first = NP - WO_SLOTS
        for p in range(NP):
            slabs = [(which, h) for h in (2 * p, 2 * p + 1) for which in range(3)]
            rows = [(lhs_q if w == 0 else lhs_kv).shape[0] for w, _ in slabs]
            if p == 0 and split_first:
                for r0 in (0, 256):
                    ticks += [(slab, (w, h, r0, 256), m) for (w, h), m in zip(slabs, rows)]
            else:
                mine = []
                if p >= first:
                    lo = (p - first) * len(wo_early) // WO_SLOTS
                    mine = wo_early[lo:(p - first + 1) * len(wo_early) // WO_SLOTS]
                for n, ((w, h), m) in enumerate(zip(slabs, rows)):
                    ticks += [(do_wo, item, wo_m)
                              for item in mine[n * len(mine) // 6:(n + 1) * len(mine) // 6]]
                    ticks.append((slab, (w, h, 0, 512), 2 * m + 8 * len(mxu_groups[p]) // 6))
            pair_end[len(ticks) - 1] = p
        ticks += [(do_wo, (h0, h0 + 4, j), wo_m)
                  for j in range(nj) for h0 in range(4 * early, HA, 4)]
        ends = []
        for _, _, dur in ticks:
            ends.append(dur + (ends[-1] if ends else 0))

        def index(t):
            return next(i for i, e in enumerate(ends) if e >= t)

        events = {}
        anchors = {}
        cursor = [0]

        def run_chunk(res, p, name, st, c0, i_done):
            done = vpu_chunk(st, c0, pltpu.bitcast(res[0:8], U32) & zero)
            anchors.setdefault(i_done, []).append(done & zero)
            if c0 + CHUNK >= 8 * (st['g'] + 1):
                og[2 * p][name], og[2 * p + 1][name] = vpu_finish(st)
                if D_R and ends[i_done - 1] + D_R < ends[-2]:
                    anchors.setdefault(index(ends[i_done - 1] + D_R) + 1, []).append(
                        pltpu.bitcast(og[2 * p][name], U32) & zero)

        def do_s(res, p):
            sc = jax.lax.dot_general(qkv[p][0], qkv[p][1], (((1,), (1,)), ((), ())),
                                     preferred_element_type=F32)
            allowed, fill = masks[ngv[p]]
            sc = jnp.where(allowed, sc, fill)
            e = jnp.exp2((sc - jnp.max(sc, axis=-1, keepdims=True)) * c_exp)
            l = jnp.sum(e, axis=-1, keepdims=True)
            pb[p] = (e * recip(l)).astype(BF16)

        def do_pv(res, p):
            o = jnp.dot(pb[p], qkv[p][2], preferred_element_type=F32)
            rm = 8 * len(mxu_groups[p])
            for i in range(2):
                for n, g in enumerate(mxu_groups[p]):
                    og[2 * p + i][g] = o[i * rm + 8 * n:i * rm + 8 * n + 8]

        def finish_pair(p, i):
            u, jobs = unpack(p, [[proj[(w, h)] for w in range(3)] for h in (2 * p, 2 * p + 1)])
            chunks = [(name, st, c0) for name, st in
                      [(name, vpu_start(*job)) for name, job in jobs.items()]
                      for c0 in range(0, 8 * (st['g'] + 1), CHUNK)]
            t_first = ends[min(pair_end)] + D_G
            t_last = ends[-2] - d_j - D_F
            gap = (t_last - t_first) / (n_chunks - 1)
            if p == NP - 1:
                gap = min(gap, (t_last - max(ends[i] + D_G, cursor[0])) / (len(chunks) - 1))
            for chunk in chunks:
                t = max(ends[i] + D_G, cursor[0])
                cursor[0] = t + gap
                g = max(index(t), i + 1)
                events.setdefault(g, []).append(
                    (run_chunk, (p,) + chunk + (index(ends[g] + d_j) + 1,)))
            qb = jnp.concatenate([u[k][0][g] for k in range(2) for g in mxu_groups[p]],
                                 axis=0).astype(BF16)
            kb = jnp.concatenate([u[0][1], u[1][1], zpad], axis=0).astype(BF16)
            vb = jnp.concatenate([u[0][2], u[1][2], zpad], axis=0).astype(BF16)
            qkv[p] = (qb, kb, vb)
            t_pv = min(ends[i] + D_PV, ends[-1] - D_O)
            events.setdefault(index(min(ends[i] + D_S, t_pv - D_SM)), []).append((do_s, (p,)))
            events.setdefault(index(t_pv), []).append((do_pv, (p,)))

        for i, (fn, args, _) in enumerate(ticks):
            res = fn(anchors.pop(i, []), *args)
            if i in pair_end:
                finish_pair(pair_end[i], i)
            for f, a in events.pop(i, []):
                f(res, *a)
        assert not events
        for j in range(nj):
            do_wo([], HA, H, j)
        return jnp.concatenate(y, axis=1)

    def pair(r0, mem):
        xf = x_v[pl.ds(r0, PAIR), :].astype(F32)
        zero = zero_v[pl.ds(0, 8), :]
        x1s = jnp.concatenate([xf[0:8], xf[32:40]], axis=0).astype(BF16)
        keep = [None] * H

        def cat(*xs):
            return jnp.concatenate(xs, axis=0)

        lhs = cat(mem, xf[8:32]).astype(BF16)

        def finish(qg, ks, vs, slot, groups):
            ws = list(cross(vs[0], vs[1]))
            return ([(qg[i], ks[i], vs[i]) for i in range(2)],
                    {g: stash(slot + n, ks, ws, g) for n, g in enumerate(groups)})

        def unpack_a(p, qkv):
            qg = [{0: q[0:8], 2: q[8:16], 3: q[16:24], 4: q[24:32]} for q, _, _ in qkv]
            ks = [cat(k[0:8], k[32:40], k[8:32]) for _, k, _ in qkv]
            vs = [cat(v[0:8], v[32:40], v[8:32]) for _, _, v in qkv]
            u, parked = finish(qg, ks, vs, NJOB * p, range(1, NGV_A[p] + 1))
            keep[p] = (parked[1], [(k[40:48], v[40:48]) for _, k, v in qkv])
            return u, {g: (qg[0][g], qg[1][g], parked[g], g) for g in range(2, NGV_A[p] + 1)}

        y_a = segment(lhs, cat(lhs, x1s), 32, NGV_A,
                      sum(g + 1 for n in NGV_A for g in range(2, n + 1)) * 8 // CHUNK, unpack_a,
                      lambda o: cat(o[0], o[2], o[3], o[4]), False, EARLY_A, D_JA, zero)

        lhs = cat(y_a[0:8], xf[40:64]).astype(BF16)

        def unpack_b(p, qkv):
            parked_a1, kv1 = keep[p]
            qg = [{0: q[0:8], 1: q[40:48], 2: q[8:16], 3: q[16:24], 4: q[24:32]}
                  for q, _, _ in qkv]
            ks = [cat(k[0:8], e[0], k[8:32]) for (_, k, _), e in zip(qkv, kv1)]
            vs = [cat(v[0:8], e[1], v[8:32]) for (_, _, v), e in zip(qkv, kv1)]
            u, parked = finish(qg, ks, vs, NJOB * p + max(NGV_A), range(1, NGV_B[p] + 1))
            jobs = {'a1': (qkv[0][0][32:40], qkv[1][0][32:40], parked_a1, 1)}
            jobs.update({g: (qg[0][g], qg[1][g], parked[g], g) for g in range(1, NGV_B[p] + 1)})
            return u, jobs

        y_b = segment(cat(lhs, x1s), lhs, 48, NGV_B,
                      sum(2 + sum(range(2, n + 2)) for n in NGV_B) * 8 // CHUNK, unpack_b,
                      lambda o: cat(o[0], o[1], o[2], o[3], o[4], o['a1']), True, EARLY_B,
                      D_JB, zero)

        a = cat(y_b[40:48], y_a[8:32], y_b[8:40])
        g = g_v[pl.ds(r0, PAIR), :]
        g = jnp.concatenate([g] * (D // 128), axis=1)
        out_v[pl.ds(r0, PAIR), :] = (g * a + h1_rows(r0, PAIR)).astype(BF16)
        return y_b[0:8]

    rows_it = UNROLL_A * PAIR

    def a_body(t, carry):
        base = pl.multiple_of(t * rows_it, rows_it)
        mem = mem_v[...]
        for u in range(UNROLL_A):
            mem = pair(pl.multiple_of(base + u * PAIR, PAIR), mem)
        mem_v[...] = mem
        pltpu.make_async_copy(out_v.at[pl.ds(base, rows_it)], out_hbm.at[pl.ds(base, rows_it)],
                              osem).start()
        return carry

    with jax.named_scope('a_body'):
        jax.lax.fori_loop(0, S // rows_it, a_body, 0)
    pltpu.make_async_copy(out_v, out_hbm, osem).wait()


@jax.jit
def pallas_gated_mix__memory_aug_recurrent_mem_tr__mixer_s_mlp__prompt_kernel(
    A_x, A_mem0, A_Wq, A_Wk, A_Wv, A_Wo, A_seg_len, B_x, B_w1, B_w2, B_w3, B_w4, gate_w,
):
    assert A_x.shape == (1, S, D) and A_Wq.shape == (D, H, DH) and A_mem0.shape == (1, M, D)
    x = A_x.reshape(S, D)
    mem0 = A_mem0.reshape(M, D)
    wq = A_Wq.reshape(D * H, DH)
    wk = A_Wk.reshape(D * H, DH)
    wv = A_Wv.reshape(D * H, DH)
    wo = A_Wo.reshape(H * DH, D)

    any_spec = pl.BlockSpec(memory_space=pl.ANY)
    out = pl.pallas_call(
        _kernel,
        out_shape=jax.ShapeDtypeStruct((S, D), BF16),
        in_specs=[any_spec] * 11,
        out_specs=any_spec,
        scratch_shapes=[
            pltpu.VMEM((S, D), BF16),
            pltpu.VMEM((NRING, 3, DP * H, DH), BF16),
            pltpu.VMEM((NRING, OP, D), BF16),
            pltpu.VMEM((3 * H * PITCH, 128), U32),
            pltpu.VMEM((D // 128, H * DH // 2, 128), U32),
            pltpu.VMEM((4, D, D // 4), BF16),
            pltpu.VMEM((4, D, D // 4), BF16),
            pltpu.VMEM((D, FF), BF16),
            pltpu.VMEM((FF, D), BF16),
            pltpu.VMEM((D // 128, S + 16, 128), F32),
            pltpu.VMEM((S + T2, D), F32),
            pltpu.VMEM((S, 128), F32),
            pltpu.VMEM((2, T1, D), BF16),
            pltpu.VMEM((2, T3, D), BF16),
            pltpu.VMEM((M, D), BF16),
            pltpu.VMEM((D,), BF16),
            pltpu.VMEM((M, D), F32),
            pltpu.VMEM((S, D), BF16),
            pltpu.VMEM((NJOB * H * 2 * (L + 8), 128), F32),
            pltpu.VMEM((16, 128), U32),
            pltpu.SemaphoreType.DMA((NSEM,)),
            pltpu.SemaphoreType.DMA(()),
        ],
        compiler_params=pltpu.CompilerParams(vmem_limit_bytes=120 * 1024 * 1024,
                                             disable_bounds_checks=True),
    )(x, mem0, wq, wk, wv, wo, B_w1, B_w2, B_w3, B_w4, gate_w)
    return out.reshape(1, S, D)
```

```python
import math

import jax
import jax.numpy as jnp
import jax.experimental.pallas as pl
import jax.experimental.pallas.tpu as pltpu

F32 = jnp.float32
BF16 = jnp.bfloat16
U32 = jnp.uint32

S = 2048
D = 1024
H = 32
DH = 128
M = 8
SEG = 32
L = M + SEG
FF = 3584
PAIR = 2 * SEG
NPAIR = S // PAIR
T1 = 256
N1 = S // T1
T2 = 512
N2 = S // T2
T3 = 256
N3 = S // T3
DP = D // N3
OP = H * DH // N3
UNROLL_A = 1
PITCH = 520
NRING = 3
NSEM = 11 + NRING
EPS = 1e-5
NCHAIN0 = 10
NCHAIN1 = 5
LN1_ROWS = 8
HOP = 4
KEYS_A = 3.0
KEYS_B = 2.0
NGV_A = [int((p + 1) * KEYS_A + 1e-6) - int(p * KEYS_A + 1e-6) for p in range(H // 2)]
NGV_B = [int((p + 1) * KEYS_B + 1e-6) - int(p * KEYS_B + 1e-6) for p in range(H // 2)]
NJOB = max(NGV_A) + max(NGV_B)
EARLY_A = 2
EARLY_B = 3
WO_SLOTS = 10
CHUNK = 8
D_G = 0
D_JA = 530
D_JB = 600
D_F = 100
D_R = 0
D_S = 500
D_PV = 1400
D_SM = 600
D_O = 170
TAIL_H = 8
NEG = -1e9


def _gelu(x):
    c = math.sqrt(2.0 / math.pi)
    return 0.5 * x * (1.0 + jnp.tanh(c * (x + 0.044715 * (x * x * x))))


def _layernorm(x):
    m = jnp.mean(x, axis=-1, keepdims=True)
    xc = x - m
    v = jnp.mean(xc * xc, axis=-1, keepdims=True)
    return xc * jax.lax.rsqrt(v + EPS)


def _slab_of(which, h):
    return which * H + (h % 2) * (H // 2) + h // 2


def _kernel(x_hbm, mem0_hbm, wq_hbm, wk_hbm, wv_hbm, wo_hbm,
            w1_hbm, w2_hbm, w3_hbm, w4_hbm, gw_hbm,
            out_hbm,
            x_v, stq_v, sto_v, wqkv_v, wo_v, w1_v, w2_v, w3_v, w4_v,
            h1_v, x1_v, g_v, ln1_v, ln3_v, mem0_v, gw_v, mem_v, out_v, kv_v, zero_v, sems, osem):
    c4 = D // 4
    xcuts = (0, 1, 2, 3, 5, N1)
    cp_x = [pltpu.make_async_copy(x_hbm.at[pl.ds(lo * T1, (hi - lo) * T1)],
                                  x_v.at[pl.ds(lo * T1, (hi - lo) * T1)], sems.at[n])
            for n, (lo, hi) in enumerate(zip(xcuts[:-1], xcuts[1:]))]
    cp_w1 = [pltpu.make_async_copy(w1_hbm.at[:, pl.ds(q * c4, c4)], w1_v.at[q], sems.at[5 + q])
             for q in range(4)]
    cp_w2 = [pltpu.make_async_copy(w2_hbm.at[:, pl.ds(q * c4, c4)], w2_v.at[q], sems.at[9])
             for q in range(4)]
    cp_ffn = [pltpu.make_async_copy(src, dst, sems.at[10])
              for src, dst in ((gw_hbm, gw_v), (mem0_hbm, mem0_v), (w3_hbm, w3_v), (w4_hbm, w4_v))]

    def piece_copies(i, slot):
        cps = [pltpu.make_async_copy(w.at[pl.ds(i * (DP * H), DP * H)], stq_v.at[slot, k],
                                     sems.at[11 + slot])
               for k, w in enumerate((wq_hbm, wk_hbm, wv_hbm))]
        cps.append(pltpu.make_async_copy(wo_hbm.at[pl.ds(i * OP, OP)], sto_v.at[slot],
                                         sems.at[11 + slot]))
        return cps

    for c in (cp_x[0:1] + cp_w1 + cp_x[1:] + cp_w2 + cp_ffn
              + piece_copies(0, 0) + piece_copies(1, 1)):
        c.start()
    x1_v[pl.ds(0, T3), :] = jnp.zeros((T3, D), F32)
    h1_v[:, pl.ds(8, 8), :] = jnp.zeros((D // 128, 8, 128), F32)
    h1_v[:, pl.ds(S, 8), :] = jnp.zeros((D // 128, 8, 128), F32)
    zero_v[...] = jnp.zeros((16, 128), U32)

    def ln_rows(x, tok, zero):
        if tok is not None:
            head = pltpu.bitcast(pltpu.bitcast(x[:, 0:128], U32) | tok, F32)
            x = jnp.concatenate([head, x[:, 128:]], axis=1)
        y = _layernorm(x)
        tok = None if zero is None else pltpu.bitcast(y[:, 0:128], U32) & zero
        return y, tok

    def ln_block(load, store, rows, nchain, gr):
        zero = zero_v[pl.ds(0, gr), :] if nchain else None
        toks = [None] * max(nchain, 1)
        for k in range(rows // gr):
            y, toks[k % len(toks)] = ln_rows(load(k * gr, gr), toks[k % len(toks)], zero)
            store(k * gr, y.astype(BF16))
        return toks[(rows // gr - 1) % len(toks)]

    def prep1(blk, slot, nchain):
        r0 = blk * T1 if isinstance(blk, int) else pl.multiple_of(blk * T1, T1)

        def store(k, y):
            ln1_v[slot, pl.ds(k, y.shape[0]), :] = y

        ln_block(lambda k, n: x_v[pl.ds(r0 + k, n), :].astype(F32), store, T1, nchain, LN1_ROWS)

    def p1_quarter(lhs, r0, q):
        h = _gelu(jnp.dot(lhs, w1_v[q], preferred_element_type=F32))
        for j in range(2):
            win = h1_v.at[2 * q + j, pl.ds(r0, T1 + 16)]
            win[pl.ds(8 + (1, -1, 2, -2)[q], T1), :] = h[:, j * 128:(j + 1) * 128]

    cp_x[0].wait()
    prep1(0, 0, 0)
    for q in range(4):
        cp_w1[q].wait()
        if q == 3:
            cp_x[1].wait()
        lhs = ln1_v[0]
        if q == 3:
            prep1(1, 1, NCHAIN0)
        p1_quarter(lhs, 0, q)

    def p1_body(i, carry):
        r0 = pl.multiple_of(i * T1, T1)
        slot = i & 1

        lhs = ln1_v[slot]
        prep1(jnp.minimum(i + 1, N1 - 1), 1 - slot, NCHAIN1)
        for q in range(4):
            p1_quarter(lhs, r0, q)
        for n in range(3, len(cp_x)):
            pl.when(i + 2 == xcuts[n])(cp_x[n].wait)
        return carry

    cp_x[2].wait()
    with jax.named_scope('p1_body'):
        jax.lax.fori_loop(1, N1, p1_body, 0)
    for c in cp_w2:
        c.wait()

    def h1_rows(r0, n):
        return jnp.concatenate([h1_v[j, pl.ds(r0, n), :] for j in range(D // 128)], axis=1)

    def prep3(src, slot):
        def store(k, y):
            ln3_v[slot, pl.ds(k, y.shape[0]), :] = y

        return ln_block(lambda k, n: src[pl.ds(k, n), :], store, T3, 1, 16)

    def p2_body(i, carry):
        r0 = pl.multiple_of(i * T2, T2)
        win = x1_v.at[pl.ds(r0, 2 * T2)]
        prep3(win, 0)
        hs = h1_rows(r0 + 8, T2).astype(BF16)
        for q in range(4):
            win[pl.ds(T2, T2), pl.ds(q * c4, c4)] = (
                jnp.dot(hs, w2_v[q], preferred_element_type=F32)
                + x_v[pl.ds(r0, T2), pl.ds(q * c4, c4)].astype(F32))
        return carry

    with jax.named_scope('p2_body'):
        jax.lax.fori_loop(0, N2, p2_body, 0)

    for c in cp_ffn + piece_copies(0, 0):
        c.wait()
    blk0 = (N2 - 2) * T2 // T3

    def p3_body(i, carry):
        r0 = pl.multiple_of((i + blk0) % N3 * T3, T3)
        r_next = pl.multiple_of((i + 1 + blk0) % N3 * T3, T3)
        slot = i & 1
        ring = i % NRING

        @pl.when(i + 2 < N3)
        def _():
            for c in piece_copies(i + 2, (i + 2) % NRING):
                c.start()

        lhs = ln3_v[slot]
        tok = prep3(x1_v.at[pl.ds(T2 + r_next, T3)], 1 - slot)
        zero = zero_v[...]
        for which in range(3):
            for j in range(DP // 2):
                blk = pltpu.bitcast(stq_v[ring, which, pl.ds(j * 64, 64), :], U32)
                a = blk[0:16] | tok
                c = blk[16:32]
                lo = (a & jnp.uint32(0xFFFF)) | (c << 16)
                a = a | (lo & zero)
                hi = (a >> 16) | (c & jnp.uint32(0xFFFF0000))
                tok = hi & zero
                if j % HOP == HOP - 1:
                    tok = pltpu.roll(tok, 1, 1)
                s0 = which * H * PITCH + i * (DP // 2) + j
                wqkv_v[pl.ds(s0, 16, stride=PITCH), :] = lo
                wqkv_v[pl.ds(s0 + 16 * PITCH, 16, stride=PITCH), :] = hi
        o0 = pl.multiple_of(i * (OP // 2), OP // 2)
        for j in range(D // 128):
            for k in range(OP // 32):
                w = pltpu.bitcast(sto_v[ring, pl.ds(k * 32, 32), pl.ds(j * 128, 128)], U32) | tok
                tok = w & zero
                if k % (2 * HOP) == 2 * HOP - 1:
                    tok = pltpu.roll(tok, 1, 1)
                wo_v[j, pl.ds(o0 + k * 16, 16), :] = w

        h = _gelu(jnp.dot(lhs, w3_v[...], preferred_element_type=F32)).astype(BF16)
        b = jnp.dot(h, w4_v[...], preferred_element_type=F32) + x1_v[pl.ds(T2 + r0, T3), :]
        gw = gw_v[...].astype(F32).reshape(1, D)
        z = jnp.sum(x_v[pl.ds(r0, T3), :].astype(F32) * gw, axis=-1, keepdims=True)
        g = 1.0 / (1.0 + jnp.exp(-z))
        g_v[pl.ds(r0, T3), :] = jnp.broadcast_to(g, (T3, 128))
        b = (1.0 - g) * b
        for j in range(D // 128):
            h1_v[j, pl.ds(r0, T3), :] = b[:, j * 128:(j + 1) * 128]

        @pl.when(i + 1 < N3)
        def _():
            for c in piece_copies(i + 1, (i + 1) % NRING):
                c.wait()

        return carry

    with jax.named_scope('p3_body'):
        jax.lax.fori_loop(0, N3, p3_body, 0)

    mem_v[...] = mem0_v[...].astype(F32)
    c_exp = (DH ** -0.5) * math.log2(math.e)
    neg_raw = NEG / (DH ** -0.5)

    L2 = 2 * L

    def make_mask(ngv):
        rm = L - 8 * ngv
        row = jax.lax.broadcasted_iota(jnp.int32, (2 * rm, 128), 0)
        col = jax.lax.broadcasted_iota(jnp.int32, (2 * rm, 128), 1)
        second = row >= rm
        rowl = jnp.where(second, row - rm, row)
        coll = jnp.where(second, col - L, col)
        real = (coll >= 0) & (coll < L)
        allowed = real & ((rowl < M) | (rowl + 8 * ngv >= coll))
        return allowed, jnp.where(real, neg_raw, -jnp.inf).astype(F32)

    masks = {n: make_mask(n) for n in set(NGV_A + NGV_B)}
    sub = jax.lax.broadcasted_iota(jnp.int32, (8, 1), 0)
    neg_c = NEG * math.log2(math.e)

    def tied(w, toks):
        for tok in toks:
            w = jnp.concatenate([w[0:56], w[56:64] | tok, w[64:]], axis=0)
        return pltpu.bitcast(w, BF16)

    zpad = jnp.zeros((128 - L2, DH), F32)

    def recip(l):
        r = pl.reciprocal(l, approx=True)
        return r * (2.0 - l * r)

    def tree(op, xs):
        xs = list(xs)
        while len(xs) > 1:
            xs = [op(xs[i], xs[i + 1]) if i + 1 < len(xs) else xs[i]
                  for i in range(0, len(xs), 2)]
        return xs[0]

    low = jax.lax.broadcasted_iota(jnp.int32, (8, 128), 1) < 64

    def cross(x0, x1):
        lo = jnp.concatenate([low] * (x0.shape[0] // 8), axis=0)
        return jnp.where(lo, x0, x1), pltpu.roll(jnp.where(lo, x1, x0), 64, 1)

    def stash(slot, ks, ws, g):
        n = 8 * (g + 2)
        starts = []
        for i, x in enumerate(ks + ws):
            base = (4 * slot + i) * (L + 8)
            kv_v[pl.ds(base, n), :] = jnp.concatenate([x[8 * g:8 * g + 8], x[0:n - 8]], axis=0)
            starts.append(base + n - 8)
        return starts, [jnp.sum(w[n - 8:L], axis=0, keepdims=True) if n - 8 < L
                        else jnp.zeros((1, DH), F32) for w in ws]

    def vpu_start(q0, q1, parked, g):
        starts, (acc_a, acc_b) = parked
        return dict(q=(q0 * c_exp, q1 * c_exp), starts=starts, g=g,
                    m=jnp.full((8, 128), neg_c, F32),
                    l=jnp.full((8, 128), float(L - 8 * (g + 1)), F32), a=acc_a, b=acc_b)

    def vpu_chunk(st, c0, gate):
        k0, k1, wa, wb = st['starts']
        g = st['g']
        q0, q1 = [pltpu.bitcast(pltpu.bitcast(q, U32) | gate, F32) for q in st['q']]
        sc = []
        for r in range(c0, min(c0 + CHUNK, 8 * (g + 1))):
            sr = jnp.where(
                low, jnp.sum(q0 * kv_v[pl.ds(k0 - r, 8), :], axis=-1, keepdims=True),
                jnp.sum(q1 * kv_v[pl.ds(k1 - r, 8), :], axis=-1, keepdims=True))
            if r > 8 * g:
                sr = jnp.where(sub >= r - 8 * g, sr, neg_c)
            sc.append(sr)
        m = jnp.maximum(tree(jnp.maximum, sc), st['m'])
        alpha = jnp.exp2(st['m'] - m)
        l, acc_a, acc_b = st['l'] * alpha, st['a'] * alpha, st['b'] * alpha
        for n, sr in enumerate(sc):
            pr = jnp.exp2(sr - m)
            l = l + pr
            acc_a = acc_a + pr * kv_v[pl.ds(wa - c0 - n, 8), :]
            acc_b = acc_b + pr * kv_v[pl.ds(wb - c0 - n, 8), :]
        st.update(m=m, l=l, a=acc_a, b=acc_b)
        return pltpu.bitcast(l, U32) | pltpu.bitcast(acc_a, U32) | pltpu.bitcast(acc_b, U32)

    def vpu_finish(st):
        r = recip(st['l'])
        oa = st['a'] * r
        ob = pltpu.roll(st['b'] * r, 64, 1)
        return jnp.where(low, oa, ob), jnp.where(low, ob, oa)

    def segment(lhs_q, lhs_kv, wo_m, ngv, n_chunks, unpack, wo_rows, split_first, early, d_j, zero):
        NP = H // 2
        nj = D // 128
        HA = H - TAIL_H
        mxu_groups = [[0] + list(range(n + 1, 5)) for n in ngv]
        proj = {}
        qkv = [None] * NP
        pb = [None] * NP
        og = [dict() for _ in range(H)]
        ocat = {}
        y = [None] * nj

        def slab(toks, which, h, r0, n):
            x = lhs_q if which == 0 else lhs_kv
            w = tied(wqkv_v[pl.ds(_slab_of(which, h) * PITCH + r0, n), :], toks)
            r = jnp.dot(x[:, 2 * r0:2 * (r0 + n)], w, preferred_element_type=F32)
            proj[(which, h)] = r + proj[(which, h)] if (which, h) in proj else r
            return proj[(which, h)]

        def do_wo(toks, h0, h1, j):
            if (h0, h1) not in ocat:
                ocat[(h0, h1)] = jnp.concatenate(
                    [wo_rows(og[h]) for h in range(h0, h1)], axis=1).astype(BF16)
            w = tied(wo_v[j, pl.ds(h0 * 64, (h1 - h0) * 64), :], toks)
            r = jnp.dot(ocat[(h0, h1)], w, preferred_element_type=F32)
            y[j] = r if y[j] is None else r + y[j]
            return y[j]

        ticks = []
        pair_end = {}
        wo_early = [(4 * c, 4 * c + 4, j) for c in range(early) for j in range(nj)]
        first = NP - WO_SLOTS
        for p in range(NP):
            slabs = [(which, h) for h in (2 * p, 2 * p + 1) for which in range(3)]
            rows = [(lhs_q if w == 0 else lhs_kv).shape[0] for w, _ in slabs]
            if p == 0 and split_first:
                for r0 in (0, 256):
                    ticks += [(slab, (w, h, r0, 256), m) for (w, h), m in zip(slabs, rows)]
            else:
                mine = []
                if p >= first:
                    lo = (p - first) * len(wo_early) // WO_SLOTS
                    mine = wo_early[lo:(p - first + 1) * len(wo_early) // WO_SLOTS]
                for n, ((w, h), m) in enumerate(zip(slabs, rows)):
                    ticks += [(do_wo, item, wo_m)
                              for item in mine[n * len(mine) // 6:(n + 1) * len(mine) // 6]]
                    ticks.append((slab, (w, h, 0, 512), 2 * m + 8 * len(mxu_groups[p]) // 6))
            pair_end[len(ticks) - 1] = p
        ticks += [(do_wo, (h0, h0 + 4, j), wo_m)
                  for j in range(nj) for h0 in range(4 * early, HA, 4)]
        ends = []
        for _, _, dur in ticks:
            ends.append(dur + (ends[-1] if ends else 0))

        def index(t):
            return next(i for i, e in enumerate(ends) if e >= t)

        events = {}
        anchors = {}
        cursor = [0]

        def run_chunk(res, p, name, st, c0, i_done):
            done = vpu_chunk(st, c0, pltpu.bitcast(res[0:8], U32) & zero)
            anchors.setdefault(i_done, []).append(done & zero)
            if c0 + CHUNK >= 8 * (st['g'] + 1):
                og[2 * p][name], og[2 * p + 1][name] = vpu_finish(st)
                if D_R and ends[i_done - 1] + D_R < ends[-2]:
                    anchors.setdefault(index(ends[i_done - 1] + D_R) + 1, []).append(
                        pltpu.bitcast(og[2 * p][name], U32) & zero)

        def do_s(res, p):
            sc = jax.lax.dot_general(qkv[p][0], qkv[p][1], (((1,), (1,)), ((), ())),
                                     preferred_element_type=F32)
            allowed, fill = masks[ngv[p]]
            sc = jnp.where(allowed, sc, fill)
            e = jnp.exp2((sc - jnp.max(sc, axis=-1, keepdims=True)) * c_exp)
            l = jnp.sum(e, axis=-1, keepdims=True)
            pb[p] = (e * recip(l)).astype(BF16)

        def do_pv(res, p):
            o = jnp.dot(pb[p], qkv[p][2], preferred_element_type=F32)
            rm = 8 * len(mxu_groups[p])
            for i in range(2):
                for n, g in enumerate(mxu_groups[p]):
                    og[2 * p + i][g] = o[i * rm + 8 * n:i * rm + 8 * n + 8]

        def finish_pair(p, i):
            u, jobs = unpack(p, [[proj[(w, h)] for w in range(3)] for h in (2 * p, 2 * p + 1)])
            chunks = [(name, st, c0) for name, st in
                      [(name, vpu_start(*job)) for name, job in jobs.items()]
                      for c0 in range(0, 8 * (st['g'] + 1), CHUNK)]
            t_first = ends[min(pair_end)] + D_G
            t_last = ends[-2] - d_j - D_F
            gap = (t_last - t_first) / (n_chunks - 1)
            if p == NP - 1:
                gap = min(gap, (t_last - max(ends[i] + D_G, cursor[0])) / (len(chunks) - 1))
            for chunk in chunks:
                t = max(ends[i] + D_G, cursor[0])
                cursor[0] = t + gap
                g = max(index(t), i + 1)
                events.setdefault(g, []).append(
                    (run_chunk, (p,) + chunk + (index(ends[g] + d_j) + 1,)))
            qb = jnp.concatenate([u[k][0][g] for k in range(2) for g in mxu_groups[p]],
                                 axis=0).astype(BF16)
            kb = jnp.concatenate([u[0][1], u[1][1], zpad], axis=0).astype(BF16)
            vb = jnp.concatenate([u[0][2], u[1][2], zpad], axis=0).astype(BF16)
            qkv[p] = (qb, kb, vb)
            t_pv = min(ends[i] + D_PV, ends[-1] - D_O)
            events.setdefault(index(min(ends[i] + D_S, t_pv - D_SM)), []).append((do_s, (p,)))
            events.setdefault(index(t_pv), []).append((do_pv, (p,)))

        for i, (fn, args, _) in enumerate(ticks):
            res = fn(anchors.pop(i, []), *args)
            if i in pair_end:
                finish_pair(pair_end[i], i)
            for f, a in events.pop(i, []):
                f(res, *a)
        assert not events
        for j in range(nj):
            do_wo([], HA, H, j)
        return jnp.concatenate(y, axis=1)

    def pair(r0, mem):
        xf = x_v[pl.ds(r0, PAIR), :].astype(F32)
        zero = zero_v[pl.ds(0, 8), :]
        x1s = jnp.concatenate([xf[0:8], xf[32:40]], axis=0).astype(BF16)
        keep = [None] * H

        def cat(*xs):
            return jnp.concatenate(xs, axis=0)

        lhs = cat(mem, xf[8:32]).astype(BF16)

        def finish(qg, ks, vs, slot, groups):
            ws = list(cross(vs[0], vs[1]))
            return ([(qg[i], ks[i], vs[i]) for i in range(2)],
                    {g: stash(slot + n, ks, ws, g) for n, g in enumerate(groups)})

        def unpack_a(p, qkv):
            qg = [{0: q[0:8], 2: q[8:16], 3: q[16:24], 4: q[24:32]} for q, _, _ in qkv]
            ks = [cat(k[0:8], k[32:40], k[8:32]) for _, k, _ in qkv]
            vs = [cat(v[0:8], v[32:40], v[8:32]) for _, _, v in qkv]
            u, parked = finish(qg, ks, vs, NJOB * p, range(1, NGV_A[p] + 1))
            keep[p] = (parked[1], [(k[40:48], v[40:48]) for _, k, v in qkv])
            return u, {g: (qg[0][g], qg[1][g], parked[g], g) for g in range(2, NGV_A[p] + 1)}

        y_a = segment(lhs, cat(lhs, x1s), 32, NGV_A,
                      sum(g + 1 for n in NGV_A for g in range(2, n + 1)) * 8 // CHUNK, unpack_a,
                      lambda o: cat(o[0], o[2], o[3], o[4]), False, EARLY_A, D_JA, zero)

        lhs = cat(y_a[0:8], xf[40:64]).astype(BF16)

        def unpack_b(p, qkv):
            parked_a1, kv1 = keep[p]
            qg = [{0: q[0:8], 1: q[40:48], 2: q[8:16], 3: q[16:24], 4: q[24:32]}
                  for q, _, _ in qkv]
            ks = [cat(k[0:8], e[0], k[8:32]) for (_, k, _), e in zip(qkv, kv1)]
            vs = [cat(v[0:8], e[1], v[8:32]) for (_, _, v), e in zip(qkv, kv1)]
            u, parked = finish(qg, ks, vs, NJOB * p + max(NGV_A), range(1, NGV_B[p] + 1))
            jobs = {'a1': (qkv[0][0][32:40], qkv[1][0][32:40], parked_a1, 1)}
            jobs.update({g: (qg[0][g], qg[1][g], parked[g], g) for g in range(1, NGV_B[p] + 1)})
            return u, jobs

        y_b = segment(cat(lhs, x1s), lhs, 48, NGV_B,
                      sum(2 + sum(range(2, n + 2)) for n in NGV_B) * 8 // CHUNK, unpack_b,
                      lambda o: cat(o[0], o[1], o[2], o[3], o[4], o['a1']), True, EARLY_B,
                      D_JB, zero)

        a = cat(y_b[40:48], y_a[8:32], y_b[8:40])
        g = g_v[pl.ds(r0, PAIR), :]
        g = jnp.concatenate([g] * (D // 128), axis=1)
        out_v[pl.ds(r0, PAIR), :] = (g * a + h1_rows(r0, PAIR)).astype(BF16)
        return y_b[0:8]

    rows_it = UNROLL_A * PAIR

    def a_body(t, carry):
        base = pl.multiple_of(t * rows_it, rows_it)
        mem = mem_v[...]
        for u in range(UNROLL_A):
            mem = pair(pl.multiple_of(base + u * PAIR, PAIR), mem)
        mem_v[...] = mem
        pltpu.make_async_copy(out_v.at[pl.ds(base, rows_it)], out_hbm.at[pl.ds(base, rows_it)],
                              osem).start()
        return carry

    with jax.named_scope('a_body'):
        jax.lax.fori_loop(0, S // rows_it, a_body, 0)
    pltpu.make_async_copy(out_v, out_hbm, osem).wait()


@jax.jit
def pallas_gated_mix__memory_aug_recurrent_mem_tr__mixer_s_mlp__prompt_kernel(
    A_x, A_mem0, A_Wq, A_Wk, A_Wv, A_Wo, A_seg_len, B_x, B_w1, B_w2, B_w3, B_w4, gate_w,
):
    assert A_x.shape == (1, S, D) and A_Wq.shape == (D, H, DH) and A_mem0.shape == (1, M, D)
    x = A_x.reshape(S, D)
    mem0 = A_mem0.reshape(M, D)
    wq = A_Wq.reshape(D * H, DH)
    wk = A_Wk.reshape(D * H, DH)
    wv = A_Wv.reshape(D * H, DH)
    wo = A_Wo.reshape(H * DH, D)

    any_spec = pl.BlockSpec(memory_space=pl.ANY)
    out = pl.pallas_call(
        _kernel,
        out_shape=jax.ShapeDtypeStruct((S, D), BF16),
        in_specs=[any_spec] * 11,
        out_specs=any_spec,
        scratch_shapes=[
            pltpu.VMEM((S, D), BF16),
            pltpu.VMEM((NRING, 3, DP * H, DH), BF16),
            pltpu.VMEM((NRING, OP, D), BF16),
            pltpu.VMEM((3 * H * PITCH, 128), U32),
            pltpu.VMEM((D // 128, H * DH // 2, 128), U32),
            pltpu.VMEM((4, D, D // 4), BF16),
            pltpu.VMEM((4, D, D // 4), BF16),
            pltpu.VMEM((D, FF), BF16),
            pltpu.VMEM((FF, D), BF16),
            pltpu.VMEM((D // 128, S + 16, 128), F32),
            pltpu.VMEM((S + T2, D), F32),
            pltpu.VMEM((S, 128), F32),
            pltpu.VMEM((2, T1, D), BF16),
            pltpu.VMEM((2, T3, D), BF16),
            pltpu.VMEM((M, D), BF16),
            pltpu.VMEM((D,), BF16),
            pltpu.VMEM((M, D), F32),
            pltpu.VMEM((S, D), BF16),
            pltpu.VMEM((NJOB * H * 2 * (L + 8), 128), F32),
            pltpu.VMEM((16, 128), U32),
            pltpu.SemaphoreType.DMA((NSEM,)),
            pltpu.SemaphoreType.DMA(()),
        ],
        compiler_params=pltpu.CompilerParams(vmem_limit_bytes=120 * 1024 * 1024,
                                             disable_bounds_checks=True),
    )(x, mem0, wq, wk, wv, wo, B_w1, B_w2, B_w3, B_w4, gate_w)
    return out.reshape(1, S, D)
```

```python
import math

import jax
import jax.numpy as jnp
import jax.experimental.pallas as pl
import jax.experimental.pallas.tpu as pltpu

F32 = jnp.float32
BF16 = jnp.bfloat16
U32 = jnp.uint32

S = 2048
D = 1024
H = 32
DH = 128
M = 8
SEG = 32
L = M + SEG
FF = 3584
PAIR = 2 * SEG
NPAIR = S // PAIR
T1 = 256
N1 = S // T1
T2 = 512
N2 = S // T2
T3 = 256
N3 = S // T3
DP = D // N3
OP = H * DH // N3
UNROLL_A = 1
PITCH = 520
NRING = 3
NSEM = 11 + NRING
EPS = 1e-5
NCHAIN0 = 10
NCHAIN1 = 5
LN1_ROWS = 8
HOP = 4
FRAC_B = 0.875
NGV_A = [3] * (H // 2)
NGV_B = [1 + 2 * (int((p + 1) * FRAC_B + 1e-6) - int(p * FRAC_B + 1e-6)) for p in range(H // 2)]
NJOB = max(NGV_A) + max(NGV_B)
EARLY_A = 2
EARLY_B = 3
WO_SLOTS = 10
CHUNK = 8
D_G = 0
D_JA = 530
D_JB = 600
D_F = 100
D_R = 0
D_S = 500
D_PV = 1400
D_SM = 600
D_O = 170
TAIL_H = 8
NEG = -1e9


def _gelu(x):
    c = math.sqrt(2.0 / math.pi)
    return 0.5 * x * (1.0 + jnp.tanh(c * (x + 0.044715 * (x * x * x))))


def _layernorm(x):
    m = jnp.mean(x, axis=-1, keepdims=True)
    xc = x - m
    v = jnp.mean(xc * xc, axis=-1, keepdims=True)
    return xc * jax.lax.rsqrt(v + EPS)


def _slab_of(which, h):
    return which * H + (h % 2) * (H // 2) + h // 2


def _kernel(x_hbm, mem0_hbm, wq_hbm, wk_hbm, wv_hbm, wo_hbm,
            w1_hbm, w2_hbm, w3_hbm, w4_hbm, gw_hbm,
            out_hbm,
            x_v, stq_v, sto_v, wqkv_v, wo_v, w1_v, w2_v, w3_v, w4_v,
            h1_v, x1_v, g_v, ln1_v, ln3_v, mem0_v, gw_v, mem_v, out_v, kv_v, zero_v, sems, osem):
    c4 = D // 4
    xcuts = (0, 1, 2, 3, 5, N1)
    cp_x = [pltpu.make_async_copy(x_hbm.at[pl.ds(lo * T1, (hi - lo) * T1)],
                                  x_v.at[pl.ds(lo * T1, (hi - lo) * T1)], sems.at[n])
            for n, (lo, hi) in enumerate(zip(xcuts[:-1], xcuts[1:]))]
    cp_w1 = [pltpu.make_async_copy(w1_hbm.at[:, pl.ds(q * c4, c4)], w1_v.at[q], sems.at[5 + q])
             for q in range(4)]
    cp_w2 = [pltpu.make_async_copy(w2_hbm.at[:, pl.ds(q * c4, c4)], w2_v.at[q], sems.at[9])
             for q in range(4)]
    cp_ffn = [pltpu.make_async_copy(src, dst, sems.at[10])
              for src, dst in ((gw_hbm, gw_v), (mem0_hbm, mem0_v), (w3_hbm, w3_v), (w4_hbm, w4_v))]

    def piece_copies(i, slot):
        cps = [pltpu.make_async_copy(w.at[pl.ds(i * (DP * H), DP * H)], stq_v.at[slot, k],
                                     sems.at[11 + slot])
               for k, w in enumerate((wq_hbm, wk_hbm, wv_hbm))]
        cps.append(pltpu.make_async_copy(wo_hbm.at[pl.ds(i * OP, OP)], sto_v.at[slot],
                                         sems.at[11 + slot]))
        return cps

    for c in (cp_x[0:1] + cp_w1 + cp_x[1:] + cp_w2 + cp_ffn
              + piece_copies(0, 0) + piece_copies(1, 1)):
        c.start()
    x1_v[pl.ds(0, T3), :] = jnp.zeros((T3, D), F32)
    h1_v[:, pl.ds(8, 8), :] = jnp.zeros((D // 128, 8, 128), F32)
    h1_v[:, pl.ds(S, 8), :] = jnp.zeros((D // 128, 8, 128), F32)
    zero_v[...] = jnp.zeros((16, 128), U32)

    def ln_rows(x, tok, zero):
        if tok is not None:
            head = pltpu.bitcast(pltpu.bitcast(x[:, 0:128], U32) | tok, F32)
            x = jnp.concatenate([head, x[:, 128:]], axis=1)
        y = _layernorm(x)
        tok = None if zero is None else pltpu.bitcast(y[:, 0:128], U32) & zero
        return y, tok

    def ln_block(load, store, rows, nchain, gr):
        zero = zero_v[pl.ds(0, gr), :] if nchain else None
        toks = [None] * max(nchain, 1)
        for k in range(rows // gr):
            y, toks[k % len(toks)] = ln_rows(load(k * gr, gr), toks[k % len(toks)], zero)
            store(k * gr, y.astype(BF16))
        return toks[(rows // gr - 1) % len(toks)]

    def prep1(blk, slot, nchain):
        r0 = blk * T1 if isinstance(blk, int) else pl.multiple_of(blk * T1, T1)

        def store(k, y):
            ln1_v[slot, pl.ds(k, y.shape[0]), :] = y

        ln_block(lambda k, n: x_v[pl.ds(r0 + k, n), :].astype(F32), store, T1, nchain, LN1_ROWS)

    def p1_quarter(lhs, r0, q):
        h = _gelu(jnp.dot(lhs, w1_v[q], preferred_element_type=F32))
        for j in range(2):
            win = h1_v.at[2 * q + j, pl.ds(r0, T1 + 16)]
            win[pl.ds(8 + (1, -1, 2, -2)[q], T1), :] = h[:, j * 128:(j + 1) * 128]

    cp_x[0].wait()
    prep1(0, 0, 0)
    for q in range(4):
        cp_w1[q].wait()
        if q == 3:
            cp_x[1].wait()
        lhs = ln1_v[0]
        if q == 3:
            prep1(1, 1, NCHAIN0)
        p1_quarter(lhs, 0, q)

    def p1_body(i, carry):
        r0 = pl.multiple_of(i * T1, T1)
        slot = i & 1

        lhs = ln1_v[slot]
        prep1(jnp.minimum(i + 1, N1 - 1), 1 - slot, NCHAIN1)
        for q in range(4):
            p1_quarter(lhs, r0, q)
        for n in range(3, len(cp_x)):
            pl.when(i + 2 == xcuts[n])(cp_x[n].wait)
        return carry

    cp_x[2].wait()
    with jax.named_scope('p1_body'):
        jax.lax.fori_loop(1, N1, p1_body, 0)
    for c in cp_w2:
        c.wait()

    def h1_rows(r0, n):
        return jnp.concatenate([h1_v[j, pl.ds(r0, n), :] for j in range(D // 128)], axis=1)

    def prep3(src, slot):
        def store(k, y):
            ln3_v[slot, pl.ds(k, y.shape[0]), :] = y

        return ln_block(lambda k, n: src[pl.ds(k, n), :], store, T3, 1, 16)

    def p2_body(i, carry):
        r0 = pl.multiple_of(i * T2, T2)
        win = x1_v.at[pl.ds(r0, 2 * T2)]
        prep3(win, 0)
        hs = h1_rows(r0 + 8, T2).astype(BF16)
        for q in range(4):
            win[pl.ds(T2, T2), pl.ds(q * c4, c4)] = (
                jnp.dot(hs, w2_v[q], preferred_element_type=F32)
                + x_v[pl.ds(r0, T2), pl.ds(q * c4, c4)].astype(F32))
        return carry

    with jax.named_scope('p2_body'):
        jax.lax.fori_loop(0, N2, p2_body, 0)

    for c in cp_ffn + piece_copies(0, 0):
        c.wait()
    blk0 = (N2 - 2) * T2 // T3

    def p3_body(i, carry):
        r0 = pl.multiple_of((i + blk0) % N3 * T3, T3)
        r_next = pl.multiple_of((i + 1 + blk0) % N3 * T3, T3)
        slot = i & 1
        ring = i % NRING

        @pl.when(i + 2 < N3)
        def _():
            for c in piece_copies(i + 2, (i + 2) % NRING):
                c.start()

        lhs = ln3_v[slot]
        tok = prep3(x1_v.at[pl.ds(T2 + r_next, T3)], 1 - slot)
        zero = zero_v[...]
        low16 = jax.lax.broadcasted_iota(jnp.int32, (16, 128), 1) < 64
        for which in range(3):
            for j in range(DP // 2):
                blk = pltpu.bitcast(stq_v[ring, which, pl.ds(j * 64, 64), :], U32)
                a = blk[0:16] | tok
                c = blk[16:32]
                lo = (a & jnp.uint32(0xFFFF)) | (c << 16)
                if which < 2:
                    a = a | (lo & zero)
                hi = (a >> 16) | (c & jnp.uint32(0xFFFF0000))
                if which < 2:
                    tok = hi & zero
                    if j % HOP == HOP - 1:
                        tok = pltpu.roll(tok, 1, 1)
                else:
                    t = pltpu.roll(jnp.where(low16, hi, lo), 64, 1)
                    lo, hi = jnp.where(low16, lo, t), jnp.where(low16, t, hi)
                    both = hi if j % 2 == 0 else both | hi
                    if j % 2 == 1:
                        tok = both & zero
                s0 = which * H * PITCH + i * (DP // 2) + j
                wqkv_v[pl.ds(s0, 16, stride=PITCH), :] = lo
                wqkv_v[pl.ds(s0 + 16 * PITCH, 16, stride=PITCH), :] = hi
        o0 = pl.multiple_of(i * (OP // 2), OP // 2)
        for j in range(D // 128):
            for k in range(OP // 32):
                w = pltpu.bitcast(sto_v[ring, pl.ds(k * 32, 32), pl.ds(j * 128, 128)], U32) | tok
                tok = w & zero
                if k % (2 * HOP) == 2 * HOP - 1:
                    tok = pltpu.roll(tok, 1, 1)
                kd = k - k % 8 + (0, 1, 4, 5, 2, 3, 6, 7)[k % 8]
                wo_v[j, pl.ds(o0 + kd * 16, 16), :] = w

        h = _gelu(jnp.dot(lhs, w3_v[...], preferred_element_type=F32)).astype(BF16)
        b = jnp.dot(h, w4_v[...], preferred_element_type=F32) + x1_v[pl.ds(T2 + r0, T3), :]
        gw = gw_v[...].astype(F32).reshape(1, D)
        z = jnp.sum(x_v[pl.ds(r0, T3), :].astype(F32) * gw, axis=-1, keepdims=True)
        g = 1.0 / (1.0 + jnp.exp(-z))
        g_v[pl.ds(r0, T3), :] = jnp.broadcast_to(g, (T3, 128))
        b = (1.0 - g) * b
        for j in range(D // 128):
            h1_v[j, pl.ds(r0, T3), :] = b[:, j * 128:(j + 1) * 128]

        @pl.when(i + 1 < N3)
        def _():
            for c in piece_copies(i + 1, (i + 1) % NRING):
                c.wait()

        return carry

    with jax.named_scope('p3_body'):
        jax.lax.fori_loop(0, N3, p3_body, 0)

    mem_v[...] = mem0_v[...].astype(F32)
    c_exp = (DH ** -0.5) * math.log2(math.e)
    neg_raw = NEG / (DH ** -0.5)

    L2 = 2 * L

    def make_mask(ngv):
        rm = L - 8 * ngv
        row = jax.lax.broadcasted_iota(jnp.int32, (2 * rm, 128), 0)
        col = jax.lax.broadcasted_iota(jnp.int32, (2 * rm, 128), 1)
        second = row >= rm
        rowl = jnp.where(second, row - rm, row)
        coll = jnp.where(second, col - L, col)
        real = (coll >= 0) & (coll < L)
        allowed = real & ((rowl < M) | (rowl + 8 * ngv >= coll))
        return allowed, jnp.where(real, neg_raw, -jnp.inf).astype(F32)

    masks = {n: make_mask(n) for n in set(NGV_A + NGV_B)}
    sub = jax.lax.broadcasted_iota(jnp.int32, (8, 1), 0)
    neg_c = NEG * math.log2(math.e)

    def tied(w, toks):
        for tok in toks:
            w = jnp.concatenate([w[0:56], w[56:64] | tok, w[64:]], axis=0)
        return pltpu.bitcast(w, BF16)

    zpad = jnp.zeros((128 - L2, DH), F32)

    def recip(l):
        r = pl.reciprocal(l, approx=True)
        return r * (2.0 - l * r)

    def tree(op, xs):
        xs = list(xs)
        while len(xs) > 1:
            xs = [op(xs[i], xs[i + 1]) if i + 1 < len(xs) else xs[i]
                  for i in range(0, len(xs), 2)]
        return xs[0]

    low = jax.lax.broadcasted_iota(jnp.int32, (8, 128), 1) < 64

    def stash(slot, ks, ws, g):
        n = 8 * (g + 2)
        starts = []
        for i, x in enumerate(ks + ws):
            base = (4 * slot + i) * (L + 8)
            kv_v[pl.ds(base, n), :] = jnp.concatenate([x[8 * g:8 * g + 8], x[0:n - 8]], axis=0)
            starts.append(base + n - 8)
        return starts, [jnp.sum(w[n - 8:L], axis=0, keepdims=True) if n - 8 < L
                        else jnp.zeros((1, DH), F32) for w in ws]

    def vpu_start(q0, q1, parked, g):
        starts, (acc_a, acc_b) = parked
        return dict(q=(q0 * c_exp, q1 * c_exp), starts=starts, g=g,
                    m=jnp.full((8, 128), neg_c, F32),
                    l=jnp.full((8, 128), float(L - 8 * (g + 1)), F32), a=acc_a, b=acc_b)

    def vpu_chunk(st, c0, gate):
        k0, k1, wa, wb = st['starts']
        g = st['g']
        q0, q1 = [pltpu.bitcast(pltpu.bitcast(q, U32) | gate, F32) for q in st['q']]
        sc = []
        for r in range(c0, min(c0 + CHUNK, 8 * (g + 1))):
            sr = jnp.where(
                low, jnp.sum(q0 * kv_v[pl.ds(k0 - r, 8), :], axis=-1, keepdims=True),
                jnp.sum(q1 * kv_v[pl.ds(k1 - r, 8), :], axis=-1, keepdims=True))
            if r > 8 * g:
                sr = jnp.where(sub >= r - 8 * g, sr, neg_c)
            sc.append(sr)
        m = jnp.maximum(tree(jnp.maximum, sc), st['m'])
        alpha = jnp.exp2(st['m'] - m)
        l, acc_a, acc_b = st['l'] * alpha, st['a'] * alpha, st['b'] * alpha
        for n, sr in enumerate(sc):
            pr = jnp.exp2(sr - m)
            l = l + pr
            acc_a = acc_a + pr * kv_v[pl.ds(wa - c0 - n, 8), :]
            acc_b = acc_b + pr * kv_v[pl.ds(wb - c0 - n, 8), :]
        st.update(m=m, l=l, a=acc_a, b=acc_b)
        return pltpu.bitcast(l, U32) | pltpu.bitcast(acc_a, U32) | pltpu.bitcast(acc_b, U32)

    def vpu_finish(st):
        r = recip(st['l'])
        return st['a'] * r, st['b'] * r

    def segment(lhs_q, lhs_kv, wo_m, ngv, n_chunks, unpack, wo_rows, split_first, early, d_j, zero):
        NP = H // 2
        nj = D // 128
        HA = H - TAIL_H
        mxu_groups = [[0] + list(range(n + 1, 5)) for n in ngv]
        proj = {}
        qkv = [None] * NP
        pb = [None] * NP
        og = [dict() for _ in range(H)]
        ocat = {}
        y = [None] * nj

        def slab(toks, which, h, r0, n):
            x = lhs_q if which == 0 else lhs_kv
            w = tied(wqkv_v[pl.ds(_slab_of(which, h) * PITCH + r0, n), :], toks)
            r = jnp.dot(x[:, 2 * r0:2 * (r0 + n)], w, preferred_element_type=F32)
            proj[(which, h)] = r + proj[(which, h)] if (which, h) in proj else r
            return proj[(which, h)]

        def do_wo(toks, h0, h1, j):
            if (h0, h1) not in ocat:
                ocat[(h0, h1)] = jnp.concatenate(
                    [wo_rows(og[h]) for h in range(h0, h1)], axis=1).astype(BF16)
            w = tied(wo_v[j, pl.ds(h0 * 64, (h1 - h0) * 64), :], toks)
            r = jnp.dot(ocat[(h0, h1)], w, preferred_element_type=F32)
            y[j] = r if y[j] is None else r + y[j]
            return y[j]

        ticks = []
        pair_end = {}
        wo_early = [(4 * c, 4 * c + 4, j) for c in range(early) for j in range(nj)]
        first = NP - WO_SLOTS
        for p in range(NP):
            slabs = [(which, h) for h in (2 * p, 2 * p + 1) for which in range(3)]
            rows = [(lhs_q if w == 0 else lhs_kv).shape[0] for w, _ in slabs]
            if p == 0 and split_first:
                for r0 in (0, 256):
                    ticks += [(slab, (w, h, r0, 256), m) for (w, h), m in zip(slabs, rows)]
            else:
                mine = []
                if p >= first:
                    lo = (p - first) * len(wo_early) // WO_SLOTS
                    mine = wo_early[lo:(p - first + 1) * len(wo_early) // WO_SLOTS]
                for n, ((w, h), m) in enumerate(zip(slabs, rows)):
                    ticks += [(do_wo, item, wo_m)
                              for item in mine[n * len(mine) // 6:(n + 1) * len(mine) // 6]]
                    ticks.append((slab, (w, h, 0, 512), 2 * m + 8 * len(mxu_groups[p]) // 6))
            pair_end[len(ticks) - 1] = p
        ticks += [(do_wo, (h0, h0 + 4, j), wo_m)
                  for j in range(nj) for h0 in range(4 * early, HA, 4)]
        ends = []
        for _, _, dur in ticks:
            ends.append(dur + (ends[-1] if ends else 0))

        def index(t):
            return next(i for i, e in enumerate(ends) if e >= t)

        events = {}
        anchors = {}
        cursor = [0]

        def run_chunk(res, p, name, st, c0, i_done):
            done = vpu_chunk(st, c0, pltpu.bitcast(res[0:8], U32) & zero)
            anchors.setdefault(i_done, []).append(done & zero)
            if c0 + CHUNK >= 8 * (st['g'] + 1):
                og[2 * p][name], og[2 * p + 1][name] = vpu_finish(st)
                if D_R and ends[i_done - 1] + D_R < ends[-2]:
                    anchors.setdefault(index(ends[i_done - 1] + D_R) + 1, []).append(
                        pltpu.bitcast(og[2 * p][name], U32) & zero)

        def do_s(res, p):
            sc = jax.lax.dot_general(qkv[p][0], qkv[p][1], (((1,), (1,)), ((), ())),
                                     preferred_element_type=F32)
            allowed, fill = masks[ngv[p]]
            sc = jnp.where(allowed, sc, fill)
            e = jnp.exp2((sc - jnp.max(sc, axis=-1, keepdims=True)) * c_exp)
            l = jnp.sum(e, axis=-1, keepdims=True)
            e = e * recip(l)
            rm = 8 * len(mxu_groups[p])
            e = e[0:rm] + e[rm:2 * rm]
            if rm % 16:
                e = jnp.concatenate([e, jnp.zeros((8, 128), F32)], axis=0)
            pb[p] = e.astype(BF16)

        def do_pv(res, p):
            for i in range(2):
                o = jnp.dot(pb[p], qkv[p][2][i], preferred_element_type=F32)
                for n, g in enumerate(mxu_groups[p]):
                    og[2 * p + i][g] = o[8 * n:8 * n + 8]

        def finish_pair(p, i):
            u, jobs = unpack(p, [[proj[(w, h)] for w in range(3)] for h in (2 * p, 2 * p + 1)])
            chunks = [(name, st, c0) for name, st in
                      [(name, vpu_start(*job)) for name, job in jobs.items()]
                      for c0 in range(0, 8 * (st['g'] + 1), CHUNK)]
            t_first = ends[min(pair_end)] + D_G
            t_last = ends[-2] - d_j - D_F
            gap = (t_last - t_first) / (n_chunks - 1)
            if p == NP - 1:
                gap = min(gap, (t_last - max(ends[i] + D_G, cursor[0])) / (len(chunks) - 1))
            for chunk in chunks:
                t = max(ends[i] + D_G, cursor[0])
                cursor[0] = t + gap
                g = max(index(t), i + 1)
                events.setdefault(g, []).append(
                    (run_chunk, (p,) + chunk + (index(ends[g] + d_j) + 1,)))
            qb = jnp.concatenate([u[k][0][g] for k in range(2) for g in mxu_groups[p]],
                                 axis=0).astype(BF16)
            kb = jnp.concatenate([u[0][1], u[1][1], zpad], axis=0).astype(BF16)
            low40 = jnp.concatenate([low] * 5, axis=0)
            vb = [jnp.concatenate([jnp.where(low40, v, 0.0), jnp.where(low40, 0.0, v), zpad],
                                  axis=0).astype(BF16) for v in (u[0][2], u[1][2])]
            qkv[p] = (qb, kb, vb)
            t_pv = min(ends[i] + D_PV, ends[-1] - D_O)
            events.setdefault(index(min(ends[i] + D_S, t_pv - D_SM)), []).append((do_s, (p,)))
            events.setdefault(index(t_pv), []).append((do_pv, (p,)))

        for i, (fn, args, _) in enumerate(ticks):
            res = fn(anchors.pop(i, []), *args)
            if i in pair_end:
                finish_pair(pair_end[i], i)
            for f, a in events.pop(i, []):
                f(res, *a)
        assert not events
        for j in range(nj):
            do_wo([], HA, H, j)
        return jnp.concatenate(y, axis=1)

    def pair(r0, mem):
        xf = x_v[pl.ds(r0, PAIR), :].astype(F32)
        zero = zero_v[pl.ds(0, 8), :]
        x1s = jnp.concatenate([xf[0:8], xf[32:40]], axis=0).astype(BF16)
        keep = [None] * H

        def cat(*xs):
            return jnp.concatenate(xs, axis=0)

        lhs = cat(mem, xf[8:32]).astype(BF16)

        def finish(qg, ks, vs, slot, groups):
            return ([(qg[i], ks[i], vs[i]) for i in range(2)],
                    {g: stash(slot + n, ks, vs, g) for n, g in enumerate(groups)})

        def unpack_a(p, qkv):
            qg = [{0: q[0:8], 2: q[8:16], 3: q[16:24], 4: q[24:32]} for q, _, _ in qkv]
            ks = [cat(k[0:8], k[32:40], k[8:32]) for _, k, _ in qkv]
            vs = [cat(v[0:8], v[32:40], v[8:32]) for _, _, v in qkv]
            u, parked = finish(qg, ks, vs, NJOB * p, range(1, NGV_A[p] + 1))
            keep[p] = (parked[1], [(k[40:48], v[40:48]) for _, k, v in qkv])
            return u, {g: (qg[0][g], qg[1][g], parked[g], g) for g in range(2, NGV_A[p] + 1)}

        y_a = segment(lhs, cat(lhs, x1s), 32, NGV_A,
                      sum(g + 1 for n in NGV_A for g in range(2, n + 1)) * 8 // CHUNK, unpack_a,
                      lambda o: cat(o[0], o[2], o[3], o[4]), False, EARLY_A, D_JA, zero)

        lhs = cat(y_a[0:8], xf[40:64]).astype(BF16)

        def unpack_b(p, qkv):
            parked_a1, kv1 = keep[p]
            qg = [{0: q[0:8], 1: q[40:48], 2: q[8:16], 3: q[16:24], 4: q[24:32]}
                  for q, _, _ in qkv]
            ks = [cat(k[0:8], e[0], k[8:32]) for (_, k, _), e in zip(qkv, kv1)]
            vs = [cat(v[0:8], e[1], v[8:32]) for (_, _, v), e in zip(qkv, kv1)]
            u, parked = finish(qg, ks, vs, NJOB * p + max(NGV_A), range(1, NGV_B[p] + 1))
            jobs = {'a1': (qkv[0][0][32:40], qkv[1][0][32:40], parked_a1, 1)}
            jobs.update({g: (qg[0][g], qg[1][g], parked[g], g) for g in range(1, NGV_B[p] + 1)})
            return u, jobs

        y_b = segment(cat(lhs, x1s), lhs, 48, NGV_B,
                      sum(2 + sum(range(2, n + 2)) for n in NGV_B) * 8 // CHUNK, unpack_b,
                      lambda o: cat(o[0], o[1], o[2], o[3], o[4], o['a1']), True, EARLY_B,
                      D_JB, zero)

        a = cat(y_b[40:48], y_a[8:32], y_b[8:40])
        g = g_v[pl.ds(r0, PAIR), :]
        g = jnp.concatenate([g] * (D // 128), axis=1)
        out_v[pl.ds(r0, PAIR), :] = (g * a + h1_rows(r0, PAIR)).astype(BF16)
        return y_b[0:8]

    rows_it = UNROLL_A * PAIR

    def a_body(t, carry):
        base = pl.multiple_of(t * rows_it, rows_it)
        mem = mem_v[...]
        for u in range(UNROLL_A):
            mem = pair(pl.multiple_of(base + u * PAIR, PAIR), mem)
        mem_v[...] = mem
        pltpu.make_async_copy(out_v.at[pl.ds(base, rows_it)], out_hbm.at[pl.ds(base, rows_it)],
                              osem).start()
        return carry

    with jax.named_scope('a_body'):
        jax.lax.fori_loop(0, S // rows_it, a_body, 0)
    pltpu.make_async_copy(out_v, out_hbm, osem).wait()


@jax.jit
def pallas_gated_mix__memory_aug_recurrent_mem_tr__mixer_s_mlp__prompt_kernel(
    A_x, A_mem0, A_Wq, A_Wk, A_Wv, A_Wo, A_seg_len, B_x, B_w1, B_w2, B_w3, B_w4, gate_w,
):
    assert A_x.shape == (1, S, D) and A_Wq.shape == (D, H, DH) and A_mem0.shape == (1, M, D)
    x = A_x.reshape(S, D)
    mem0 = A_mem0.reshape(M, D)
    wq = A_Wq.reshape(D * H, DH)
    wk = A_Wk.reshape(D * H, DH)
    wv = A_Wv.reshape(D * H, DH)
    wo = A_Wo.reshape(H * DH, D)

    any_spec = pl.BlockSpec(memory_space=pl.ANY)
    out = pl.pallas_call(
        _kernel,
        out_shape=jax.ShapeDtypeStruct((S, D), BF16),
        in_specs=[any_spec] * 11,
        out_specs=any_spec,
        scratch_shapes=[
            pltpu.VMEM((S, D), BF16),
            pltpu.VMEM((NRING, 3, DP * H, DH), BF16),
            pltpu.VMEM((NRING, OP, D), BF16),
            pltpu.VMEM((3 * H * PITCH, 128), U32),
            pltpu.VMEM((D // 128, H * DH // 2, 128), U32),
            pltpu.VMEM((4, D, D // 4), BF16),
            pltpu.VMEM((4, D, D // 4), BF16),
            pltpu.VMEM((D, FF), BF16),
            pltpu.VMEM((FF, D), BF16),
            pltpu.VMEM((D // 128, S + 16, 128), F32),
            pltpu.VMEM((S + T2, D), F32),
            pltpu.VMEM((S, 128), F32),
            pltpu.VMEM((2, T1, D), BF16),
            pltpu.VMEM((2, T3, D), BF16),
            pltpu.VMEM((M, D), BF16),
            pltpu.VMEM((D,), BF16),
            pltpu.VMEM((M, D), F32),
            pltpu.VMEM((S, D), BF16),
            pltpu.VMEM((NJOB * H * 2 * (L + 8), 128), F32),
            pltpu.VMEM((16, 128), U32),
            pltpu.SemaphoreType.DMA((NSEM,)),
            pltpu.SemaphoreType.DMA(()),
        ],
        compiler_params=pltpu.CompilerParams(vmem_limit_bytes=120 * 1024 * 1024,
                                             disable_bounds_checks=True),
    )(x, mem0, wq, wk, wv, wo, B_w1, B_w2, B_w3, B_w4, gate_w)
    return out.reshape(1, S, D)
```

```python
import math

import jax
import jax.numpy as jnp
import jax.experimental.pallas as pl
import jax.experimental.pallas.tpu as pltpu

F32 = jnp.float32
BF16 = jnp.bfloat16
U32 = jnp.uint32

S = 2048
D = 1024
H = 32
DH = 128
M = 8
SEG = 32
L = M + SEG
FF = 3584
PAIR = 2 * SEG
NPAIR = S // PAIR
T1 = 256
N1 = S // T1
T2 = 512
N2 = S // T2
T3 = 256
N3 = S // T3
DP = D // N3
OP = H * DH // N3
UNROLL_A = 1
PITCH = 520
NRING = 3
NSEM = 11 + NRING
EPS = 1e-5
NCHAIN0 = 10
NCHAIN1 = 5
LN1_ROWS = 8
HOP = 4
FRAC_B = 0.875
NGV_A = [3] * (H // 2)
NGV_B = [1 + 2 * (int((p + 1) * FRAC_B + 1e-6) - int(p * FRAC_B + 1e-6)) for p in range(H // 2)]
NJOB = max(NGV_A) + max(NGV_B)
EARLY_A = 2
EARLY_B = 3
WO_SLOTS = 10
CHUNK = 8
D_G = 0
D_JA = 530
D_JB = 600
D_F = 50
D_R = 0
D_S = 500
D_PV = 1400
D_SM = 600
D_O = 170
TAIL_H = 8
NEG = -1e9


def _gelu(x):
    c = math.sqrt(2.0 / math.pi)
    return 0.5 * x * (1.0 + jnp.tanh(c * (x + 0.044715 * (x * x * x))))


def _layernorm(x):
    m = jnp.mean(x, axis=-1, keepdims=True)
    xc = x - m
    v = jnp.mean(xc * xc, axis=-1, keepdims=True)
    return xc * jax.lax.rsqrt(v + EPS)


def _slab_of(which, h):
    return which * H + (h % 2) * (H // 2) + h // 2


def _kernel(x_hbm, mem0_hbm, wq_hbm, wk_hbm, wv_hbm, wo_hbm,
            w1_hbm, w2_hbm, w3_hbm, w4_hbm, gw_hbm,
            out_hbm,
            x_v, stq_v, sto_v, wqkv_v, wo_v, w1_v, w2_v, w3_v, w4_v,
            h1_v, x1_v, g_v, ln1_v, ln3_v, mem0_v, gw_v, mem_v, out_v, kv_v, zero_v, sems, osem):
    c4 = D // 4
    xcuts = (0, 1, 2, 3, 5, N1)
    cp_x = [pltpu.make_async_copy(x_hbm.at[pl.ds(lo * T1, (hi - lo) * T1)],
                                  x_v.at[pl.ds(lo * T1, (hi - lo) * T1)], sems.at[n])
            for n, (lo, hi) in enumerate(zip(xcuts[:-1], xcuts[1:]))]
    cp_w1 = [pltpu.make_async_copy(w1_hbm.at[:, pl.ds(q * c4, c4)], w1_v.at[q], sems.at[5 + q])
             for q in range(4)]
    cp_w2 = [pltpu.make_async_copy(w2_hbm.at[:, pl.ds(q * c4, c4)], w2_v.at[q], sems.at[9])
             for q in range(4)]
    cp_ffn = [pltpu.make_async_copy(src, dst, sems.at[10])
              for src, dst in ((gw_hbm, gw_v), (mem0_hbm, mem0_v), (w3_hbm, w3_v), (w4_hbm, w4_v))]

    def piece_copies(i, slot):
        cps = [pltpu.make_async_copy(w.at[pl.ds(i * (DP * H), DP * H)], stq_v.at[slot, k],
                                     sems.at[11 + slot])
               for k, w in enumerate((wq_hbm, wk_hbm, wv_hbm))]
        cps.append(pltpu.make_async_copy(wo_hbm.at[pl.ds(i * OP, OP)], sto_v.at[slot],
                                         sems.at[11 + slot]))
        return cps

    for c in (cp_x[0:1] + cp_w1 + cp_x[1:] + cp_w2 + cp_ffn
              + piece_copies(0, 0) + piece_copies(1, 1)):
        c.start()
    x1_v[pl.ds(0, T3), :] = jnp.zeros((T3, D), F32)
    h1_v[:, pl.ds(8, 8), :] = jnp.zeros((D // 128, 8, 128), F32)
    h1_v[:, pl.ds(S, 8), :] = jnp.zeros((D // 128, 8, 128), F32)
    zero_v[...] = jnp.zeros((16, 128), U32)

    def ln_rows(x, tok, zero):
        if tok is not None:
            head = pltpu.bitcast(pltpu.bitcast(x[:, 0:128], U32) | tok, F32)
            x = jnp.concatenate([head, x[:, 128:]], axis=1)
        y = _layernorm(x)
        tok = None if zero is None else pltpu.bitcast(y[:, 0:128], U32) & zero
        return y, tok

    def ln_block(load, store, rows, nchain, gr):
        zero = zero_v[pl.ds(0, gr), :] if nchain else None
        toks = [None] * max(nchain, 1)
        for k in range(rows // gr):
            y, toks[k % len(toks)] = ln_rows(load(k * gr, gr), toks[k % len(toks)], zero)
            store(k * gr, y.astype(BF16))
        return toks[(rows // gr - 1) % len(toks)]

    def prep1(blk, slot, nchain):
        r0 = blk * T1 if isinstance(blk, int) else pl.multiple_of(blk * T1, T1)

        def store(k, y):
            ln1_v[slot, pl.ds(k, y.shape[0]), :] = y

        ln_block(lambda k, n: x_v[pl.ds(r0 + k, n), :].astype(F32), store, T1, nchain, LN1_ROWS)

    def p1_quarter(lhs, r0, q):
        h = _gelu(jnp.dot(lhs, w1_v[q], preferred_element_type=F32))
        for j in range(2):
            win = h1_v.at[2 * q + j, pl.ds(r0, T1 + 16)]
            win[pl.ds(8 + (1, -1, 2, -2)[q], T1), :] = h[:, j * 128:(j + 1) * 128]

    cp_x[0].wait()
    prep1(0, 0, 0)
    for q in range(4):
        cp_w1[q].wait()
        if q == 3:
            cp_x[1].wait()
        lhs = ln1_v[0]
        if q == 3:
            prep1(1, 1, NCHAIN0)
        p1_quarter(lhs, 0, q)

    def p1_body(i, carry):
        r0 = pl.multiple_of(i * T1, T1)
        slot = i & 1

        lhs = ln1_v[slot]
        prep1(jnp.minimum(i + 1, N1 - 1), 1 - slot, NCHAIN1)
        for q in range(4):
            p1_quarter(lhs, r0, q)
        for n in range(3, len(cp_x)):
            pl.when(i + 2 == xcuts[n])(cp_x[n].wait)
        return carry

    cp_x[2].wait()
    with jax.named_scope('p1_body'):
        jax.lax.fori_loop(1, N1, p1_body, 0)
    for c in cp_w2:
        c.wait()

    def h1_rows(r0, n):
        return jnp.concatenate([h1_v[j, pl.ds(r0, n), :] for j in range(D // 128)], axis=1)

    def prep3(src, slot):
        def store(k, y):
            ln3_v[slot, pl.ds(k, y.shape[0]), :] = y

        return ln_block(lambda k, n: src[pl.ds(k, n), :], store, T3, 1, 16)

    def p2_body(i, carry):
        r0 = pl.multiple_of(i * T2, T2)
        win = x1_v.at[pl.ds(r0, 2 * T2)]
        prep3(win, 0)
        hs = h1_rows(r0 + 8, T2).astype(BF16)
        for q in range(4):
            win[pl.ds(T2, T2), pl.ds(q * c4, c4)] = (
                jnp.dot(hs, w2_v[q], preferred_element_type=F32)
                + x_v[pl.ds(r0, T2), pl.ds(q * c4, c4)].astype(F32))
        return carry

    with jax.named_scope('p2_body'):
        jax.lax.fori_loop(0, N2, p2_body, 0)

    for c in cp_ffn + piece_copies(0, 0):
        c.wait()
    blk0 = (N2 - 2) * T2 // T3

    def p3_body(i, carry):
        r0 = pl.multiple_of((i + blk0) % N3 * T3, T3)
        r_next = pl.multiple_of((i + 1 + blk0) % N3 * T3, T3)
        slot = i & 1
        ring = i % NRING

        @pl.when(i + 2 < N3)
        def _():
            for c in piece_copies(i + 2, (i + 2) % NRING):
                c.start()

        lhs = ln3_v[slot]
        tok = prep3(x1_v.at[pl.ds(T2 + r_next, T3)], 1 - slot)
        zero = zero_v[...]
        low16 = jax.lax.broadcasted_iota(jnp.int32, (16, 128), 1) < 64
        for which in range(3):
            for j in range(DP // 2):
                blk = pltpu.bitcast(stq_v[ring, which, pl.ds(j * 64, 64), :], U32)
                a = blk[0:16] | tok
                c = blk[16:32]
                lo = (a & jnp.uint32(0xFFFF)) | (c << 16)
                if which < 2:
                    a = a | (lo & zero)
                hi = (a >> 16) | (c & jnp.uint32(0xFFFF0000))
                if which < 2:
                    tok = hi & zero
                    if j % HOP == HOP - 1:
                        tok = pltpu.roll(tok, 1, 1)
                else:
                    t = pltpu.roll(jnp.where(low16, hi, lo), 64, 1)
                    lo, hi = jnp.where(low16, lo, t), jnp.where(low16, t, hi)
                    both = hi if j % 2 == 0 else both | hi
                    if j % 2 == 1:
                        tok = both & zero
                s0 = which * H * PITCH + i * (DP // 2) + j
                wqkv_v[pl.ds(s0, 16, stride=PITCH), :] = lo
                wqkv_v[pl.ds(s0 + 16 * PITCH, 16, stride=PITCH), :] = hi
        o0 = pl.multiple_of(i * (OP // 2), OP // 2)
        for j in range(D // 128):
            for k in range(OP // 32):
                w = pltpu.bitcast(sto_v[ring, pl.ds(k * 32, 32), pl.ds(j * 128, 128)], U32) | tok
                tok = w & zero
                if k % (2 * HOP) == 2 * HOP - 1:
                    tok = pltpu.roll(tok, 1, 1)
                kd = k - k % 8 + (0, 1, 4, 5, 2, 3, 6, 7)[k % 8]
                wo_v[j, pl.ds(o0 + kd * 16, 16), :] = w

        h = _gelu(jnp.dot(lhs, w3_v[...], preferred_element_type=F32)).astype(BF16)
        b = jnp.dot(h, w4_v[...], preferred_element_type=F32) + x1_v[pl.ds(T2 + r0, T3), :]
        gw = gw_v[...].astype(F32).reshape(1, D)
        z = jnp.sum(x_v[pl.ds(r0, T3), :].astype(F32) * gw, axis=-1, keepdims=True)
        g = 1.0 / (1.0 + jnp.exp(-z))
        g_v[pl.ds(r0, T3), :] = jnp.broadcast_to(g, (T3, 128))
        b = (1.0 - g) * b
        for j in range(D // 128):
            h1_v[j, pl.ds(r0, T3), :] = b[:, j * 128:(j + 1) * 128]

        @pl.when(i + 1 < N3)
        def _():
            for c in piece_copies(i + 1, (i + 1) % NRING):
                c.wait()

        return carry

    with jax.named_scope('p3_body'):
        jax.lax.fori_loop(0, N3, p3_body, 0)

    mem_v[...] = mem0_v[...].astype(F32)
    c_exp = (DH ** -0.5) * math.log2(math.e)
    neg_raw = NEG / (DH ** -0.5)

    L2 = 2 * L

    def make_mask(ngv):
        rm = L - 8 * ngv
        row = jax.lax.broadcasted_iota(jnp.int32, (2 * rm, 128), 0)
        col = jax.lax.broadcasted_iota(jnp.int32, (2 * rm, 128), 1)
        second = row >= rm
        rowl = jnp.where(second, row - rm, row)
        coll = jnp.where(second, col - L, col)
        real = (coll >= 0) & (coll < L)
        allowed = real & ((rowl < M) | (rowl + 8 * ngv >= coll))
        return allowed, jnp.where(real, neg_raw, -jnp.inf).astype(F32)

    masks = {n: make_mask(n) for n in set(NGV_A + NGV_B)}
    neg_c = NEG * math.log2(math.e)

    def tied(w, toks):
        for tok in toks:
            w = jnp.concatenate([w[0:56], w[56:64] | tok, w[64:]], axis=0)
        return pltpu.bitcast(w, BF16)

    zpad = jnp.zeros((128 - L2, DH), F32)

    def recip(l):
        r = pl.reciprocal(l, approx=True)
        return r * (2.0 - l * r)

    def tree(op, x):
        while x.shape[0] > 1:
            x = op(x[0:x.shape[0] // 2], x[x.shape[0] // 2:])
        return x[0]

    causal = (jax.lax.broadcasted_iota(jnp.int32, (7, 8, 128), 1)
              > jax.lax.broadcasted_iota(jnp.int32, (7, 8, 128), 0))
    low = jax.lax.broadcasted_iota(jnp.int32, (8, 128), 1) < 64

    def stash(buf, slot, ks, ws, g):
        n = 8 * (g + 2)
        starts = []
        for i, x in enumerate(ks + ws):
            base = (4 * slot + i) * (L + 8)
            buf[pl.ds(base, n), :] = jnp.concatenate([x[8 * g:8 * g + 8], x[0:n - 8]], axis=0)
            starts.append(base + n - 8)
        return buf, starts, [jnp.sum(w[n - 8:L], axis=0, keepdims=True) if n - 8 < L
                             else jnp.zeros((1, DH), F32) for w in ws]

    def vpu_start(q0, q1, parked, g):
        buf, starts, (acc_a, acc_b) = parked
        return dict(q=(q0 * c_exp, q1 * c_exp), buf=buf, starts=starts, g=g,
                    m=jnp.full((8, 128), neg_c, F32),
                    l=jnp.full((8, 128), float(L - 8 * (g + 1)), F32), a=acc_a, b=acc_b)

    def vpu_chunk(st, c0, gate):
        def windows(start):
            return jnp.concatenate([st['buf'][pl.ds(start - r, 8), :]
                                    for r in range(c0, c0 + CHUNK)], axis=0).reshape(CHUNK, 8, 128)

        k0, k1, wa, wb = st['starts']
        q0, q1 = [pltpu.bitcast(pltpu.bitcast(q, U32) | gate, F32) for q in st['q']]
        sc = jnp.where(low, jnp.sum(q0 * windows(k0), axis=-1, keepdims=True),
                       jnp.sum(q1 * windows(k1), axis=-1, keepdims=True))
        if c0 == 8 * st['g']:
            sc = jnp.concatenate([sc[0:1], jnp.where(causal, sc[1:], neg_c)], axis=0)
        m = jnp.maximum(tree(jnp.maximum, sc), st['m'])
        alpha = jnp.exp2(st['m'] - m)
        pr = jnp.exp2(sc - m)
        new = []
        for old, x in ((st['l'], pr), (st['a'], pr * windows(wa)), (st['b'], pr * windows(wb))):
            new.append(jnp.sum(jnp.concatenate([(old * alpha)[None], x], axis=0), axis=0))
        st.update(m=m, l=new[0], a=new[1], b=new[2])
        return (pltpu.bitcast(new[0], U32) | pltpu.bitcast(new[1], U32)
                | pltpu.bitcast(new[2], U32))

    def vpu_finish(st):
        r = recip(st['l'])
        return st['a'] * r, st['b'] * r

    def segment(lhs_q, lhs_kv, wo_m, ngv, n_chunks, unpack, wo_rows, split_first, early, d_j, zero):
        NP = H // 2
        nj = D // 128
        HA = H - TAIL_H
        mxu_groups = [[0] + list(range(n + 1, 5)) for n in ngv]
        proj = {}
        qkv = [None] * NP
        pb = [None] * NP
        og = [dict() for _ in range(H)]
        ocat = {}
        y = [None] * nj

        def slab(toks, which, h, r0, n):
            x = lhs_q if which == 0 else lhs_kv
            w = tied(wqkv_v[pl.ds(_slab_of(which, h) * PITCH + r0, n), :], toks)
            r = jnp.dot(x[:, 2 * r0:2 * (r0 + n)], w, preferred_element_type=F32)
            proj[(which, h)] = r + proj[(which, h)] if (which, h) in proj else r
            return proj[(which, h)]

        def do_wo(toks, h0, h1, j):
            if (h0, h1) not in ocat:
                ocat[(h0, h1)] = jnp.concatenate(
                    [wo_rows(og[h]) for h in range(h0, h1)], axis=1).astype(BF16)
            w = tied(wo_v[j, pl.ds(h0 * 64, (h1 - h0) * 64), :], toks)
            r = jnp.dot(ocat[(h0, h1)], w, preferred_element_type=F32)
            y[j] = r if y[j] is None else r + y[j]
            return y[j]

        ticks = []
        pair_end = {}
        wo_early = [(4 * c, 4 * c + 4, j) for c in range(early) for j in range(nj)]
        first = NP - WO_SLOTS
        for p in range(NP):
            slabs = [(which, h) for h in (2 * p, 2 * p + 1) for which in range(3)]
            rows = [(lhs_q if w == 0 else lhs_kv).shape[0] for w, _ in slabs]
            if p == 0 and split_first:
                for r0 in (0, 256):
                    ticks += [(slab, (w, h, r0, 256), m) for (w, h), m in zip(slabs, rows)]
            else:
                mine = []
                if p >= first:
                    lo = (p - first) * len(wo_early) // WO_SLOTS
                    mine = wo_early[lo:(p - first + 1) * len(wo_early) // WO_SLOTS]
                for n, ((w, h), m) in enumerate(zip(slabs, rows)):
                    ticks += [(do_wo, item, wo_m)
                              for item in mine[n * len(mine) // 6:(n + 1) * len(mine) // 6]]
                    ticks.append((slab, (w, h, 0, 512), 2 * m + 8 * len(mxu_groups[p]) // 6))
            pair_end[len(ticks) - 1] = p
        ticks += [(do_wo, (h0, h0 + 4, j), wo_m)
                  for j in range(nj) for h0 in range(4 * early, HA, 4)]
        ends = []
        for _, _, dur in ticks:
            ends.append(dur + (ends[-1] if ends else 0))

        def index(t):
            return next(i for i, e in enumerate(ends) if e >= t)

        events = {}
        anchors = {}
        cursor = [0]

        def run_chunk(res, p, name, st, c0, i_done):
            done = vpu_chunk(st, c0, pltpu.bitcast(res[0:8], U32) & zero)
            anchors.setdefault(i_done, []).append(done & zero)
            if c0 + CHUNK >= 8 * (st['g'] + 1):
                og[2 * p][name], og[2 * p + 1][name] = vpu_finish(st)
                if D_R and ends[i_done - 1] + D_R < ends[-2]:
                    anchors.setdefault(index(ends[i_done - 1] + D_R) + 1, []).append(
                        pltpu.bitcast(og[2 * p][name], U32) & zero)

        def do_s(res, p):
            sc = jax.lax.dot_general(qkv[p][0], qkv[p][1], (((1,), (1,)), ((), ())),
                                     preferred_element_type=F32)
            allowed, fill = masks[ngv[p]]
            sc = jnp.where(allowed, sc, fill)
            e = jnp.exp2((sc - jnp.max(sc, axis=-1, keepdims=True)) * c_exp)
            l = jnp.sum(e, axis=-1, keepdims=True)
            e = e * recip(l)
            rm = 8 * len(mxu_groups[p])
            e = e[0:rm] + e[rm:2 * rm]
            if rm % 16:
                e = jnp.concatenate([e, jnp.zeros((8, 128), F32)], axis=0)
            pb[p] = e.astype(BF16)

        def do_pv(res, p):
            for i in range(2):
                o = jnp.dot(pb[p], qkv[p][2][i], preferred_element_type=F32)
                for n, g in enumerate(mxu_groups[p]):
                    og[2 * p + i][g] = o[8 * n:8 * n + 8]

        def finish_pair(p, i):
            u, jobs = unpack(p, [[proj[(w, h)] for w in range(3)] for h in (2 * p, 2 * p + 1)])
            chunks = [(name, st, c0) for name, st in
                      [(name, vpu_start(*job)) for name, job in jobs.items()]
                      for c0 in range(0, 8 * (st['g'] + 1), CHUNK)]
            t_first = ends[min(pair_end)] + D_G
            t_last = ends[-2] - d_j - D_F
            gap = (t_last - t_first) / (n_chunks - 1)
            if p == NP - 1:
                gap = min(gap, (t_last - max(ends[i] + D_G, cursor[0])) / (len(chunks) - 1))
            for chunk in chunks:
                t = max(ends[i] + D_G, cursor[0])
                cursor[0] = t + gap
                g = max(index(t), i + 1)
                events.setdefault(g, []).append(
                    (run_chunk, (p,) + chunk + (index(ends[g] + d_j) + 1,)))
            qb = jnp.concatenate([u[k][0][g] for k in range(2) for g in mxu_groups[p]],
                                 axis=0).astype(BF16)
            kb = jnp.concatenate([u[0][1], u[1][1], zpad], axis=0).astype(BF16)
            low40 = jnp.concatenate([low] * 5, axis=0)
            vb = [jnp.concatenate([jnp.where(low40, v, 0.0), jnp.where(low40, 0.0, v), zpad],
                                  axis=0).astype(BF16) for v in (u[0][2], u[1][2])]
            qkv[p] = (qb, kb, vb)
            t_pv = min(ends[i] + D_PV, ends[-1] - D_O)
            events.setdefault(index(min(ends[i] + D_S, t_pv - D_SM)), []).append((do_s, (p,)))
            events.setdefault(index(t_pv), []).append((do_pv, (p,)))

        for i, (fn, args, _) in enumerate(ticks):
            res = fn(anchors.pop(i, []), *args)
            if i in pair_end:
                finish_pair(pair_end[i], i)
            for f, a in events.pop(i, []):
                f(res, *a)
        assert not events
        for j in range(nj):
            do_wo([], HA, H, j)
        return jnp.concatenate(y, axis=1)

    def pair(r0, mem):
        xf = x_v[pl.ds(r0, PAIR), :].astype(F32)
        zero = zero_v[pl.ds(0, 8), :]
        x1s = jnp.concatenate([xf[0:8], xf[32:40]], axis=0).astype(BF16)
        keep = [None] * H

        def cat(*xs):
            return jnp.concatenate(xs, axis=0)

        lhs = cat(mem, xf[8:32]).astype(BF16)

        def finish(p, qg, ks, vs, slot, groups):
            return ([(qg[i], ks[i], vs[i]) for i in range(2)],
                    {g: stash(kv_v[p], slot + n, ks, vs, g) for n, g in enumerate(groups)})

        def unpack_a(p, qkv):
            qg = [{0: q[0:8], 2: q[8:16], 3: q[16:24], 4: q[24:32]} for q, _, _ in qkv]
            ks = [cat(k[0:8], k[32:40], k[8:32]) for _, k, _ in qkv]
            vs = [cat(v[0:8], v[32:40], v[8:32]) for _, _, v in qkv]
            u, parked = finish(p, qg, ks, vs, 0, range(1, NGV_A[p] + 1))
            keep[p] = (parked[1], [(k[40:48], v[40:48]) for _, k, v in qkv])
            return u, {g: (qg[0][g], qg[1][g], parked[g], g) for g in range(2, NGV_A[p] + 1)}

        y_a = segment(lhs, cat(lhs, x1s), 32, NGV_A,
                      sum(g + 1 for n in NGV_A for g in range(2, n + 1)) * 8 // CHUNK, unpack_a,
                      lambda o: cat(o[0], o[2], o[3], o[4]), False, EARLY_A, D_JA, zero)

        lhs = cat(y_a[0:8], xf[40:64]).astype(BF16)

        def unpack_b(p, qkv):
            parked_a1, kv1 = keep[p]
            qg = [{0: q[0:8], 1: q[40:48], 2: q[8:16], 3: q[16:24], 4: q[24:32]}
                  for q, _, _ in qkv]
            ks = [cat(k[0:8], e[0], k[8:32]) for (_, k, _), e in zip(qkv, kv1)]
            vs = [cat(v[0:8], e[1], v[8:32]) for (_, _, v), e in zip(qkv, kv1)]
            u, parked = finish(p, qg, ks, vs, max(NGV_A), range(1, NGV_B[p] + 1))
            jobs = {'a1': (qkv[0][0][32:40], qkv[1][0][32:40], parked_a1, 1)}
            jobs.update({g: (qg[0][g], qg[1][g], parked[g], g) for g in range(1, NGV_B[p] + 1)})
            return u, jobs

        y_b = segment(cat(lhs, x1s), lhs, 48, NGV_B,
                      sum(2 + sum(range(2, n + 2)) for n in NGV_B) * 8 // CHUNK, unpack_b,
                      lambda o: cat(o[0], o[1], o[2], o[3], o[4], o['a1']), True, EARLY_B,
                      D_JB, zero)

        a = cat(y_b[40:48], y_a[8:32], y_b[8:40])
        g = g_v[pl.ds(r0, PAIR), :]
        g = jnp.concatenate([g] * (D // 128), axis=1)
        out_v[pl.ds(r0, PAIR), :] = (g * a + h1_rows(r0, PAIR)).astype(BF16)
        return y_b[0:8]

    rows_it = UNROLL_A * PAIR

    def a_body(t, carry):
        base = pl.multiple_of(t * rows_it, rows_it)
        mem = mem_v[...]
        for u in range(UNROLL_A):
            mem = pair(pl.multiple_of(base + u * PAIR, PAIR), mem)
        mem_v[...] = mem
        pltpu.make_async_copy(out_v.at[pl.ds(base, rows_it)], out_hbm.at[pl.ds(base, rows_it)],
                              osem).start()
        return carry

    with jax.named_scope('a_body'):
        jax.lax.fori_loop(0, S // rows_it, a_body, 0)
    pltpu.make_async_copy(out_v, out_hbm, osem).wait()


@jax.jit
def pallas_gated_mix__memory_aug_recurrent_mem_tr__mixer_s_mlp__prompt_kernel(
    A_x, A_mem0, A_Wq, A_Wk, A_Wv, A_Wo, A_seg_len, B_x, B_w1, B_w2, B_w3, B_w4, gate_w,
):
    assert A_x.shape == (1, S, D) and A_Wq.shape == (D, H, DH) and A_mem0.shape == (1, M, D)
    x = A_x.reshape(S, D)
    mem0 = A_mem0.reshape(M, D)
    wq = A_Wq.reshape(D * H, DH)
    wk = A_Wk.reshape(D * H, DH)
    wv = A_Wv.reshape(D * H, DH)
    wo = A_Wo.reshape(H * DH, D)

    any_spec = pl.BlockSpec(memory_space=pl.ANY)
    out = pl.pallas_call(
        _kernel,
        out_shape=jax.ShapeDtypeStruct((S, D), BF16),
        in_specs=[any_spec] * 11,
        out_specs=any_spec,
        scratch_shapes=[
            pltpu.VMEM((S, D), BF16),
            pltpu.VMEM((NRING, 3, DP * H, DH), BF16),
            pltpu.VMEM((NRING, OP, D), BF16),
            pltpu.VMEM((3 * H * PITCH, 128), U32),
            pltpu.VMEM((D // 128, H * DH // 2, 128), U32),
            pltpu.VMEM((4, D, D // 4), BF16),
            pltpu.VMEM((4, D, D // 4), BF16),
            pltpu.VMEM((D, FF), BF16),
            pltpu.VMEM((FF, D), BF16),
            pltpu.VMEM((D // 128, S + 16, 128), F32),
            pltpu.VMEM((S + T2, D), F32),
            pltpu.VMEM((S, 128), F32),
            pltpu.VMEM((2, T1, D), BF16),
            pltpu.VMEM((2, T3, D), BF16),
            pltpu.VMEM((M, D), BF16),
            pltpu.VMEM((D,), BF16),
            pltpu.VMEM((M, D), F32),
            pltpu.VMEM((S, D), BF16),
            [pltpu.VMEM((NJOB * 4 * (L + 8), 128), F32)] * (H // 2),
            pltpu.VMEM((16, 128), U32),
            pltpu.SemaphoreType.DMA((NSEM,)),
            pltpu.SemaphoreType.DMA(()),
        ],
        compiler_params=pltpu.CompilerParams(vmem_limit_bytes=120 * 1024 * 1024,
                                             disable_bounds_checks=True),
    )(x, mem0, wq, wk, wv, wo, B_w1, B_w2, B_w3, B_w4, gate_w)
    return out.reshape(1, S, D)
```

```python
import math

import jax
import jax.numpy as jnp
import jax.experimental.pallas as pl
import jax.experimental.pallas.tpu as pltpu

F32 = jnp.float32
BF16 = jnp.bfloat16
U32 = jnp.uint32

S = 2048
D = 1024
H = 32
DH = 128
M = 8
SEG = 32
L = M + SEG
FF = 3584
PAIR = 2 * SEG
NPAIR = S // PAIR
T1 = 256
N1 = S // T1
T2 = 512
N2 = S // T2
T3 = 256
N3 = S // T3
DP = D // N3
OP = H * DH // N3
UNROLL_A = 1
PITCH = 520
NRING = 3
NSEM = 11 + NRING
EPS = 1e-5
NCHAIN0 = 10
NCHAIN1 = 5
LN1_ROWS = 8
HOP = 4
NGV_A = [3] * (H // 2)
NGV_B = [3, 3, 1, 3, 3, 3, 1, 3, 3, 3, 3, 3, 1, 3, 3, 3]
NJOB = max(NGV_A) + max(NGV_B)
EARLY_A = 2
EARLY_B = 3
WO_SLOTS = 10
CHUNK = 8
D_G = 0
D_JA = 510
D_JB = 650
D_F = 50
D_R = 0
D_S = 250
D_PV = 1000
D_SM = 600
D_O = 140
TAIL_H = 8
NEG = -1e9


def _gelu(x):
    c = math.sqrt(2.0 / math.pi)
    return 0.5 * x * (1.0 + jnp.tanh(c * (x + 0.044715 * (x * x * x))))


def _layernorm(x):
    m = jnp.mean(x, axis=-1, keepdims=True)
    xc = x - m
    v = jnp.mean(xc * xc, axis=-1, keepdims=True)
    return xc * jax.lax.rsqrt(v + EPS)


def _slab_of(which, h):
    return which * H + (h % 2) * (H // 2) + h // 2


def _kernel(x_hbm, mem0_hbm, wq_hbm, wk_hbm, wv_hbm, wo_hbm,
            w1_hbm, w2_hbm, w3_hbm, w4_hbm, gw_hbm,
            out_hbm,
            x_v, stq_v, sto_v, wqkv_v, wo_v, w1_v, w2_v, w3_v, w4_v,
            h1_v, x1_v, g_v, ln1_v, ln3_v, mem0_v, gw_v, mem_v, out_v, kv_v, zero_v, sems, osem):
    c4 = D // 4
    xcuts = (0, 1, 2, 3, 5, N1)
    cp_x = [pltpu.make_async_copy(x_hbm.at[pl.ds(lo * T1, (hi - lo) * T1)],
                                  x_v.at[pl.ds(lo * T1, (hi - lo) * T1)], sems.at[n])
            for n, (lo, hi) in enumerate(zip(xcuts[:-1], xcuts[1:]))]
    cp_w1 = [pltpu.make_async_copy(w1_hbm.at[:, pl.ds(q * c4, c4)], w1_v.at[q], sems.at[5 + q])
             for q in range(4)]
    cp_w2 = [pltpu.make_async_copy(w2_hbm.at[:, pl.ds(q * c4, c4)], w2_v.at[q], sems.at[9])
             for q in range(4)]
    cp_ffn = [pltpu.make_async_copy(src, dst, sems.at[10])
              for src, dst in ((gw_hbm, gw_v), (mem0_hbm, mem0_v), (w3_hbm, w3_v), (w4_hbm, w4_v))]

    def piece_copies(i, slot):
        cps = [pltpu.make_async_copy(w.at[pl.ds(i * (DP * H), DP * H)], stq_v.at[slot, k],
                                     sems.at[11 + slot])
               for k, w in enumerate((wq_hbm, wk_hbm, wv_hbm))]
        cps.append(pltpu.make_async_copy(wo_hbm.at[pl.ds(i * OP, OP)], sto_v.at[slot],
                                         sems.at[11 + slot]))
        return cps

    for c in (cp_x[0:1] + cp_w1 + cp_x[1:] + cp_w2 + cp_ffn
              + piece_copies(0, 0) + piece_copies(1, 1)):
        c.start()
    x1_v[pl.ds(0, T3), :] = jnp.zeros((T3, D), F32)
    h1_v[:, pl.ds(8, 8), :] = jnp.zeros((D // 128, 8, 128), F32)
    h1_v[:, pl.ds(S, 8), :] = jnp.zeros((D // 128, 8, 128), F32)
    zero_v[...] = jnp.zeros((16, 128), U32)

    def ln_rows(x, tok, zero):
        if tok is not None:
            head = pltpu.bitcast(pltpu.bitcast(x[:, 0:128], U32) | tok, F32)
            x = jnp.concatenate([head, x[:, 128:]], axis=1)
        y = _layernorm(x)
        tok = None if zero is None else pltpu.bitcast(y[:, 0:128], U32) & zero
        return y, tok

    def ln_block(load, store, rows, nchain, gr):
        zero = zero_v[pl.ds(0, gr), :] if nchain else None
        toks = [None] * max(nchain, 1)
        for k in range(rows // gr):
            y, toks[k % len(toks)] = ln_rows(load(k * gr, gr), toks[k % len(toks)], zero)
            store(k * gr, y.astype(BF16))
        return toks[(rows // gr - 1) % len(toks)]

    def prep1(blk, slot, nchain):
        r0 = blk * T1 if isinstance(blk, int) else pl.multiple_of(blk * T1, T1)

        def store(k, y):
            ln1_v[slot, pl.ds(k, y.shape[0]), :] = y

        ln_block(lambda k, n: x_v[pl.ds(r0 + k, n), :].astype(F32), store, T1, nchain, LN1_ROWS)

    def p1_quarter(lhs, r0, q):
        h = _gelu(jnp.dot(lhs, w1_v[q], preferred_element_type=F32))
        for j in range(2):
            win = h1_v.at[2 * q + j, pl.ds(r0, T1 + 16)]
            win[pl.ds(8 + (1, -1, 2, -2)[q], T1), :] = h[:, j * 128:(j + 1) * 128]

    cp_x[0].wait()
    prep1(0, 0, 0)
    for q in range(4):
        cp_w1[q].wait()
        if q == 3:
            cp_x[1].wait()
        lhs = ln1_v[0]
        if q == 3:
            prep1(1, 1, NCHAIN0)
        p1_quarter(lhs, 0, q)

    def p1_body(i, carry):
        r0 = pl.multiple_of(i * T1, T1)
        slot = i & 1

        lhs = ln1_v[slot]
        prep1(jnp.minimum(i + 1, N1 - 1), 1 - slot, NCHAIN1)
        for q in range(4):
            p1_quarter(lhs, r0, q)
        for n in range(3, len(cp_x)):
            pl.when(i + 2 == xcuts[n])(cp_x[n].wait)
        return carry

    cp_x[2].wait()
    with jax.named_scope('p1_body'):
        jax.lax.fori_loop(1, N1, p1_body, 0)
    for c in cp_w2:
        c.wait()

    def h1_rows(r0, n):
        return jnp.concatenate([h1_v[j, pl.ds(r0, n), :] for j in range(D // 128)], axis=1)

    def prep3(src, slot):
        def store(k, y):
            ln3_v[slot, pl.ds(k, y.shape[0]), :] = y

        return ln_block(lambda k, n: src[pl.ds(k, n), :], store, T3, 1, 16)

    def p2_body(i, carry):
        r0 = pl.multiple_of(i * T2, T2)
        win = x1_v.at[pl.ds(r0, 2 * T2)]
        prep3(win, 0)
        hs = h1_rows(r0 + 8, T2).astype(BF16)
        for q in range(4):
            win[pl.ds(T2, T2), pl.ds(q * c4, c4)] = (
                jnp.dot(hs, w2_v[q], preferred_element_type=F32)
                + x_v[pl.ds(r0, T2), pl.ds(q * c4, c4)].astype(F32))
        return carry

    with jax.named_scope('p2_body'):
        jax.lax.fori_loop(0, N2, p2_body, 0)

    for c in cp_ffn + piece_copies(0, 0):
        c.wait()
    blk0 = (N2 - 2) * T2 // T3

    def p3_body(i, carry):
        r0 = pl.multiple_of((i + blk0) % N3 * T3, T3)
        r_next = pl.multiple_of((i + 1 + blk0) % N3 * T3, T3)
        slot = i & 1
        ring = i % NRING

        @pl.when(i + 2 < N3)
        def _():
            for c in piece_copies(i + 2, (i + 2) % NRING):
                c.start()

        lhs = ln3_v[slot]
        tok = prep3(x1_v.at[pl.ds(T2 + r_next, T3)], 1 - slot)
        zero = zero_v[...]
        low16 = jax.lax.broadcasted_iota(jnp.int32, (16, 128), 1) < 64
        for which in range(3):
            for j in range(DP // 2):
                blk = pltpu.bitcast(stq_v[ring, which, pl.ds(j * 64, 64), :], U32)
                a = blk[0:16] | tok
                c = blk[16:32]
                lo = (a & jnp.uint32(0xFFFF)) | (c << 16)
                if which < 2:
                    a = a | (lo & zero)
                hi = (a >> 16) | (c & jnp.uint32(0xFFFF0000))
                if which < 2:
                    tok = hi & zero
                    if j % HOP == HOP - 1:
                        tok = pltpu.roll(tok, 1, 1)
                else:
                    t = pltpu.roll(jnp.where(low16, hi, lo), 64, 1)
                    lo, hi = jnp.where(low16, lo, t), jnp.where(low16, t, hi)
                    both = hi if j % 2 == 0 else both | hi
                    if j % 2 == 1:
                        tok = both & zero
                s0 = which * H * PITCH + i * (DP // 2) + j
                wqkv_v[pl.ds(s0, 16, stride=PITCH), :] = lo
                wqkv_v[pl.ds(s0 + 16 * PITCH, 16, stride=PITCH), :] = hi
        o0 = pl.multiple_of(i * (OP // 2), OP // 2)
        for j in range(D // 128):
            for k in range(OP // 32):
                w = pltpu.bitcast(sto_v[ring, pl.ds(k * 32, 32), pl.ds(j * 128, 128)], U32) | tok
                tok = w & zero
                if k % (2 * HOP) == 2 * HOP - 1:
                    tok = pltpu.roll(tok, 1, 1)
                kd = k - k % 8 + (0, 1, 4, 5, 2, 3, 6, 7)[k % 8]
                wo_v[j, pl.ds(o0 + kd * 16, 16), :] = w

        h = _gelu(jnp.dot(lhs, w3_v[...], preferred_element_type=F32)).astype(BF16)
        b = jnp.dot(h, w4_v[...], preferred_element_type=F32) + x1_v[pl.ds(T2 + r0, T3), :]
        gw = gw_v[...].astype(F32).reshape(1, D)
        z = jnp.sum(x_v[pl.ds(r0, T3), :].astype(F32) * gw, axis=-1, keepdims=True)
        g = 1.0 / (1.0 + jnp.exp(-z))
        g_v[pl.ds(r0, T3), :] = jnp.broadcast_to(g, (T3, 128))
        b = (1.0 - g) * b
        for j in range(D // 128):
            h1_v[j, pl.ds(r0, T3), :] = b[:, j * 128:(j + 1) * 128]

        @pl.when(i + 1 < N3)
        def _():
            for c in piece_copies(i + 1, (i + 1) % NRING):
                c.wait()

        return carry

    with jax.named_scope('p3_body'):
        jax.lax.fori_loop(0, N3, p3_body, 0)

    mem_v[...] = mem0_v[...].astype(F32)
    c_exp = (DH ** -0.5) * math.log2(math.e)
    neg_raw = NEG / (DH ** -0.5)

    L2 = 2 * L

    def make_mask(ngv):
        rm = L - 8 * ngv
        row = jax.lax.broadcasted_iota(jnp.int32, (2 * rm, 128), 0)
        col = jax.lax.broadcasted_iota(jnp.int32, (2 * rm, 128), 1)
        second = row >= rm
        rowl = jnp.where(second, row - rm, row)
        coll = jnp.where(second, col - L, col)
        real = (coll >= 0) & (coll < L)
        allowed = real & ((rowl < M) | (rowl + 8 * ngv >= coll))
        return allowed, jnp.where(real, neg_raw, -jnp.inf).astype(F32)

    masks = {n: make_mask(n) for n in set(NGV_A + NGV_B)}
    neg_c = NEG * math.log2(math.e)

    def tied(w, toks):
        for tok in toks:
            w = jnp.concatenate([w[0:56], w[56:64] | tok, w[64:]], axis=0)
        return pltpu.bitcast(w, BF16)

    zpad = jnp.zeros((128 - L2, DH), F32)

    def recip(l):
        r = pl.reciprocal(l, approx=True)
        return r * (2.0 - l * r)

    def tree(op, x):
        while x.shape[0] > 1:
            x = op(x[0:x.shape[0] // 2], x[x.shape[0] // 2:])
        return x[0]

    causal = (jax.lax.broadcasted_iota(jnp.int32, (7, 8, 128), 1)
              > jax.lax.broadcasted_iota(jnp.int32, (7, 8, 128), 0))
    low = jax.lax.broadcasted_iota(jnp.int32, (8, 128), 1) < 64

    def stash(buf, slot, ks, ws, g):
        n = 8 * (g + 2)
        starts = []
        for i, x in enumerate(ks + ws):
            base = (4 * slot + i) * (L + 8)
            buf[pl.ds(base, n), :] = jnp.concatenate([x[8 * g:8 * g + 8], x[0:n - 8]], axis=0)
            starts.append(base + n - 8)
        return buf, starts, [jnp.sum(w[n - 8:L], axis=0, keepdims=True) if n - 8 < L
                             else jnp.zeros((1, DH), F32) for w in ws]

    def vpu_start(q0, q1, parked, g):
        buf, starts, (acc_a, acc_b) = parked
        return dict(q=(q0 * c_exp, q1 * c_exp), buf=buf, starts=starts, g=g,
                    m=jnp.full((8, 128), neg_c, F32),
                    l=jnp.full((8, 128), float(L - 8 * (g + 1)), F32), a=acc_a, b=acc_b)

    def vpu_chunk(st, c0, gate):
        def windows(start):
            return jnp.concatenate([st['buf'][pl.ds(start - r, 8), :]
                                    for r in range(c0, c0 + CHUNK)], axis=0).reshape(CHUNK, 8, 128)

        k0, k1, wa, wb = st['starts']
        q0, q1 = [pltpu.bitcast(pltpu.bitcast(q, U32) | gate, F32) for q in st['q']]
        sc = jnp.where(low, jnp.sum(q0 * windows(k0), axis=-1, keepdims=True),
                       jnp.sum(q1 * windows(k1), axis=-1, keepdims=True))
        if c0 == 8 * st['g']:
            sc = jnp.concatenate([sc[0:1], jnp.where(causal, sc[1:], neg_c)], axis=0)
        m = jnp.maximum(tree(jnp.maximum, sc), st['m'])
        alpha = jnp.exp2(st['m'] - m)
        pr = jnp.exp2(sc - m)
        new = []
        for old, x in ((st['l'], pr), (st['a'], pr * windows(wa)), (st['b'], pr * windows(wb))):
            new.append(jnp.sum(jnp.concatenate([(old * alpha)[None], x], axis=0), axis=0))
        st.update(m=m, l=new[0], a=new[1], b=new[2])
        return (pltpu.bitcast(new[0], U32) | pltpu.bitcast(new[1], U32)
                | pltpu.bitcast(new[2], U32))

    def vpu_finish(st):
        r = recip(st['l'])
        return st['a'] * r, st['b'] * r

    def segment(lhs_q, lhs_kv, wo_m, ngv, n_chunks, unpack, wo_rows, split_first, early, d_j, zero):
        NP = H // 2
        nj = D // 128
        HA = H - TAIL_H
        mxu_groups = [[0] + list(range(n + 1, 5)) for n in ngv]
        proj = {}
        qkv = [None] * NP
        pb = [None] * NP
        og = [dict() for _ in range(H)]
        ocat = {}
        y = [None] * nj

        def slab(toks, which, h, r0, n):
            x = lhs_q if which == 0 else lhs_kv
            w = tied(wqkv_v[pl.ds(_slab_of(which, h) * PITCH + r0, n), :], toks)
            r = jnp.dot(x[:, 2 * r0:2 * (r0 + n)], w, preferred_element_type=F32)
            proj[(which, h)] = r + proj[(which, h)] if (which, h) in proj else r
            return proj[(which, h)]

        def do_wo(toks, h0, h1, j):
            if (h0, h1) not in ocat:
                ocat[(h0, h1)] = jnp.concatenate(
                    [wo_rows(og[h]) for h in range(h0, h1)], axis=1).astype(BF16)
            w = tied(wo_v[j, pl.ds(h0 * 64, (h1 - h0) * 64), :], toks)
            r = jnp.dot(ocat[(h0, h1)], w, preferred_element_type=F32)
            y[j] = r if y[j] is None else r + y[j]
            return y[j]

        ticks = []
        pair_end = {}
        wo_early = [(4 * c, 4 * c + 4, j) for c in range(early) for j in range(nj)]
        first = NP - WO_SLOTS
        for p in range(NP):
            slabs = [(which, h) for h in (2 * p, 2 * p + 1) for which in range(3)]
            rows = [(lhs_q if w == 0 else lhs_kv).shape[0] for w, _ in slabs]
            if p == 0 and split_first:
                for r0 in (0, 256):
                    ticks += [(slab, (w, h, r0, 256), m) for (w, h), m in zip(slabs, rows)]
            else:
                mine = []
                if p >= first:
                    lo = (p - first) * len(wo_early) // WO_SLOTS
                    mine = wo_early[lo:(p - first + 1) * len(wo_early) // WO_SLOTS]
                for n, ((w, h), m) in enumerate(zip(slabs, rows)):
                    ticks += [(do_wo, item, wo_m)
                              for item in mine[n * len(mine) // 6:(n + 1) * len(mine) // 6]]
                    ticks.append((slab, (w, h, 0, 512), 2 * m + 8 * len(mxu_groups[p]) // 6))
            pair_end[len(ticks) - 1] = p
        ticks += [(do_wo, (h0, h0 + 4, j), wo_m)
                  for j in range(nj) for h0 in range(4 * early, HA, 4)]
        ends = []
        for _, _, dur in ticks:
            ends.append(dur + (ends[-1] if ends else 0))

        def index(t):
            return next(i for i, e in enumerate(ends) if e >= t)

        events = {}
        anchors = {}
        cursor = [0]

        def run_chunk(res, p, name, st, c0, i_done):
            done = vpu_chunk(st, c0, pltpu.bitcast(res[0:8], U32) & zero)
            anchors.setdefault(i_done, []).append(done & zero)
            if c0 + CHUNK >= 8 * (st['g'] + 1):
                og[2 * p][name], og[2 * p + 1][name] = vpu_finish(st)
                if D_R and ends[i_done - 1] + D_R < ends[-2]:
                    anchors.setdefault(index(ends[i_done - 1] + D_R) + 1, []).append(
                        pltpu.bitcast(og[2 * p][name], U32) & zero)

        def do_s(res, p):
            sc = jax.lax.dot_general(qkv[p][0], qkv[p][1], (((1,), (1,)), ((), ())),
                                     preferred_element_type=F32)
            allowed, fill = masks[ngv[p]]
            sc = jnp.where(allowed, sc, fill)
            e = jnp.exp2((sc - jnp.max(sc, axis=-1, keepdims=True)) * c_exp)
            l = jnp.sum(e, axis=-1, keepdims=True)
            e = e * recip(l)
            rm = 8 * len(mxu_groups[p])
            e = e[0:rm] + e[rm:2 * rm]
            if rm % 16:
                e = jnp.concatenate([e, jnp.zeros((8, 128), F32)], axis=0)
            pb[p] = e.astype(BF16)

        def do_pv(res, p):
            for i in range(2):
                o = jnp.dot(pb[p], qkv[p][2][i], preferred_element_type=F32)
                for n, g in enumerate(mxu_groups[p]):
                    og[2 * p + i][g] = o[8 * n:8 * n + 8]

        def finish_pair(p, i):
            u, jobs = unpack(p, [[proj[(w, h)] for w in range(3)] for h in (2 * p, 2 * p + 1)])
            chunks = [(name, st, c0) for name, st in
                      [(name, vpu_start(*job)) for name, job in jobs.items()]
                      for c0 in range(0, 8 * (st['g'] + 1), CHUNK)]
            t_first = ends[min(pair_end)] + D_G
            t_last = ends[-2] - d_j - D_F
            gap = (t_last - t_first) / (n_chunks - 1)
            if p == NP - 1:
                gap = min(gap, (t_last - max(ends[i] + D_G, cursor[0])) / (len(chunks) - 1))
            for chunk in chunks:
                t = max(ends[i] + D_G, cursor[0])
                cursor[0] = t + gap
                g = max(index(t), i + 1)
                events.setdefault(g, []).append(
                    (run_chunk, (p,) + chunk + (index(ends[g] + d_j) + 1,)))
            qb = jnp.concatenate([u[k][0][g] for k in range(2) for g in mxu_groups[p]],
                                 axis=0).astype(BF16)
            kb = jnp.concatenate([u[0][1], u[1][1], zpad], axis=0).astype(BF16)
            low40 = jnp.concatenate([low] * 5, axis=0)
            vb = [jnp.concatenate([jnp.where(low40, v, 0.0), jnp.where(low40, 0.0, v), zpad],
                                  axis=0).astype(BF16) for v in (u[0][2], u[1][2])]
            qkv[p] = (qb, kb, vb)
            t_pv = min(ends[i] + D_PV, ends[-1] - D_O)
            events.setdefault(index(min(ends[i] + D_S, t_pv - D_SM)), []).append((do_s, (p,)))
            events.setdefault(index(t_pv), []).append((do_pv, (p,)))

        for i, (fn, args, _) in enumerate(ticks):
            res = fn(anchors.pop(i, []), *args)
            if i in pair_end:
                finish_pair(pair_end[i], i)
            for f, a in events.pop(i, []):
                f(res, *a)
        assert not events
        for j in range(nj):
            do_wo([], HA, H, j)
        return jnp.concatenate(y, axis=1)

    def pair(r0, mem):
        xf = x_v[pl.ds(r0, PAIR), :].astype(F32)
        zero = zero_v[pl.ds(0, 8), :]
        x1s = jnp.concatenate([xf[0:8], xf[32:40]], axis=0).astype(BF16)
        keep = [None] * H

        def cat(*xs):
            return jnp.concatenate(xs, axis=0)

        lhs = cat(mem, xf[8:32]).astype(BF16)

        def finish(p, qg, ks, vs, slot, groups):
            return ([(qg[i], ks[i], vs[i]) for i in range(2)],
                    {g: stash(kv_v[p], slot + n, ks, vs, g) for n, g in enumerate(groups)})

        def unpack_a(p, qkv):
            qg = [{0: q[0:8], 2: q[8:16], 3: q[16:24], 4: q[24:32]} for q, _, _ in qkv]
            ks = [cat(k[0:8], k[32:40], k[8:32]) for _, k, _ in qkv]
            vs = [cat(v[0:8], v[32:40], v[8:32]) for _, _, v in qkv]
            u, parked = finish(p, qg, ks, vs, 0, range(1, NGV_A[p] + 1))
            keep[p] = (parked[1], [(k[40:48], v[40:48]) for _, k, v in qkv])
            return u, {g: (qg[0][g], qg[1][g], parked[g], g) for g in range(2, NGV_A[p] + 1)}

        y_a = segment(lhs, cat(lhs, x1s), 32, NGV_A,
                      sum(g + 1 for n in NGV_A for g in range(2, n + 1)) * 8 // CHUNK, unpack_a,
                      lambda o: cat(o[0], o[2], o[3], o[4]), False, EARLY_A, D_JA, zero)

        lhs = cat(y_a[0:8], xf[40:64]).astype(BF16)

        def unpack_b(p, qkv):
            parked_a1, kv1 = keep[p]
            qg = [{0: q[0:8], 1: q[40:48], 2: q[8:16], 3: q[16:24], 4: q[24:32]}
                  for q, _, _ in qkv]
            ks = [cat(k[0:8], e[0], k[8:32]) for (_, k, _), e in zip(qkv, kv1)]
            vs = [cat(v[0:8], e[1], v[8:32]) for (_, _, v), e in zip(qkv, kv1)]
            u, parked = finish(p, qg, ks, vs, max(NGV_A), range(1, NGV_B[p] + 1))
            jobs = {'a1': (qkv[0][0][32:40], qkv[1][0][32:40], parked_a1, 1)}
            jobs.update({g: (qg[0][g], qg[1][g], parked[g], g) for g in range(1, NGV_B[p] + 1)})
            return u, jobs

        y_b = segment(cat(lhs, x1s), lhs, 48, NGV_B,
                      sum(2 + sum(range(2, n + 2)) for n in NGV_B) * 8 // CHUNK, unpack_b,
                      lambda o: cat(o[0], o[1], o[2], o[3], o[4], o['a1']), True, EARLY_B,
                      D_JB, zero)

        a = cat(y_b[40:48], y_a[8:32], y_b[8:40])
        g = g_v[pl.ds(r0, PAIR), :]
        g = jnp.concatenate([g] * (D // 128), axis=1)
        out_v[pl.ds(r0, PAIR), :] = (g * a + h1_rows(r0, PAIR)).astype(BF16)
        return y_b[0:8]

    rows_it = UNROLL_A * PAIR

    def a_body(t, carry):
        base = pl.multiple_of(t * rows_it, rows_it)
        mem = mem_v[...]
        for u in range(UNROLL_A):
            mem = pair(pl.multiple_of(base + u * PAIR, PAIR), mem)
        mem_v[...] = mem
        pltpu.make_async_copy(out_v.at[pl.ds(base, rows_it)], out_hbm.at[pl.ds(base, rows_it)],
                              osem).start()
        return carry

    with jax.named_scope('a_body'):
        jax.lax.fori_loop(0, S // rows_it, a_body, 0)
    pltpu.make_async_copy(out_v, out_hbm, osem).wait()


@jax.jit
def pallas_gated_mix__memory_aug_recurrent_mem_tr__mixer_s_mlp__prompt_kernel(
    A_x, A_mem0, A_Wq, A_Wk, A_Wv, A_Wo, A_seg_len, B_x, B_w1, B_w2, B_w3, B_w4, gate_w,
):
    assert A_x.shape == (1, S, D) and A_Wq.shape == (D, H, DH) and A_mem0.shape == (1, M, D)
    x = A_x.reshape(S, D)
    mem0 = A_mem0.reshape(M, D)
    wq = A_Wq.reshape(D * H, DH)
    wk = A_Wk.reshape(D * H, DH)
    wv = A_Wv.reshape(D * H, DH)
    wo = A_Wo.reshape(H * DH, D)

    any_spec = pl.BlockSpec(memory_space=pl.ANY)
    out = pl.pallas_call(
        _kernel,
        out_shape=jax.ShapeDtypeStruct((S, D), BF16),
        in_specs=[any_spec] * 11,
        out_specs=any_spec,
        scratch_shapes=[
            pltpu.VMEM((S, D), BF16),
            pltpu.VMEM((NRING, 3, DP * H, DH), BF16),
            pltpu.VMEM((NRING, OP, D), BF16),
            pltpu.VMEM((3 * H * PITCH, 128), U32),
            pltpu.VMEM((D // 128, H * DH // 2, 128), U32),
            pltpu.VMEM((4, D, D // 4), BF16),
            pltpu.VMEM((4, D, D // 4), BF16),
            pltpu.VMEM((D, FF), BF16),
            pltpu.VMEM((FF, D), BF16),
            pltpu.VMEM((D // 128, S + 16, 128), F32),
            pltpu.VMEM((S + T2, D), F32),
            pltpu.VMEM((S, 128), F32),
            pltpu.VMEM((2, T1, D), BF16),
            pltpu.VMEM((2, T3, D), BF16),
            pltpu.VMEM((M, D), BF16),
            pltpu.VMEM((D,), BF16),
            pltpu.VMEM((M, D), F32),
            pltpu.VMEM((S, D), BF16),
            [pltpu.VMEM((NJOB * 4 * (L + 8), 128), F32)] * (H // 2),
            pltpu.VMEM((16, 128), U32),
            pltpu.SemaphoreType.DMA((NSEM,)),
            pltpu.SemaphoreType.DMA(()),
        ],
        compiler_params=pltpu.CompilerParams(vmem_limit_bytes=120 * 1024 * 1024,
                                             disable_bounds_checks=True),
    )(x, mem0, wq, wk, wv, wo, B_w1, B_w2, B_w3, B_w4, gate_w)
    return out.reshape(1, S, D)
```

```python
import math

import jax
import jax.numpy as jnp
import jax.experimental.pallas as pl
import jax.experimental.pallas.tpu as pltpu

F32 = jnp.float32
BF16 = jnp.bfloat16
U32 = jnp.uint32

S = 2048
D = 1024
H = 32
DH = 128
M = 8
SEG = 32
L = M + SEG
FF = 3584
PAIR = 2 * SEG
NPAIR = S // PAIR
T1 = 256
N1 = S // T1
T2 = 512
N2 = S // T2
T3 = 256
N3 = S // T3
DP = D // N3
OP = H * DH // N3
UNROLL_A = 1
PITCH = 520
NRING = 3
NSEM = 11 + NRING
EPS = 1e-5
NCHAIN0 = 10
NCHAIN1 = 5
LN1_ROWS = 8
HOP = 4
NGV_A = [3] * (H // 2)
NGV_B = [3, 3, 1, 3, 3, 3, 1, 3, 3, 3, 3, 3, 1, 3, 3, 3]
NJOB = max(NGV_A) + max(NGV_B)
EARLY_A = 2
EARLY_B = 3
WO_SLOTS = 10
CHUNK = 8
D_G = 0
D_JA = 510
D_JB = 650
D_F = 50
D_R = 0
HALF_A = False
HALF_B = False
TAIL_CM = False
ORDER_A = (0, 1, 2, 3, 4, 5)
ORDER_B = (0, 1, 2, 3, 4, 5)
D_S = 250
D_PV = 1000
D_SM = 600
D_O = 140
TAIL_H = 8
NEG = -1e9


def _gelu(x):
    c = math.sqrt(2.0 / math.pi)
    return 0.5 * x * (1.0 + jnp.tanh(c * (x + 0.044715 * (x * x * x))))


def _layernorm(x):
    m = jnp.mean(x, axis=-1, keepdims=True)
    xc = x - m
    v = jnp.mean(xc * xc, axis=-1, keepdims=True)
    return xc * jax.lax.rsqrt(v + EPS)


def _slab_of(which, h):
    return which * H + (h % 2) * (H // 2) + h // 2


def _kernel(x_hbm, mem0_hbm, wq_hbm, wk_hbm, wv_hbm, wo_hbm,
            w1_hbm, w2_hbm, w3_hbm, w4_hbm, gw_hbm,
            out_hbm,
            x_v, stq_v, sto_v, wqkv_v, wo_v, w1_v, w2_v, w3_v, w4_v,
            h1_v, x1_v, g_v, ln1_v, ln3_v, mem0_v, gw_v, mem_v, out_v, kv_v, zero_v, sems, osem):
    c4 = D // 4
    xcuts = (0, 1, 2, 3, 5, N1)
    cp_x = [pltpu.make_async_copy(x_hbm.at[pl.ds(lo * T1, (hi - lo) * T1)],
                                  x_v.at[pl.ds(lo * T1, (hi - lo) * T1)], sems.at[n])
            for n, (lo, hi) in enumerate(zip(xcuts[:-1], xcuts[1:]))]
    cp_w1 = [pltpu.make_async_copy(w1_hbm.at[:, pl.ds(q * c4, c4)], w1_v.at[q], sems.at[5 + q])
             for q in range(4)]
    cp_w2 = [pltpu.make_async_copy(w2_hbm.at[:, pl.ds(q * c4, c4)], w2_v.at[q], sems.at[9])
             for q in range(4)]
    cp_ffn = [pltpu.make_async_copy(src, dst, sems.at[10])
              for src, dst in ((gw_hbm, gw_v), (mem0_hbm, mem0_v), (w3_hbm, w3_v), (w4_hbm, w4_v))]

    def piece_copies(i, slot):
        cps = [pltpu.make_async_copy(w.at[pl.ds(i * (DP * H), DP * H)], stq_v.at[slot, k],
                                     sems.at[11 + slot])
               for k, w in enumerate((wq_hbm, wk_hbm, wv_hbm))]
        cps.append(pltpu.make_async_copy(wo_hbm.at[pl.ds(i * OP, OP)], sto_v.at[slot],
                                         sems.at[11 + slot]))
        return cps

    for c in (cp_x[0:1] + cp_w1 + cp_x[1:] + cp_w2 + cp_ffn
              + piece_copies(0, 0) + piece_copies(1, 1)):
        c.start()
    x1_v[pl.ds(0, T3), :] = jnp.zeros((T3, D), F32)
    h1_v[:, pl.ds(8, 8), :] = jnp.zeros((D // 128, 8, 128), F32)
    h1_v[:, pl.ds(S, 8), :] = jnp.zeros((D // 128, 8, 128), F32)
    zero_v[...] = jnp.zeros((16, 128), U32)

    def ln_rows(x, tok, zero):
        if tok is not None:
            head = pltpu.bitcast(pltpu.bitcast(x[:, 0:128], U32) | tok, F32)
            x = jnp.concatenate([head, x[:, 128:]], axis=1)
        y = _layernorm(x)
        tok = None if zero is None else pltpu.bitcast(y[:, 0:128], U32) & zero
        return y, tok

    def ln_block(load, store, rows, nchain, gr):
        zero = zero_v[pl.ds(0, gr), :] if nchain else None
        toks = [None] * max(nchain, 1)
        for k in range(rows // gr):
            y, toks[k % len(toks)] = ln_rows(load(k * gr, gr), toks[k % len(toks)], zero)
            store(k * gr, y.astype(BF16))
        return toks[(rows // gr - 1) % len(toks)]

    def prep1(blk, slot, nchain):
        r0 = blk * T1 if isinstance(blk, int) else pl.multiple_of(blk * T1, T1)

        def store(k, y):
            ln1_v[slot, pl.ds(k, y.shape[0]), :] = y

        ln_block(lambda k, n: x_v[pl.ds(r0 + k, n), :].astype(F32), store, T1, nchain, LN1_ROWS)

    def p1_quarter(lhs, r0, q):
        h = _gelu(jnp.dot(lhs, w1_v[q], preferred_element_type=F32))
        for j in range(2):
            win = h1_v.at[2 * q + j, pl.ds(r0, T1 + 16)]
            win[pl.ds(8 + (1, -1, 2, -2)[q], T1), :] = h[:, j * 128:(j + 1) * 128]

    cp_x[0].wait()
    prep1(0, 0, 0)
    for q in range(4):
        cp_w1[q].wait()
        if q == 3:
            cp_x[1].wait()
        lhs = ln1_v[0]
        if q == 3:
            prep1(1, 1, NCHAIN0)
        p1_quarter(lhs, 0, q)

    def p1_body(i, carry):
        r0 = pl.multiple_of(i * T1, T1)
        slot = i & 1

        lhs = ln1_v[slot]
        prep1(jnp.minimum(i + 1, N1 - 1), 1 - slot, NCHAIN1)
        for q in range(4):
            p1_quarter(lhs, r0, q)
        for n in range(3, len(cp_x)):
            pl.when(i + 2 == xcuts[n])(cp_x[n].wait)
        return carry

    cp_x[2].wait()
    with jax.named_scope('p1_body'):
        jax.lax.fori_loop(1, N1, p1_body, 0)
    for c in cp_w2:
        c.wait()

    def h1_rows(r0, n):
        return jnp.concatenate([h1_v[j, pl.ds(r0, n), :] for j in range(D // 128)], axis=1)

    def prep3(src, slot):
        def store(k, y):
            ln3_v[slot, pl.ds(k, y.shape[0]), :] = y

        return ln_block(lambda k, n: src[pl.ds(k, n), :], store, T3, 1, 16)

    def p2_body(i, carry):
        r0 = pl.multiple_of(i * T2, T2)
        win = x1_v.at[pl.ds(r0, 2 * T2)]
        prep3(win, 0)
        hs = h1_rows(r0 + 8, T2).astype(BF16)
        for q in range(4):
            win[pl.ds(T2, T2), pl.ds(q * c4, c4)] = (
                jnp.dot(hs, w2_v[q], preferred_element_type=F32)
                + x_v[pl.ds(r0, T2), pl.ds(q * c4, c4)].astype(F32))
        return carry

    with jax.named_scope('p2_body'):
        jax.lax.fori_loop(0, N2, p2_body, 0)

    for c in cp_ffn + piece_copies(0, 0):
        c.wait()
    blk0 = (N2 - 2) * T2 // T3

    def p3_body(i, carry):
        r0 = pl.multiple_of((i + blk0) % N3 * T3, T3)
        r_next = pl.multiple_of((i + 1 + blk0) % N3 * T3, T3)
        slot = i & 1
        ring = i % NRING

        @pl.when(i + 2 < N3)
        def _():
            for c in piece_copies(i + 2, (i + 2) % NRING):
                c.start()

        lhs = ln3_v[slot]
        tok = prep3(x1_v.at[pl.ds(T2 + r_next, T3)], 1 - slot)
        zero = zero_v[...]
        low16 = jax.lax.broadcasted_iota(jnp.int32, (16, 128), 1) < 64
        for which in range(3):
            for j in range(DP // 2):
                blk = pltpu.bitcast(stq_v[ring, which, pl.ds(j * 64, 64), :], U32)
                a = blk[0:16] | tok
                c = blk[16:32]
                lo = (a & jnp.uint32(0xFFFF)) | (c << 16)
                if which < 2:
                    a = a | (lo & zero)
                hi = (a >> 16) | (c & jnp.uint32(0xFFFF0000))
                if which < 2:
                    tok = hi & zero
                    if j % HOP == HOP - 1:
                        tok = pltpu.roll(tok, 1, 1)
                else:
                    t = pltpu.roll(jnp.where(low16, hi, lo), 64, 1)
                    lo, hi = jnp.where(low16, lo, t), jnp.where(low16, t, hi)
                    both = hi if j % 2 == 0 else both | hi
                    if j % 2 == 1:
                        tok = both & zero
                s0 = which * H * PITCH + i * (DP // 2) + j
                wqkv_v[pl.ds(s0, 16, stride=PITCH), :] = lo
                wqkv_v[pl.ds(s0 + 16 * PITCH, 16, stride=PITCH), :] = hi
        o0 = pl.multiple_of(i * (OP // 2), OP // 2)
        for j in range(D // 128):
            for k in range(OP // 32):
                w = pltpu.bitcast(sto_v[ring, pl.ds(k * 32, 32), pl.ds(j * 128, 128)], U32) | tok
                tok = w & zero
                if k % (2 * HOP) == 2 * HOP - 1:
                    tok = pltpu.roll(tok, 1, 1)
                kd = k - k % 8 + (0, 1, 4, 5, 2, 3, 6, 7)[k % 8]
                wo_v[j, pl.ds(o0 + kd * 16, 16), :] = w

        h = _gelu(jnp.dot(lhs, w3_v[...], preferred_element_type=F32)).astype(BF16)
        b = jnp.dot(h, w4_v[...], preferred_element_type=F32) + x1_v[pl.ds(T2 + r0, T3), :]
        gw = gw_v[...].astype(F32).reshape(1, D)
        z = jnp.sum(x_v[pl.ds(r0, T3), :].astype(F32) * gw, axis=-1, keepdims=True)
        g = 1.0 / (1.0 + jnp.exp(-z))
        g_v[pl.ds(r0, T3), :] = jnp.broadcast_to(g, (T3, 128))
        b = (1.0 - g) * b
        for j in range(D // 128):
            h1_v[j, pl.ds(r0, T3), :] = b[:, j * 128:(j + 1) * 128]

        @pl.when(i + 1 < N3)
        def _():
            for c in piece_copies(i + 1, (i + 1) % NRING):
                c.wait()

        return carry

    with jax.named_scope('p3_body'):
        jax.lax.fori_loop(0, N3, p3_body, 0)

    mem_v[...] = mem0_v[...].astype(F32)
    c_exp = (DH ** -0.5) * math.log2(math.e)
    neg_raw = NEG / (DH ** -0.5)

    L2 = 2 * L

    def make_mask(ngv):
        rm = L - 8 * ngv
        row = jax.lax.broadcasted_iota(jnp.int32, (2 * rm, 128), 0)
        col = jax.lax.broadcasted_iota(jnp.int32, (2 * rm, 128), 1)
        second = row >= rm
        rowl = jnp.where(second, row - rm, row)
        coll = jnp.where(second, col - L, col)
        real = (coll >= 0) & (coll < L)
        allowed = real & ((rowl < M) | (rowl + 8 * ngv >= coll))
        fill = jnp.where(allowed, 0.0, jnp.where(real, neg_raw, -jnp.inf)).astype(F32)
        return jnp.where(allowed, jnp.uint32(0xFFFFFFFF), jnp.uint32(0)), pltpu.bitcast(fill, U32)

    masks = {n: make_mask(n) for n in set(NGV_A + NGV_B)}
    neg_c = NEG * math.log2(math.e)

    def tied(w, toks):
        for tok in toks:
            w = jnp.concatenate([w[0:56], w[56:64] | tok, w[64:]], axis=0)
        return pltpu.bitcast(w, BF16)

    zpad = jnp.zeros((128 - L2, DH), F32)

    def recip(l):
        r = pl.reciprocal(l, approx=True)
        return r * (2.0 - l * r)

    def tree(op, x):
        while x.shape[0] > 1:
            x = op(x[0:x.shape[0] // 2], x[x.shape[0] // 2:])
        return x[0]

    causal = (jax.lax.broadcasted_iota(jnp.int32, (7, 8, 128), 1)
              > jax.lax.broadcasted_iota(jnp.int32, (7, 8, 128), 0))
    low = jax.lax.broadcasted_iota(jnp.int32, (8, 128), 1) < 64

    def stash(buf, slot, ks, ws, g):
        n = 8 * (g + 2)
        starts = []
        for i, x in enumerate(ks + ws):
            base = (4 * slot + i) * (L + 8)
            buf[pl.ds(base, n), :] = jnp.concatenate([x[8 * g:8 * g + 8], x[0:n - 8]], axis=0)
            starts.append(base + n - 8)
        return buf, starts, [jnp.sum(w[n - 8:L], axis=0, keepdims=True) if n - 8 < L
                             else jnp.zeros((1, DH), F32) for w in ws]

    def vpu_start(q0, q1, parked, g):
        buf, starts, (acc_a, acc_b) = parked
        return dict(q=(q0 * c_exp, q1 * c_exp), buf=buf, starts=starts, g=g,
                    m=jnp.full((8, 128), neg_c, F32),
                    l=jnp.full((8, 128), float(L - 8 * (g + 1)), F32), a=acc_a, b=acc_b)

    def vpu_chunk(st, c0, gate):
        def windows(start):
            return jnp.concatenate([st['buf'][pl.ds(start - r, 8), :]
                                    for r in range(c0, c0 + CHUNK)], axis=0).reshape(CHUNK, 8, 128)

        k0, k1, wa, wb = st['starts']
        q0, q1 = [pltpu.bitcast(pltpu.bitcast(q, U32) | gate, F32) for q in st['q']]
        sc = jnp.where(low, jnp.sum(q0 * windows(k0), axis=-1, keepdims=True),
                       jnp.sum(q1 * windows(k1), axis=-1, keepdims=True))
        if c0 == 8 * st['g']:
            sc = jnp.concatenate([sc[0:1], jnp.where(causal, sc[1:], neg_c)], axis=0)
        m = jnp.maximum(tree(jnp.maximum, sc), st['m'])
        alpha = jnp.exp2(st['m'] - m)
        pr = jnp.exp2(sc - m)
        new = []
        for old, x in ((st['l'], pr), (st['a'], pr * windows(wa)), (st['b'], pr * windows(wb))):
            new.append(jnp.sum(jnp.concatenate([(old * alpha)[None], x], axis=0), axis=0))
        st.update(m=m, l=new[0], a=new[1], b=new[2])
        return (pltpu.bitcast(new[0], U32) | pltpu.bitcast(new[1], U32)
                | pltpu.bitcast(new[2], U32))

    def vpu_finish(st):
        r = recip(st['l'])
        return st['a'] * r, st['b'] * r

    def segment(lhs_q, lhs_kv, wo_m, ngv, n_chunks, unpack, wo_rows, split_first, early, d_j, order, half, zero):
        NP = H // 2
        nj = D // 128
        HA = H - TAIL_H
        mxu_groups = [[0] + list(range(n + 1, 5)) for n in ngv]
        proj = {}
        qkv = [None] * NP
        pb = [None] * NP
        og = [dict() for _ in range(H)]
        ocat = {}
        y = [None] * nj

        def slab(toks, which, h, r0, n):
            x = lhs_q if which == 0 else lhs_kv
            w = tied(wqkv_v[pl.ds(_slab_of(which, h) * PITCH + r0, n), :], toks)
            r = jnp.dot(x[:, 2 * r0:2 * (r0 + n)], w, preferred_element_type=F32)
            proj[(which, h)] = r + proj[(which, h)] if (which, h) in proj else r
            return proj[(which, h)]

        def do_wo(toks, h0, h1, j):
            if (h0, h1) not in ocat:
                ocat[(h0, h1)] = jnp.concatenate(
                    [wo_rows(og[h]) for h in range(h0, h1)], axis=1).astype(BF16)
            w = tied(wo_v[j, pl.ds(h0 * 64, (h1 - h0) * 64), :], toks)
            r = jnp.dot(ocat[(h0, h1)], w, preferred_element_type=F32)
            y[j] = r if y[j] is None else r + y[j]
            return y[j]

        ticks = []
        pair_end = {}
        wo_early = [(4 * c, 4 * c + 4, j) for c in range(early) for j in range(nj)]
        first = NP - WO_SLOTS
        for p in range(NP):
            slabs = [(k % 3, 2 * p + k // 3) for k in order]
            rows = [(lhs_q if w == 0 else lhs_kv).shape[0] for w, _ in slabs]
            if p == 0 and split_first:
                for r0 in (0, 256):
                    ticks += [(slab, (w, h, r0, 256), m) for (w, h), m in zip(slabs, rows)]
            else:
                mine = []
                if p >= first:
                    lo = (p - first) * len(wo_early) // WO_SLOTS
                    mine = wo_early[lo:(p - first + 1) * len(wo_early) // WO_SLOTS]
                att = 8 * len(mxu_groups[p])
                if half:
                    units = [(slab, slabs[k] + (r0, 256), rows[k] + att / 12)
                             for k0 in (0, 3) for r0 in (0, 256) for k in range(k0, k0 + 3)]
                else:
                    units = [(slab, slabs[k] + (0, 512), 2 * rows[k] + att // 6) for k in range(6)]
                for n, unit in enumerate(units):
                    ticks += [(do_wo, item, wo_m) for item in
                              mine[n * len(mine) // len(units):(n + 1) * len(mine) // len(units)]]
                    ticks.append(unit)
            pair_end[len(ticks) - 1] = p
        tail = [(h0, h0 + 4, j) for j in range(nj) for h0 in range(4 * early, HA, 4)]
        ticks += [(do_wo, item, wo_m) for item in (sorted(tail) if TAIL_CM else tail)]
        ends = []
        for _, _, dur in ticks:
            ends.append(dur + (ends[-1] if ends else 0))

        def index(t):
            return next(i for i, e in enumerate(ends) if e >= t)

        events = {}
        anchors = {}
        cursor = [0]

        def run_chunk(res, p, name, st, c0, i_done):
            done = vpu_chunk(st, c0, pltpu.bitcast(res[0:8], U32) & zero)
            anchors.setdefault(i_done, []).append(done & zero)
            if c0 + CHUNK >= 8 * (st['g'] + 1):
                og[2 * p][name], og[2 * p + 1][name] = vpu_finish(st)
                if D_R and ends[i_done - 1] + D_R < ends[-2]:
                    anchors.setdefault(index(ends[i_done - 1] + D_R) + 1, []).append(
                        pltpu.bitcast(og[2 * p][name], U32) & zero)

        def do_s(res, p):
            sc = jax.lax.dot_general(qkv[p][0], qkv[p][1], (((1,), (1,)), ((), ())),
                                     preferred_element_type=F32)
            keep, fill = masks[ngv[p]]
            sc = pltpu.bitcast((pltpu.bitcast(sc, U32) & keep) | fill, F32)
            e = jnp.exp2((sc - jnp.max(sc, axis=-1, keepdims=True)) * c_exp)
            l = jnp.sum(e, axis=-1, keepdims=True)
            e = e * recip(l)
            rm = 8 * len(mxu_groups[p])
            e = e[0:rm] + e[rm:2 * rm]
            if rm % 16:
                e = jnp.concatenate([e, jnp.zeros((8, 128), F32)], axis=0)
            pb[p] = e.astype(BF16)

        def do_pv(res, p):
            for i in range(2):
                o = jnp.dot(pb[p], qkv[p][2][i], preferred_element_type=F32)
                for n, g in enumerate(mxu_groups[p]):
                    og[2 * p + i][g] = o[8 * n:8 * n + 8]

        def finish_pair(p, i):
            u, jobs = unpack(p, [[proj[(w, h)] for w in range(3)] for h in (2 * p, 2 * p + 1)])
            chunks = [(name, st, c0) for name, st in
                      [(name, vpu_start(*job)) for name, job in jobs.items()]
                      for c0 in range(0, 8 * (st['g'] + 1), CHUNK)]
            t_first = ends[min(pair_end)] + D_G
            t_last = ends[-2] - d_j - D_F
            gap = (t_last - t_first) / (n_chunks - 1)
            if p == NP - 1:
                gap = min(gap, (t_last - max(ends[i] + D_G, cursor[0])) / (len(chunks) - 1))
            for chunk in chunks:
                t = max(ends[i] + D_G, cursor[0])
                cursor[0] = t + gap
                g = max(index(t), i + 1)
                events.setdefault(g, []).append(
                    (run_chunk, (p,) + chunk + (index(ends[g] + d_j) + 1,)))
            qb = jnp.concatenate([u[k][0][g] for k in range(2) for g in mxu_groups[p]],
                                 axis=0).astype(BF16)
            kb = jnp.concatenate([u[0][1], u[1][1], zpad], axis=0).astype(BF16)
            low40 = jnp.concatenate([low] * 5, axis=0)
            vb = [jnp.concatenate([jnp.where(low40, v, 0.0), jnp.where(low40, 0.0, v), zpad],
                                  axis=0).astype(BF16) for v in (u[0][2], u[1][2])]
            qkv[p] = (qb, kb, vb)
            t_pv = min(ends[i] + D_PV, ends[-1] - D_O)
            events.setdefault(index(min(ends[i] + D_S, t_pv - D_SM)), []).append((do_s, (p,)))
            events.setdefault(index(t_pv), []).append((do_pv, (p,)))

        for i, (fn, args, _) in enumerate(ticks):
            res = fn(anchors.pop(i, []), *args)
            if i in pair_end:
                finish_pair(pair_end[i], i)
            for f, a in events.pop(i, []):
                f(res, *a)
        assert not events
        for j in range(nj):
            do_wo([], HA, H, j)
        return jnp.concatenate(y, axis=1)

    def pair(r0, mem):
        xf = x_v[pl.ds(r0, PAIR), :].astype(F32)
        zero = zero_v[pl.ds(0, 8), :]
        x1s = jnp.concatenate([xf[0:8], xf[32:40]], axis=0).astype(BF16)
        keep = [None] * H

        def cat(*xs):
            return jnp.concatenate(xs, axis=0)

        lhs = cat(mem, xf[8:32]).astype(BF16)

        def finish(p, qg, ks, vs, slot, groups):
            return ([(qg[i], ks[i], vs[i]) for i in range(2)],
                    {g: stash(kv_v[p], slot + n, ks, vs, g) for n, g in enumerate(groups)})

        def unpack_a(p, qkv):
            qg = [{0: q[0:8], 2: q[8:16], 3: q[16:24], 4: q[24:32]} for q, _, _ in qkv]
            ks = [cat(k[0:8], k[32:40], k[8:32]) for _, k, _ in qkv]
            vs = [cat(v[0:8], v[32:40], v[8:32]) for _, _, v in qkv]
            u, parked = finish(p, qg, ks, vs, 0, range(1, NGV_A[p] + 1))
            keep[p] = (parked[1], [(k[40:48], v[40:48]) for _, k, v in qkv])
            return u, {g: (qg[0][g], qg[1][g], parked[g], g) for g in range(2, NGV_A[p] + 1)}

        y_a = segment(lhs, cat(lhs, x1s), 32, NGV_A,
                      sum(g + 1 for n in NGV_A for g in range(2, n + 1)) * 8 // CHUNK, unpack_a,
                      lambda o: cat(o[0], o[2], o[3], o[4]), False, EARLY_A, D_JA, ORDER_A, HALF_A, zero)

        lhs = cat(y_a[0:8], xf[40:64]).astype(BF16)

        def unpack_b(p, qkv):
            parked_a1, kv1 = keep[p]
            qg = [{0: q[0:8], 1: q[40:48], 2: q[8:16], 3: q[16:24], 4: q[24:32]}
                  for q, _, _ in qkv]
            ks = [cat(k[0:8], e[0], k[8:32]) for (_, k, _), e in zip(qkv, kv1)]
            vs = [cat(v[0:8], e[1], v[8:32]) for (_, _, v), e in zip(qkv, kv1)]
            u, parked = finish(p, qg, ks, vs, max(NGV_A), range(1, NGV_B[p] + 1))
            jobs = {'a1': (qkv[0][0][32:40], qkv[1][0][32:40], parked_a1, 1)}
            jobs.update({g: (qg[0][g], qg[1][g], parked[g], g) for g in range(1, NGV_B[p] + 1)})
            return u, jobs

        y_b = segment(cat(lhs, x1s), lhs, 48, NGV_B,
                      sum(2 + sum(range(2, n + 2)) for n in NGV_B) * 8 // CHUNK, unpack_b,
                      lambda o: cat(o[0], o[1], o[2], o[3], o[4], o['a1']), True, EARLY_B,
                      D_JB, ORDER_B, HALF_B, zero)

        a = cat(y_b[40:48], y_a[8:32], y_b[8:40])
        g = g_v[pl.ds(r0, PAIR), :]
        g = jnp.concatenate([g] * (D // 128), axis=1)
        out_v[pl.ds(r0, PAIR), :] = (g * a + h1_rows(r0, PAIR)).astype(BF16)
        return y_b[0:8]

    rows_it = UNROLL_A * PAIR

    def a_body(t, carry):
        base = pl.multiple_of(t * rows_it, rows_it)
        mem = mem_v[...]
        for u in range(UNROLL_A):
            mem = pair(pl.multiple_of(base + u * PAIR, PAIR), mem)
        mem_v[...] = mem
        pltpu.make_async_copy(out_v.at[pl.ds(base, rows_it)], out_hbm.at[pl.ds(base, rows_it)],
                              osem).start()
        return carry

    with jax.named_scope('a_body'):
        jax.lax.fori_loop(0, S // rows_it, a_body, 0)
    pltpu.make_async_copy(out_v, out_hbm, osem).wait()


@jax.jit
def pallas_gated_mix__memory_aug_recurrent_mem_tr__mixer_s_mlp__prompt_kernel(
    A_x, A_mem0, A_Wq, A_Wk, A_Wv, A_Wo, A_seg_len, B_x, B_w1, B_w2, B_w3, B_w4, gate_w,
):
    assert A_x.shape == (1, S, D) and A_Wq.shape == (D, H, DH) and A_mem0.shape == (1, M, D)
    x = A_x.reshape(S, D)
    mem0 = A_mem0.reshape(M, D)
    wq = A_Wq.reshape(D * H, DH)
    wk = A_Wk.reshape(D * H, DH)
    wv = A_Wv.reshape(D * H, DH)
    wo = A_Wo.reshape(H * DH, D)

    any_spec = pl.BlockSpec(memory_space=pl.ANY)
    out = pl.pallas_call(
        _kernel,
        out_shape=jax.ShapeDtypeStruct((S, D), BF16),
        in_specs=[any_spec] * 11,
        out_specs=any_spec,
        scratch_shapes=[
            pltpu.VMEM((S, D), BF16),
            pltpu.VMEM((NRING, 3, DP * H, DH), BF16),
            pltpu.VMEM((NRING, OP, D), BF16),
            pltpu.VMEM((3 * H * PITCH, 128), U32),
            pltpu.VMEM((D // 128, H * DH // 2, 128), U32),
            pltpu.VMEM((4, D, D // 4), BF16),
            pltpu.VMEM((4, D, D // 4), BF16),
            pltpu.VMEM((D, FF), BF16),
            pltpu.VMEM((FF, D), BF16),
            pltpu.VMEM((D // 128, S + 16, 128), F32),
            pltpu.VMEM((S + T2, D), F32),
            pltpu.VMEM((S, 128), F32),
            pltpu.VMEM((2, T1, D), BF16),
            pltpu.VMEM((2, T3, D), BF16),
            pltpu.VMEM((M, D), BF16),
            pltpu.VMEM((D,), BF16),
            pltpu.VMEM((M, D), F32),
            pltpu.VMEM((S, D), BF16),
            [pltpu.VMEM((NJOB * 4 * (L + 8), 128), F32)] * (H // 2),
            pltpu.VMEM((16, 128), U32),
            pltpu.SemaphoreType.DMA((NSEM,)),
            pltpu.SemaphoreType.DMA(()),
        ],
        compiler_params=pltpu.CompilerParams(vmem_limit_bytes=120 * 1024 * 1024,
                                             disable_bounds_checks=True),
    )(x, mem0, wq, wk, wv, wo, B_w1, B_w2, B_w3, B_w4, gate_w)
    return out.reshape(1, S, D)
```

```python
import math

import jax
import jax.numpy as jnp
import jax.experimental.pallas as pl
import jax.experimental.pallas.tpu as pltpu

F32 = jnp.float32
BF16 = jnp.bfloat16
U32 = jnp.uint32

S = 2048
D = 1024
H = 32
DH = 128
M = 8
SEG = 32
L = M + SEG
FF = 3584
PAIR = 2 * SEG
NPAIR = S // PAIR
T1 = 256
N1 = S // T1
T2 = 512
N2 = S // T2
T3 = 256
N3 = S // T3
DP = D // N3
OP = H * DH // N3
UNROLL_A = 1
PITCH = 520
NRING = 3
NSEM = 11 + NRING
EPS = 1e-5
NCHAIN0 = 10
NCHAIN1 = 5
LN1_ROWS = 8
HOP = 4
NGV_A = [3] * (H // 2)
NGV_B = [3, 3, 1, 3, 3, 3, 1, 3, 3, 3, 3, 3, 1, 3, 3, 3]
NJOB = max(NGV_A) + max(NGV_B)
EARLY_A = 2
EARLY_B = 3
WO_SLOTS = 10
CHUNK = 8
D_G = 0
D_JA = 510
D_JB = 530
D_F = 50
D_R = 0
HALF_A = True
HALF_B = True
TAIL_CM = True
ORDER_A = (0, 1, 2, 3, 4, 5)
ORDER_B = (0, 1, 2, 3, 4, 5)
D_S = 250
D_PV = 1400
D_SM = 600
D_O = 170
TAIL_H = 8
NEG = -1e9


def _gelu(x):
    c = math.sqrt(2.0 / math.pi)
    return 0.5 * x * (1.0 + jnp.tanh(c * (x + 0.044715 * (x * x * x))))


def _layernorm(x):
    m = jnp.mean(x, axis=-1, keepdims=True)
    xc = x - m
    v = jnp.mean(xc * xc, axis=-1, keepdims=True)
    return xc * jax.lax.rsqrt(v + EPS)


def _slab_of(which, h):
    return which * H + (h % 2) * (H // 2) + h // 2


def _kernel(x_hbm, mem0_hbm, wq_hbm, wk_hbm, wv_hbm, wo_hbm,
            w1_hbm, w2_hbm, w3_hbm, w4_hbm, gw_hbm,
            out_hbm,
            x_v, stq_v, sto_v, wqkv_v, wo_v, w1_v, w2_v, w3_v, w4_v,
            h1_v, x1_v, g_v, ln1_v, ln3_v, mem0_v, gw_v, mem_v, out_v, kv_v, zero_v, sems, osem):
    c4 = D // 4
    xcuts = (0, 1, 2, 3, 5, N1)
    cp_x = [pltpu.make_async_copy(x_hbm.at[pl.ds(lo * T1, (hi - lo) * T1)],
                                  x_v.at[pl.ds(lo * T1, (hi - lo) * T1)], sems.at[n])
            for n, (lo, hi) in enumerate(zip(xcuts[:-1], xcuts[1:]))]
    cp_w1 = [pltpu.make_async_copy(w1_hbm.at[:, pl.ds(q * c4, c4)], w1_v.at[q], sems.at[5 + q])
             for q in range(4)]
    cp_w2 = [pltpu.make_async_copy(w2_hbm.at[:, pl.ds(q * c4, c4)], w2_v.at[q], sems.at[9])
             for q in range(4)]
    cp_ffn = [pltpu.make_async_copy(src, dst, sems.at[10])
              for src, dst in ((gw_hbm, gw_v), (mem0_hbm, mem0_v), (w3_hbm, w3_v), (w4_hbm, w4_v))]

    def piece_copies(i, slot):
        cps = [pltpu.make_async_copy(w.at[pl.ds(i * (DP * H), DP * H)], stq_v.at[slot, k],
                                     sems.at[11 + slot])
               for k, w in enumerate((wq_hbm, wk_hbm, wv_hbm))]
        cps.append(pltpu.make_async_copy(wo_hbm.at[pl.ds(i * OP, OP)], sto_v.at[slot],
                                         sems.at[11 + slot]))
        return cps

    for c in (cp_x[0:1] + cp_w1 + cp_x[1:] + cp_w2 + cp_ffn
              + piece_copies(0, 0) + piece_copies(1, 1)):
        c.start()
    x1_v[pl.ds(0, T3), :] = jnp.zeros((T3, D), F32)
    h1_v[:, pl.ds(8, 8), :] = jnp.zeros((D // 128, 8, 128), F32)
    h1_v[:, pl.ds(S, 8), :] = jnp.zeros((D // 128, 8, 128), F32)
    zero_v[...] = jnp.zeros((16, 128), U32)

    def ln_rows(x, tok, zero):
        if tok is not None:
            head = pltpu.bitcast(pltpu.bitcast(x[:, 0:128], U32) | tok, F32)
            x = jnp.concatenate([head, x[:, 128:]], axis=1)
        y = _layernorm(x)
        tok = None if zero is None else pltpu.bitcast(y[:, 0:128], U32) & zero
        return y, tok

    def ln_block(load, store, rows, nchain, gr):
        zero = zero_v[pl.ds(0, gr), :] if nchain else None
        toks = [None] * max(nchain, 1)
        for k in range(rows // gr):
            y, toks[k % len(toks)] = ln_rows(load(k * gr, gr), toks[k % len(toks)], zero)
            store(k * gr, y.astype(BF16))
        return toks[(rows // gr - 1) % len(toks)]

    def prep1(blk, slot, nchain):
        r0 = blk * T1 if isinstance(blk, int) else pl.multiple_of(blk * T1, T1)

        def store(k, y):
            ln1_v[slot, pl.ds(k, y.shape[0]), :] = y

        ln_block(lambda k, n: x_v[pl.ds(r0 + k, n), :].astype(F32), store, T1, nchain, LN1_ROWS)

    def p1_quarter(lhs, r0, q):
        h = _gelu(jnp.dot(lhs, w1_v[q], preferred_element_type=F32))
        for j in range(2):
            win = h1_v.at[2 * q + j, pl.ds(r0, T1 + 16)]
            win[pl.ds(8 + (1, -1, 2, -2)[q], T1), :] = h[:, j * 128:(j + 1) * 128]

    cp_x[0].wait()
    prep1(0, 0, 0)
    for q in range(4):
        cp_w1[q].wait()
        if q == 3:
            cp_x[1].wait()
        lhs = ln1_v[0]
        if q == 3:
            prep1(1, 1, NCHAIN0)
        p1_quarter(lhs, 0, q)

    def p1_body(i, carry):
        r0 = pl.multiple_of(i * T1, T1)
        slot = i & 1

        lhs = ln1_v[slot]
        prep1(jnp.minimum(i + 1, N1 - 1), 1 - slot, NCHAIN1)
        for q in range(4):
            p1_quarter(lhs, r0, q)
        for n in range(3, len(cp_x)):
            pl.when(i + 2 == xcuts[n])(cp_x[n].wait)
        return carry

    cp_x[2].wait()
    with jax.named_scope('p1_body'):
        jax.lax.fori_loop(1, N1, p1_body, 0)
    for c in cp_w2:
        c.wait()

    def h1_rows(r0, n):
        return jnp.concatenate([h1_v[j, pl.ds(r0, n), :] for j in range(D // 128)], axis=1)

    def prep3(src, slot):
        def store(k, y):
            ln3_v[slot, pl.ds(k, y.shape[0]), :] = y

        return ln_block(lambda k, n: src[pl.ds(k, n), :], store, T3, 1, 16)

    def p2_body(i, carry):
        r0 = pl.multiple_of(i * T2, T2)
        win = x1_v.at[pl.ds(r0, 2 * T2)]
        prep3(win, 0)
        hs = h1_rows(r0 + 8, T2).astype(BF16)
        for q in range(4):
            win[pl.ds(T2, T2), pl.ds(q * c4, c4)] = (
                jnp.dot(hs, w2_v[q], preferred_element_type=F32)
                + x_v[pl.ds(r0, T2), pl.ds(q * c4, c4)].astype(F32))
        return carry

    with jax.named_scope('p2_body'):
        jax.lax.fori_loop(0, N2, p2_body, 0)

    for c in cp_ffn + piece_copies(0, 0):
        c.wait()
    blk0 = (N2 - 2) * T2 // T3

    def p3_body(i, carry):
        r0 = pl.multiple_of((i + blk0) % N3 * T3, T3)
        r_next = pl.multiple_of((i + 1 + blk0) % N3 * T3, T3)
        slot = i & 1
        ring = i % NRING

        @pl.when(i + 2 < N3)
        def _():
            for c in piece_copies(i + 2, (i + 2) % NRING):
                c.start()

        lhs = ln3_v[slot]
        tok = prep3(x1_v.at[pl.ds(T2 + r_next, T3)], 1 - slot)
        zero = zero_v[...]
        low16 = jax.lax.broadcasted_iota(jnp.int32, (16, 128), 1) < 64
        for which in range(3):
            for j in range(DP // 2):
                blk = pltpu.bitcast(stq_v[ring, which, pl.ds(j * 64, 64), :], U32)
                a = blk[0:16] | tok
                c = blk[16:32]
                lo = (a & jnp.uint32(0xFFFF)) | (c << 16)
                if which < 2:
                    a = a | (lo & zero)
                hi = (a >> 16) | (c & jnp.uint32(0xFFFF0000))
                if which < 2:
                    tok = hi & zero
                    if j % HOP == HOP - 1:
                        tok = pltpu.roll(tok, 1, 1)
                else:
                    t = pltpu.roll(jnp.where(low16, hi, lo), 64, 1)
                    lo, hi = jnp.where(low16, lo, t), jnp.where(low16, t, hi)
                    both = hi if j % 2 == 0 else both | hi
                    if j % 2 == 1:
                        tok = both & zero
                s0 = which * H * PITCH + i * (DP // 2) + j
                wqkv_v[pl.ds(s0, 16, stride=PITCH), :] = lo
                wqkv_v[pl.ds(s0 + 16 * PITCH, 16, stride=PITCH), :] = hi
        o0 = pl.multiple_of(i * (OP // 2), OP // 2)
        for j in range(D // 128):
            for k in range(OP // 32):
                w = pltpu.bitcast(sto_v[ring, pl.ds(k * 32, 32), pl.ds(j * 128, 128)], U32) | tok
                tok = w & zero
                if k % (2 * HOP) == 2 * HOP - 1:
                    tok = pltpu.roll(tok, 1, 1)
                kd = k - k % 8 + (0, 1, 4, 5, 2, 3, 6, 7)[k % 8]
                wo_v[j, pl.ds(o0 + kd * 16, 16), :] = w

        h = _gelu(jnp.dot(lhs, w3_v[...], preferred_element_type=F32)).astype(BF16)
        b = jnp.dot(h, w4_v[...], preferred_element_type=F32) + x1_v[pl.ds(T2 + r0, T3), :]
        gw = gw_v[...].astype(F32).reshape(1, D)
        z = jnp.sum(x_v[pl.ds(r0, T3), :].astype(F32) * gw, axis=-1, keepdims=True)
        g = 1.0 / (1.0 + jnp.exp(-z))
        g_v[pl.ds(r0, T3), :] = jnp.broadcast_to(g, (T3, 128))
        b = (1.0 - g) * b
        for j in range(D // 128):
            h1_v[j, pl.ds(r0, T3), :] = b[:, j * 128:(j + 1) * 128]

        @pl.when(i + 1 < N3)
        def _():
            for c in piece_copies(i + 1, (i + 1) % NRING):
                c.wait()

        return carry

    with jax.named_scope('p3_body'):
        jax.lax.fori_loop(0, N3, p3_body, 0)

    mem_v[...] = mem0_v[...].astype(F32)
    c_exp = (DH ** -0.5) * math.log2(math.e)
    neg_raw = NEG / (DH ** -0.5)

    L2 = 2 * L

    def make_mask(ngv):
        rm = L - 8 * ngv
        row = jax.lax.broadcasted_iota(jnp.int32, (2 * rm, 128), 0)
        col = jax.lax.broadcasted_iota(jnp.int32, (2 * rm, 128), 1)
        second = row >= rm
        rowl = jnp.where(second, row - rm, row)
        coll = jnp.where(second, col - L, col)
        real = (coll >= 0) & (coll < L)
        allowed = real & ((rowl < M) | (rowl + 8 * ngv >= coll))
        fill = jnp.where(allowed, 0.0, jnp.where(real, neg_raw, -jnp.inf)).astype(F32)
        return jnp.where(allowed, jnp.uint32(0xFFFFFFFF), jnp.uint32(0)), pltpu.bitcast(fill, U32)

    masks = {n: make_mask(n) for n in set(NGV_A + NGV_B)}
    neg_c = NEG * math.log2(math.e)

    def tied(w, toks):
        for tok in toks:
            w = jnp.concatenate([w[0:56], w[56:64] | tok, w[64:]], axis=0)
        return pltpu.bitcast(w, BF16)

    zpad = jnp.zeros((128 - L2, DH), F32)

    def recip(l):
        r = pl.reciprocal(l, approx=True)
        return r * (2.0 - l * r)

    def tree(op, x):
        while x.shape[0] > 1:
            x = op(x[0:x.shape[0] // 2], x[x.shape[0] // 2:])
        return x[0]

    causal = (jax.lax.broadcasted_iota(jnp.int32, (7, 8, 128), 1)
              > jax.lax.broadcasted_iota(jnp.int32, (7, 8, 128), 0))
    low = jax.lax.broadcasted_iota(jnp.int32, (8, 128), 1) < 64

    def stash(buf, slot, ks, ws, g):
        n = 8 * (g + 2)
        starts = []
        for i, x in enumerate(ks + ws):
            base = (4 * slot + i) * (L + 8)
            buf[pl.ds(base, n), :] = jnp.concatenate([x[8 * g:8 * g + 8], x[0:n - 8]], axis=0)
            starts.append(base + n - 8)
        return buf, starts, [jnp.sum(w[n - 8:L], axis=0, keepdims=True) if n - 8 < L
                             else jnp.zeros((1, DH), F32) for w in ws]

    def vpu_start(q0, q1, parked, g):
        buf, starts, (acc_a, acc_b) = parked
        return dict(q=(q0 * c_exp, q1 * c_exp), buf=buf, starts=starts, g=g,
                    m=jnp.full((8, 128), neg_c, F32),
                    l=jnp.full((8, 128), float(L - 8 * (g + 1)), F32), a=acc_a, b=acc_b)

    def vpu_chunk(st, c0, gate):
        def windows(start):
            return jnp.concatenate([st['buf'][pl.ds(start - r, 8), :]
                                    for r in range(c0, c0 + CHUNK)], axis=0).reshape(CHUNK, 8, 128)

        k0, k1, wa, wb = st['starts']
        q0, q1 = [pltpu.bitcast(pltpu.bitcast(q, U32) | gate, F32) for q in st['q']]
        sc = jnp.where(low, jnp.sum(q0 * windows(k0), axis=-1, keepdims=True),
                       jnp.sum(q1 * windows(k1), axis=-1, keepdims=True))
        if c0 == 8 * st['g']:
            sc = jnp.concatenate([sc[0:1], jnp.where(causal, sc[1:], neg_c)], axis=0)
        m = jnp.maximum(tree(jnp.maximum, sc), st['m'])
        alpha = jnp.exp2(st['m'] - m)
        pr = jnp.exp2(sc - m)
        new = []
        for old, x in ((st['l'], pr), (st['a'], pr * windows(wa)), (st['b'], pr * windows(wb))):
            new.append(jnp.sum(jnp.concatenate([(old * alpha)[None], x], axis=0), axis=0))
        st.update(m=m, l=new[0], a=new[1], b=new[2])
        return (pltpu.bitcast(new[0], U32) | pltpu.bitcast(new[1], U32)
                | pltpu.bitcast(new[2], U32))

    def vpu_finish(st):
        r = recip(st['l'])
        return st['a'] * r, st['b'] * r

    def segment(lhs_q, lhs_kv, wo_m, ngv, n_chunks, unpack, wo_rows, split_first, early, d_j, order, half, zero):
        NP = H // 2
        nj = D // 128
        HA = H - TAIL_H
        mxu_groups = [[0] + list(range(n + 1, 5)) for n in ngv]
        proj = {}
        qkv = [None] * NP
        pb = [None] * NP
        og = [dict() for _ in range(H)]
        ocat = {}
        y = [None] * nj

        def slab(toks, which, h, r0, n):
            x = lhs_q if which == 0 else lhs_kv
            w = tied(wqkv_v[pl.ds(_slab_of(which, h) * PITCH + r0, n), :], toks)
            r = jnp.dot(x[:, 2 * r0:2 * (r0 + n)], w, preferred_element_type=F32)
            proj[(which, h)] = r + proj[(which, h)] if (which, h) in proj else r
            return proj[(which, h)]

        def do_wo(toks, h0, h1, j):
            if (h0, h1) not in ocat:
                ocat[(h0, h1)] = jnp.concatenate(
                    [wo_rows(og[h]) for h in range(h0, h1)], axis=1).astype(BF16)
            w = tied(wo_v[j, pl.ds(h0 * 64, (h1 - h0) * 64), :], toks)
            r = jnp.dot(ocat[(h0, h1)], w, preferred_element_type=F32)
            y[j] = r if y[j] is None else r + y[j]
            return y[j]

        ticks = []
        pair_end = {}
        wo_early = [(4 * c, 4 * c + 4, j) for c in range(early) for j in range(nj)]
        first = NP - WO_SLOTS
        for p in range(NP):
            slabs = [(k % 3, 2 * p + k // 3) for k in order]
            rows = [(lhs_q if w == 0 else lhs_kv).shape[0] for w, _ in slabs]
            if p == 0 and split_first:
                for r0 in (0, 256):
                    ticks += [(slab, (w, h, r0, 256), m) for (w, h), m in zip(slabs, rows)]
            else:
                mine = []
                if p >= first:
                    lo = (p - first) * len(wo_early) // WO_SLOTS
                    mine = wo_early[lo:(p - first + 1) * len(wo_early) // WO_SLOTS]
                att = 8 * len(mxu_groups[p])
                if half:
                    units = [(slab, slabs[k] + (r0, 256), rows[k] + att / 12)
                             for k0 in (0, 3) for r0 in (0, 256) for k in range(k0, k0 + 3)]
                else:
                    units = [(slab, slabs[k] + (0, 512), 2 * rows[k] + att // 6) for k in range(6)]
                for n, unit in enumerate(units):
                    ticks += [(do_wo, item, wo_m) for item in
                              mine[n * len(mine) // len(units):(n + 1) * len(mine) // len(units)]]
                    ticks.append(unit)
            pair_end[len(ticks) - 1] = p
        tail = [(h0, h0 + 4, j) for j in range(nj) for h0 in range(4 * early, HA, 4)]
        ticks += [(do_wo, item, wo_m) for item in (sorted(tail) if TAIL_CM else tail)]
        ends = []
        for _, _, dur in ticks:
            ends.append(dur + (ends[-1] if ends else 0))

        def index(t):
            return next(i for i, e in enumerate(ends) if e >= t)

        events = {}
        anchors = {}
        cursor = [0]

        def run_chunk(res, p, name, st, c0, i_done):
            done = vpu_chunk(st, c0, pltpu.bitcast(res[0:8], U32) & zero)
            anchors.setdefault(i_done, []).append(done & zero)
            if c0 + CHUNK >= 8 * (st['g'] + 1):
                og[2 * p][name], og[2 * p + 1][name] = vpu_finish(st)
                if D_R and ends[i_done - 1] + D_R < ends[-2]:
                    anchors.setdefault(index(ends[i_done - 1] + D_R) + 1, []).append(
                        pltpu.bitcast(og[2 * p][name], U32) & zero)

        def do_s(res, p):
            sc = jax.lax.dot_general(qkv[p][0], qkv[p][1], (((1,), (1,)), ((), ())),
                                     preferred_element_type=F32)
            keep, fill = masks[ngv[p]]
            sc = pltpu.bitcast((pltpu.bitcast(sc, U32) & keep) | fill, F32)
            e = jnp.exp2((sc - jnp.max(sc, axis=-1, keepdims=True)) * c_exp)
            l = jnp.sum(e, axis=-1, keepdims=True)
            e = e * recip(l)
            rm = 8 * len(mxu_groups[p])
            e = e[0:rm] + e[rm:2 * rm]
            if rm % 16:
                e = jnp.concatenate([e, jnp.zeros((8, 128), F32)], axis=0)
            pb[p] = e.astype(BF16)

        def do_pv(res, p):
            for i in range(2):
                o = jnp.dot(pb[p], qkv[p][2][i], preferred_element_type=F32)
                for n, g in enumerate(mxu_groups[p]):
                    og[2 * p + i][g] = o[8 * n:8 * n + 8]

        def finish_pair(p, i):
            u, jobs = unpack(p, [[proj[(w, h)] for w in range(3)] for h in (2 * p, 2 * p + 1)])
            chunks = [(name, st, c0) for name, st in
                      [(name, vpu_start(*job)) for name, job in jobs.items()]
                      for c0 in range(0, 8 * (st['g'] + 1), CHUNK)]
            t_first = ends[min(pair_end)] + D_G
            t_last = ends[-2] - d_j - D_F
            gap = (t_last - t_first) / (n_chunks - 1)
            if p == NP - 1:
                gap = min(gap, (t_last - max(ends[i] + D_G, cursor[0])) / (len(chunks) - 1))
            for chunk in chunks:
                t = max(ends[i] + D_G, cursor[0])
                cursor[0] = t + gap
                g = max(index(t), i + 1)
                events.setdefault(g, []).append(
                    (run_chunk, (p,) + chunk + (index(ends[g] + d_j) + 1,)))
            qb = jnp.concatenate([u[k][0][g] for k in range(2) for g in mxu_groups[p]],
                                 axis=0).astype(BF16)
            kb = jnp.concatenate([u[0][1], u[1][1], zpad], axis=0).astype(BF16)
            low40 = jnp.concatenate([low] * 5, axis=0)
            vb = [jnp.concatenate([jnp.where(low40, v, 0.0), jnp.where(low40, 0.0, v), zpad],
                                  axis=0).astype(BF16) for v in (u[0][2], u[1][2])]
            qkv[p] = (qb, kb, vb)
            t_pv = min(ends[i] + D_PV, ends[-1] - D_O)
            events.setdefault(index(min(ends[i] + D_S, t_pv - D_SM)), []).append((do_s, (p,)))
            events.setdefault(index(t_pv), []).append((do_pv, (p,)))

        for i, (fn, args, _) in enumerate(ticks):
            res = fn(anchors.pop(i, []), *args)
            if i in pair_end:
                finish_pair(pair_end[i], i)
            for f, a in events.pop(i, []):
                f(res, *a)
        assert not events
        for j in range(nj):
            do_wo([], HA, H, j)
        return jnp.concatenate(y, axis=1)

    def pair(r0, mem):
        xf = x_v[pl.ds(r0, PAIR), :].astype(F32)
        zero = zero_v[pl.ds(0, 8), :]
        x1s = jnp.concatenate([xf[0:8], xf[32:40]], axis=0).astype(BF16)
        keep = [None] * H

        def cat(*xs):
            return jnp.concatenate(xs, axis=0)

        lhs = cat(mem, xf[8:32]).astype(BF16)

        def finish(p, qg, ks, vs, slot, groups):
            return ([(qg[i], ks[i], vs[i]) for i in range(2)],
                    {g: stash(kv_v[p], slot + n, ks, vs, g) for n, g in enumerate(groups)})

        def unpack_a(p, qkv):
            qg = [{0: q[0:8], 2: q[8:16], 3: q[16:24], 4: q[24:32]} for q, _, _ in qkv]
            ks = [cat(k[0:8], k[32:40], k[8:32]) for _, k, _ in qkv]
            vs = [cat(v[0:8], v[32:40], v[8:32]) for _, _, v in qkv]
            u, parked = finish(p, qg, ks, vs, 0, range(1, NGV_A[p] + 1))
            keep[p] = (parked[1], [(k[40:48], v[40:48]) for _, k, v in qkv])
            return u, {g: (qg[0][g], qg[1][g], parked[g], g) for g in range(2, NGV_A[p] + 1)}

        y_a = segment(lhs, cat(lhs, x1s), 32, NGV_A,
                      sum(g + 1 for n in NGV_A for g in range(2, n + 1)) * 8 // CHUNK, unpack_a,
                      lambda o: cat(o[0], o[2], o[3], o[4]), False, EARLY_A, D_JA, ORDER_A, HALF_A, zero)

        lhs = cat(y_a[0:8], xf[40:64]).astype(BF16)

        def unpack_b(p, qkv):
            parked_a1, kv1 = keep[p]
            qg = [{0: q[0:8], 1: q[40:48], 2: q[8:16], 3: q[16:24], 4: q[24:32]}
                  for q, _, _ in qkv]
            ks = [cat(k[0:8], e[0], k[8:32]) for (_, k, _), e in zip(qkv, kv1)]
            vs = [cat(v[0:8], e[1], v[8:32]) for (_, _, v), e in zip(qkv, kv1)]
            u, parked = finish(p, qg, ks, vs, max(NGV_A), range(1, NGV_B[p] + 1))
            jobs = {'a1': (qkv[0][0][32:40], qkv[1][0][32:40], parked_a1, 1)}
            jobs.update({g: (qg[0][g], qg[1][g], parked[g], g) for g in range(1, NGV_B[p] + 1)})
            return u, jobs

        y_b = segment(cat(lhs, x1s), lhs, 48, NGV_B,
                      sum(2 + sum(range(2, n + 2)) for n in NGV_B) * 8 // CHUNK, unpack_b,
                      lambda o: cat(o[0], o[1], o[2], o[3], o[4], o['a1']), True, EARLY_B,
                      D_JB, ORDER_B, HALF_B, zero)

        a = cat(y_b[40:48], y_a[8:32], y_b[8:40])
        g = g_v[pl.ds(r0, PAIR), :]
        g = jnp.concatenate([g] * (D // 128), axis=1)
        out_v[pl.ds(r0, PAIR), :] = (g * a + h1_rows(r0, PAIR)).astype(BF16)
        return y_b[0:8]

    rows_it = UNROLL_A * PAIR

    def a_body(t, carry):
        base = pl.multiple_of(t * rows_it, rows_it)
        mem = mem_v[...]
        for u in range(UNROLL_A):
            mem = pair(pl.multiple_of(base + u * PAIR, PAIR), mem)
        mem_v[...] = mem
        pltpu.make_async_copy(out_v.at[pl.ds(base, rows_it)], out_hbm.at[pl.ds(base, rows_it)],
                              osem).start()
        return carry

    with jax.named_scope('a_body'):
        jax.lax.fori_loop(0, S // rows_it, a_body, 0)
    pltpu.make_async_copy(out_v, out_hbm, osem).wait()


@jax.jit
def pallas_gated_mix__memory_aug_recurrent_mem_tr__mixer_s_mlp__prompt_kernel(
    A_x, A_mem0, A_Wq, A_Wk, A_Wv, A_Wo, A_seg_len, B_x, B_w1, B_w2, B_w3, B_w4, gate_w,
):
    assert A_x.shape == (1, S, D) and A_Wq.shape == (D, H, DH) and A_mem0.shape == (1, M, D)
    x = A_x.reshape(S, D)
    mem0 = A_mem0.reshape(M, D)
    wq = A_Wq.reshape(D * H, DH)
    wk = A_Wk.reshape(D * H, DH)
    wv = A_Wv.reshape(D * H, DH)
    wo = A_Wo.reshape(H * DH, D)

    any_spec = pl.BlockSpec(memory_space=pl.ANY)
    out = pl.pallas_call(
        _kernel,
        out_shape=jax.ShapeDtypeStruct((S, D), BF16),
        in_specs=[any_spec] * 11,
        out_specs=any_spec,
        scratch_shapes=[
            pltpu.VMEM((S, D), BF16),
            pltpu.VMEM((NRING, 3, DP * H, DH), BF16),
            pltpu.VMEM((NRING, OP, D), BF16),
            pltpu.VMEM((3 * H * PITCH, 128), U32),
            pltpu.VMEM((D // 128, H * DH // 2, 128), U32),
            pltpu.VMEM((4, D, D // 4), BF16),
            pltpu.VMEM((4, D, D // 4), BF16),
            pltpu.VMEM((D, FF), BF16),
            pltpu.VMEM((FF, D), BF16),
            pltpu.VMEM((D // 128, S + 16, 128), F32),
            pltpu.VMEM((S + T2, D), F32),
            pltpu.VMEM((S, 128), F32),
            pltpu.VMEM((2, T1, D), BF16),
            pltpu.VMEM((2, T3, D), BF16),
            pltpu.VMEM((M, D), BF16),
            pltpu.VMEM((D,), BF16),
            pltpu.VMEM((M, D), F32),
            pltpu.VMEM((S, D), BF16),
            [pltpu.VMEM((NJOB * 4 * (L + 8), 128), F32)] * (H // 2),
            pltpu.VMEM((16, 128), U32),
            pltpu.SemaphoreType.DMA((NSEM,)),
            pltpu.SemaphoreType.DMA(()),
        ],
        compiler_params=pltpu.CompilerParams(vmem_limit_bytes=120 * 1024 * 1024,
                                             disable_bounds_checks=True),
    )(x, mem0, wq, wk, wv, wo, B_w1, B_w2, B_w3, B_w4, gate_w)
    return out.reshape(1, S, D)
```

```python
import math

import jax
import jax.numpy as jnp
import jax.experimental.pallas as pl
import jax.experimental.pallas.tpu as pltpu

F32 = jnp.float32
BF16 = jnp.bfloat16
U32 = jnp.uint32

S = 2048
D = 1024
H = 32
DH = 128
M = 8
SEG = 32
L = M + SEG
FF = 3584
EPS = 1e-5
NEG = -1e9

PAIR = 2 * SEG
T1 = 256
N1 = S // T1
T2 = 512
N2 = S // T2
T3 = 256
N3 = S // T3
DP = D // N3
OP = H * DH // N3
PITCH = 520
NRING = 3
NSEM = 11 + NRING

NCHAIN0 = 10
NCHAIN1 = 5
LN1_ROWS = 8
HOP = 4
NGV_A = [3] * (H // 2)
NGV_B = [3, 3, 1, 3, 3, 3, 1, 3, 3, 3, 3, 3, 1, 3, 3, 3]
NJOB = max(NGV_A) + max(NGV_B)
CHUNK = 8
EARLY_A = 2
EARLY_B = 3
WO_SLOTS = 10
TAIL_H = 8
D_G = 0
D_JA = 510
D_JB = 530
D_F = 50
D_S = 250
D_PV = 1400
D_SM = 600
D_O = 170


def _gelu(x):
    c = math.sqrt(2.0 / math.pi)
    return 0.5 * x * (1.0 + jnp.tanh(c * (x + 0.044715 * (x * x * x))))


def _layernorm(x):
    m = jnp.mean(x, axis=-1, keepdims=True)
    xc = x - m
    v = jnp.mean(xc * xc, axis=-1, keepdims=True)
    return xc * jax.lax.rsqrt(v + EPS)


def _slab_of(which, h):
    return which * H + (h % 2) * (H // 2) + h // 2


def _kernel(x_hbm, mem0_hbm, wq_hbm, wk_hbm, wv_hbm, wo_hbm,
            w1_hbm, w2_hbm, w3_hbm, w4_hbm, gw_hbm,
            out_hbm,
            x_v, stq_v, sto_v, wqkv_v, wo_v, w1_v, w2_v, w3_v, w4_v,
            h1_v, x1_v, g_v, ln1_v, ln3_v, mem0_v, gw_v, mem_v, out_v, kv_v, zero_v, sems, osem):
    c4 = D // 4
    xcuts = (0, 1, 2, 3, 5, N1)
    cp_x = [pltpu.make_async_copy(x_hbm.at[pl.ds(lo * T1, (hi - lo) * T1)],
                                  x_v.at[pl.ds(lo * T1, (hi - lo) * T1)], sems.at[n])
            for n, (lo, hi) in enumerate(zip(xcuts[:-1], xcuts[1:]))]
    cp_w1 = [pltpu.make_async_copy(w1_hbm.at[:, pl.ds(q * c4, c4)], w1_v.at[q], sems.at[5 + q])
             for q in range(4)]
    cp_w2 = [pltpu.make_async_copy(w2_hbm.at[:, pl.ds(q * c4, c4)], w2_v.at[q], sems.at[9])
             for q in range(4)]
    cp_ffn = [pltpu.make_async_copy(src, dst, sems.at[10])
              for src, dst in ((gw_hbm, gw_v), (mem0_hbm, mem0_v), (w3_hbm, w3_v), (w4_hbm, w4_v))]

    def piece_copies(i, slot):
        cps = [pltpu.make_async_copy(w.at[pl.ds(i * (DP * H), DP * H)], stq_v.at[slot, k],
                                     sems.at[11 + slot])
               for k, w in enumerate((wq_hbm, wk_hbm, wv_hbm))]
        cps.append(pltpu.make_async_copy(wo_hbm.at[pl.ds(i * OP, OP)], sto_v.at[slot],
                                         sems.at[11 + slot]))
        return cps

    for c in (cp_x[0:1] + cp_w1 + cp_x[1:] + cp_w2 + cp_ffn
              + piece_copies(0, 0) + piece_copies(1, 1)):
        c.start()
    x1_v[pl.ds(0, T3), :] = jnp.zeros((T3, D), F32)
    h1_v[:, pl.ds(8, 8), :] = jnp.zeros((D // 128, 8, 128), F32)
    h1_v[:, pl.ds(S, 8), :] = jnp.zeros((D // 128, 8, 128), F32)
    zero_v[...] = jnp.zeros((16, 128), U32)

    def ln_rows(x, tok, zero):
        if tok is not None:
            head = pltpu.bitcast(pltpu.bitcast(x[:, 0:128], U32) | tok, F32)
            x = jnp.concatenate([head, x[:, 128:]], axis=1)
        y = _layernorm(x)
        tok = None if zero is None else pltpu.bitcast(y[:, 0:128], U32) & zero
        return y, tok

    def ln_block(load, store, rows, nchain, gr):
        zero = zero_v[pl.ds(0, gr), :] if nchain else None
        toks = [None] * max(nchain, 1)
        for k in range(rows // gr):
            y, toks[k % len(toks)] = ln_rows(load(k * gr, gr), toks[k % len(toks)], zero)
            store(k * gr, y.astype(BF16))
        return toks[(rows // gr - 1) % len(toks)]

    def prep1(blk, slot, nchain):
        r0 = blk * T1 if isinstance(blk, int) else pl.multiple_of(blk * T1, T1)

        def store(k, y):
            ln1_v[slot, pl.ds(k, y.shape[0]), :] = y

        ln_block(lambda k, n: x_v[pl.ds(r0 + k, n), :].astype(F32), store, T1, nchain, LN1_ROWS)

    def p1_quarter(lhs, r0, q):
        h = _gelu(jnp.dot(lhs, w1_v[q], preferred_element_type=F32))
        for j in range(2):
            win = h1_v.at[2 * q + j, pl.ds(r0, T1 + 16)]
            win[pl.ds(8 + (1, -1, 2, -2)[q], T1), :] = h[:, j * 128:(j + 1) * 128]

    cp_x[0].wait()
    prep1(0, 0, 0)
    for q in range(4):
        cp_w1[q].wait()
        if q == 3:
            cp_x[1].wait()
        lhs = ln1_v[0]
        if q == 3:
            prep1(1, 1, NCHAIN0)
        p1_quarter(lhs, 0, q)

    def p1_body(i, carry):
        r0 = pl.multiple_of(i * T1, T1)
        slot = i & 1

        lhs = ln1_v[slot]
        prep1(jnp.minimum(i + 1, N1 - 1), 1 - slot, NCHAIN1)
        for q in range(4):
            p1_quarter(lhs, r0, q)
        for n in range(3, len(cp_x)):
            pl.when(i + 2 == xcuts[n])(cp_x[n].wait)
        return carry

    cp_x[2].wait()
    with jax.named_scope('p1_body'):
        jax.lax.fori_loop(1, N1, p1_body, 0)
    for c in cp_w2:
        c.wait()

    def h1_rows(r0, n):
        return jnp.concatenate([h1_v[j, pl.ds(r0, n), :] for j in range(D // 128)], axis=1)

    def prep3(src, slot):
        def store(k, y):
            ln3_v[slot, pl.ds(k, y.shape[0]), :] = y

        return ln_block(lambda k, n: src[pl.ds(k, n), :], store, T3, 1, 16)

    def p2_body(i, carry):
        r0 = pl.multiple_of(i * T2, T2)
        win = x1_v.at[pl.ds(r0, 2 * T2)]
        prep3(win, 0)
        hs = h1_rows(r0 + 8, T2).astype(BF16)
        for q in range(4):
            win[pl.ds(T2, T2), pl.ds(q * c4, c4)] = (
                jnp.dot(hs, w2_v[q], preferred_element_type=F32)
                + x_v[pl.ds(r0, T2), pl.ds(q * c4, c4)].astype(F32))
        return carry

    with jax.named_scope('p2_body'):
        jax.lax.fori_loop(0, N2, p2_body, 0)

    for c in cp_ffn + piece_copies(0, 0):
        c.wait()
    blk0 = (N2 - 2) * T2 // T3

    def p3_body(i, carry):
        r0 = pl.multiple_of((i + blk0) % N3 * T3, T3)
        r_next = pl.multiple_of((i + 1 + blk0) % N3 * T3, T3)
        slot = i & 1
        ring = i % NRING

        @pl.when(i + 2 < N3)
        def _():
            for c in piece_copies(i + 2, (i + 2) % NRING):
                c.start()

        lhs = ln3_v[slot]
        tok = prep3(x1_v.at[pl.ds(T2 + r_next, T3)], 1 - slot)
        zero = zero_v[...]
        low16 = jax.lax.broadcasted_iota(jnp.int32, (16, 128), 1) < 64
        for which in range(3):
            for j in range(DP // 2):
                blk = pltpu.bitcast(stq_v[ring, which, pl.ds(j * 64, 64), :], U32)
                a = blk[0:16] | tok
                c = blk[16:32]
                lo = (a & jnp.uint32(0xFFFF)) | (c << 16)
                if which < 2:
                    a = a | (lo & zero)
                hi = (a >> 16) | (c & jnp.uint32(0xFFFF0000))
                if which < 2:
                    tok = hi & zero
                    if j % HOP == HOP - 1:
                        tok = pltpu.roll(tok, 1, 1)
                else:
                    t = pltpu.roll(jnp.where(low16, hi, lo), 64, 1)
                    lo, hi = jnp.where(low16, lo, t), jnp.where(low16, t, hi)
                    both = hi if j % 2 == 0 else both | hi
                    if j % 2 == 1:
                        tok = both & zero
                s0 = which * H * PITCH + i * (DP // 2) + j
                wqkv_v[pl.ds(s0, 16, stride=PITCH), :] = lo
                wqkv_v[pl.ds(s0 + 16 * PITCH, 16, stride=PITCH), :] = hi
        o0 = pl.multiple_of(i * (OP // 2), OP // 2)
        for j in range(D // 128):
            for k in range(OP // 32):
                w = pltpu.bitcast(sto_v[ring, pl.ds(k * 32, 32), pl.ds(j * 128, 128)], U32) | tok
                tok = w & zero
                if k % (2 * HOP) == 2 * HOP - 1:
                    tok = pltpu.roll(tok, 1, 1)
                kd = k - k % 8 + (0, 1, 4, 5, 2, 3, 6, 7)[k % 8]
                wo_v[j, pl.ds(o0 + kd * 16, 16), :] = w

        h = _gelu(jnp.dot(lhs, w3_v[...], preferred_element_type=F32)).astype(BF16)
        b = jnp.dot(h, w4_v[...], preferred_element_type=F32) + x1_v[pl.ds(T2 + r0, T3), :]
        gw = gw_v[...].astype(F32).reshape(1, D)
        z = jnp.sum(x_v[pl.ds(r0, T3), :].astype(F32) * gw, axis=-1, keepdims=True)
        g = 1.0 / (1.0 + jnp.exp(-z))
        g_v[pl.ds(r0, T3), :] = jnp.broadcast_to(g, (T3, 128))
        b = (1.0 - g) * b
        for j in range(D // 128):
            h1_v[j, pl.ds(r0, T3), :] = b[:, j * 128:(j + 1) * 128]

        @pl.when(i + 1 < N3)
        def _():
            for c in piece_copies(i + 1, (i + 1) % NRING):
                c.wait()

        return carry

    with jax.named_scope('p3_body'):
        jax.lax.fori_loop(0, N3, p3_body, 0)

    mem_v[...] = mem0_v[...].astype(F32)
    c_exp = (DH ** -0.5) * math.log2(math.e)
    neg_raw = NEG / (DH ** -0.5)

    L2 = 2 * L

    def make_mask(ngv):
        rm = L - 8 * ngv
        row = jax.lax.broadcasted_iota(jnp.int32, (2 * rm, 128), 0)
        col = jax.lax.broadcasted_iota(jnp.int32, (2 * rm, 128), 1)
        second = row >= rm
        rowl = jnp.where(second, row - rm, row)
        coll = jnp.where(second, col - L, col)
        real = (coll >= 0) & (coll < L)
        allowed = real & ((rowl < M) | (rowl + 8 * ngv >= coll))
        fill = jnp.where(allowed, 0.0, jnp.where(real, neg_raw, -jnp.inf)).astype(F32)
        return jnp.where(allowed, jnp.uint32(0xFFFFFFFF), jnp.uint32(0)), pltpu.bitcast(fill, U32)

    masks = {n: make_mask(n) for n in set(NGV_A + NGV_B)}
    neg_c = NEG * math.log2(math.e)

    def tied(w, toks):
        for tok in toks:
            w = jnp.concatenate([w[0:56], w[56:64] | tok, w[64:]], axis=0)
        return pltpu.bitcast(w, BF16)

    zpad = jnp.zeros((128 - L2, DH), F32)

    def recip(l):
        r = pl.reciprocal(l, approx=True)
        return r * (2.0 - l * r)

    def tree(op, x):
        while x.shape[0] > 1:
            x = op(x[0:x.shape[0] // 2], x[x.shape[0] // 2:])
        return x[0]

    causal = (jax.lax.broadcasted_iota(jnp.int32, (7, 8, 128), 1)
              > jax.lax.broadcasted_iota(jnp.int32, (7, 8, 128), 0))
    low = jax.lax.broadcasted_iota(jnp.int32, (8, 128), 1) < 64

    def stash(buf, slot, ks, ws, g):
        n = 8 * (g + 2)
        starts = []
        for i, x in enumerate(ks + ws):
            base = (4 * slot + i) * (L + 8)
            buf[pl.ds(base, n), :] = jnp.concatenate([x[8 * g:8 * g + 8], x[0:n - 8]], axis=0)
            starts.append(base + n - 8)
        return buf, starts, [jnp.sum(w[n - 8:L], axis=0, keepdims=True) if n - 8 < L
                             else jnp.zeros((1, DH), F32) for w in ws]

    def vpu_start(q0, q1, parked, g):
        buf, starts, (acc_a, acc_b) = parked
        return dict(q=(q0 * c_exp, q1 * c_exp), buf=buf, starts=starts, g=g,
                    m=jnp.full((8, 128), neg_c, F32),
                    l=jnp.full((8, 128), float(L - 8 * (g + 1)), F32), a=acc_a, b=acc_b)

    def vpu_chunk(st, c0, gate):
        def windows(start):
            return jnp.concatenate([st['buf'][pl.ds(start - r, 8), :]
                                    for r in range(c0, c0 + CHUNK)], axis=0).reshape(CHUNK, 8, 128)

        k0, k1, wa, wb = st['starts']
        q0, q1 = [pltpu.bitcast(pltpu.bitcast(q, U32) | gate, F32) for q in st['q']]
        sc = jnp.where(low, jnp.sum(q0 * windows(k0), axis=-1, keepdims=True),
                       jnp.sum(q1 * windows(k1), axis=-1, keepdims=True))
        if c0 == 8 * st['g']:
            sc = jnp.concatenate([sc[0:1], jnp.where(causal, sc[1:], neg_c)], axis=0)
        m = jnp.maximum(tree(jnp.maximum, sc), st['m'])
        alpha = jnp.exp2(st['m'] - m)
        pr = jnp.exp2(sc - m)
        new = []
        for old, x in ((st['l'], pr), (st['a'], pr * windows(wa)), (st['b'], pr * windows(wb))):
            new.append(jnp.sum(jnp.concatenate([(old * alpha)[None], x], axis=0), axis=0))
        st.update(m=m, l=new[0], a=new[1], b=new[2])
        return (pltpu.bitcast(new[0], U32) | pltpu.bitcast(new[1], U32)
                | pltpu.bitcast(new[2], U32))

    def vpu_finish(st):
        r = recip(st['l'])
        return st['a'] * r, st['b'] * r

    def segment(lhs_q, lhs_kv, wo_m, ngv, n_chunks, unpack, wo_rows, split_first, early, d_j,
                zero):
        NP = H // 2
        nj = D // 128
        HA = H - TAIL_H
        mxu_groups = [[0] + list(range(n + 1, 5)) for n in ngv]
        proj = {}
        qkv = [None] * NP
        pb = [None] * NP
        og = [dict() for _ in range(H)]
        ocat = {}
        y = [None] * nj

        def slab(toks, which, h, r0, n):
            x = lhs_q if which == 0 else lhs_kv
            w = tied(wqkv_v[pl.ds(_slab_of(which, h) * PITCH + r0, n), :], toks)
            r = jnp.dot(x[:, 2 * r0:2 * (r0 + n)], w, preferred_element_type=F32)
            proj[(which, h)] = r + proj[(which, h)] if (which, h) in proj else r
            return proj[(which, h)]

        def do_wo(toks, h0, h1, j):
            if (h0, h1) not in ocat:
                ocat[(h0, h1)] = jnp.concatenate(
                    [wo_rows(og[h]) for h in range(h0, h1)], axis=1).astype(BF16)
            w = tied(wo_v[j, pl.ds(h0 * 64, (h1 - h0) * 64), :], toks)
            r = jnp.dot(ocat[(h0, h1)], w, preferred_element_type=F32)
            y[j] = r if y[j] is None else r + y[j]
            return y[j]

        ticks = []
        pair_end = {}
        wo_early = [(4 * c, 4 * c + 4, j) for c in range(early) for j in range(nj)]
        first = NP - WO_SLOTS
        for p in range(NP):
            slabs = [(which, h) for h in (2 * p, 2 * p + 1) for which in range(3)]
            rows = [(lhs_q if w == 0 else lhs_kv).shape[0] for w, _ in slabs]
            if p == 0 and split_first:
                for r0 in (0, 256):
                    ticks += [(slab, (w, h, r0, 256), m) for (w, h), m in zip(slabs, rows)]
            else:
                mine = []
                if p >= first:
                    lo = (p - first) * len(wo_early) // WO_SLOTS
                    mine = wo_early[lo:(p - first + 1) * len(wo_early) // WO_SLOTS]
                att = 8 * len(mxu_groups[p])
                units = [(slab, slabs[k] + (r0, 256), rows[k] + att / 12)
                         for k0 in (0, 3) for r0 in (0, 256) for k in range(k0, k0 + 3)]
                for n, unit in enumerate(units):
                    ticks += [(do_wo, item, wo_m) for item in
                              mine[n * len(mine) // len(units):(n + 1) * len(mine) // len(units)]]
                    ticks.append(unit)
            pair_end[len(ticks) - 1] = p
        ticks += [(do_wo, (h0, h0 + 4, j), wo_m)
                  for h0 in range(4 * early, HA, 4) for j in range(nj)]
        ends = []
        for _, _, dur in ticks:
            ends.append(dur + (ends[-1] if ends else 0))

        def index(t):
            return next(i for i, e in enumerate(ends) if e >= t)

        events = {}
        anchors = {}
        cursor = [0]

        def run_chunk(res, p, name, st, c0, i_done):
            done = vpu_chunk(st, c0, pltpu.bitcast(res[0:8], U32) & zero)
            anchors.setdefault(i_done, []).append(done & zero)
            if c0 + CHUNK >= 8 * (st['g'] + 1):
                og[2 * p][name], og[2 * p + 1][name] = vpu_finish(st)

        def do_s(res, p):
            sc = jax.lax.dot_general(qkv[p][0], qkv[p][1], (((1,), (1,)), ((), ())),
                                     preferred_element_type=F32)
            keep, fill = masks[ngv[p]]
            sc = pltpu.bitcast((pltpu.bitcast(sc, U32) & keep) | fill, F32)
            e = jnp.exp2((sc - jnp.max(sc, axis=-1, keepdims=True)) * c_exp)
            l = jnp.sum(e, axis=-1, keepdims=True)
            e = e * recip(l)
            rm = 8 * len(mxu_groups[p])
            e = e[0:rm] + e[rm:2 * rm]
            if rm % 16:
                e = jnp.concatenate([e, jnp.zeros((8, 128), F32)], axis=0)
            pb[p] = e.astype(BF16)

        def do_pv(res, p):
            for i in range(2):
                o = jnp.dot(pb[p], qkv[p][2][i], preferred_element_type=F32)
                for n, g in enumerate(mxu_groups[p]):
                    og[2 * p + i][g] = o[8 * n:8 * n + 8]

        def finish_pair(p, i):
            u, jobs = unpack(p, [[proj[(w, h)] for w in range(3)] for h in (2 * p, 2 * p + 1)])
            chunks = [(name, st, c0) for name, st in
                      [(name, vpu_start(*job)) for name, job in jobs.items()]
                      for c0 in range(0, 8 * (st['g'] + 1), CHUNK)]
            t_first = ends[min(pair_end)] + D_G
            t_last = ends[-2] - d_j - D_F
            gap = (t_last - t_first) / (n_chunks - 1)
            if p == NP - 1:
                gap = min(gap, (t_last - max(ends[i] + D_G, cursor[0])) / (len(chunks) - 1))
            for chunk in chunks:
                t = max(ends[i] + D_G, cursor[0])
                cursor[0] = t + gap
                g = max(index(t), i + 1)
                events.setdefault(g, []).append(
                    (run_chunk, (p,) + chunk + (index(ends[g] + d_j) + 1,)))
            qb = jnp.concatenate([u[k][0][g] for k in range(2) for g in mxu_groups[p]],
                                 axis=0).astype(BF16)
            kb = jnp.concatenate([u[0][1], u[1][1], zpad], axis=0).astype(BF16)
            low40 = jnp.concatenate([low] * 5, axis=0)
            vb = [jnp.concatenate([jnp.where(low40, v, 0.0), jnp.where(low40, 0.0, v), zpad],
                                  axis=0).astype(BF16) for v in (u[0][2], u[1][2])]
            qkv[p] = (qb, kb, vb)
            t_pv = min(ends[i] + D_PV, ends[-1] - D_O)
            events.setdefault(index(min(ends[i] + D_S, t_pv - D_SM)), []).append((do_s, (p,)))
            events.setdefault(index(t_pv), []).append((do_pv, (p,)))

        for i, (fn, args, _) in enumerate(ticks):
            res = fn(anchors.pop(i, []), *args)
            if i in pair_end:
                finish_pair(pair_end[i], i)
            for f, a in events.pop(i, []):
                f(res, *a)
        assert not events
        for j in range(nj):
            do_wo([], HA, H, j)
        return jnp.concatenate(y, axis=1)

    def pair(r0, mem):
        xf = x_v[pl.ds(r0, PAIR), :].astype(F32)
        zero = zero_v[pl.ds(0, 8), :]
        x1s = jnp.concatenate([xf[0:8], xf[32:40]], axis=0).astype(BF16)
        keep = [None] * (H // 2)

        def cat(*xs):
            return jnp.concatenate(xs, axis=0)

        lhs = cat(mem, xf[8:32]).astype(BF16)

        def finish(p, qg, ks, vs, slot, groups):
            return ([(qg[i], ks[i], vs[i]) for i in range(2)],
                    {g: stash(kv_v[p], slot + n, ks, vs, g) for n, g in enumerate(groups)})

        def unpack_a(p, qkv):
            qg = [{0: q[0:8], 2: q[8:16], 3: q[16:24], 4: q[24:32]} for q, _, _ in qkv]
            ks = [cat(k[0:8], k[32:40], k[8:32]) for _, k, _ in qkv]
            vs = [cat(v[0:8], v[32:40], v[8:32]) for _, _, v in qkv]
            u, parked = finish(p, qg, ks, vs, 0, range(1, NGV_A[p] + 1))
            keep[p] = (parked[1], [(k[40:48], v[40:48]) for _, k, v in qkv])
            return u, {g: (qg[0][g], qg[1][g], parked[g], g) for g in range(2, NGV_A[p] + 1)}

        y_a = segment(lhs, cat(lhs, x1s), 32, NGV_A,
                      sum(g + 1 for n in NGV_A for g in range(2, n + 1)) * 8 // CHUNK, unpack_a,
                      lambda o: cat(o[0], o[2], o[3], o[4]), False, EARLY_A, D_JA, zero)

        lhs = cat(y_a[0:8], xf[40:64]).astype(BF16)

        def unpack_b(p, qkv):
            parked_a1, kv1 = keep[p]
            qg = [{0: q[0:8], 1: q[40:48], 2: q[8:16], 3: q[16:24], 4: q[24:32]}
                  for q, _, _ in qkv]
            ks = [cat(k[0:8], e[0], k[8:32]) for (_, k, _), e in zip(qkv, kv1)]
            vs = [cat(v[0:8], e[1], v[8:32]) for (_, _, v), e in zip(qkv, kv1)]
            u, parked = finish(p, qg, ks, vs, max(NGV_A), range(1, NGV_B[p] + 1))
            jobs = {'a1': (qkv[0][0][32:40], qkv[1][0][32:40], parked_a1, 1)}
            jobs.update({g: (qg[0][g], qg[1][g], parked[g], g) for g in range(1, NGV_B[p] + 1)})
            return u, jobs

        y_b = segment(cat(lhs, x1s), lhs, 48, NGV_B,
                      sum(2 + sum(range(2, n + 2)) for n in NGV_B) * 8 // CHUNK, unpack_b,
                      lambda o: cat(o[0], o[1], o[2], o[3], o[4], o['a1']), True, EARLY_B,
                      D_JB, zero)

        a = cat(y_b[40:48], y_a[8:32], y_b[8:40])
        g = g_v[pl.ds(r0, PAIR), :]
        g = jnp.concatenate([g] * (D // 128), axis=1)
        out_v[pl.ds(r0, PAIR), :] = (g * a + h1_rows(r0, PAIR)).astype(BF16)
        return y_b[0:8]

    def a_body(t, carry):
        r0 = pl.multiple_of(t * PAIR, PAIR)
        mem_v[...] = pair(r0, mem_v[...])
        pltpu.make_async_copy(out_v.at[pl.ds(r0, PAIR)], out_hbm.at[pl.ds(r0, PAIR)],
                              osem).start()
        return carry

    with jax.named_scope('a_body'):
        jax.lax.fori_loop(0, S // PAIR, a_body, 0)
    pltpu.make_async_copy(out_v, out_hbm, osem).wait()


@jax.jit
def pallas_gated_mix__memory_aug_recurrent_mem_tr__mixer_s_mlp__prompt_kernel(
    A_x, A_mem0, A_Wq, A_Wk, A_Wv, A_Wo, A_seg_len, B_x, B_w1, B_w2, B_w3, B_w4, gate_w,
):
    assert A_x.shape == (1, S, D) and A_Wq.shape == (D, H, DH) and A_mem0.shape == (1, M, D)
    x = A_x.reshape(S, D)
    mem0 = A_mem0.reshape(M, D)
    wq = A_Wq.reshape(D * H, DH)
    wk = A_Wk.reshape(D * H, DH)
    wv = A_Wv.reshape(D * H, DH)
    wo = A_Wo.reshape(H * DH, D)

    any_spec = pl.BlockSpec(memory_space=pl.ANY)
    out = pl.pallas_call(
        _kernel,
        out_shape=jax.ShapeDtypeStruct((S, D), BF16),
        in_specs=[any_spec] * 11,
        out_specs=any_spec,
        scratch_shapes=[
            pltpu.VMEM((S, D), BF16),
            pltpu.VMEM((NRING, 3, DP * H, DH), BF16),
            pltpu.VMEM((NRING, OP, D), BF16),
            pltpu.VMEM((3 * H * PITCH + 544, 128), U32),
            pltpu.VMEM((D // 128, H * DH // 2, 128), U32),
            pltpu.VMEM((4, D, D // 4), BF16),
            pltpu.VMEM((4, D, D // 4), BF16),
            pltpu.VMEM((D, FF), BF16),
            pltpu.VMEM((FF, D), BF16),
            pltpu.VMEM((D // 128, S + 16, 128), F32),
            pltpu.VMEM((S + T2, D), F32),
            pltpu.VMEM((S, 128), F32),
            pltpu.VMEM((2, T1, D), BF16),
            pltpu.VMEM((2, T3, D), BF16),
            pltpu.VMEM((M, D), BF16),
            pltpu.VMEM((D,), BF16),
            pltpu.VMEM((M, D), F32),
            pltpu.VMEM((S, D), BF16),
            [pltpu.VMEM((NJOB * 4 * (L + 8), 128), F32)] * (H // 2),
            pltpu.VMEM((16, 128), U32),
            pltpu.SemaphoreType.DMA((NSEM,)),
            pltpu.SemaphoreType.DMA(()),
        ],
        compiler_params=pltpu.CompilerParams(vmem_limit_bytes=120 * 1024 * 1024,
                                             disable_bounds_checks=True),
    )(x, mem0, wq, wk, wv, wo, B_w1, B_w2, B_w3, B_w4, gate_w)
    return out.reshape(1, S, D)
```

```python
import math

import jax
import jax.numpy as jnp
import jax.experimental.pallas as pl
import jax.experimental.pallas.tpu as pltpu

F32 = jnp.float32
BF16 = jnp.bfloat16
U32 = jnp.uint32

S = 2048
D = 1024
H = 32
DH = 128
M = 8
SEG = 32
L = M + SEG
FF = 3584
EPS = 1e-5
NEG = -1e9

PAIR = 2 * SEG
T1 = 256
N1 = S // T1
T2 = 512
N2 = S // T2
T3 = 256
N3 = S // T3
DP = D // N3
OP = H * DH // N3
PITCH = 520
NRING = 3
NSEM = 11 + NRING

NCHAIN0 = 10
NCHAIN1 = 5
LN1_ROWS = 8
HOP = 4
NGV_A = [3] * (H // 2)
NGV_B = [3, 3, 1, 3, 3, 3, 1, 3, 3, 3, 3, 3, 1, 3, 3, 3]
NJOB = max(NGV_A) + max(NGV_B)
CHUNK = 8
KVP = 44
AR = 40
D_SM = 600
KNOBS_A = dict(early=2, slots=10, tail_h=8, d_j=600, d_f=150, d_s=250, d_pv=1400, d_o=200)
KNOBS_B = dict(early=3, slots=10, tail_h=4, d_j=530, d_f=50, d_s=250, d_pv=1400, d_o=170)


def _gelu(x):
    c = math.sqrt(2.0 / math.pi)
    return 0.5 * x * (1.0 + jnp.tanh(c * (x + 0.044715 * (x * x * x))))


def _layernorm(x):
    m = jnp.mean(x, axis=-1, keepdims=True)
    xc = x - m
    v = jnp.mean(xc * xc, axis=-1, keepdims=True)
    return xc * jax.lax.rsqrt(v + EPS)


def _slab_of(which, h):
    return which * H + (h % 2) * (H // 2) + h // 2


def _kernel(x_hbm, mem0_hbm, wq_hbm, wk_hbm, wv_hbm, wo_hbm,
            w1_hbm, w2_hbm, w3_hbm, w4_hbm, gw_hbm,
            out_hbm,
            x_v, stq_v, sto_v, wqkv_v, wo_v, w1_v, w2_v, w3_v, w4_v,
            h1_v, x1_v, g_v, ln1_v, ln3_v, mem0_v, gw_v, mem_v, out_v, kv_v, zero_v, sems, osem):
    c4 = D // 4
    xcuts = (0, 1, 2, 3, 5, N1)
    cp_x = [pltpu.make_async_copy(x_hbm.at[pl.ds(lo * T1, (hi - lo) * T1)],
                                  x_v.at[pl.ds(lo * T1, (hi - lo) * T1)], sems.at[n])
            for n, (lo, hi) in enumerate(zip(xcuts[:-1], xcuts[1:]))]
    cp_w1 = [pltpu.make_async_copy(w1_hbm.at[:, pl.ds(q * c4, c4)], w1_v.at[q], sems.at[5 + q])
             for q in range(4)]
    cp_w2 = [pltpu.make_async_copy(w2_hbm.at[:, pl.ds(q * c4, c4)], w2_v.at[q], sems.at[9])
             for q in range(4)]
    cp_ffn = [pltpu.make_async_copy(src, dst, sems.at[10])
              for src, dst in ((gw_hbm, gw_v), (mem0_hbm, mem0_v), (w3_hbm, w3_v), (w4_hbm, w4_v))]

    def piece_copies(i, slot):
        cps = [pltpu.make_async_copy(w.at[pl.ds(i * (DP * H), DP * H)], stq_v.at[slot, k],
                                     sems.at[11 + slot])
               for k, w in enumerate((wq_hbm, wk_hbm, wv_hbm))]
        cps.append(pltpu.make_async_copy(wo_hbm.at[pl.ds(i * OP, OP)], sto_v.at[slot],
                                         sems.at[11 + slot]))
        return cps

    for c in (cp_x[0:1] + cp_w1 + cp_x[1:] + cp_w2 + cp_ffn
              + piece_copies(0, 0) + piece_copies(1, 1)):
        c.start()
    x1_v[pl.ds(0, T3), :] = jnp.zeros((T3, D), F32)
    h1_v[:, pl.ds(8, 8), :] = jnp.zeros((D // 128, 8, 128), F32)
    h1_v[:, pl.ds(S, 8), :] = jnp.zeros((D // 128, 8, 128), F32)
    zero_v[...] = jnp.zeros((16, 128), U32)

    def ln_rows(x, tok, zero):
        if tok is not None:
            head = pltpu.bitcast(pltpu.bitcast(x[:, 0:128], U32) | tok, F32)
            x = jnp.concatenate([head, x[:, 128:]], axis=1)
        y = _layernorm(x)
        tok = None if zero is None else pltpu.bitcast(y[:, 0:128], U32) & zero
        return y, tok

    def ln_block(load, store, rows, nchain, gr):
        zero = zero_v[pl.ds(0, gr), :] if nchain else None
        toks = [None] * max(nchain, 1)
        for k in range(rows // gr):
            y, toks[k % len(toks)] = ln_rows(load(k * gr, gr), toks[k % len(toks)], zero)
            store(k * gr, y.astype(BF16))

    def prep1(blk, slot, nchain):
        r0 = blk * T1 if isinstance(blk, int) else pl.multiple_of(blk * T1, T1)

        def store(k, y):
            ln1_v[slot, pl.ds(k, y.shape[0]), :] = y

        ln_block(lambda k, n: x_v[pl.ds(r0 + k, n), :].astype(F32), store, T1, nchain, LN1_ROWS)

    def p1_quarter(lhs, r0, q):
        h = _gelu(jnp.dot(lhs, w1_v[q], preferred_element_type=F32))
        for j in range(2):
            win = h1_v.at[2 * q + j, pl.ds(r0, T1 + 16)]
            win[pl.ds(8 + (1, -1, 2, -2)[q], T1), :] = h[:, j * 128:(j + 1) * 128]

    cp_x[0].wait()
    prep1(0, 0, 0)
    for q in range(4):
        cp_w1[q].wait()
        if q == 3:
            cp_x[1].wait()
        lhs = ln1_v[0]
        if q == 3:
            prep1(1, 1, NCHAIN0)
        p1_quarter(lhs, 0, q)

    def p1_body(i, carry):
        r0 = pl.multiple_of(i * T1, T1)
        slot = i & 1

        lhs = ln1_v[slot]
        prep1(jnp.minimum(i + 1, N1 - 1), 1 - slot, NCHAIN1)
        for q in range(4):
            p1_quarter(lhs, r0, q)
        for n in range(3, len(cp_x)):
            pl.when(i + 2 == xcuts[n])(cp_x[n].wait)
        return carry

    cp_x[2].wait()
    with jax.named_scope('p1_body'):
        jax.lax.fori_loop(1, N1, p1_body, 0)
    for c in cp_w2:
        c.wait()

    def h1_rows(r0, n):
        return jnp.concatenate([h1_v[j, pl.ds(r0, n), :] for j in range(D // 128)], axis=1)

    def prep3(src, slot):
        def store(k, y):
            ln3_v[slot, pl.ds(k, y.shape[0]), :] = y

        ln_block(lambda k, n: src[pl.ds(k, n), :], store, T3, 1, 16)

    def p2_body(i, carry):
        r0 = pl.multiple_of(i * T2, T2)
        win = x1_v.at[pl.ds(r0, 2 * T2)]
        prep3(win, 0)
        hs = h1_rows(r0 + 8, T2).astype(BF16)
        for q in range(4):
            win[pl.ds(T2, T2), pl.ds(q * c4, c4)] = (
                jnp.dot(hs, w2_v[q], preferred_element_type=F32)
                + x_v[pl.ds(r0, T2), pl.ds(q * c4, c4)].astype(F32))
        return carry

    with jax.named_scope('p2_body'):
        jax.lax.fori_loop(0, N2, p2_body, 0)

    for c in cp_ffn + piece_copies(0, 0):
        c.wait()
    blk0 = (N2 - 2) * T2 // T3

    def p3_body(i, carry):
        r0 = pl.multiple_of((i + blk0) % N3 * T3, T3)
        r_next = pl.multiple_of((i + 1 + blk0) % N3 * T3, T3)
        slot = i & 1
        ring = i % NRING

        @pl.when(i + 2 < N3)
        def _():
            for c in piece_copies(i + 2, (i + 2) % NRING):
                c.start()

        lhs = ln3_v[slot]
        prep3(x1_v.at[pl.ds(T2 + r_next, T3)], 1 - slot)
        zero = zero_v[...]
        low16 = jax.lax.broadcasted_iota(jnp.int32, (16, 128), 1) < 64
        for which in range(3):
            tok = zero
            for j in range(DP // 2):
                blk = pltpu.bitcast(stq_v[ring, which, pl.ds(j * 64, 64), :], U32)
                a = blk[0:16] | tok
                c = blk[16:32]
                lo = (a & jnp.uint32(0xFFFF)) | (c << 16)
                hi = (a >> 16) | (c & jnp.uint32(0xFFFF0000))
                if which < 2:
                    tok = pltpu.roll((lo | hi) & zero, 1, 1)
                else:
                    t = pltpu.roll(jnp.where(low16, hi, lo), 64, 1)
                    lo, hi = jnp.where(low16, lo, t), jnp.where(low16, t, hi)
                    tok = hi & zero
                s0 = which * H * PITCH + i * (DP // 2) + j
                wqkv_v[pl.ds(s0, 16, stride=PITCH), :] = lo
                wqkv_v[pl.ds(s0 + 16 * PITCH, 16, stride=PITCH), :] = hi
        o0 = pl.multiple_of(i * (OP // 2), OP // 2)
        tok = zero
        for j in range(D // 128):
            for k in range(OP // 32):
                w = pltpu.bitcast(sto_v[ring, pl.ds(k * 32, 32), pl.ds(j * 128, 128)], U32) | tok
                tok = w & zero
                if k % HOP == HOP - 1:
                    tok = pltpu.roll(tok, 1, 1)
                kd = k - k % 8 + (0, 1, 4, 5, 2, 3, 6, 7)[k % 8]
                wo_v[j, pl.ds(o0 + kd * 16, 16), :] = w

        h = _gelu(jnp.dot(lhs, w3_v[...], preferred_element_type=F32)).astype(BF16)
        b = jnp.dot(h, w4_v[...], preferred_element_type=F32) + x1_v[pl.ds(T2 + r0, T3), :]
        gw = gw_v[...].astype(F32).reshape(1, D)
        z = jnp.sum(x_v[pl.ds(r0, T3), :].astype(F32) * gw, axis=-1, keepdims=True)
        g = 1.0 / (1.0 + jnp.exp(-z))
        g_v[pl.ds(r0, T3), :] = jnp.broadcast_to(g, (T3, 128))
        b = (1.0 - g) * b
        for j in range(D // 128):
            h1_v[j, pl.ds(r0, T3), :] = b[:, j * 128:(j + 1) * 128]

        @pl.when(i + 1 < N3)
        def _():
            for c in piece_copies(i + 1, (i + 1) % NRING):
                c.wait()

        return carry

    with jax.named_scope('p3_body'):
        jax.lax.fori_loop(0, N3, p3_body, 0)

    mem_v[...] = mem0_v[...].astype(F32)
    c_exp = (DH ** -0.5) * math.log2(math.e)
    neg_raw = NEG / (DH ** -0.5)

    L2 = 2 * L

    def make_mask(ngv):
        rm = L - 8 * ngv
        row = jax.lax.broadcasted_iota(jnp.int32, (2 * rm, 128), 0)
        col = jax.lax.broadcasted_iota(jnp.int32, (2 * rm, 128), 1)
        second = row >= rm
        rowl = jnp.where(second, row - rm, row)
        coll = jnp.where(second, col - L, col)
        real = (coll >= 0) & (coll < L)
        allowed = real & ((rowl < M) | (rowl + 8 * ngv >= coll))
        fill = jnp.where(allowed, 0.0, jnp.where(real, neg_raw, -jnp.inf)).astype(F32)
        return jnp.where(allowed, jnp.uint32(0xFFFFFFFF), jnp.uint32(0)), pltpu.bitcast(fill, U32)

    masks = {n: make_mask(n) for n in set(NGV_A + NGV_B)}
    neg_c = NEG * math.log2(math.e)

    def tied(w, toks):
        for tok in toks:
            w = jnp.concatenate([w[0:AR], w[AR:AR + 8] | tok, w[AR + 8:]], axis=0)
        return pltpu.bitcast(w, BF16)

    zpad = jnp.zeros((128 - L2, DH), F32)

    def recip(l):
        r = pl.reciprocal(l, approx=True)
        return r * (2.0 - l * r)

    def tree(op, x):
        while x.shape[0] > 1:
            x = op(x[0:x.shape[0] // 2], x[x.shape[0] // 2:])
        return x[0]

    causal = (jax.lax.broadcasted_iota(jnp.int32, (7, 8, 128), 1)
              > jax.lax.broadcasted_iota(jnp.int32, (7, 8, 128), 0))
    low = jax.lax.broadcasted_iota(jnp.int32, (8, 128), 1) < 64

    def stash(buf, slot, ks, ws, g):
        n = 8 * (g + 2)
        starts = []
        for i, x in enumerate(ks + ws):
            base = (4 * slot + i) * KVP
            buf[pl.ds(base, n), :] = jnp.concatenate([x[8 * g:8 * g + 8], x[0:n - 8]], axis=0)
            starts.append(base + n - 8)
        return buf, starts, [jnp.sum(w[n - 8:L], axis=0, keepdims=True) for w in ws]

    def vpu_start(q0, q1, parked, g):
        buf, starts, (acc_a, acc_b) = parked
        return dict(q=(q0 * c_exp, q1 * c_exp), buf=buf, starts=starts, g=g,
                    m=jnp.full((8, 128), neg_c, F32),
                    l=jnp.full((8, 128), float(L - 8 * (g + 1)), F32), a=acc_a, b=acc_b)

    def vpu_chunk(st, c0, gate):
        def windows(start):
            return jnp.concatenate([st['buf'][pl.ds(start - r, 8), :]
                                    for r in range(c0, c0 + CHUNK)], axis=0).reshape(CHUNK, 8, 128)

        k0, k1, wa, wb = st['starts']
        q0, q1 = [pltpu.bitcast(pltpu.bitcast(q, U32) | gate, F32) for q in st['q']]
        sc = jnp.where(low, jnp.sum(q0 * windows(k0), axis=-1, keepdims=True),
                       jnp.sum(q1 * windows(k1), axis=-1, keepdims=True))
        if c0 == 8 * st['g']:
            sc = jnp.concatenate([sc[0:1], jnp.where(causal, sc[1:], neg_c)], axis=0)
        m = jnp.maximum(tree(jnp.maximum, sc), st['m'])
        alpha = jnp.exp2(st['m'] - m)
        pr = jnp.exp2(sc - m)
        new = []
        for old, x in ((st['l'], pr), (st['a'], pr * windows(wa)), (st['b'], pr * windows(wb))):
            new.append(jnp.sum(jnp.concatenate([(old * alpha)[None], x], axis=0), axis=0))
        st.update(m=m, l=new[0], a=new[1], b=new[2])
        return (pltpu.bitcast(new[0], U32) | pltpu.bitcast(new[1], U32)
                | pltpu.bitcast(new[2], U32))

    def vpu_finish(st):
        r = recip(st['l'])
        return st['a'] * r, st['b'] * r

    def segment(lhs_q, lhs_kv, wo_m, ngv, n_chunks, unpack, wo_rows, split_first, zero,
                early, slots, tail_h, d_j, d_f, d_s, d_pv, d_o):
        NP = H // 2
        nj = D // 128
        HA = H - tail_h
        mxu_groups = [[0] + list(range(n + 1, 5)) for n in ngv]
        proj = {}
        qkv = [None] * NP
        pb = [None] * NP
        og = [dict() for _ in range(H)]
        ocat = {}
        y = [None] * nj

        def slab(toks, which, h, r0, n):
            x = lhs_q if which == 0 else lhs_kv
            w = tied(wqkv_v[pl.ds(_slab_of(which, h) * PITCH + r0, n), :], toks)
            r = jnp.dot(x[:, 2 * r0:2 * (r0 + n)], w, preferred_element_type=F32)
            proj[(which, h)] = r + proj[(which, h)] if (which, h) in proj else r
            return proj[(which, h)]

        def do_wo(toks, h0, h1, j):
            if (h0, h1) not in ocat:
                ocat[(h0, h1)] = jnp.concatenate(
                    [wo_rows(og[h]) for h in range(h0, h1)], axis=1).astype(BF16)
            w = tied(wo_v[j, pl.ds(h0 * 64, (h1 - h0) * 64), :], toks)
            r = jnp.dot(ocat[(h0, h1)], w, preferred_element_type=F32)
            y[j] = r if y[j] is None else r + y[j]
            return y[j]

        ticks = []
        pair_end = {}
        wo_early = [(4 * c, 4 * c + 4, j) for c in range(early) for j in range(nj)]
        first = NP - slots
        for p in range(NP):
            slabs = [(which, h) for h in (2 * p, 2 * p + 1) for which in range(3)]
            rows = [(lhs_q if w == 0 else lhs_kv).shape[0] for w, _ in slabs]
            if p == 0 and split_first:
                for r0 in (0, 256):
                    ticks += [(slab, (w, h, r0, 256), m) for (w, h), m in zip(slabs, rows)]
            else:
                mine = []
                if p >= first:
                    lo = (p - first) * len(wo_early) // slots
                    mine = wo_early[lo:(p - first + 1) * len(wo_early) // slots]
                att = 8 * len(mxu_groups[p])
                units = [(slab, slabs[k] + (r0, 256), rows[k] + att / 12)
                         for k0 in (0, 3) for r0 in (0, 256) for k in range(k0, k0 + 3)]
                for n, unit in enumerate(units):
                    ticks += [(do_wo, item, wo_m) for item in
                              mine[n * len(mine) // len(units):(n + 1) * len(mine) // len(units)]]
                    ticks.append(unit)
            pair_end[len(ticks) - 1] = p
        ticks += [(do_wo, (h0, h0 + 4, j), wo_m)
                  for h0 in range(4 * early, HA, 4) for j in range(nj)]
        ends = []
        for _, _, dur in ticks:
            ends.append(dur + (ends[-1] if ends else 0))

        def index(t):
            return next(i for i, e in enumerate(ends) if e >= t)

        events = {}
        anchors = {}
        cursor = [0]

        def run_chunk(res, p, name, st, c0, i_done):
            done = vpu_chunk(st, c0, pltpu.bitcast(res[0:8], U32) & zero)
            anchors.setdefault(i_done, []).append(done & zero)
            if c0 + CHUNK >= 8 * (st['g'] + 1):
                og[2 * p][name], og[2 * p + 1][name] = vpu_finish(st)

        def do_s(res, p):
            sc = jax.lax.dot_general(qkv[p][0], qkv[p][1], (((1,), (1,)), ((), ())),
                                     preferred_element_type=F32)
            keep, fill = masks[ngv[p]]
            sc = pltpu.bitcast((pltpu.bitcast(sc, U32) & keep) | fill, F32)
            e = jnp.exp2((sc - jnp.max(sc, axis=-1, keepdims=True)) * c_exp)
            l = jnp.sum(e, axis=-1, keepdims=True)
            e = e * recip(l)
            rm = 8 * len(mxu_groups[p])
            e = e[0:rm] + e[rm:2 * rm]
            if rm % 16:
                e = jnp.concatenate([e, jnp.zeros((8, 128), F32)], axis=0)
            pb[p] = e.astype(BF16)

        def do_pv(res, p):
            for i in range(2):
                o = jnp.dot(pb[p], qkv[p][2][i], preferred_element_type=F32)
                for n, g in enumerate(mxu_groups[p]):
                    og[2 * p + i][g] = o[8 * n:8 * n + 8]

        def finish_pair(p, i):
            u, jobs = unpack(p, [[proj[(w, h)] for w in range(3)] for h in (2 * p, 2 * p + 1)])
            chunks = [(name, st, c0) for name, st in
                      [(name, vpu_start(*job)) for name, job in jobs.items()]
                      for c0 in range(0, 8 * (st['g'] + 1), CHUNK)]
            t_first = ends[min(pair_end)]
            t_last = ends[-2] - d_j - d_f
            gap = (t_last - t_first) / (n_chunks - 1)
            if p == NP - 1:
                gap = min(gap, (t_last - max(ends[i], cursor[0])) / (len(chunks) - 1))
            for chunk in chunks:
                t = max(ends[i], cursor[0])
                cursor[0] = t + gap
                g = max(index(t), i + 1)
                events.setdefault(g, []).append(
                    (run_chunk, (p,) + chunk + (index(ends[g] + d_j) + 1,)))
            qb = jnp.concatenate([u[k][0][g] for k in range(2) for g in mxu_groups[p]],
                                 axis=0).astype(BF16)
            kb = jnp.concatenate([u[0][1], u[1][1], zpad], axis=0).astype(BF16)
            low40 = jnp.concatenate([low] * 5, axis=0)
            vb = [jnp.concatenate([jnp.where(low40, v, 0.0), jnp.where(low40, 0.0, v), zpad],
                                  axis=0).astype(BF16) for v in (u[0][2], u[1][2])]
            qkv[p] = (qb, kb, vb)
            t_pv = min(ends[i] + d_pv, ends[-1] - d_o)
            events.setdefault(index(min(ends[i] + d_s, t_pv - D_SM)), []).append((do_s, (p,)))
            events.setdefault(index(t_pv), []).append((do_pv, (p,)))

        for i, (fn, args, _) in enumerate(ticks):
            res = fn(anchors.pop(i, []), *args)
            if i in pair_end:
                finish_pair(pair_end[i], i)
            for f, a in events.pop(i, []):
                f(res, *a)
        assert not events
        for j in range(nj):
            do_wo([], HA, H, j)
        return jnp.concatenate(y, axis=1)

    def pair(r0, mem):
        xf = x_v[pl.ds(r0, PAIR), :].astype(F32)
        zero = zero_v[pl.ds(0, 8), :]
        x1s = jnp.concatenate([xf[0:8], xf[32:40]], axis=0).astype(BF16)
        keep = [None] * (H // 2)

        def cat(*xs):
            return jnp.concatenate(xs, axis=0)

        lhs = cat(mem, xf[8:32]).astype(BF16)

        def finish(p, qg, ks, vs, slot, groups):
            return ([(qg[i], ks[i], vs[i]) for i in range(2)],
                    {g: stash(kv_v[p], slot + n, ks, vs, g) for n, g in enumerate(groups)})

        def unpack_a(p, qkv):
            qg = [{0: q[0:8], 2: q[8:16], 3: q[16:24], 4: q[24:32]} for q, _, _ in qkv]
            ks = [cat(k[0:8], k[32:40], k[8:32]) for _, k, _ in qkv]
            vs = [cat(v[0:8], v[32:40], v[8:32]) for _, _, v in qkv]
            u, parked = finish(p, qg, ks, vs, 0, range(1, NGV_A[p] + 1))
            keep[p] = (parked[1], [(k[40:48], v[40:48]) for _, k, v in qkv])
            return u, {g: (qg[0][g], qg[1][g], parked[g], g) for g in range(2, NGV_A[p] + 1)}

        y_a = segment(lhs, cat(lhs, x1s), 32, NGV_A,
                      sum(g + 1 for n in NGV_A for g in range(2, n + 1)) * 8 // CHUNK, unpack_a,
                      lambda o: cat(o[0], o[2], o[3], o[4]), False, zero, **KNOBS_A)

        lhs = cat(y_a[0:8], xf[40:64]).astype(BF16)

        def unpack_b(p, qkv):
            parked_a1, kv1 = keep[p]
            qg = [{0: q[0:8], 1: q[40:48], 2: q[8:16], 3: q[16:24], 4: q[24:32]}
                  for q, _, _ in qkv]
            ks = [cat(k[0:8], e[0], k[8:32]) for (_, k, _), e in zip(qkv, kv1)]
            vs = [cat(v[0:8], e[1], v[8:32]) for (_, _, v), e in zip(qkv, kv1)]
            u, parked = finish(p, qg, ks, vs, max(NGV_A), range(1, NGV_B[p] + 1))
            jobs = {'a1': (qkv[0][0][32:40], qkv[1][0][32:40], parked_a1, 1)}
            jobs.update({g: (qg[0][g], qg[1][g], parked[g], g) for g in range(1, NGV_B[p] + 1)})
            return u, jobs

        y_b = segment(cat(lhs, x1s), lhs, 48, NGV_B,
                      sum(2 + sum(range(2, n + 2)) for n in NGV_B) * 8 // CHUNK, unpack_b,
                      lambda o: cat(o[0], o[1], o[2], o[3], o[4], o['a1']), True, zero,
                      **KNOBS_B)

        a = cat(y_b[40:48], y_a[8:32], y_b[8:40])
        g = g_v[pl.ds(r0, PAIR), :]
        g = jnp.concatenate([g] * (D // 128), axis=1)
        out_v[pl.ds(r0, PAIR), :] = (g * a + h1_rows(r0, PAIR)).astype(BF16)
        return y_b[0:8]

    def a_body(t, carry):
        r0 = pl.multiple_of(t * PAIR, PAIR)
        mem_v[...] = pair(r0, mem_v[...])
        pltpu.make_async_copy(out_v.at[pl.ds(r0, PAIR)], out_hbm.at[pl.ds(r0, PAIR)],
                              osem).start()
        return carry

    with jax.named_scope('a_body'):
        jax.lax.fori_loop(0, S // PAIR, a_body, 0)
    pltpu.make_async_copy(out_v, out_hbm, osem).wait()


@jax.jit
def pallas_gated_mix__memory_aug_recurrent_mem_tr__mixer_s_mlp__prompt_kernel(
    A_x, A_mem0, A_Wq, A_Wk, A_Wv, A_Wo, A_seg_len, B_x, B_w1, B_w2, B_w3, B_w4, gate_w,
):
    assert A_x.shape == (1, S, D) and A_Wq.shape == (D, H, DH) and A_mem0.shape == (1, M, D)
    x = A_x.reshape(S, D)
    mem0 = A_mem0.reshape(M, D)
    wq = A_Wq.reshape(D * H, DH)
    wk = A_Wk.reshape(D * H, DH)
    wv = A_Wv.reshape(D * H, DH)
    wo = A_Wo.reshape(H * DH, D)

    any_spec = pl.BlockSpec(memory_space=pl.ANY)
    out = pl.pallas_call(
        _kernel,
        out_shape=jax.ShapeDtypeStruct((S, D), BF16),
        in_specs=[any_spec] * 11,
        out_specs=any_spec,
        scratch_shapes=[
            pltpu.VMEM((S, D), BF16),
            pltpu.VMEM((NRING, 3, DP * H, DH), BF16),
            pltpu.VMEM((NRING, OP, D), BF16),
            pltpu.VMEM((3 * H * PITCH + 544, 128), U32),
            pltpu.VMEM((D // 128, H * DH // 2, 128), U32),
            pltpu.VMEM((4, D, D // 4), BF16),
            pltpu.VMEM((4, D, D // 4), BF16),
            pltpu.VMEM((D, FF), BF16),
            pltpu.VMEM((FF, D), BF16),
            pltpu.VMEM((D // 128, S + 16, 128), F32),
            pltpu.VMEM((S + T2, D), F32),
            pltpu.VMEM((S, 128), F32),
            pltpu.VMEM((2, T1, D), BF16),
            pltpu.VMEM((2, T3, D), BF16),
            pltpu.VMEM((M, D), BF16),
            pltpu.VMEM((D,), BF16),
            pltpu.VMEM((M, D), F32),
            pltpu.VMEM((S, D), BF16),
            [pltpu.VMEM((NJOB * 4 * KVP, 128), F32)] * (H // 2),
            pltpu.VMEM((16, 128), U32),
            pltpu.SemaphoreType.DMA((NSEM,)),
            pltpu.SemaphoreType.DMA(()),
        ],
        compiler_params=pltpu.CompilerParams(vmem_limit_bytes=120 * 1024 * 1024,
                                             disable_bounds_checks=True),
    )(x, mem0, wq, wk, wv, wo, B_w1, B_w2, B_w3, B_w4, gate_w)
    return out.reshape(1, S, D)
```

```python
import math

import jax
import jax.numpy as jnp
import jax.experimental.pallas as pl
import jax.experimental.pallas.tpu as pltpu

F32 = jnp.float32
BF16 = jnp.bfloat16
U32 = jnp.uint32

S = 2048
D = 1024
H = 32
DH = 128
M = 8
SEG = 32
L = M + SEG
FF = 3584
EPS = 1e-5
NEG = -1e9

PAIR = 2 * SEG
T1 = 256
N1 = S // T1
T2 = 512
N2 = S // T2
T3 = 256
N3 = S // T3
DP = D // N3
OP = H * DH // N3
PITCH = 520
NRING = 3
NSEM = 11 + NRING

NCHAIN0 = 10
NCHAIN1 = 5
LN1_ROWS = 8
HOP = 4
NGV = 3
CHUNK = 8
KVP = 48
AR = 40
GR = 24
TAIL_H = 8
WO_SLOTS = 10
D_SM = 560
D_PP = 200
KNOBS_A = dict(early=2, d_g=80, d_j=700, d_f=50, d_s=350, d_pv=1050, d_o=200)
KNOBS_B = dict(early=3, d_g=0, d_j=530, d_f=50, d_s=200, d_pv=1000, d_o=170)


def _gelu(x):
    c = math.sqrt(2.0 / math.pi)
    return 0.5 * x * (1.0 + jnp.tanh(c * (x + 0.044715 * (x * x * x))))


def _layernorm(x):
    m = jnp.mean(x, axis=-1, keepdims=True)
    xc = x - m
    v = jnp.mean(xc * xc, axis=-1, keepdims=True)
    return xc * jax.lax.rsqrt(v + EPS)


def _slab_of(which, h):
    return which * H + (h % 2) * (H // 2) + h // 2


def _kernel(x_hbm, mem0_hbm, wq_hbm, wk_hbm, wv_hbm, wo_hbm,
            w1_hbm, w2_hbm, w3_hbm, w4_hbm, gw_hbm,
            out_hbm,
            x_v, stq_v, sto_v, wqkv_v, wo_v, w1_v, w2_v, w3_v, w4_v,
            h1_v, x1_v, g_v, ln1_v, ln3_v, mem0_v, gw_v, mem_v, out_v, kv_v, zero_v, sems, osem):
    c4 = D // 4
    xcuts = (0, 1, 2, 3, 5, N1)
    cp_x = [pltpu.make_async_copy(x_hbm.at[pl.ds(lo * T1, (hi - lo) * T1)],
                                  x_v.at[pl.ds(lo * T1, (hi - lo) * T1)], sems.at[n])
            for n, (lo, hi) in enumerate(zip(xcuts[:-1], xcuts[1:]))]
    cp_w1 = [pltpu.make_async_copy(w1_hbm.at[:, pl.ds(q * c4, c4)], w1_v.at[q], sems.at[5 + q])
             for q in range(4)]
    cp_w2 = [pltpu.make_async_copy(w2_hbm.at[:, pl.ds(q * c4, c4)], w2_v.at[q], sems.at[9])
             for q in range(4)]
    cp_ffn = [pltpu.make_async_copy(src, dst, sems.at[10])
              for src, dst in ((gw_hbm, gw_v), (mem0_hbm, mem0_v), (w3_hbm, w3_v), (w4_hbm, w4_v))]

    def piece_copies(i, slot):
        cps = [pltpu.make_async_copy(w.at[pl.ds(i * (DP * H), DP * H)], stq_v.at[slot, k],
                                     sems.at[11 + slot])
               for k, w in enumerate((wq_hbm, wk_hbm, wv_hbm))]
        cps.append(pltpu.make_async_copy(wo_hbm.at[pl.ds(i * OP, OP)], sto_v.at[slot],
                                         sems.at[11 + slot]))
        return cps

    for c in (cp_x[0:1] + cp_w1 + cp_x[1:] + cp_w2 + cp_ffn
              + piece_copies(0, 0) + piece_copies(1, 1)):
        c.start()
    x1_v[pl.ds(0, T3), :] = jnp.zeros((T3, D), F32)
    h1_v[:, pl.ds(8, 8), :] = jnp.zeros((D // 128, 8, 128), F32)
    h1_v[:, pl.ds(S, 8), :] = jnp.zeros((D // 128, 8, 128), F32)
    zero_v[...] = jnp.zeros((16, 128), U32)

    def ln_rows(x, tok, zero):
        if tok is not None:
            head = pltpu.bitcast(pltpu.bitcast(x[:, 0:128], U32) | tok, F32)
            x = jnp.concatenate([head, x[:, 128:]], axis=1)
        y = _layernorm(x)
        tok = None if zero is None else pltpu.bitcast(y[:, 0:128], U32) & zero
        return y, tok

    def ln_block(load, store, rows, nchain, gr):
        zero = zero_v[pl.ds(0, gr), :] if nchain else None
        toks = [None] * max(nchain, 1)
        for k in range(rows // gr):
            y, toks[k % len(toks)] = ln_rows(load(k * gr, gr), toks[k % len(toks)], zero)
            store(k * gr, y.astype(BF16))

    def prep1(blk, slot, nchain):
        r0 = blk * T1 if isinstance(blk, int) else pl.multiple_of(blk * T1, T1)

        def store(k, y):
            ln1_v[slot, pl.ds(k, y.shape[0]), :] = y

        ln_block(lambda k, n: x_v[pl.ds(r0 + k, n), :].astype(F32), store, T1, nchain, LN1_ROWS)

    def p1_quarter(lhs, r0, q):
        h = _gelu(jnp.dot(lhs, w1_v[q], preferred_element_type=F32))
        for j in range(2):
            win = h1_v.at[2 * q + j, pl.ds(r0, T1 + 16)]
            win[pl.ds(8 + (1, -1, 2, -2)[q], T1), :] = h[:, j * 128:(j + 1) * 128]

    cp_x[0].wait()
    prep1(0, 0, 0)
    for q in range(4):
        cp_w1[q].wait()
        if q == 3:
            cp_x[1].wait()
        lhs = ln1_v[0]
        if q == 3:
            prep1(1, 1, NCHAIN0)
        p1_quarter(lhs, 0, q)

    def p1_body(i, carry):
        r0 = pl.multiple_of(i * T1, T1)
        slot = i & 1

        lhs = ln1_v[slot]
        prep1(jnp.minimum(i + 1, N1 - 1), 1 - slot, NCHAIN1)
        for q in range(4):
            p1_quarter(lhs, r0, q)
        for n in range(3, len(cp_x)):
            pl.when(i + 2 == xcuts[n])(cp_x[n].wait)
        return carry

    cp_x[2].wait()
    with jax.named_scope('p1_body'):
        jax.lax.fori_loop(1, N1, p1_body, 0)
    for c in cp_w2:
        c.wait()

    def h1_rows(r0, n):
        return jnp.concatenate([h1_v[j, pl.ds(r0, n), :] for j in range(D // 128)], axis=1)

    def prep3(src, slot):
        def store(k, y):
            ln3_v[slot, pl.ds(k, y.shape[0]), :] = y

        ln_block(lambda k, n: src[pl.ds(k, n), :], store, T3, 1, 16)

    def p2_body(i, carry):
        r0 = pl.multiple_of(i * T2, T2)
        win = x1_v.at[pl.ds(r0, 2 * T2)]
        prep3(win, 0)
        hs = h1_rows(r0 + 8, T2).astype(BF16)
        for q in range(4):
            win[pl.ds(T2, T2), pl.ds(q * c4, c4)] = (
                jnp.dot(hs, w2_v[q], preferred_element_type=F32)
                + x_v[pl.ds(r0, T2), pl.ds(q * c4, c4)].astype(F32))
        return carry

    with jax.named_scope('p2_body'):
        jax.lax.fori_loop(0, N2, p2_body, 0)

    for c in cp_ffn + piece_copies(0, 0):
        c.wait()
    blk0 = (N2 - 2) * T2 // T3

    def p3_body(i, carry):
        r0 = pl.multiple_of((i + blk0) % N3 * T3, T3)
        r_next = pl.multiple_of((i + 1 + blk0) % N3 * T3, T3)
        slot = i & 1
        ring = i % NRING

        @pl.when(i + 2 < N3)
        def _():
            for c in piece_copies(i + 2, (i + 2) % NRING):
                c.start()

        lhs = ln3_v[slot]
        prep3(x1_v.at[pl.ds(T2 + r_next, T3)], 1 - slot)
        zero = zero_v[...]
        low16 = jax.lax.broadcasted_iota(jnp.int32, (16, 128), 1) < 64
        for which in range(3):
            tok = zero
            for j in range(DP // 2):
                blk = pltpu.bitcast(stq_v[ring, which, pl.ds(j * 64, 64), :], U32)
                a = blk[0:16] | tok
                c = blk[16:32]
                lo = (a & jnp.uint32(0xFFFF)) | (c << 16)
                hi = (a >> 16) | (c & jnp.uint32(0xFFFF0000))
                if which < 2:
                    tok = pltpu.roll((lo | hi) & zero, 1, 1)
                else:
                    t = pltpu.roll(jnp.where(low16, hi, lo), 64, 1)
                    lo, hi = jnp.where(low16, lo, t), jnp.where(low16, t, hi)
                    tok = hi & zero
                s0 = which * H * PITCH + i * (DP // 2) + j
                wqkv_v[pl.ds(s0, 16, stride=PITCH), :] = lo
                wqkv_v[pl.ds(s0 + 16 * PITCH, 16, stride=PITCH), :] = hi
        o0 = pl.multiple_of(i * (OP // 2), OP // 2)
        tok = zero
        for j in range(D // 128):
            for k in range(OP // 32):
                w = pltpu.bitcast(sto_v[ring, pl.ds(k * 32, 32), pl.ds(j * 128, 128)], U32) | tok
                tok = w & zero
                if k % HOP == HOP - 1:
                    tok = pltpu.roll(tok, 1, 1)
                kd = k - k % 8 + (0, 1, 4, 5, 2, 3, 6, 7)[k % 8]
                wo_v[j, pl.ds(o0 + kd * 16, 16), :] = w

        h = _gelu(jnp.dot(lhs, w3_v[...], preferred_element_type=F32)).astype(BF16)
        b = jnp.dot(h, w4_v[...], preferred_element_type=F32) + x1_v[pl.ds(T2 + r0, T3), :]
        gw = gw_v[...].astype(F32).reshape(1, D)
        z = jnp.sum(x_v[pl.ds(r0, T3), :].astype(F32) * gw, axis=-1, keepdims=True)
        g = 1.0 / (1.0 + jnp.exp(-z))
        g_v[pl.ds(r0, T3), :] = jnp.broadcast_to(g, (T3, 128))
        b = (1.0 - g) * b
        for j in range(D // 128):
            h1_v[j, pl.ds(r0, T3), :] = b[:, j * 128:(j + 1) * 128]

        @pl.when(i + 1 < N3)
        def _():
            for c in piece_copies(i + 1, (i + 1) % NRING):
                c.wait()

        return carry

    with jax.named_scope('p3_body'):
        jax.lax.fori_loop(0, N3, p3_body, 0)

    mem_v[...] = mem0_v[...].astype(F32)
    c_exp = (DH ** -0.5) * math.log2(math.e)
    neg_raw = NEG / (DH ** -0.5)

    L2 = 2 * L
    mxu_groups = [0] + list(range(NGV + 1, 5))
    rm = 8 * len(mxu_groups)
    row = jax.lax.broadcasted_iota(jnp.int32, (2 * rm, 128), 0)
    col = jax.lax.broadcasted_iota(jnp.int32, (2 * rm, 128), 1)
    second = row >= rm
    rowl = jnp.where(second, row - rm, row)
    coll = jnp.where(second, col - L, col)
    real = (coll >= 0) & (coll < L)
    allowed = real & ((rowl < M) | (rowl + 8 * NGV >= coll))
    keep = jnp.where(allowed, jnp.uint32(0xFFFFFFFF), jnp.uint32(0))
    fill = pltpu.bitcast(
        jnp.where(allowed, 0.0, jnp.where(real, neg_raw, -jnp.inf)).astype(F32), U32)
    neg_c = NEG * math.log2(math.e)

    def tied(w, toks):
        for tok in toks:
            w = jnp.concatenate([w[0:AR], w[AR:AR + 8] | tok, w[AR + 8:]], axis=0)
        return pltpu.bitcast(w, BF16)

    zpad = jnp.zeros((128 - L2, DH), F32)

    def recip(l):
        r = pl.reciprocal(l, approx=True)
        return r * (2.0 - l * r)

    def tree(op, x):
        while x.shape[0] > 1:
            x = x.reshape(x.shape[0] // 2, 16, 128)
            x = op(x[:, 0:8], x[:, 8:16])
        return x[0]

    causal = (jax.lax.broadcasted_iota(jnp.int32, (7, 8, 128), 1)
              > jax.lax.broadcasted_iota(jnp.int32, (7, 8, 128), 0))
    low = jax.lax.broadcasted_iota(jnp.int32, (8, 128), 1) < 64

    def stash(buf, slot, ks, ws, g):
        n = 8 * (g + 2)
        starts = []
        for i, x in enumerate(ks + ws):
            base = (4 * slot + i) * KVP
            buf[pl.ds(base, n), :] = jnp.concatenate([x[8 * g:8 * g + 8], x[0:n - 8]], axis=0)
            starts.append(base + n - 8)
        return buf, starts, [jnp.sum(w[n - 8:L], axis=0, keepdims=True) for w in ws]

    def vpu_start(q0, q1, parked, g):
        buf, starts, (acc_a, acc_b) = parked
        return dict(q=(q0 * c_exp, q1 * c_exp), buf=buf, starts=starts, g=g,
                    m=jnp.full((8, 128), neg_c, F32),
                    l=jnp.full((8, 128), float(L - 8 * (g + 1)), F32), a=acc_a, b=acc_b)

    def vpu_chunk(st, c0, gate):
        def windows(*starts):
            return jnp.concatenate(
                [st['buf'][pl.ds(k - r, 8), :] for r in range(c0, c0 + CHUNK) for k in starts],
                axis=0).reshape(CHUNK, 8 * len(starts), 128)

        k0, k1, wa, wb = st['starts']
        q = jnp.concatenate([pltpu.bitcast(pltpu.bitcast(x, U32) | gate, F32) for x in st['q']],
                            axis=0)
        sc = jnp.sum(q * windows(k0, k1), axis=-1, keepdims=True)
        sc = jnp.where(low, sc[:, 0:8], sc[:, 8:16])
        if c0 == 8 * st['g']:
            sc = jnp.concatenate([sc[0:1], jnp.where(causal, sc[1:], neg_c)], axis=0)
        m = jnp.maximum(tree(jnp.maximum, sc), st['m'])
        alpha = jnp.exp2(st['m'] - m)
        pr = jnp.exp2(sc - m)
        new = []
        for old, x in ((st['l'], pr), (st['a'], pr * windows(wa)), (st['b'], pr * windows(wb))):
            new.append(jnp.sum(jnp.concatenate([(old * alpha)[None], x], axis=0), axis=0))
        st.update(m=m, l=new[0], a=new[1], b=new[2])
        return (pltpu.bitcast(new[0], U32) | pltpu.bitcast(new[1], U32)
                | pltpu.bitcast(new[2], U32))

    def vpu_finish(st):
        r = recip(st['l'])
        return st['a'] * r, st['b'] * r

    def segment(lhs_q, lhs_kv, wo_m, unpack, wo_rows, split_first, zero,
                early, d_g, d_j, d_f, d_s, d_pv, d_o):
        NP = H // 2
        nj = D // 128
        HA = H - TAIL_H
        proj = {}
        qkv = [None] * NP
        pb = [None] * NP
        og = [dict() for _ in range(H)]
        ocat = {}
        y = [None] * nj

        def slab(toks, which, h, r0, n):
            x = lhs_q if which == 0 else lhs_kv
            w = tied(wqkv_v[pl.ds(_slab_of(which, h) * PITCH + r0, n), :], toks)
            r = jnp.dot(x[:, 2 * r0:2 * (r0 + n)], w, preferred_element_type=F32)
            proj[(which, h)] = r + proj[(which, h)] if (which, h) in proj else r
            return proj[(which, h)]

        def do_wo(toks, h0, h1, j):
            if (h0, h1) not in ocat:
                ocat[(h0, h1)] = jnp.concatenate(
                    [wo_rows(og[h]) for h in range(h0, h1)], axis=1).astype(BF16)
            w = tied(wo_v[j, pl.ds(h0 * 64, (h1 - h0) * 64), :], toks)
            r = jnp.dot(ocat[(h0, h1)], w, preferred_element_type=F32)
            y[j] = r if y[j] is None else r + y[j]
            return y[j]

        ticks = []
        pair_end = {}
        wo_early = [(4 * c, 4 * c + 4, j) for c in range(early) for j in range(nj)]
        first = NP - WO_SLOTS
        for p in range(NP):
            slabs = [(which, h) for h in (2 * p, 2 * p + 1) for which in range(3)]
            rows = [(lhs_q if w == 0 else lhs_kv).shape[0] for w, _ in slabs]
            if p == 0 and split_first:
                for r0 in (0, 256):
                    ticks += [(slab, (w, h, r0, 256), m) for (w, h), m in zip(slabs, rows)]
            else:
                mine = []
                if p >= first:
                    lo = (p - first) * len(wo_early) // WO_SLOTS
                    mine = wo_early[lo:(p - first + 1) * len(wo_early) // WO_SLOTS]
                units = [(slab, slabs[k] + (r0, 256), rows[k] + rm / 12)
                         for k0 in (0, 3) for r0 in (0, 256) for k in range(k0, k0 + 3)]
                for n, unit in enumerate(units):
                    ticks += [(do_wo, item, wo_m) for item in
                              mine[n * len(mine) // len(units):(n + 1) * len(mine) // len(units)]]
                    ticks.append(unit)
            pair_end[len(ticks) - 1] = p
        ticks += [(do_wo, (h0, h0 + 4, j), wo_m)
                  for h0 in range(4 * early, HA, 4) for j in range(nj)]
        ends = []
        for _, _, dur in ticks:
            ends.append(dur + (ends[-1] if ends else 0))

        def index(t):
            return next(i for i, e in enumerate(ends) if e >= t)

        events = {}
        anchors = {}
        cursor = [0]

        def run_chunk(res, p, name, st, c0, i_done):
            done = vpu_chunk(st, c0, pltpu.bitcast(res[GR:GR + 8], U32) & zero)
            anchors.setdefault(i_done, []).append(done & zero)
            if c0 + CHUNK >= 8 * (st['g'] + 1):
                og[2 * p][name], og[2 * p + 1][name] = vpu_finish(st)

        def do_s(res, p):
            sc = jax.lax.dot_general(qkv[p][0], qkv[p][1], (((1,), (1,)), ((), ())),
                                     preferred_element_type=F32)
            sc = pltpu.bitcast((pltpu.bitcast(sc, U32) & keep) | fill, F32)
            e = jnp.exp2((sc - jnp.max(sc, axis=-1, keepdims=True)) * c_exp)
            l = jnp.sum(e, axis=-1, keepdims=True)
            e = e * recip(l)
            pb[p] = (e[0:rm] + e[rm:2 * rm]).astype(BF16)

        def do_pv(res, p):
            for i in range(2):
                o = jnp.dot(pb[p], qkv[p][2][i], preferred_element_type=F32)
                for n, g in enumerate(mxu_groups):
                    og[2 * p + i][g] = o[8 * n:8 * n + 8]

        def finish_pair(p, i):
            u, jobs = unpack(p, [[proj[(w, h)] for w in range(3)] for h in (2 * p, 2 * p + 1)])
            chunks = [(name, st, c0) for name, st in
                      [(name, vpu_start(*job)) for name, job in jobs.items()]
                      for c0 in range(0, 8 * (st['g'] + 1), CHUNK)]
            t_first = ends[min(pair_end)] + d_g
            t_last = ends[-2] - d_j - d_f
            gap = (t_last - t_first) / (NP * len(chunks) - 1)
            if p == NP - 1:
                gap = min(gap, (t_last - max(ends[i] + d_g, cursor[0])) / (len(chunks) - 1))
            for chunk in chunks:
                t = max(ends[i] + d_g, cursor[0])
                cursor[0] = t + gap
                g = max(index(t), i + 1)
                events.setdefault(g, []).append(
                    (run_chunk, (p,) + chunk + (index(ends[g] + d_j) + 1,)))
            qb = jnp.concatenate([u[k][0][g] for k in range(2) for g in mxu_groups],
                                 axis=0).astype(BF16)
            kb = jnp.concatenate([u[0][1], u[1][1], zpad], axis=0).astype(BF16)
            low40 = jnp.concatenate([low] * 5, axis=0)
            vb = [jnp.concatenate([jnp.where(low40, v, 0.0), jnp.where(low40, 0.0, v), zpad],
                                  axis=0).astype(BF16) for v in (u[0][2], u[1][2])]
            qkv[p] = (qb, kb, vb)
            if p % 4 == 3:
                t2 = min(ends[i] + d_pv, ends[-1] - d_o)
                t1 = t2 - D_PP
                events.setdefault(index(min(ends[i] + d_s, t1 - D_SM)), []).extend(
                    (do_s, (k,)) for k in range(p - 3, p + 1))
                events.setdefault(index(t1), []).extend((do_pv, (k,)) for k in (p - 3, p - 2))
                events.setdefault(index(t2), []).extend((do_pv, (k,)) for k in (p - 1, p))

        for i, (fn, args, _) in enumerate(ticks):
            res = fn(anchors.pop(i, []), *args)
            if i in pair_end:
                finish_pair(pair_end[i], i)
            for f, a in events.pop(i, []):
                f(res, *a)
        assert not events
        for j in range(nj):
            do_wo([], HA, H, j)
        return jnp.concatenate(y, axis=1)

    def pair(r0, mem):
        xf = x_v[pl.ds(r0, PAIR), :].astype(F32)
        zero = zero_v[pl.ds(0, 8), :]
        x1s = jnp.concatenate([xf[0:8], xf[32:40]], axis=0).astype(BF16)
        carry = [None] * (H // 2)

        def cat(*xs):
            return jnp.concatenate(xs, axis=0)

        lhs = cat(mem, xf[8:32]).astype(BF16)

        def park(p, ks, vs, slot):
            return {g: stash(kv_v[p], slot + g - 1, ks, vs, g) for g in range(1, NGV + 1)}

        def unpack_a(p, qkv):
            qg = [{0: q[0:8], 2: q[8:16], 3: q[16:24], 4: q[24:32]} for q, _, _ in qkv]
            ks = [cat(k[0:8], k[32:40], k[8:32]) for _, k, _ in qkv]
            vs = [cat(v[0:8], v[32:40], v[8:32]) for _, _, v in qkv]
            parked = park(p, ks, vs, 0)
            carry[p] = (parked[1], [(k[40:48], v[40:48]) for _, k, v in qkv])
            return (list(zip(qg, ks, vs)),
                    {g: (qg[0][g], qg[1][g], parked[g], g) for g in range(2, NGV + 1)})

        y_a = segment(lhs, cat(lhs, x1s), 32, unpack_a, lambda o: cat(o[0], o[2], o[3], o[4]),
                      False, zero, **KNOBS_A)

        lhs = cat(y_a[0:8], xf[40:64]).astype(BF16)

        def unpack_b(p, qkv):
            parked_a1, kv1 = carry[p]
            qg = [{0: q[0:8], 1: q[40:48], 2: q[8:16], 3: q[16:24], 4: q[24:32]}
                  for q, _, _ in qkv]
            ks = [cat(k[0:8], e[0], k[8:32]) for (_, k, _), e in zip(qkv, kv1)]
            vs = [cat(v[0:8], e[1], v[8:32]) for (_, _, v), e in zip(qkv, kv1)]
            parked = park(p, ks, vs, NGV)
            jobs = {'a1': (qkv[0][0][32:40], qkv[1][0][32:40], parked_a1, 1)}
            jobs.update({g: (qg[0][g], qg[1][g], parked[g], g) for g in range(1, NGV + 1)})
            return list(zip(qg, ks, vs)), jobs

        y_b = segment(cat(lhs, x1s), lhs, 48, unpack_b,
                      lambda o: cat(o[0], o[1], o[2], o[3], o[4], o['a1']),
                      True, zero, **KNOBS_B)

        a = cat(y_b[40:48], y_a[8:32], y_b[8:40])
        g = g_v[pl.ds(r0, PAIR), :]
        g = jnp.concatenate([g] * (D // 128), axis=1)
        out_v[pl.ds(r0, PAIR), :] = (g * a + h1_rows(r0, PAIR)).astype(BF16)
        return y_b[0:8]

    def a_body(t, carry):
        r0 = pl.multiple_of(t * PAIR, PAIR)
        mem_v[...] = pair(r0, mem_v[...])
        pltpu.make_async_copy(out_v.at[pl.ds(r0, PAIR)], out_hbm.at[pl.ds(r0, PAIR)],
                              osem).start()
        return carry

    with jax.named_scope('a_body'):
        jax.lax.fori_loop(0, S // PAIR, a_body, 0)
    pltpu.make_async_copy(out_v, out_hbm, osem).wait()


@jax.jit
def pallas_gated_mix__memory_aug_recurrent_mem_tr__mixer_s_mlp__prompt_kernel(
    A_x, A_mem0, A_Wq, A_Wk, A_Wv, A_Wo, A_seg_len, B_x, B_w1, B_w2, B_w3, B_w4, gate_w,
):
    assert A_x.shape == (1, S, D) and A_Wq.shape == (D, H, DH) and A_mem0.shape == (1, M, D)
    x = A_x.reshape(S, D)
    mem0 = A_mem0.reshape(M, D)
    wq = A_Wq.reshape(D * H, DH)
    wk = A_Wk.reshape(D * H, DH)
    wv = A_Wv.reshape(D * H, DH)
    wo = A_Wo.reshape(H * DH, D)

    any_spec = pl.BlockSpec(memory_space=pl.ANY)
    out = pl.pallas_call(
        _kernel,
        out_shape=jax.ShapeDtypeStruct((S, D), BF16),
        in_specs=[any_spec] * 11,
        out_specs=any_spec,
        scratch_shapes=[
            pltpu.VMEM((S, D), BF16),
            pltpu.VMEM((NRING, 3, DP * H, DH), BF16),
            pltpu.VMEM((NRING, OP, D), BF16),
            pltpu.VMEM((3 * H * PITCH + 544, 128), U32),
            pltpu.VMEM((D // 128, H * DH // 2, 128), U32),
            pltpu.VMEM((4, D, D // 4), BF16),
            pltpu.VMEM((4, D, D // 4), BF16),
            pltpu.VMEM((D, FF), BF16),
            pltpu.VMEM((FF, D), BF16),
            pltpu.VMEM((D // 128, S + 16, 128), F32),
            pltpu.VMEM((S + T2, D), F32),
            pltpu.VMEM((S, 128), F32),
            pltpu.VMEM((2, T1, D), BF16),
            pltpu.VMEM((2, T3, D), BF16),
            pltpu.VMEM((M, D), BF16),
            pltpu.VMEM((D,), BF16),
            pltpu.VMEM((M, D), F32),
            pltpu.VMEM((S, D), BF16),
            [pltpu.VMEM((2 * NGV * 4 * KVP, 128), F32)] * (H // 2),
            pltpu.VMEM((16, 128), U32),
            pltpu.SemaphoreType.DMA((NSEM,)),
            pltpu.SemaphoreType.DMA(()),
        ],
        compiler_params=pltpu.CompilerParams(vmem_limit_bytes=120 * 1024 * 1024,
                                             disable_bounds_checks=True),
    )(x, mem0, wq, wk, wv, wo, B_w1, B_w2, B_w3, B_w4, gate_w)
    return out.reshape(1, S, D)
```

```python
import math

import jax
import jax.numpy as jnp
import jax.experimental.pallas as pl
import jax.experimental.pallas.tpu as pltpu

F32 = jnp.float32
BF16 = jnp.bfloat16
U32 = jnp.uint32

S = 2048
D = 1024
H = 32
DH = 128
M = 8
SEG = 32
L = M + SEG
FF = 3584
EPS = 1e-5
NEG = -1e9

PAIR = 2 * SEG
T1 = 256
N1 = S // T1
T2 = 512
N2 = S // T2
T3 = 256
N3 = S // T3
DP = D // N3
OP = H * DH // N3
PITCH = 520
NRING = 3
NSEM = 11 + NRING

NCHAIN0 = 10
NCHAIN1 = 5
LN1_ROWS = 8
HOP = 4
NGV = 3
CHUNK = 8
KVP = 48
AR = 40
GR = 24
TAIL_H = 8
WO_SLOTS = 10
D_SM = 560
D_PP = 200
ORDER_A = ((0, 0), (1, 0), (2, 0), (0, 1), (1, 1), (2, 1))
ORDER_B = ((0, 0), (1, 0), (1, 1), (0, 1), (2, 0), (2, 1))
KNOBS_A = dict(order=ORDER_A, early=2, d_g=40, d_j=700, d_f=50, d_s=350, d_pv=900, d_o=200)
KNOBS_B = dict(order=ORDER_B, early=3, d_g=0, d_j=530, d_f=50, d_s=200, d_pv=1000, d_o=170)


def _gelu(x):
    c = math.sqrt(2.0 / math.pi)
    return 0.5 * x * (1.0 + jnp.tanh(c * (x + 0.044715 * (x * x * x))))


def _layernorm(x):
    m = jnp.mean(x, axis=-1, keepdims=True)
    xc = x - m
    v = jnp.mean(xc * xc, axis=-1, keepdims=True)
    return xc * jax.lax.rsqrt(v + EPS)


def _slab_of(which, h):
    return which * H + (h % 2) * (H // 2) + h // 2


def _kernel(x_hbm, mem0_hbm, wq_hbm, wk_hbm, wv_hbm, wo_hbm,
            w1_hbm, w2_hbm, w3_hbm, w4_hbm, gw_hbm,
            out_hbm,
            x_v, stq_v, sto_v, wqkv_v, wo_v, w1_v, w2_v, w3_v, w4_v,
            h1_v, x1_v, g_v, ln1_v, ln3_v, mem0_v, gw_v, mem_v, out_v, kv_v, zero_v, sems, osem):
    c4 = D // 4
    xcuts = (0, 1, 2, 3, 5, N1)
    cp_x = [pltpu.make_async_copy(x_hbm.at[pl.ds(lo * T1, (hi - lo) * T1)],
                                  x_v.at[pl.ds(lo * T1, (hi - lo) * T1)], sems.at[n])
            for n, (lo, hi) in enumerate(zip(xcuts[:-1], xcuts[1:]))]
    cp_w1 = [pltpu.make_async_copy(w1_hbm.at[:, pl.ds(q * c4, c4)], w1_v.at[q], sems.at[5 + q])
             for q in range(4)]
    cp_w2 = [pltpu.make_async_copy(w2_hbm.at[:, pl.ds(q * c4, c4)], w2_v.at[q], sems.at[9])
             for q in range(4)]
    cp_ffn = [pltpu.make_async_copy(src, dst, sems.at[10])
              for src, dst in ((gw_hbm, gw_v), (mem0_hbm, mem0_v), (w3_hbm, w3_v), (w4_hbm, w4_v))]

    def piece_copies(i, slot):
        cps = [pltpu.make_async_copy(w.at[pl.ds(i * (DP * H), DP * H)], stq_v.at[slot, k],
                                     sems.at[11 + slot])
               for k, w in enumerate((wq_hbm, wk_hbm, wv_hbm))]
        cps.append(pltpu.make_async_copy(wo_hbm.at[pl.ds(i * OP, OP)], sto_v.at[slot],
                                         sems.at[11 + slot]))
        return cps

    for c in (cp_x[0:1] + cp_w1 + cp_x[1:] + cp_w2 + cp_ffn
              + piece_copies(0, 0) + piece_copies(1, 1)):
        c.start()
    x1_v[pl.ds(0, T3), :] = jnp.zeros((T3, D), F32)
    h1_v[:, pl.ds(8, 8), :] = jnp.zeros((D // 128, 8, 128), F32)
    h1_v[:, pl.ds(S, 8), :] = jnp.zeros((D // 128, 8, 128), F32)
    zero_v[...] = jnp.zeros((16, 128), U32)

    def ln_rows(x, tok, zero):
        if tok is not None:
            head = pltpu.bitcast(pltpu.bitcast(x[:, 0:128], U32) | tok, F32)
            x = jnp.concatenate([head, x[:, 128:]], axis=1)
        y = _layernorm(x)
        tok = None if zero is None else pltpu.bitcast(y[:, 0:128], U32) & zero
        return y, tok

    def ln_block(load, store, rows, nchain, gr):
        zero = zero_v[pl.ds(0, gr), :] if nchain else None
        toks = [None] * max(nchain, 1)
        for k in range(rows // gr):
            y, toks[k % len(toks)] = ln_rows(load(k * gr, gr), toks[k % len(toks)], zero)
            store(k * gr, y.astype(BF16))

    def prep1(blk, slot, nchain):
        r0 = blk * T1 if isinstance(blk, int) else pl.multiple_of(blk * T1, T1)

        def store(k, y):
            ln1_v[slot, pl.ds(k, y.shape[0]), :] = y

        ln_block(lambda k, n: x_v[pl.ds(r0 + k, n), :].astype(F32), store, T1, nchain, LN1_ROWS)

    def p1_quarter(lhs, r0, q):
        h = _gelu(jnp.dot(lhs, w1_v[q], preferred_element_type=F32))
        for j in range(2):
            win = h1_v.at[2 * q + j, pl.ds(r0, T1 + 16)]
            win[pl.ds(8 + (1, -1, 2, -2)[q], T1), :] = h[:, j * 128:(j + 1) * 128]

    cp_x[0].wait()
    prep1(0, 0, 0)
    for q in range(4):
        cp_w1[q].wait()
        if q == 3:
            cp_x[1].wait()
        lhs = ln1_v[0]
        if q == 3:
            prep1(1, 1, NCHAIN0)
        p1_quarter(lhs, 0, q)

    def p1_body(i, carry):
        r0 = pl.multiple_of(i * T1, T1)
        slot = i & 1

        lhs = ln1_v[slot]
        prep1(jnp.minimum(i + 1, N1 - 1), 1 - slot, NCHAIN1)
        for q in range(4):
            p1_quarter(lhs, r0, q)
        for n in range(3, len(cp_x)):
            pl.when(i + 2 == xcuts[n])(cp_x[n].wait)
        return carry

    cp_x[2].wait()
    with jax.named_scope('p1_body'):
        jax.lax.fori_loop(1, N1, p1_body, 0)
    for c in cp_w2:
        c.wait()

    def h1_rows(r0, n):
        return jnp.concatenate([h1_v[j, pl.ds(r0, n), :] for j in range(D // 128)], axis=1)

    def prep3(src, slot):
        def store(k, y):
            ln3_v[slot, pl.ds(k, y.shape[0]), :] = y

        ln_block(lambda k, n: src[pl.ds(k, n), :], store, T3, 1, 16)

    def p2_body(i, carry):
        r0 = pl.multiple_of(i * T2, T2)
        win = x1_v.at[pl.ds(r0, 2 * T2)]
        prep3(win, 0)
        hs = h1_rows(r0 + 8, T2).astype(BF16)
        for q in range(4):
            win[pl.ds(T2, T2), pl.ds(q * c4, c4)] = (
                jnp.dot(hs, w2_v[q], preferred_element_type=F32)
                + x_v[pl.ds(r0, T2), pl.ds(q * c4, c4)].astype(F32))
        return carry

    with jax.named_scope('p2_body'):
        jax.lax.fori_loop(0, N2, p2_body, 0)

    for c in cp_ffn + piece_copies(0, 0):
        c.wait()
    blk0 = (N2 - 2) * T2 // T3

    def p3_body(i, carry):
        r0 = pl.multiple_of((i + blk0) % N3 * T3, T3)
        r_next = pl.multiple_of((i + 1 + blk0) % N3 * T3, T3)
        slot = i & 1
        ring = i % NRING

        @pl.when(i + 2 < N3)
        def _():
            for c in piece_copies(i + 2, (i + 2) % NRING):
                c.start()

        lhs = ln3_v[slot]
        prep3(x1_v.at[pl.ds(T2 + r_next, T3)], 1 - slot)
        zero = zero_v[...]
        low16 = jax.lax.broadcasted_iota(jnp.int32, (16, 128), 1) < 64
        for which in range(3):
            tok = zero
            for j in range(DP // 2):
                blk = pltpu.bitcast(stq_v[ring, which, pl.ds(j * 64, 64), :], U32)
                a = blk[0:16] | tok
                c = blk[16:32]
                lo = (a & jnp.uint32(0xFFFF)) | (c << 16)
                hi = (a >> 16) | (c & jnp.uint32(0xFFFF0000))
                if which < 2:
                    tok = pltpu.roll((lo | hi) & zero, 1, 1)
                else:
                    t = pltpu.roll(jnp.where(low16, hi, lo), 64, 1)
                    lo, hi = jnp.where(low16, lo, t), jnp.where(low16, t, hi)
                    tok = hi & zero
                s0 = which * H * PITCH + i * (DP // 2) + j
                wqkv_v[pl.ds(s0, 16, stride=PITCH), :] = lo
                wqkv_v[pl.ds(s0 + 16 * PITCH, 16, stride=PITCH), :] = hi
        o0 = pl.multiple_of(i * (OP // 2), OP // 2)
        tok = zero
        for j in range(D // 128):
            for k in range(OP // 32):
                w = pltpu.bitcast(sto_v[ring, pl.ds(k * 32, 32), pl.ds(j * 128, 128)], U32) | tok
                tok = w & zero
                if k % HOP == HOP - 1:
                    tok = pltpu.roll(tok, 1, 1)
                kd = k - k % 8 + (0, 1, 4, 5, 2, 3, 6, 7)[k % 8]
                wo_v[j, pl.ds(o0 + kd * 16, 16), :] = w

        h = _gelu(jnp.dot(lhs, w3_v[...], preferred_element_type=F32)).astype(BF16)
        b = jnp.dot(h, w4_v[...], preferred_element_type=F32) + x1_v[pl.ds(T2 + r0, T3), :]
        gw = gw_v[...].astype(F32).reshape(1, D)
        z = jnp.sum(x_v[pl.ds(r0, T3), :].astype(F32) * gw, axis=-1, keepdims=True)
        g = 1.0 / (1.0 + jnp.exp(-z))
        g_v[pl.ds(r0, T3), :] = jnp.broadcast_to(g, (T3, 128))
        b = (1.0 - g) * b
        for j in range(D // 128):
            h1_v[j, pl.ds(r0, T3), :] = b[:, j * 128:(j + 1) * 128]

        @pl.when(i + 1 < N3)
        def _():
            for c in piece_copies(i + 1, (i + 1) % NRING):
                c.wait()

        return carry

    with jax.named_scope('p3_body'):
        jax.lax.fori_loop(0, N3, p3_body, 0)

    mem_v[...] = mem0_v[...].astype(F32)
    c_exp = (DH ** -0.5) * math.log2(math.e)
    neg_raw = NEG / (DH ** -0.5)

    L2 = 2 * L
    mxu_groups = [0] + list(range(NGV + 1, 5))
    rm = 8 * len(mxu_groups)
    row = jax.lax.broadcasted_iota(jnp.int32, (2 * rm, 128), 0)
    col = jax.lax.broadcasted_iota(jnp.int32, (2 * rm, 128), 1)
    second = row >= rm
    rowl = jnp.where(second, row - rm, row)
    coll = jnp.where(second, col - L, col)
    real = (coll >= 0) & (coll < L)
    allowed = real & ((rowl < M) | (rowl + 8 * NGV >= coll))
    keep = jnp.where(allowed, jnp.uint32(0xFFFFFFFF), jnp.uint32(0))
    fill = pltpu.bitcast(
        jnp.where(allowed, 0.0, jnp.where(real, neg_raw, -jnp.inf)).astype(F32), U32)
    neg_c = NEG * math.log2(math.e)

    def tied(w, toks):
        for tok in toks:
            w = jnp.concatenate([w[0:AR], w[AR:AR + 8] | tok, w[AR + 8:]], axis=0)
        return pltpu.bitcast(w, BF16)

    zpad = jnp.zeros((128 - L2, DH), F32)

    def recip(l):
        r = pl.reciprocal(l, approx=True)
        return r * (2.0 - l * r)

    def tree(op, x):
        while x.shape[0] > 1:
            x = x.reshape(x.shape[0] // 2, 16, 128)
            x = op(x[:, 0:8], x[:, 8:16])
        return x[0]

    causal = (jax.lax.broadcasted_iota(jnp.int32, (7, 8, 128), 1)
              > jax.lax.broadcasted_iota(jnp.int32, (7, 8, 128), 0))
    low = jax.lax.broadcasted_iota(jnp.int32, (8, 128), 1) < 64

    def stash(buf, slot, ks, ws, g):
        n = 8 * (g + 2)
        starts = []
        for i, x in enumerate(ks + ws):
            base = (4 * slot + i) * KVP
            buf[pl.ds(base, n), :] = jnp.concatenate([x[8 * g:8 * g + 8], x[0:n - 8]], axis=0)
            starts.append(base + n - 8)
        return buf, starts, [jnp.sum(w[n - 8:L], axis=0, keepdims=True) for w in ws]

    def vpu_start(q0, q1, parked, g):
        buf, starts, (acc_a, acc_b) = parked
        return dict(q=(q0 * c_exp, q1 * c_exp), buf=buf, starts=starts, g=g,
                    m=jnp.full((8, 128), neg_c, F32),
                    l=jnp.full((8, 128), float(L - 8 * (g + 1)), F32), a=acc_a, b=acc_b)

    def vpu_chunk(st, c0, gate):
        def windows(*starts):
            return jnp.concatenate(
                [st['buf'][pl.ds(k - r, 8), :] for r in range(c0, c0 + CHUNK) for k in starts],
                axis=0).reshape(CHUNK, 8 * len(starts), 128)

        k0, k1, wa, wb = st['starts']
        q = jnp.concatenate([pltpu.bitcast(pltpu.bitcast(x, U32) | gate, F32) for x in st['q']],
                            axis=0)
        sc = jnp.sum(q * windows(k0, k1), axis=-1, keepdims=True)
        sc = jnp.where(low, sc[:, 0:8], sc[:, 8:16])
        if c0 == 8 * st['g']:
            sc = jnp.concatenate([sc[0:1], jnp.where(causal, sc[1:], neg_c)], axis=0)
        m = jnp.maximum(tree(jnp.maximum, sc), st['m'])
        alpha = jnp.exp2(st['m'] - m)
        pr = jnp.exp2(sc - m)
        new = []
        for old, x in ((st['l'], pr), (st['a'], pr * windows(wa)), (st['b'], pr * windows(wb))):
            new.append(jnp.sum(jnp.concatenate([(old * alpha)[None], x], axis=0), axis=0))
        st.update(m=m, l=new[0], a=new[1], b=new[2])
        return (pltpu.bitcast(new[0], U32) | pltpu.bitcast(new[1], U32)
                | pltpu.bitcast(new[2], U32))

    def vpu_finish(st):
        r = recip(st['l'])
        return st['a'] * r, st['b'] * r

    def segment(lhs_q, lhs_kv, wo_m, unpack, wo_rows, split_first, zero,
                order, early, d_g, d_j, d_f, d_s, d_pv, d_o):
        NP = H // 2
        nj = D // 128
        HA = H - TAIL_H
        proj = {}
        qkv = [None] * NP
        pb = [None] * NP
        og = [dict() for _ in range(H)]
        ocat = {}
        y = [None] * nj

        def slab(toks, which, h, r0, n):
            x = lhs_q if which == 0 else lhs_kv
            w = tied(wqkv_v[pl.ds(_slab_of(which, h) * PITCH + r0, n), :], toks)
            r = jnp.dot(x[:, 2 * r0:2 * (r0 + n)], w, preferred_element_type=F32)
            proj[(which, h)] = r + proj[(which, h)] if (which, h) in proj else r
            return proj[(which, h)]

        def do_wo(toks, h0, h1, j):
            if (h0, h1) not in ocat:
                ocat[(h0, h1)] = jnp.concatenate(
                    [wo_rows(og[h]) for h in range(h0, h1)], axis=1).astype(BF16)
            w = tied(wo_v[j, pl.ds(h0 * 64, (h1 - h0) * 64), :], toks)
            r = jnp.dot(ocat[(h0, h1)], w, preferred_element_type=F32)
            y[j] = r if y[j] is None else r + y[j]
            return y[j]

        ticks = []
        pair_end = {}
        wo_early = [(4 * c, 4 * c + 4, j) for c in range(early) for j in range(nj)]
        first = NP - WO_SLOTS
        for p in range(NP):
            slabs = [(which, h) for h in (2 * p, 2 * p + 1) for which in range(3)]
            rows = [(lhs_q if w == 0 else lhs_kv).shape[0] for w, _ in slabs]
            if p == 0 and split_first:
                for r0 in (0, 256):
                    ticks += [(slab, (w, h, r0, 256), m) for (w, h), m in zip(slabs, rows)]
            else:
                mine = []
                if p >= first:
                    lo = (p - first) * len(wo_early) // WO_SLOTS
                    mine = wo_early[lo:(p - first + 1) * len(wo_early) // WO_SLOTS]
                units = [(slab, slabs[k0 + k] + (256 * half, 256), rows[k0 + k] + rm / 12)
                         for k0 in (0, 3) for k, half in order]
                for n, unit in enumerate(units):
                    ticks += [(do_wo, item, wo_m) for item in
                              mine[n * len(mine) // len(units):(n + 1) * len(mine) // len(units)]]
                    ticks.append(unit)
            pair_end[len(ticks) - 1] = p
        ticks += [(do_wo, (h0, h0 + 4, j), wo_m)
                  for h0 in range(4 * early, HA, 4) for j in range(nj)]
        ends = []
        for _, _, dur in ticks:
            ends.append(dur + (ends[-1] if ends else 0))

        def index(t):
            return next(i for i, e in enumerate(ends) if e >= t)

        events = {}
        anchors = {}
        cursor = [0]

        def run_chunk(res, p, name, st, c0, i_done):
            done = vpu_chunk(st, c0, pltpu.bitcast(res[GR:GR + 8], U32) & zero)
            anchors.setdefault(i_done, []).append(done & zero)
            if c0 + CHUNK >= 8 * (st['g'] + 1):
                og[2 * p][name], og[2 * p + 1][name] = vpu_finish(st)

        def do_s(res, p):
            sc = jax.lax.dot_general(qkv[p][0], qkv[p][1], (((1,), (1,)), ((), ())),
                                     preferred_element_type=F32)
            sc = pltpu.bitcast((pltpu.bitcast(sc, U32) & keep) | fill, F32)
            e = jnp.exp2((sc - jnp.max(sc, axis=-1, keepdims=True)) * c_exp)
            l = jnp.sum(e, axis=-1, keepdims=True)
            e = e * recip(l)
            pb[p] = (e[0:rm] + e[rm:2 * rm]).astype(BF16)

        def do_pv(res, p):
            for i in range(2):
                o = jnp.dot(pb[p], qkv[p][2][i], preferred_element_type=F32)
                for n, g in enumerate(mxu_groups):
                    og[2 * p + i][g] = o[8 * n:8 * n + 8]

        def finish_pair(p, i):
            u, jobs = unpack(p, [[proj[(w, h)] for w in range(3)] for h in (2 * p, 2 * p + 1)])
            chunks = [(name, st, c0) for name, st in
                      [(name, vpu_start(*job)) for name, job in jobs.items()]
                      for c0 in range(0, 8 * (st['g'] + 1), CHUNK)]
            t_first = ends[min(pair_end)] + d_g
            t_last = ends[-2] - d_j - d_f
            gap = (t_last - t_first) / (NP * len(chunks) - 1)
            if p == NP - 1:
                gap = min(gap, (t_last - max(ends[i] + d_g, cursor[0])) / (len(chunks) - 1))
            for chunk in chunks:
                t = max(ends[i] + d_g, cursor[0])
                cursor[0] = t + gap
                g = max(index(t), i + 1)
                events.setdefault(g, []).append(
                    (run_chunk, (p,) + chunk + (index(ends[g] + d_j) + 1,)))
            qb = jnp.concatenate([u[k][0][g] for k in range(2) for g in mxu_groups],
                                 axis=0).astype(BF16)
            kb = jnp.concatenate([u[0][1], u[1][1], zpad], axis=0).astype(BF16)
            low40 = jnp.concatenate([low] * 5, axis=0)
            vb = [jnp.concatenate([jnp.where(low40, v, 0.0), jnp.where(low40, 0.0, v), zpad],
                                  axis=0).astype(BF16) for v in (u[0][2], u[1][2])]
            qkv[p] = (qb, kb, vb)
            if p % 4 == 3:
                t2 = min(ends[i] + d_pv, ends[-1] - d_o)
                t1 = t2 - D_PP
                events.setdefault(index(min(ends[i] + d_s, t1 - D_SM)), []).extend(
                    (do_s, (k,)) for k in range(p - 3, p + 1))
                events.setdefault(index(t1), []).extend((do_pv, (k,)) for k in (p - 3, p - 2))
                events.setdefault(index(t2), []).extend((do_pv, (k,)) for k in (p - 1, p))

        for i, (fn, args, _) in enumerate(ticks):
            res = fn(anchors.pop(i, []), *args)
            if i in pair_end:
                finish_pair(pair_end[i], i)
            for f, a in events.pop(i, []):
                f(res, *a)
        assert not events
        for j in range(nj):
            do_wo([], HA, H, j)
        return jnp.concatenate(y, axis=1)

    def pair(r0, mem):
        xf = x_v[pl.ds(r0, PAIR), :].astype(F32)
        zero = zero_v[pl.ds(0, 8), :]
        x1s = jnp.concatenate([xf[0:8], xf[32:40]], axis=0).astype(BF16)
        carry = [None] * (H // 2)

        def cat(*xs):
            return jnp.concatenate(xs, axis=0)

        lhs = cat(mem, xf[8:32]).astype(BF16)

        def park(p, ks, vs, slot):
            return {g: stash(kv_v[p], slot + g - 1, ks, vs, g) for g in range(1, NGV + 1)}

        def unpack_a(p, qkv):
            qg = [{0: q[0:8], 2: q[8:16], 3: q[16:24], 4: q[24:32]} for q, _, _ in qkv]
            ks = [cat(k[0:8], k[32:40], k[8:32]) for _, k, _ in qkv]
            vs = [cat(v[0:8], v[32:40], v[8:32]) for _, _, v in qkv]
            parked = park(p, ks, vs, 0)
            carry[p] = (parked[1], [(k[40:48], v[40:48]) for _, k, v in qkv])
            return (list(zip(qg, ks, vs)),
                    {g: (qg[0][g], qg[1][g], parked[g], g) for g in range(2, NGV + 1)})

        y_a = segment(lhs, cat(lhs, x1s), 32, unpack_a, lambda o: cat(o[0], o[2], o[3], o[4]),
                      False, zero, **KNOBS_A)

        lhs = cat(y_a[0:8], xf[40:64]).astype(BF16)

        def unpack_b(p, qkv):
            parked_a1, kv1 = carry[p]
            qg = [{0: q[0:8], 1: q[40:48], 2: q[8:16], 3: q[16:24], 4: q[24:32]}
                  for q, _, _ in qkv]
            ks = [cat(k[0:8], e[0], k[8:32]) for (_, k, _), e in zip(qkv, kv1)]
            vs = [cat(v[0:8], e[1], v[8:32]) for (_, _, v), e in zip(qkv, kv1)]
            parked = park(p, ks, vs, NGV)
            jobs = {'a1': (qkv[0][0][32:40], qkv[1][0][32:40], parked_a1, 1)}
            jobs.update({g: (qg[0][g], qg[1][g], parked[g], g) for g in range(1, NGV + 1)})
            return list(zip(qg, ks, vs)), jobs

        y_b = segment(cat(lhs, x1s), lhs, 48, unpack_b,
                      lambda o: cat(o[0], o[1], o[2], o[3], o[4], o['a1']),
                      True, zero, **KNOBS_B)

        a = cat(y_b[40:48], y_a[8:32], y_b[8:40])
        g = g_v[pl.ds(r0, PAIR), :]
        g = jnp.concatenate([g] * (D // 128), axis=1)
        out_v[pl.ds(r0, PAIR), :] = (g * a + h1_rows(r0, PAIR)).astype(BF16)
        return y_b[0:8]

    def a_body(t, carry):
        r0 = pl.multiple_of(t * PAIR, PAIR)
        mem_v[...] = pair(r0, mem_v[...])
        pltpu.make_async_copy(out_v.at[pl.ds(r0, PAIR)], out_hbm.at[pl.ds(r0, PAIR)],
                              osem).start()
        return carry

    with jax.named_scope('a_body'):
        jax.lax.fori_loop(0, S // PAIR, a_body, 0)
    pltpu.make_async_copy(out_v, out_hbm, osem).wait()


@jax.jit
def pallas_gated_mix__memory_aug_recurrent_mem_tr__mixer_s_mlp__prompt_kernel(
    A_x, A_mem0, A_Wq, A_Wk, A_Wv, A_Wo, A_seg_len, B_x, B_w1, B_w2, B_w3, B_w4, gate_w,
):
    assert A_x.shape == (1, S, D) and A_Wq.shape == (D, H, DH) and A_mem0.shape == (1, M, D)
    x = A_x.reshape(S, D)
    mem0 = A_mem0.reshape(M, D)
    wq = A_Wq.reshape(D * H, DH)
    wk = A_Wk.reshape(D * H, DH)
    wv = A_Wv.reshape(D * H, DH)
    wo = A_Wo.reshape(H * DH, D)

    any_spec = pl.BlockSpec(memory_space=pl.ANY)
    out = pl.pallas_call(
        _kernel,
        out_shape=jax.ShapeDtypeStruct((S, D), BF16),
        in_specs=[any_spec] * 11,
        out_specs=any_spec,
        scratch_shapes=[
            pltpu.VMEM((S, D), BF16),
            pltpu.VMEM((NRING, 3, DP * H, DH), BF16),
            pltpu.VMEM((NRING, OP, D), BF16),
            pltpu.VMEM((3 * H * PITCH + 544, 128), U32),
            pltpu.VMEM((D // 128, H * DH // 2, 128), U32),
            pltpu.VMEM((4, D, D // 4), BF16),
            pltpu.VMEM((4, D, D // 4), BF16),
            pltpu.VMEM((D, FF), BF16),
            pltpu.VMEM((FF, D), BF16),
            pltpu.VMEM((D // 128, S + 16, 128), F32),
            pltpu.VMEM((S + T2, D), F32),
            pltpu.VMEM((S, 128), F32),
            pltpu.VMEM((2, T1, D), BF16),
            pltpu.VMEM((2, T3, D), BF16),
            pltpu.VMEM((M, D), BF16),
            pltpu.VMEM((D,), BF16),
            pltpu.VMEM((M, D), F32),
            pltpu.VMEM((S, D), BF16),
            [pltpu.VMEM((2 * NGV * 4 * KVP, 128), F32)] * (H // 2),
            pltpu.VMEM((16, 128), U32),
            pltpu.SemaphoreType.DMA((NSEM,)),
            pltpu.SemaphoreType.DMA(()),
        ],
        compiler_params=pltpu.CompilerParams(vmem_limit_bytes=120 * 1024 * 1024,
                                             disable_bounds_checks=True),
    )(x, mem0, wq, wk, wv, wo, B_w1, B_w2, B_w3, B_w4, gate_w)
    return out.reshape(1, S, D)
```

```python
import math

import jax
import jax.numpy as jnp
import jax.experimental.pallas as pl
import jax.experimental.pallas.tpu as pltpu

F32 = jnp.float32
BF16 = jnp.bfloat16
U32 = jnp.uint32

S = 2048
D = 1024
H = 32
DH = 128
M = 8
SEG = 32
L = M + SEG
FF = 3584
EPS = 1e-5
NEG = -1e9

PAIR = 2 * SEG
T1 = 256
N1 = S // T1
T2 = 512
N2 = S // T2
T3 = 256
N3 = S // T3
DP = D // N3
OP = H * DH // N3
PITCH = 520
NRING = 3
NSEM = 11 + NRING

NCHAIN0 = 10
NCHAIN1 = 5
LN1_ROWS = 8
HOP = 4
NGV = 3
FULL_A = (1, 5, 8, 11)
CHUNK = 8
AR = 40
GR = 24
TAIL_H = 8
D_SM = 560
D_PP = 200
ORDER_A = ((0, 0), (1, 0), (2, 0), (0, 1), (1, 1), (2, 1))
ORDER_B = ((0, 0), (1, 0), (1, 1), (0, 1), (2, 0), (2, 1))
KNOBS_A = dict(order=ORDER_A, early=2, slots=2, d_g=80, d_j=620, d_f=50, d_s=350, d_pv=1050, d_o=200)
KNOBS_B = dict(order=ORDER_B, early=3, slots=10, d_g=0, d_j=530, d_f=50, d_s=200, d_pv=1000, d_o=200)
KV_ROWS = 8 * (L + 8) + 4 * NGV * 16


def _gelu(x):
    c = math.sqrt(2.0 / math.pi)
    return 0.5 * x * (1.0 + jnp.tanh(c * (x + 0.044715 * (x * x * x))))


def _layernorm(x):
    m = jnp.mean(x, axis=-1, keepdims=True)
    xc = x - m
    v = jnp.mean(xc * xc, axis=-1, keepdims=True)
    return xc * jax.lax.rsqrt(v + EPS)


def _slab_of(which, h):
    return which * H + (h % 2) * (H // 2) + h // 2


def key0_row(seg, i):
    return (4 * seg + i) * (L + 8) + 8


def _kernel(x_hbm, mem0_hbm, wq_hbm, wk_hbm, wv_hbm, wo_hbm,
            w1_hbm, w2_hbm, w3_hbm, w4_hbm, gw_hbm,
            out_hbm,
            x_v, stq_v, sto_v, wqkv_v, wo_v, w1_v, w2_v, w3_v, w4_v,
            h1_v, x1_v, g_v, ln1_v, ln3_v, mem0_v, gw_v, mem_v, out_v, kv_v, zero_v, sems, osem):
    c4 = D // 4
    xcuts = (0, 1, 2, 3, 5, N1)
    cp_x = [pltpu.make_async_copy(x_hbm.at[pl.ds(lo * T1, (hi - lo) * T1)],
                                  x_v.at[pl.ds(lo * T1, (hi - lo) * T1)], sems.at[n])
            for n, (lo, hi) in enumerate(zip(xcuts[:-1], xcuts[1:]))]
    cp_w1 = [pltpu.make_async_copy(w1_hbm.at[:, pl.ds(q * c4, c4)], w1_v.at[q], sems.at[5 + q])
             for q in range(4)]
    cp_w2 = [pltpu.make_async_copy(w2_hbm.at[:, pl.ds(q * c4, c4)], w2_v.at[q], sems.at[9])
             for q in range(4)]
    cp_ffn = [pltpu.make_async_copy(src, dst, sems.at[10])
              for src, dst in ((gw_hbm, gw_v), (mem0_hbm, mem0_v), (w3_hbm, w3_v), (w4_hbm, w4_v))]

    def piece_copies(i, slot):
        cps = [pltpu.make_async_copy(w.at[pl.ds(i * (DP * H), DP * H)], stq_v.at[slot, k],
                                     sems.at[11 + slot])
               for k, w in enumerate((wq_hbm, wk_hbm, wv_hbm))]
        cps.append(pltpu.make_async_copy(wo_hbm.at[pl.ds(i * OP, OP)], sto_v.at[slot],
                                         sems.at[11 + slot]))
        return cps

    for c in (cp_x[0:1] + cp_w1 + cp_x[1:] + cp_w2 + cp_ffn
              + piece_copies(0, 0) + piece_copies(1, 1)):
        c.start()
    x1_v[pl.ds(0, T3), :] = jnp.zeros((T3, D), F32)
    h1_v[:, pl.ds(8, 8), :] = jnp.zeros((D // 128, 8, 128), F32)
    h1_v[:, pl.ds(S, 8), :] = jnp.zeros((D // 128, 8, 128), F32)
    zero_v[...] = jnp.zeros((16, 128), U32)
    for buf in kv_v:
        for seg in range(2):
            for i in range(2):
                buf[pl.ds(key0_row(seg, i) - 8, 8), :] = jnp.zeros((8, 128), F32)

    def ln_rows(x, tok, zero):
        if tok is not None:
            head = pltpu.bitcast(pltpu.bitcast(x[:, 0:128], U32) | tok, F32)
            x = jnp.concatenate([head, x[:, 128:]], axis=1)
        y = _layernorm(x)
        tok = None if zero is None else pltpu.bitcast(y[:, 0:128], U32) & zero
        return y, tok

    def ln_block(load, store, rows, nchain, gr):
        zero = zero_v[pl.ds(0, gr), :] if nchain else None
        toks = [None] * max(nchain, 1)
        for k in range(rows // gr):
            y, toks[k % len(toks)] = ln_rows(load(k * gr, gr), toks[k % len(toks)], zero)
            store(k * gr, y.astype(BF16))

    def prep1(blk, slot, nchain):
        r0 = blk * T1 if isinstance(blk, int) else pl.multiple_of(blk * T1, T1)

        def store(k, y):
            ln1_v[slot, pl.ds(k, y.shape[0]), :] = y

        ln_block(lambda k, n: x_v[pl.ds(r0 + k, n), :].astype(F32), store, T1, nchain, LN1_ROWS)

    def p1_quarter(lhs, r0, q):
        h = _gelu(jnp.dot(lhs, w1_v[q], preferred_element_type=F32))
        for j in range(2):
            win = h1_v.at[2 * q + j, pl.ds(r0, T1 + 16)]
            win[pl.ds(8 + (1, -1, 2, -2)[q], T1), :] = h[:, j * 128:(j + 1) * 128]

    cp_x[0].wait()
    prep1(0, 0, 0)
    for q in range(4):
        cp_w1[q].wait()
        if q == 3:
            cp_x[1].wait()
        lhs = ln1_v[0]
        if q == 3:
            prep1(1, 1, NCHAIN0)
        p1_quarter(lhs, 0, q)

    def p1_body(i, carry):
        r0 = pl.multiple_of(i * T1, T1)
        slot = i & 1

        lhs = ln1_v[slot]
        prep1(jnp.minimum(i + 1, N1 - 1), 1 - slot, NCHAIN1)
        for q in range(4):
            p1_quarter(lhs, r0, q)
        for n in range(3, len(cp_x)):
            pl.when(i + 2 == xcuts[n])(cp_x[n].wait)
        return carry

    cp_x[2].wait()
    with jax.named_scope('p1_body'):
        jax.lax.fori_loop(1, N1, p1_body, 0)
    for c in cp_w2:
        c.wait()

    def h1_rows(r0, n):
        return jnp.concatenate([h1_v[j, pl.ds(r0, n), :] for j in range(D // 128)], axis=1)

    def prep3(src, slot):
        def store(k, y):
            ln3_v[slot, pl.ds(k, y.shape[0]), :] = y

        ln_block(lambda k, n: src[pl.ds(k, n), :], store, T3, 1, 16)

    def p2_body(i, carry):
        r0 = pl.multiple_of(i * T2, T2)
        win = x1_v.at[pl.ds(r0, 2 * T2)]
        prep3(win, 0)
        hs = h1_rows(r0 + 8, T2).astype(BF16)
        for q in range(4):
            win[pl.ds(T2, T2), pl.ds(q * c4, c4)] = (
                jnp.dot(hs, w2_v[q], preferred_element_type=F32)
                + x_v[pl.ds(r0, T2), pl.ds(q * c4, c4)].astype(F32))
        return carry

    with jax.named_scope('p2_body'):
        jax.lax.fori_loop(0, N2, p2_body, 0)

    for c in cp_ffn + piece_copies(0, 0):
        c.wait()
    blk0 = (N2 - 2) * T2 // T3

    def p3_body(i, carry):
        r0 = pl.multiple_of((i + blk0) % N3 * T3, T3)
        r_next = pl.multiple_of((i + 1 + blk0) % N3 * T3, T3)
        slot = i & 1
        ring = i % NRING

        @pl.when(i + 2 < N3)
        def _():
            for c in piece_copies(i + 2, (i + 2) % NRING):
                c.start()

        lhs = ln3_v[slot]
        prep3(x1_v.at[pl.ds(T2 + r_next, T3)], 1 - slot)
        zero = zero_v[...]
        low16 = jax.lax.broadcasted_iota(jnp.int32, (16, 128), 1) < 64
        for which in range(3):
            tok = zero
            for j in range(DP // 2):
                blk = pltpu.bitcast(stq_v[ring, which, pl.ds(j * 64, 64), :], U32)
                a = blk[0:16] | tok
                c = blk[16:32]
                lo = (a & jnp.uint32(0xFFFF)) | (c << 16)
                hi = (a >> 16) | (c & jnp.uint32(0xFFFF0000))
                if which < 2:
                    tok = pltpu.roll((lo | hi) & zero, 1, 1)
                else:
                    t = pltpu.roll(jnp.where(low16, hi, lo), 64, 1)
                    lo, hi = jnp.where(low16, lo, t), jnp.where(low16, t, hi)
                    tok = hi & zero
                s0 = which * H * PITCH + i * (DP // 2) + j
                wqkv_v[pl.ds(s0, 16, stride=PITCH), :] = lo
                wqkv_v[pl.ds(s0 + 16 * PITCH, 16, stride=PITCH), :] = hi
        o0 = pl.multiple_of(i * (OP // 2), OP // 2)
        tok = zero
        for j in range(D // 128):
            for k in range(OP // 32):
                w = pltpu.bitcast(sto_v[ring, pl.ds(k * 32, 32), pl.ds(j * 128, 128)], U32) | tok
                tok = w & zero
                if k % HOP == HOP - 1:
                    tok = pltpu.roll(tok, 1, 1)
                kd = k - k % 8 + (0, 1, 4, 5, 2, 3, 6, 7)[k % 8]
                wo_v[j, pl.ds(o0 + kd * 16, 16), :] = w

        h = _gelu(jnp.dot(lhs, w3_v[...], preferred_element_type=F32)).astype(BF16)
        b = jnp.dot(h, w4_v[...], preferred_element_type=F32) + x1_v[pl.ds(T2 + r0, T3), :]
        gw = gw_v[...].astype(F32).reshape(1, D)
        z = jnp.sum(x_v[pl.ds(r0, T3), :].astype(F32) * gw, axis=-1, keepdims=True)
        g = 1.0 / (1.0 + jnp.exp(-z))
        g_v[pl.ds(r0, T3), :] = jnp.broadcast_to(g, (T3, 128))
        b = (1.0 - g) * b
        for j in range(D // 128):
            h1_v[j, pl.ds(r0, T3), :] = b[:, j * 128:(j + 1) * 128]

        @pl.when(i + 1 < N3)
        def _():
            for c in piece_copies(i + 1, (i + 1) % NRING):
                c.wait()

        return carry

    with jax.named_scope('p3_body'):
        jax.lax.fori_loop(0, N3, p3_body, 0)

    mem_v[...] = mem0_v[...].astype(F32)
    c_exp = (DH ** -0.5) * math.log2(math.e)
    neg_raw = NEG / (DH ** -0.5)

    L2 = 2 * L
    mxu_groups = [0] + list(range(NGV + 1, 5))
    rm = 8 * len(mxu_groups)
    row = jax.lax.broadcasted_iota(jnp.int32, (2 * rm, 128), 0)
    col = jax.lax.broadcasted_iota(jnp.int32, (2 * rm, 128), 1)
    second = row >= rm
    rowl = jnp.where(second, row - rm, row)
    coll = jnp.where(second, col - L, col)
    real = (coll >= 0) & (coll < L)
    allowed = real & ((rowl < M) | (rowl + 8 * NGV >= coll))
    keep = jnp.where(allowed, jnp.uint32(0xFFFFFFFF), jnp.uint32(0))
    fill = pltpu.bitcast(
        jnp.where(allowed, 0.0, jnp.where(real, neg_raw, -jnp.inf)).astype(F32), U32)
    neg_c = NEG * math.log2(math.e)

    def tied(w, toks):
        for tok in toks:
            w = jnp.concatenate([w[0:AR], w[AR:AR + 8] | tok, w[AR + 8:]], axis=0)
        return pltpu.bitcast(w, BF16)

    zpad = jnp.zeros((128 - L2, DH), F32)

    def recip(l):
        r = pl.reciprocal(l, approx=True)
        return r * (2.0 - l * r)

    def tree(op, x):
        while x.shape[0] > 1:
            x = x.reshape(x.shape[0] // 2, 16, 128)
            x = op(x[:, 0:8], x[:, 8:16])
        return x[0]

    causal = (jax.lax.broadcasted_iota(jnp.int32, (7, 8, 128), 1)
              > jax.lax.broadcasted_iota(jnp.int32, (7, 8, 128), 0))
    low = jax.lax.broadcasted_iota(jnp.int32, (8, 128), 1) < 64

    def park(buf, seg, ks, vs, top):
        base = [key0_row(seg, i) for i in range(4)]
        for i, x in enumerate(ks + vs):
            buf[pl.ds(base[i], 8 * top + 8), :] = x[0:8 * top + 8]
            if top == 4 or i >= 2:
                buf[pl.ds(base[i] - 8, 8), :] = x[8 * top:8 * top + 8]
        out = {}
        for g in range(1, top + 1):
            last = list(base)
            if g < top:
                for i, v in enumerate(vs):
                    last[2 + i] = 8 * (L + 8) + ((NGV * seg + g - 1) * 2 + i) * 16 + 8
                    buf[pl.ds(last[2 + i] - 8, 16), :] = jnp.concatenate(
                        [v[8 * g:8 * g + 8], v[0:8]], axis=0)
            out[g] = (buf, base, last, [jnp.sum(v[8 * g + 8:L], axis=0, keepdims=True)
                                        if g < 4 else None for v in vs])
        return out

    def vpu_start(q0, q1, parked, g, masked=True):
        buf, base, last, (acc_a, acc_b) = parked
        st = dict(q=(q0 * c_exp, q1 * c_exp), buf=buf, base=base, last=last, g=g, masked=masked,
                  m=None)
        if g < 4:
            st.update(m=jnp.full((8, 128), neg_c, F32),
                      l=jnp.full((8, 128), float(L - 8 * (g + 1)), F32), a=acc_a, b=acc_b)
        return st

    def vpu_chunk(st, c0, gate):
        final = c0 == 8 * st['g']

        def windows(*rows):
            return jnp.concatenate(
                [st['buf'][pl.ds(k + 8 * st['g'] - r, 8), :]
                 for r in range(c0, c0 + CHUNK) for k in rows],
                axis=0).reshape(CHUNK, 8 * len(rows), 128)

        k0, k1, wa, wb = st['last' if final else 'base']
        q = jnp.concatenate([pltpu.bitcast(pltpu.bitcast(x, U32) | gate, F32) for x in st['q']],
                            axis=0)
        sc = jnp.sum(q * windows(k0, k1), axis=-1, keepdims=True)
        sc = jnp.where(low, sc[:, 0:8], sc[:, 8:16])
        if final and st['masked']:
            sc = jnp.concatenate([sc[0:1], jnp.where(causal, sc[1:], neg_c)], axis=0)
        m = tree(jnp.maximum, sc)
        if st['m'] is not None:
            m = jnp.maximum(m, st['m'])
            alpha = jnp.exp2(st['m'] - m)
        pr = jnp.exp2(sc - m)
        new = []
        for key, x in (('l', pr), ('a', pr * windows(wa)), ('b', pr * windows(wb))):
            if st['m'] is not None:
                x = jnp.concatenate([(st[key] * alpha)[None], x], axis=0)
            new.append(jnp.sum(x, axis=0))
        st.update(m=m, l=new[0], a=new[1], b=new[2])
        return (pltpu.bitcast(new[0], U32) | pltpu.bitcast(new[1], U32)
                | pltpu.bitcast(new[2], U32))

    def vpu_finish(st):
        r = recip(st['l'])
        return st['a'] * r, st['b'] * r

    def segment(lhs_q, lhs_kv, wo_m, full, n_chunks, unpack, wo_rows, split_first, zero,
                order, early, slots, d_g, d_j, d_f, d_s, d_pv, d_o):
        NP = H // 2
        nj = D // 128
        HA = H - TAIL_H
        mxu_pairs = [p for p in range(NP) if p not in full]
        proj = {}
        qkv = [None] * NP
        pb = [None] * NP
        og = [dict() for _ in range(H)]
        ocat = {}
        y = [None] * nj

        def slab(toks, which, h, r0, n):
            x = lhs_q if which == 0 else lhs_kv
            w = tied(wqkv_v[pl.ds(_slab_of(which, h) * PITCH + r0, n), :], toks)
            r = jnp.dot(x[:, 2 * r0:2 * (r0 + n)], w, preferred_element_type=F32)
            proj[(which, h)] = r + proj[(which, h)] if (which, h) in proj else r
            return proj[(which, h)]

        def do_wo(toks, h0, h1, j):
            if (h0, h1) not in ocat:
                ocat[(h0, h1)] = jnp.concatenate(
                    [wo_rows(og[h]) for h in range(h0, h1)], axis=1).astype(BF16)
            w = tied(wo_v[j, pl.ds(h0 * 64, (h1 - h0) * 64), :], toks)
            r = jnp.dot(ocat[(h0, h1)], w, preferred_element_type=F32)
            y[j] = r if y[j] is None else r + y[j]
            return y[j]

        ticks = []
        pair_end = {}
        wo_early = [(4 * c, 4 * c + 4, j) for c in range(early) for j in range(nj)]
        first = NP - slots
        for p in range(NP):
            slabs = [(which, h) for h in (2 * p, 2 * p + 1) for which in range(3)]
            rows = [(lhs_q if w == 0 else lhs_kv).shape[0] for w, _ in slabs]
            if p == 0 and split_first:
                for r0 in (0, 256):
                    ticks += [(slab, (w, h, r0, 256), m) for (w, h), m in zip(slabs, rows)]
            else:
                mine = []
                if p >= first:
                    lo = (p - first) * len(wo_early) // slots
                    mine = wo_early[lo:(p - first + 1) * len(wo_early) // slots]
                att = 0 if p in full else rm / 12
                units = [(slab, slabs[k0 + k] + (256 * half, 256), rows[k0 + k] + att)
                         for k0 in (0, 3) for k, half in order]
                for n, unit in enumerate(units):
                    ticks += [(do_wo, item, wo_m) for item in
                              mine[n * len(mine) // len(units):(n + 1) * len(mine) // len(units)]]
                    ticks.append(unit)
            pair_end[len(ticks) - 1] = p
        ticks += [(do_wo, (h0, h0 + 4, j), wo_m)
                  for h0 in range(4 * early, HA, 4) for j in range(nj)]
        ends = []
        for _, _, dur in ticks:
            ends.append(dur + (ends[-1] if ends else 0))

        def index(t):
            return next(i for i, e in enumerate(ends) if e >= t)

        events = {}
        anchors = {}
        cursor = [0]

        def run_chunk(res, p, name, st, c0, i_done):
            done = vpu_chunk(st, c0, pltpu.bitcast(res[GR:GR + 8], U32) & zero)
            anchors.setdefault(i_done, []).append(done & zero)
            if c0 + CHUNK >= 8 * (st['g'] + 1):
                og[2 * p][name], og[2 * p + 1][name] = vpu_finish(st)

        def do_s(res, p):
            sc = jax.lax.dot_general(qkv[p][0], qkv[p][1], (((1,), (1,)), ((), ())),
                                     preferred_element_type=F32)
            sc = pltpu.bitcast((pltpu.bitcast(sc, U32) & keep) | fill, F32)
            e = jnp.exp2((sc - jnp.max(sc, axis=-1, keepdims=True)) * c_exp)
            l = jnp.sum(e, axis=-1, keepdims=True)
            e = e * recip(l)
            pb[p] = (e[0:rm] + e[rm:2 * rm]).astype(BF16)

        def do_pv(res, p):
            for i in range(2):
                o = jnp.dot(pb[p], qkv[p][2][i], preferred_element_type=F32)
                for n, g in enumerate(mxu_groups):
                    og[2 * p + i][g] = o[8 * n:8 * n + 8]

        def finish_pair(p, i):
            u, jobs = unpack(p, [[proj[(w, h)] for w in range(3)] for h in (2 * p, 2 * p + 1)])
            chunks = [(name, st, c0) for name, st in
                      [(name, vpu_start(*job)) for name, job in jobs.items()]
                      for c0 in range(0, 8 * (st['g'] + 1), CHUNK)]
            t_first = ends[min(pair_end)] + d_g
            t_last = ends[-2] - d_j - d_f
            gap = (t_last - t_first) / (n_chunks - 1)
            if p == NP - 1:
                gap = min(gap, (t_last - max(ends[i] + d_g, cursor[0])) / (len(chunks) - 1))
            for chunk in chunks:
                t = max(ends[i] + d_g, cursor[0])
                cursor[0] = t + gap
                g = max(index(t), i + 1)
                events.setdefault(g, []).append(
                    (run_chunk, (p,) + chunk + (index(ends[g] + d_j) + 1,)))
            if p in full:
                return
            qb = jnp.concatenate([u[k][0][g] for k in range(2) for g in mxu_groups],
                                 axis=0).astype(BF16)
            kb = jnp.concatenate([u[0][1], u[1][1], zpad], axis=0).astype(BF16)
            low40 = jnp.concatenate([low] * 5, axis=0)
            vb = [jnp.concatenate([jnp.where(low40, v, 0.0), jnp.where(low40, 0.0, v), zpad],
                                  axis=0).astype(BF16) for v in (u[0][2], u[1][2])]
            qkv[p] = (qb, kb, vb)
            n = mxu_pairs.index(p)
            if n % 4 == 3:
                four = mxu_pairs[n - 3:n + 1]
                t2 = min(ends[i] + d_pv, ends[-1] - d_o)
                t1 = t2 - D_PP
                events.setdefault(index(min(ends[i] + d_s, t1 - D_SM)), []).extend(
                    (do_s, (k,)) for k in four)
                events.setdefault(index(t1), []).extend((do_pv, (k,)) for k in four[0:2])
                events.setdefault(index(t2), []).extend((do_pv, (k,)) for k in four[2:4])

        for i, (fn, args, _) in enumerate(ticks):
            res = fn(anchors.pop(i, []), *args)
            if i in pair_end:
                finish_pair(pair_end[i], i)
            for f, a in events.pop(i, []):
                f(res, *a)
        assert not events
        for j in range(nj):
            do_wo([], HA, H, j)
        return jnp.concatenate(y, axis=1)

    def pair(r0, mem):
        xf = x_v[pl.ds(r0, PAIR), :].astype(F32)
        zero = zero_v[pl.ds(0, 8), :]
        x1s = jnp.concatenate([xf[0:8], xf[32:40]], axis=0).astype(BF16)
        carry = [None] * (H // 2)

        def cat(*xs):
            return jnp.concatenate(xs, axis=0)

        lhs = cat(mem, xf[8:32]).astype(BF16)

        def unpack_a(p, qkv):
            qg = [{0: q[0:8], 2: q[8:16], 3: q[16:24], 4: q[24:32]} for q, _, _ in qkv]
            ks = [cat(k[0:8], k[32:40], k[8:32]) for _, k, _ in qkv]
            vs = [cat(v[0:8], v[32:40], v[8:32]) for _, _, v in qkv]
            top = 4 if p in FULL_A else NGV
            parked = park(kv_v[p], 0, ks, vs, top)
            carry[p] = (parked[1], [(k[40:48], v[40:48]) for _, k, v in qkv])
            jobs = {0: (qg[0][0], qg[1][0], parked[4], 4, False)} if top == 4 else {}
            jobs.update({g: (qg[0][g], qg[1][g], parked[g], g) for g in range(top, 1, -1)})
            return list(zip(qg, ks, vs)), jobs

        y_a = segment(lhs, cat(lhs, x1s), 32, FULL_A, 7 * (H // 2) + 10 * len(FULL_A), unpack_a,
                      lambda o: cat(o[0], o[2], o[3], o[4]), False, zero, **KNOBS_A)

        lhs = cat(y_a[0:8], xf[40:64]).astype(BF16)

        def unpack_b(p, qkv):
            parked_a1, kv1 = carry[p]
            qg = [{0: q[0:8], 1: q[40:48], 2: q[8:16], 3: q[16:24], 4: q[24:32]}
                  for q, _, _ in qkv]
            ks = [cat(k[0:8], e[0], k[8:32]) for (_, k, _), e in zip(qkv, kv1)]
            vs = [cat(v[0:8], e[1], v[8:32]) for (_, _, v), e in zip(qkv, kv1)]
            parked = park(kv_v[p], 1, ks, vs, NGV)
            jobs = {'a1': (qkv[0][0][32:40], qkv[1][0][32:40], parked_a1, 1)}
            jobs.update({g: (qg[0][g], qg[1][g], parked[g], g) for g in range(1, NGV + 1)})
            return list(zip(qg, ks, vs)), jobs

        y_b = segment(cat(lhs, x1s), lhs, 48, (), 11 * (H // 2), unpack_b,
                      lambda o: cat(o[0], o[1], o[2], o[3], o[4], o['a1']),
                      True, zero, **KNOBS_B)

        a = cat(y_b[40:48], y_a[8:32], y_b[8:40])
        g = g_v[pl.ds(r0, PAIR), :]
        g = jnp.concatenate([g] * (D // 128), axis=1)
        out_v[pl.ds(r0, PAIR), :] = (g * a + h1_rows(r0, PAIR)).astype(BF16)
        return y_b[0:8]

    def a_body(t, carry):
        r0 = pl.multiple_of(t * PAIR, PAIR)
        mem_v[...] = pair(r0, mem_v[...])
        pltpu.make_async_copy(out_v.at[pl.ds(r0, PAIR)], out_hbm.at[pl.ds(r0, PAIR)],
                              osem).start()
        return carry

    with jax.named_scope('a_body'):
        jax.lax.fori_loop(0, S // PAIR, a_body, 0)
    pltpu.make_async_copy(out_v, out_hbm, osem).wait()


@jax.jit
def pallas_gated_mix__memory_aug_recurrent_mem_tr__mixer_s_mlp__prompt_kernel(
    A_x, A_mem0, A_Wq, A_Wk, A_Wv, A_Wo, A_seg_len, B_x, B_w1, B_w2, B_w3, B_w4, gate_w,
):
    assert A_x.shape == (1, S, D) and A_Wq.shape == (D, H, DH) and A_mem0.shape == (1, M, D)
    x = A_x.reshape(S, D)
    mem0 = A_mem0.reshape(M, D)
    wq = A_Wq.reshape(D * H, DH)
    wk = A_Wk.reshape(D * H, DH)
    wv = A_Wv.reshape(D * H, DH)
    wo = A_Wo.reshape(H * DH, D)

    any_spec = pl.BlockSpec(memory_space=pl.ANY)
    out = pl.pallas_call(
        _kernel,
        out_shape=jax.ShapeDtypeStruct((S, D), BF16),
        in_specs=[any_spec] * 11,
        out_specs=any_spec,
        scratch_shapes=[
            pltpu.VMEM((S, D), BF16),
            pltpu.VMEM((NRING, 3, DP * H, DH), BF16),
            pltpu.VMEM((NRING, OP, D), BF16),
            pltpu.VMEM((3 * H * PITCH + 544, 128), U32),
            pltpu.VMEM((D // 128, H * DH // 2, 128), U32),
            pltpu.VMEM((4, D, D // 4), BF16),
            pltpu.VMEM((4, D, D // 4), BF16),
            pltpu.VMEM((D, FF), BF16),
            pltpu.VMEM((FF, D), BF16),
            pltpu.VMEM((D // 128, S + 16, 128), F32),
            pltpu.VMEM((S + T2, D), F32),
            pltpu.VMEM((S, 128), F32),
            pltpu.VMEM((2, T1, D), BF16),
            pltpu.VMEM((2, T3, D), BF16),
            pltpu.VMEM((M, D), BF16),
            pltpu.VMEM((D,), BF16),
            pltpu.VMEM((M, D), F32),
            pltpu.VMEM((S, D), BF16),
            [pltpu.VMEM((KV_ROWS, 128), F32)] * (H // 2),
            pltpu.VMEM((16, 128), U32),
            pltpu.SemaphoreType.DMA((NSEM,)),
            pltpu.SemaphoreType.DMA(()),
        ],
        compiler_params=pltpu.CompilerParams(vmem_limit_bytes=120 * 1024 * 1024,
                                             disable_bounds_checks=True),
    )(x, mem0, wq, wk, wv, wo, B_w1, B_w2, B_w3, B_w4, gate_w)
    return out.reshape(1, S, D)
```

```python
import math

import jax
import jax.numpy as jnp
import jax.experimental.pallas as pl
import jax.experimental.pallas.tpu as pltpu

F32 = jnp.float32
BF16 = jnp.bfloat16
U32 = jnp.uint32

S = 2048
D = 1024
H = 32
DH = 128
M = 8
SEG = 32
L = M + SEG
FF = 3584
EPS = 1e-5
NEG = -1e9

PAIR = 2 * SEG
T1 = 256
N1 = S // T1
T2 = 512
N2 = S // T2
T3 = 256
N3 = S // T3
DP = D // N3
OP = H * DH // N3
PITCH = 520
NRING = 3
NSEM = 11 + NRING + N2

NCHAIN0 = 10
NCHAIN1 = 5
LN1_ROWS = 8
HOP = 4
NGV = 3
FULL_A = (1, 5, 8, 11)
CHUNK = 8
AR = 40
GR = 24
TAIL_H = 8
D_SM = 560
D_PP = 200
ORDER_A = ((0, 0), (1, 0), (2, 0), (0, 1), (1, 1), (2, 1))
ORDER_B = ((0, 0), (1, 0), (1, 1), (0, 1), (2, 0), (2, 1))
KNOBS_A = dict(order=ORDER_A, early=2, slots=2, d_g=80, d_j=620, d_f=50, d_s=350, d_pv=1050, d_o=200)
KNOBS_B = dict(order=ORDER_B, early=3, slots=10, d_g=0, d_j=530, d_f=50, d_s=200, d_pv=1000, d_o=200)
KV_ROWS = 8 * (L + 8) + 4 * NGV * 16


def _gelu(x):
    c = math.sqrt(2.0 / math.pi)
    return 0.5 * x * (1.0 + jnp.tanh(c * (x + 0.044715 * (x * x * x))))


def _layernorm(x):
    m = jnp.mean(x, axis=-1, keepdims=True)
    xc = x - m
    v = jnp.mean(xc * xc, axis=-1, keepdims=True)
    return xc * jax.lax.rsqrt(v + EPS)


def _strassen_lhs(a11, a12, a21, a22):
    return [a11 + a22, a21 + a22, a11, a22, a11 + a12, a21 - a11, a12 - a22]


def _slab_of(which, h):
    return which * H + (h % 2) * (H // 2) + h // 2


def key0_row(seg, i):
    return (4 * seg + i) * (L + 8) + 8


def _kernel(x_hbm, mem0_hbm, wq_hbm, wk_hbm, wv_hbm, wo_hbm,
            w1_hbm, w2_hbm, w3_hbm, w4_hbm, gw_hbm,
            out_hbm,
            x_v, stq_v, sto_v, wqkv_v, wo_v, w1_v, w2_v, w3_v, w4_v, e3_v, e4_v,
            h1_v, x1_v, g_v, ln1_v, ln3_v, mem0_v, gw_v, mem_v, out_v, kv_v, zero_v, sems, osem):
    c4 = D // 4
    xcuts = (0, 1, 2, 3, 5, N1)
    cp_x = [pltpu.make_async_copy(x_hbm.at[pl.ds(lo * T1, (hi - lo) * T1)],
                                  x_v.at[pl.ds(lo * T1, (hi - lo) * T1)], sems.at[n])
            for n, (lo, hi) in enumerate(zip(xcuts[:-1], xcuts[1:]))]
    cp_w1 = [pltpu.make_async_copy(w1_hbm.at[:, pl.ds(q * c4, c4)], w1_v.at[q], sems.at[5 + q])
             for q in range(4)]
    cp_w2 = [pltpu.make_async_copy(w2_hbm.at[:, pl.ds(q * c4, c4)], w2_v.at[q], sems.at[9])
             for q in range(4)]
    cp_small = [pltpu.make_async_copy(src, dst, sems.at[10])
                for src, dst in ((gw_hbm, gw_v), (mem0_hbm, mem0_v))]

    def ffn_copies(q):
        cps = []
        for src, dst, k in ((w3_hbm, w3_v, D), (w4_hbm, w4_v, FF)):
            for half in range(2):
                rows = pl.ds(half * (k // 2) + q * (k // 8), k // 8)
                cps.append(pltpu.make_async_copy(src.at[rows], dst.at[rows],
                                                 sems.at[11 + NRING + q]))
        return cps

    def piece_copies(i, slot):
        cps = [pltpu.make_async_copy(w.at[pl.ds(i * (DP * H), DP * H)], stq_v.at[slot, k],
                                     sems.at[11 + slot])
               for k, w in enumerate((wq_hbm, wk_hbm, wv_hbm))]
        cps.append(pltpu.make_async_copy(wo_hbm.at[pl.ds(i * OP, OP)], sto_v.at[slot],
                                         sems.at[11 + slot]))
        return cps

    for c in (cp_x[0:1] + cp_w1 + cp_x[1:] + cp_w2 + cp_small
              + [c for q in range(N2) for c in ffn_copies(q)]
              + piece_copies(0, 0) + piece_copies(1, 1)):
        c.start()
    x1_v[pl.ds(0, T3), :] = jnp.zeros((T3, D), F32)
    h1_v[:, pl.ds(8, 8), :] = jnp.zeros((D // 128, 8, 128), F32)
    h1_v[:, pl.ds(S, 8), :] = jnp.zeros((D // 128, 8, 128), F32)
    zero_v[...] = jnp.zeros((16, 128), U32)
    for buf in kv_v:
        for seg in range(2):
            for i in range(2):
                buf[pl.ds(key0_row(seg, i) - 8, 8), :] = jnp.zeros((8, 128), F32)

    def ln_rows(x, tok, zero):
        if tok is not None:
            head = pltpu.bitcast(pltpu.bitcast(x[:, 0:128], U32) | tok, F32)
            x = jnp.concatenate([head, x[:, 128:]], axis=1)
        y = _layernorm(x)
        tok = None if zero is None else pltpu.bitcast(y[:, 0:128], U32) & zero
        return y, tok

    def ln_block(load, store, rows, nchain, gr):
        zero = zero_v[pl.ds(0, gr), :] if nchain else None
        toks = [None] * max(nchain, 1)
        for k in range(rows // gr):
            y, toks[k % len(toks)] = ln_rows(load(k * gr, gr), toks[k % len(toks)], zero)
            store(k * gr, y.astype(BF16))

    def prep1(blk, slot, nchain):
        r0 = blk * T1 if isinstance(blk, int) else pl.multiple_of(blk * T1, T1)

        def store(k, y):
            ln1_v[slot, pl.ds(k, y.shape[0]), :] = y

        ln_block(lambda k, n: x_v[pl.ds(r0 + k, n), :].astype(F32), store, T1, nchain, LN1_ROWS)

    def p1_quarter(lhs, r0, q):
        h = _gelu(jnp.dot(lhs, w1_v[q], preferred_element_type=F32))
        for j in range(2):
            win = h1_v.at[2 * q + j, pl.ds(r0, T1 + 16)]
            win[pl.ds(8 + (1, -1, 2, -2)[q], T1), :] = h[:, j * 128:(j + 1) * 128]

    cp_x[0].wait()
    prep1(0, 0, 0)
    for q in range(4):
        cp_w1[q].wait()
        if q == 3:
            cp_x[1].wait()
        lhs = ln1_v[0]
        if q == 3:
            prep1(1, 1, NCHAIN0)
        p1_quarter(lhs, 0, q)

    def p1_body(i, carry):
        r0 = pl.multiple_of(i * T1, T1)
        slot = i & 1

        lhs = ln1_v[slot]
        prep1(jnp.minimum(i + 1, N1 - 1), 1 - slot, NCHAIN1)
        for q in range(4):
            p1_quarter(lhs, r0, q)
        for n in range(3, len(cp_x)):
            pl.when(i + 2 == xcuts[n])(cp_x[n].wait)
        return carry

    cp_x[2].wait()
    with jax.named_scope('p1_body'):
        jax.lax.fori_loop(1, N1, p1_body, 0)
    for c in cp_w2 + ffn_copies(0):
        c.wait()

    def h1_rows(r0, n):
        return jnp.concatenate([h1_v[j, pl.ds(r0, n), :] for j in range(D // 128)], axis=1)

    def prep3(src, slot):
        zero = zero_v[...]
        tok = None
        for k in range(0, T3 // 2, 8):
            x = jnp.concatenate([src[pl.ds(k, 8), :], src[pl.ds(T3 // 2 + k, 8), :]], axis=0)
            y, tok = ln_rows(x, tok, zero)
            ops = _strassen_lhs(y[0:8, 0:D // 2], y[0:8, D // 2:], y[8:16, 0:D // 2], y[8:16, D // 2:])
            for n, op in enumerate(ops):
                ln3_v[slot, n, pl.ds(k, 8), :] = op.astype(BF16)

    def weight_sums(w_v, e_v, q, zero):
        kh, nh = w_v.shape[0] // 2, w_v.shape[1] // 2
        r0 = pl.multiple_of(q * (kh // 4), 16)
        w = w_v.at[pl.ds(r0, kh + kh // 4)]
        tok = zero
        for r in range(0, kh // 4, 16):
            for c in range(0, nh, 256):
                b11, b12, b21, b22 = [
                    w[pl.ds(i * kh + r, 16), pl.ds(j * nh + c, 256)].astype(F32)
                    for i in range(2) for j in range(2)]
                head = pltpu.bitcast(pltpu.bitcast(b11[:, 0:128], U32) | tok, F32)
                b11 = jnp.concatenate([head, b11[:, 128:]], axis=1)
                sums = [b11 + b22, b11 + b12, b21 + b22, b12 - b22, b21 - b11]
                for n in range(3):
                    e_v[n, pl.ds(r0 + r, 16), pl.ds(c, 256)] = sums[n].astype(BF16)
                w[pl.ds(r, 16), pl.ds(nh + c, 256)] = sums[3].astype(BF16)
                w[pl.ds(kh + r, 16), pl.ds(c, 256)] = sums[4].astype(BF16)
                t = pltpu.bitcast(sums[1] + sums[2], U32)
                tok = pltpu.roll((t[:, 0:128] | t[:, 128:]) & zero, 1, 1)

    def strassen(lhs, w_v, e_v, n, init=None):
        kh, nh = w_v.shape[0] // 2, w_v.shape[1] // 2

        def mul(i, rhs):
            return jnp.dot(lhs(i), rhs, preferred_element_type=F32)

        def blk(i, j):
            return w_v[pl.ds(i * kh, kh), pl.ds(j * nh + n * 128, 128)]

        def ext(k):
            return e_v[k, :, pl.ds(n * 128, 128)]

        m1 = mul(0, ext(0))
        m2 = mul(1, blk(0, 0))
        m4 = mul(3, blk(1, 0))
        c21, c11, c22 = m2 + m4, m1 + m4, m1 - m2
        m5 = mul(4, blk(1, 1))
        c11 = c11 - m5
        m3 = mul(2, blk(0, 1))
        c12, c22 = m3 + m5, c22 + m3
        c22 = mul(5, ext(1)) + c22
        c11 = mul(6, ext(2)) + c11
        return c11, c12, c21, c22

    def p2_body(i, carry):
        r0 = pl.multiple_of(i * T2, T2)
        win = x1_v.at[pl.ds(r0, 2 * T2)]
        prep3(win, 0)
        zero = zero_v[...]
        weight_sums(w3_v, e3_v, i, zero)
        weight_sums(w4_v, e4_v, i, zero)
        hs = h1_rows(r0 + 8, T2).astype(BF16)
        for q in range(4):
            win[pl.ds(T2, T2), pl.ds(q * c4, c4)] = (
                jnp.dot(hs, w2_v[q], preferred_element_type=F32)
                + x_v[pl.ds(r0, T2), pl.ds(q * c4, c4)].astype(F32))

        @pl.when(i + 1 < N2)
        def _():
            for c in ffn_copies(i + 1):
                c.wait()

        return carry

    with jax.named_scope('p2_body'):
        jax.lax.fori_loop(0, N2, p2_body, 0)

    for c in cp_small + piece_copies(0, 0):
        c.wait()
    blk0 = (N2 - 2) * T2 // T3

    def p3_body(i, carry):
        r0 = pl.multiple_of((i + blk0) % N3 * T3, T3)
        r_next = pl.multiple_of((i + 1 + blk0) % N3 * T3, T3)
        slot = i & 1
        ring = i % NRING

        @pl.when(i + 2 < N3)
        def _():
            for c in piece_copies(i + 2, (i + 2) % NRING):
                c.start()

        lhs = [ln3_v[slot, n] for n in range(7)]
        prep3(x1_v.at[pl.ds(T2 + r_next, T3)], 1 - slot)
        zero = zero_v[...]
        low16 = jax.lax.broadcasted_iota(jnp.int32, (16, 128), 1) < 64
        for which in range(3):
            tok = zero
            for j in range(DP // 2):
                blk = pltpu.bitcast(stq_v[ring, which, pl.ds(j * 64, 64), :], U32)
                a = blk[0:16] | tok
                c = blk[16:32]
                lo = (a & jnp.uint32(0xFFFF)) | (c << 16)
                hi = (a >> 16) | (c & jnp.uint32(0xFFFF0000))
                if which < 2:
                    tok = pltpu.roll((lo | hi) & zero, 1, 1)
                else:
                    t = pltpu.roll(jnp.where(low16, hi, lo), 64, 1)
                    lo, hi = jnp.where(low16, lo, t), jnp.where(low16, t, hi)
                    tok = hi & zero
                s0 = which * H * PITCH + i * (DP // 2) + j
                wqkv_v[pl.ds(s0, 16, stride=PITCH), :] = lo
                wqkv_v[pl.ds(s0 + 16 * PITCH, 16, stride=PITCH), :] = hi
        o0 = pl.multiple_of(i * (OP // 2), OP // 2)
        tok = zero
        for j in range(D // 128):
            for k in range(OP // 32):
                w = pltpu.bitcast(sto_v[ring, pl.ds(k * 32, 32), pl.ds(j * 128, 128)], U32) | tok
                tok = w & zero
                if k % HOP == HOP - 1:
                    tok = pltpu.roll(tok, 1, 1)
                kd = k - k % 8 + (0, 1, 4, 5, 2, 3, 6, 7)[k % 8]
                wo_v[j, pl.ds(o0 + kd * 16, 16), :] = w

        hops = []
        for n in range(FF // 256):
            c = strassen(lambda k: lhs[k], w3_v, e3_v, n)
            hops.append(_strassen_lhs(*[_gelu(x) for x in c]))
        hops = [jnp.concatenate([h[k] for h in hops], axis=1).astype(BF16) for k in range(7)]
        c = [strassen(lambda k: hops[k], w4_v, e4_v, n) for n in range(D // 256)]
        b = jnp.concatenate(
            [jnp.concatenate([x[2 * i + j] for j in range(2) for x in c], axis=1)
             for i in range(2)], axis=0) + x1_v[pl.ds(T2 + r0, T3), :]
        gw = gw_v[...].astype(F32).reshape(1, D)
        z = jnp.sum(x_v[pl.ds(r0, T3), :].astype(F32) * gw, axis=-1, keepdims=True)
        g = 1.0 / (1.0 + jnp.exp(-z))
        g_v[pl.ds(r0, T3), :] = jnp.broadcast_to(g, (T3, 128))
        b = (1.0 - g) * b
        for j in range(D // 128):
            h1_v[j, pl.ds(r0, T3), :] = b[:, j * 128:(j + 1) * 128]

        @pl.when(i + 1 < N3)
        def _():
            for c in piece_copies(i + 1, (i + 1) % NRING):
                c.wait()

        return carry

    with jax.named_scope('p3_body'):
        jax.lax.fori_loop(0, N3, p3_body, 0)

    mem_v[...] = mem0_v[...].astype(F32)
    c_exp = (DH ** -0.5) * math.log2(math.e)
    neg_raw = NEG / (DH ** -0.5)

    L2 = 2 * L
    mxu_groups = [0] + list(range(NGV + 1, 5))
    rm = 8 * len(mxu_groups)
    row = jax.lax.broadcasted_iota(jnp.int32, (2 * rm, 128), 0)
    col = jax.lax.broadcasted_iota(jnp.int32, (2 * rm, 128), 1)
    second = row >= rm
    rowl = jnp.where(second, row - rm, row)
    coll = jnp.where(second, col - L, col)
    real = (coll >= 0) & (coll < L)
    allowed = real & ((rowl < M) | (rowl + 8 * NGV >= coll))
    keep = jnp.where(allowed, jnp.uint32(0xFFFFFFFF), jnp.uint32(0))
    fill = pltpu.bitcast(
        jnp.where(allowed, 0.0, jnp.where(real, neg_raw, -jnp.inf)).astype(F32), U32)
    neg_c = NEG * math.log2(math.e)

    def tied(w, toks):
        for tok in toks:
            w = jnp.concatenate([w[0:AR], w[AR:AR + 8] | tok, w[AR + 8:]], axis=0)
        return pltpu.bitcast(w, BF16)

    zpad = jnp.zeros((128 - L2, DH), F32)

    def recip(l):
        r = pl.reciprocal(l, approx=True)
        return r * (2.0 - l * r)

    def tree(op, x):
        while x.shape[0] > 1:
            x = x.reshape(x.shape[0] // 2, 16, 128)
            x = op(x[:, 0:8], x[:, 8:16])
        return x[0]

    causal = (jax.lax.broadcasted_iota(jnp.int32, (7, 8, 128), 1)
              > jax.lax.broadcasted_iota(jnp.int32, (7, 8, 128), 0))
    low = jax.lax.broadcasted_iota(jnp.int32, (8, 128), 1) < 64

    def park(buf, seg, ks, vs, top):
        base = [key0_row(seg, i) for i in range(4)]
        for i, x in enumerate(ks + vs):
            buf[pl.ds(base[i], 8 * top + 8), :] = x[0:8 * top + 8]
            if top == 4 or i >= 2:
                buf[pl.ds(base[i] - 8, 8), :] = x[8 * top:8 * top + 8]
        out = {}
        for g in range(1, top + 1):
            last = list(base)
            if g < top:
                for i, v in enumerate(vs):
                    last[2 + i] = 8 * (L + 8) + ((NGV * seg + g - 1) * 2 + i) * 16 + 8
                    buf[pl.ds(last[2 + i] - 8, 16), :] = jnp.concatenate(
                        [v[8 * g:8 * g + 8], v[0:8]], axis=0)
            out[g] = (buf, base, last, [jnp.sum(v[8 * g + 8:L], axis=0, keepdims=True)
                                        if g < 4 else None for v in vs])
        return out

    def vpu_start(q0, q1, parked, g, masked=True):
        buf, base, last, (acc_a, acc_b) = parked
        st = dict(q=(q0 * c_exp, q1 * c_exp), buf=buf, base=base, last=last, g=g, masked=masked,
                  m=None)
        if g < 4:
            st.update(m=jnp.full((8, 128), neg_c, F32),
                      l=jnp.full((8, 128), float(L - 8 * (g + 1)), F32), a=acc_a, b=acc_b)
        return st

    def vpu_chunk(st, c0, gate):
        final = c0 == 8 * st['g']

        def windows(*rows):
            return jnp.concatenate(
                [st['buf'][pl.ds(k + 8 * st['g'] - r, 8), :]
                 for r in range(c0, c0 + CHUNK) for k in rows],
                axis=0).reshape(CHUNK, 8 * len(rows), 128)

        k0, k1, wa, wb = st['last' if final else 'base']
        q = jnp.concatenate([pltpu.bitcast(pltpu.bitcast(x, U32) | gate, F32) for x in st['q']],
                            axis=0)
        sc = jnp.sum(q * windows(k0, k1), axis=-1, keepdims=True)
        sc = jnp.where(low, sc[:, 0:8], sc[:, 8:16])
        if final and st['masked']:
            sc = jnp.concatenate([sc[0:1], jnp.where(causal, sc[1:], neg_c)], axis=0)
        m = tree(jnp.maximum, sc)
        if st['m'] is not None:
            m = jnp.maximum(m, st['m'])
            alpha = jnp.exp2(st['m'] - m)
        pr = jnp.exp2(sc - m)
        new = []
        for key, x in (('l', pr), ('a', pr * windows(wa)), ('b', pr * windows(wb))):
            if st['m'] is not None:
                x = jnp.concatenate([(st[key] * alpha)[None], x], axis=0)
            new.append(jnp.sum(x, axis=0))
        st.update(m=m, l=new[0], a=new[1], b=new[2])
        return (pltpu.bitcast(new[0], U32) | pltpu.bitcast(new[1], U32)
                | pltpu.bitcast(new[2], U32))

    def vpu_finish(st):
        r = recip(st['l'])
        return st['a'] * r, st['b'] * r

    def segment(lhs_q, lhs_kv, wo_m, full, n_chunks, unpack, wo_rows, split_first, zero,
                order, early, slots, d_g, d_j, d_f, d_s, d_pv, d_o):
        NP = H // 2
        nj = D // 128
        HA = H - TAIL_H
        mxu_pairs = [p for p in range(NP) if p not in full]
        proj = {}
        qkv = [None] * NP
        pb = [None] * NP
        og = [dict() for _ in range(H)]
        ocat = {}
        y = [None] * nj

        def slab(toks, which, h, r0, n):
            x = lhs_q if which == 0 else lhs_kv
            w = tied(wqkv_v[pl.ds(_slab_of(which, h) * PITCH + r0, n), :], toks)
            r = jnp.dot(x[:, 2 * r0:2 * (r0 + n)], w, preferred_element_type=F32)
            proj[(which, h)] = r + proj[(which, h)] if (which, h) in proj else r
            return proj[(which, h)]

        def do_wo(toks, h0, h1, j):
            if (h0, h1) not in ocat:
                ocat[(h0, h1)] = jnp.concatenate(
                    [wo_rows(og[h]) for h in range(h0, h1)], axis=1).astype(BF16)
            w = tied(wo_v[j, pl.ds(h0 * 64, (h1 - h0) * 64), :], toks)
            r = jnp.dot(ocat[(h0, h1)], w, preferred_element_type=F32)
            y[j] = r if y[j] is None else r + y[j]
            return y[j]

        ticks = []
        pair_end = {}
        wo_early = [(4 * c, 4 * c + 4, j) for c in range(early) for j in range(nj)]
        first = NP - slots
        for p in range(NP):
            slabs = [(which, h) for h in (2 * p, 2 * p + 1) for which in range(3)]
            rows = [(lhs_q if w == 0 else lhs_kv).shape[0] for w, _ in slabs]
            if p == 0 and split_first:
                for r0 in (0, 256):
                    ticks += [(slab, (w, h, r0, 256), m) for (w, h), m in zip(slabs, rows)]
            else:
                mine = []
                if p >= first:
                    lo = (p - first) * len(wo_early) // slots
                    mine = wo_early[lo:(p - first + 1) * len(wo_early) // slots]
                att = 0 if p in full else rm / 12
                units = [(slab, slabs[k0 + k] + (256 * half, 256), rows[k0 + k] + att)
                         for k0 in (0, 3) for k, half in order]
                for n, unit in enumerate(units):
                    ticks += [(do_wo, item, wo_m) for item in
                              mine[n * len(mine) // len(units):(n + 1) * len(mine) // len(units)]]
                    ticks.append(unit)
            pair_end[len(ticks) - 1] = p
        ticks += [(do_wo, (h0, h0 + 4, j), wo_m)
                  for h0 in range(4 * early, HA, 4) for j in range(nj)]
        ends = []
        for _, _, dur in ticks:
            ends.append(dur + (ends[-1] if ends else 0))

        def index(t):
            return next(i for i, e in enumerate(ends) if e >= t)

        events = {}
        anchors = {}
        cursor = [0]

        def run_chunk(res, p, name, st, c0, i_done):
            done = vpu_chunk(st, c0, pltpu.bitcast(res[GR:GR + 8], U32) & zero)
            anchors.setdefault(i_done, []).append(done & zero)
            if c0 + CHUNK >= 8 * (st['g'] + 1):
                og[2 * p][name], og[2 * p + 1][name] = vpu_finish(st)

        def do_s(res, p):
            sc = jax.lax.dot_general(qkv[p][0], qkv[p][1], (((1,), (1,)), ((), ())),
                                     preferred_element_type=F32)
            sc = pltpu.bitcast((pltpu.bitcast(sc, U32) & keep) | fill, F32)
            e = jnp.exp2((sc - jnp.max(sc, axis=-1, keepdims=True)) * c_exp)
            l = jnp.sum(e, axis=-1, keepdims=True)
            e = e * recip(l)
            pb[p] = (e[0:rm] + e[rm:2 * rm]).astype(BF16)

        def do_pv(res, p):
            for i in range(2):
                o = jnp.dot(pb[p], qkv[p][2][i], preferred_element_type=F32)
                for n, g in enumerate(mxu_groups):
                    og[2 * p + i][g] = o[8 * n:8 * n + 8]

        def finish_pair(p, i):
            u, jobs = unpack(p, [[proj[(w, h)] for w in range(3)] for h in (2 * p, 2 * p + 1)])
            chunks = [(name, st, c0) for name, st in
                      [(name, vpu_start(*job)) for name, job in jobs.items()]
                      for c0 in range(0, 8 * (st['g'] + 1), CHUNK)]
            t_first = ends[min(pair_end)] + d_g
            t_last = ends[-2] - d_j - d_f
            gap = (t_last - t_first) / (n_chunks - 1)
            if p == NP - 1:
                gap = min(gap, (t_last - max(ends[i] + d_g, cursor[0])) / (len(chunks) - 1))
            for chunk in chunks:
                t = max(ends[i] + d_g, cursor[0])
                cursor[0] = t + gap
                g = max(index(t), i + 1)
                events.setdefault(g, []).append(
                    (run_chunk, (p,) + chunk + (index(ends[g] + d_j) + 1,)))
            if p in full:
                return
            qb = jnp.concatenate([u[k][0][g] for k in range(2) for g in mxu_groups],
                                 axis=0).astype(BF16)
            kb = jnp.concatenate([u[0][1], u[1][1], zpad], axis=0).astype(BF16)
            low40 = jnp.concatenate([low] * 5, axis=0)
            vb = [jnp.concatenate([jnp.where(low40, v, 0.0), jnp.where(low40, 0.0, v), zpad],
                                  axis=0).astype(BF16) for v in (u[0][2], u[1][2])]
            qkv[p] = (qb, kb, vb)
            n = mxu_pairs.index(p)
            if n % 4 == 3:
                four = mxu_pairs[n - 3:n + 1]
                t2 = min(ends[i] + d_pv, ends[-1] - d_o)
                t1 = t2 - D_PP
                events.setdefault(index(min(ends[i] + d_s, t1 - D_SM)), []).extend(
                    (do_s, (k,)) for k in four)
                events.setdefault(index(t1), []).extend((do_pv, (k,)) for k in four[0:2])
                events.setdefault(index(t2), []).extend((do_pv, (k,)) for k in four[2:4])

        for i, (fn, args, _) in enumerate(ticks):
            res = fn(anchors.pop(i, []), *args)
            if i in pair_end:
                finish_pair(pair_end[i], i)
            for f, a in events.pop(i, []):
                f(res, *a)
        assert not events
        for j in range(nj):
            do_wo([], HA, H, j)
        return jnp.concatenate(y, axis=1)

    def pair(r0, mem):
        xf = x_v[pl.ds(r0, PAIR), :].astype(F32)
        zero = zero_v[pl.ds(0, 8), :]
        x1s = jnp.concatenate([xf[0:8], xf[32:40]], axis=0).astype(BF16)
        carry = [None] * (H // 2)

        def cat(*xs):
            return jnp.concatenate(xs, axis=0)

        lhs = cat(mem, xf[8:32]).astype(BF16)

        def unpack_a(p, qkv):
            qg = [{0: q[0:8], 2: q[8:16], 3: q[16:24], 4: q[24:32]} for q, _, _ in qkv]
            ks = [cat(k[0:8], k[32:40], k[8:32]) for _, k, _ in qkv]
            vs = [cat(v[0:8], v[32:40], v[8:32]) for _, _, v in qkv]
            top = 4 if p in FULL_A else NGV
            parked = park(kv_v[p], 0, ks, vs, top)
            carry[p] = (parked[1], [(k[40:48], v[40:48]) for _, k, v in qkv])
            jobs = {0: (qg[0][0], qg[1][0], parked[4], 4, False)} if top == 4 else {}
            jobs.update({g: (qg[0][g], qg[1][g], parked[g], g) for g in range(top, 1, -1)})
            return list(zip(qg, ks, vs)), jobs

        y_a = segment(lhs, cat(lhs, x1s), 32, FULL_A, 7 * (H // 2) + 10 * len(FULL_A), unpack_a,
                      lambda o: cat(o[0], o[2], o[3], o[4]), False, zero, **KNOBS_A)

        lhs = cat(y_a[0:8], xf[40:64]).astype(BF16)

        def unpack_b(p, qkv):
            parked_a1, kv1 = carry[p]
            qg = [{0: q[0:8], 1: q[40:48], 2: q[8:16], 3: q[16:24], 4: q[24:32]}
                  for q, _, _ in qkv]
            ks = [cat(k[0:8], e[0], k[8:32]) for (_, k, _), e in zip(qkv, kv1)]
            vs = [cat(v[0:8], e[1], v[8:32]) for (_, _, v), e in zip(qkv, kv1)]
            parked = park(kv_v[p], 1, ks, vs, NGV)
            jobs = {'a1': (qkv[0][0][32:40], qkv[1][0][32:40], parked_a1, 1)}
            jobs.update({g: (qg[0][g], qg[1][g], parked[g], g) for g in range(1, NGV + 1)})
            return list(zip(qg, ks, vs)), jobs

        y_b = segment(cat(lhs, x1s), lhs, 48, (), 11 * (H // 2), unpack_b,
                      lambda o: cat(o[0], o[1], o[2], o[3], o[4], o['a1']),
                      True, zero, **KNOBS_B)

        a = cat(y_b[40:48], y_a[8:32], y_b[8:40])
        g = g_v[pl.ds(r0, PAIR), :]
        g = jnp.concatenate([g] * (D // 128), axis=1)
        out_v[pl.ds(r0, PAIR), :] = (g * a + h1_rows(r0, PAIR)).astype(BF16)
        return y_b[0:8]

    def a_body(t, carry):
        r0 = pl.multiple_of(t * PAIR, PAIR)
        mem_v[...] = pair(r0, mem_v[...])
        pltpu.make_async_copy(out_v.at[pl.ds(r0, PAIR)], out_hbm.at[pl.ds(r0, PAIR)],
                              osem).start()
        return carry

    with jax.named_scope('a_body'):
        jax.lax.fori_loop(0, S // PAIR, a_body, 0)
    pltpu.make_async_copy(out_v, out_hbm, osem).wait()


@jax.jit
def pallas_gated_mix__memory_aug_recurrent_mem_tr__mixer_s_mlp__prompt_kernel(
    A_x, A_mem0, A_Wq, A_Wk, A_Wv, A_Wo, A_seg_len, B_x, B_w1, B_w2, B_w3, B_w4, gate_w,
):
    assert A_x.shape == (1, S, D) and A_Wq.shape == (D, H, DH) and A_mem0.shape == (1, M, D)
    x = A_x.reshape(S, D)
    mem0 = A_mem0.reshape(M, D)
    wq = A_Wq.reshape(D * H, DH)
    wk = A_Wk.reshape(D * H, DH)
    wv = A_Wv.reshape(D * H, DH)
    wo = A_Wo.reshape(H * DH, D)

    any_spec = pl.BlockSpec(memory_space=pl.ANY)
    out = pl.pallas_call(
        _kernel,
        out_shape=jax.ShapeDtypeStruct((S, D), BF16),
        in_specs=[any_spec] * 11,
        out_specs=any_spec,
        scratch_shapes=[
            pltpu.VMEM((S, D), BF16),
            pltpu.VMEM((NRING, 3, DP * H, DH), BF16),
            pltpu.VMEM((NRING, OP, D), BF16),
            pltpu.VMEM((3 * H * PITCH + 544, 128), U32),
            pltpu.VMEM((D // 128, H * DH // 2, 128), U32),
            pltpu.VMEM((4, D, D // 4), BF16),
            pltpu.VMEM((4, D, D // 4), BF16),
            pltpu.VMEM((D, FF), BF16),
            pltpu.VMEM((FF, D), BF16),
            pltpu.VMEM((3, D // 2, FF // 2), BF16),
            pltpu.VMEM((3, FF // 2, D // 2), BF16),
            pltpu.VMEM((D // 128, S + 16, 128), F32),
            pltpu.VMEM((S + T2, D), F32),
            pltpu.VMEM((S, 128), F32),
            pltpu.VMEM((2, T1, D), BF16),
            pltpu.VMEM((2, 7, T3 // 2, D // 2), BF16),
            pltpu.VMEM((M, D), BF16),
            pltpu.VMEM((D,), BF16),
            pltpu.VMEM((M, D), F32),
            pltpu.VMEM((S, D), BF16),
            [pltpu.VMEM((KV_ROWS, 128), F32)] * (H // 2),
            pltpu.VMEM((16, 128), U32),
            pltpu.SemaphoreType.DMA((NSEM,)),
            pltpu.SemaphoreType.DMA(()),
        ],
        compiler_params=pltpu.CompilerParams(vmem_limit_bytes=120 * 1024 * 1024,
                                             disable_bounds_checks=True),
    )(x, mem0, wq, wk, wv, wo, B_w1, B_w2, B_w3, B_w4, gate_w)
    return out.reshape(1, S, D)
```
